```python
import jax
import jax.numpy as jnp

def _softmax(x, axis=-1):
    return jax.nn.softmax(x, axis=axis)

def _gelu(x):
    return jax.nn.gelu(x, approximate=True)

def _silu(x):
    return jax.nn.silu(x)

def _sigmoid(x):
    return jax.nn.sigmoid(x)

def _layernorm(x, axis=-1, eps=1e-05):
    m = jnp.mean(x, axis=axis, keepdims=True)
    v = jnp.var(x, axis=axis, keepdims=True)
    return (x - m) / jnp.sqrt(v + eps)

def _scatter_add(tgt, idx, src, axis=0):
    return tgt.at[idx].add(src)

def _segment_sum(src, seg, n):
    return jax.ops.segment_sum(src, seg, n)

class _Rng:

    def __init__(self, key):
        self._k = key

    def _next(self):
        self._k, sub = jax.random.split(self._k)
        return sub

    def normal(self, shape):
        return jax.random.normal(self._next(), shape, dtype=jnp.bfloat16)

    def randint(self, lo, hi, shape):
        return jax.random.randint(self._next(), shape, lo, hi, dtype=jnp.int32)

    def uniform(self, shape, lo=0.0, hi=1.0):
        return jax.random.uniform(self._next(), shape, jnp.bfloat16, lo, hi)

    def permutation(self, n):
        return jax.random.permutation(self._next(), n)
kernel_name = 'gated_mix__sliding_local_dilated__memory_aug_recurrent_mem_tr__prompt'

def setup_inputs():
    _rng = _Rng(jax.random.key(int.from_bytes(__import__("os").urandom(4), "little")))
    _w = lambda a: (lambda t: t.astype(jnp.bfloat16) if jnp.issubdtype(t.dtype, jnp.floating) else t)(jnp.asarray(a))

    def _A_setup():
        B, S, D = (1, 2048, 576)
        return {'x': _w((lambda *s: _rng.normal(s) * 0.05)(B, S, D)), 'wqkv': _w((lambda *s: _rng.normal(s) * 0.05)(D, 3 * D)), 'wo': _w((lambda *s: _rng.normal(s) * 0.05)(D, D))}
    _A_in = _A_setup()

    def _B_setup():
        B, S, Dm = (1, 2048, 576)
        H, Dh = (32, 128)
        M, seg = (8, 32)
        seg = min(seg, S)
        S = S // seg * seg
        return {'x': _w((lambda *s: _rng.normal(s) * 0.05)(B, S, Dm)), 'mem0': _w((lambda *s: _rng.normal(s) * 0.05)(B, M, Dm)), 'Wq': _w((lambda *s: _rng.normal(s) * 0.05)(Dm, H, Dh) * Dm ** (-0.5)), 'Wk': _w((lambda *s: _rng.normal(s) * 0.05)(Dm, H, Dh) * Dm ** (-0.5)), 'Wv': _w((lambda *s: _rng.normal(s) * 0.05)(Dm, H, Dh) * Dm ** (-0.5)), 'Wo': _w((lambda *s: _rng.normal(s) * 0.05)(H, Dh, Dm) * (H * Dh) ** (-0.5)), 'seg_len': seg}
    _B_in = _B_setup()
    return {'A_x': _A_in['x'], 'A_wqkv': _A_in['wqkv'], 'A_wo': _A_in['wo'], 'B_x': _B_in['x'], 'B_mem0': _B_in['mem0'], 'B_Wq': _B_in['Wq'], 'B_Wk': _B_in['Wk'], 'B_Wv': _B_in['Wv'], 'B_Wo': _B_in['Wo'], 'B_seg_len': _B_in['seg_len'], 'gate_w': _w((lambda *s: _rng.normal(s) * 0.05)(576))}

def reference(A_x, A_wqkv, A_wo, B_x, B_mem0, B_Wq, B_Wk, B_Wv, B_Wo, B_seg_len, gate_w):

    def _A_ref(x, wqkv, wo):
        B, S, D = x.shape
        H = 32
        Dh = D // H
        W, dil = (8, 2)
        qkv = (lambda x, *d: x.transpose(*d))((x @ wqkv).reshape(B, S, 3, H, Dh), 2, 0, 3, 1, 4)
        q, k, v = (qkv[0], qkv[1], qkv[2])
        scale = Dh ** (-0.5)
        pos = jnp.arange(S)
        off = jnp.arange(W) * dil
        idx = pos[:, None] - off[None, :]
        mask = idx >= 0
        idx_c = jnp.where(mask, idx, 0).reshape(-1)
        kg = k[:, :, idx_c, :].reshape(B, H, S, W, Dh)
        vg = v[:, :, idx_c, :].reshape(B, H, S, W, Dh)
        logits = jnp.einsum('bhsd,bhswd->bhsw', q, kg) * scale
        logits = jnp.where(mask[None, None, :, :], logits, -1000000000.0)
        attn = _softmax(logits, axis=-1)
        o = jnp.einsum('bhsw,bhswd->bhsd', attn, vg)
        return (lambda x, *d: x.transpose(*d))(o, 0, 2, 1, 3).reshape(B, S, D) @ wo

    def _B_ref(x, mem0, Wq, Wk, Wv, Wo, seg_len):
        B, S, Dm = x.shape
        H, Dh = (Wq.shape[1], Wq.shape[2])
        M = mem0.shape[1]
        scale = Dh ** (-0.5)
        n_seg = S // seg_len
        L = M + seg_len
        idx = jnp.arange(L)
        mask = (idx[:, None] < M) | (idx[:, None] >= idx[None, :])
        mem = mem0
        outs = []
        for s in range(n_seg):
            xs = x[:, s * seg_len:(s + 1) * seg_len, :].copy()
            h = jnp.concatenate([mem, xs], axis=1)
            q = jnp.einsum('btd,dhe->bhte', h, Wq)
            k = jnp.einsum('btd,dhe->bhte', h, Wk)
            v = jnp.einsum('btd,dhe->bhte', h, Wv)
            scores = jnp.einsum('bhqe,bhke->bhqk', q, k) * scale
            scores = jnp.where(mask[None, None], scores, -1000000000.0)
            p = _softmax(scores, axis=-1)
            o = jnp.einsum('bhqk,bhke->bhqe', p, v)
            o = jnp.einsum('bhte,hed->btd', o, Wo)
            mem = o[:, :M, :].copy()
            outs.append(o[:, M:, :])
        return jnp.concatenate(outs, axis=1)
    x = A_x
    g = _sigmoid((x * gate_w).sum(-1, keepdims=True))
    a = _A_ref(x, A_wqkv, A_wo)
    b = _B_ref(x, B_mem0, B_Wq, B_Wk, B_Wv, B_Wo, B_seg_len)
    return g * a + (1 - g) * b
```

```python
import functools

import jax
import jax.numpy as jnp
from jax import lax
import jax.experimental.pallas as pl
import jax.experimental.pallas.tpu as pltpu

F32, BF16, U32 = jnp.float32, jnp.bfloat16, jnp.uint32

D = 576
LANES = 128
HA, DA = 32, 18
WIN, DIL = 8, 2
HB, DB = 32, 128
NP = HB // 2
NEG = -1000000000.0
NG = HA // 8
RA = 3 * (DA // 2) * 8


def _dot(a, b):
    return lax.dot_general(a, b, (((1,), (0,)), ((), ())), preferred_element_type=F32)


def _dot_nt(a, b):
    return lax.dot_general(a, b, (((1,), (1,)), ((), ())), preferred_element_type=F32)


def _low_half(rows):
    return lax.broadcasted_iota(jnp.int32, (rows, LANES), 1) < 64


def _pair_tiles(w1, w2):
    a1, b1, c1 = w1[384:448], w1[448:512], w1[512:576]
    a2, b2, c2 = w2[384:448], w2[448:512], w2[512:576]
    cat = lambda u, v: jnp.concatenate([u, v], axis=0)
    return ([w1[i * 128:(i + 1) * 128] for i in range(3)] + [cat(c1, b1 - b2)]
            + [w2[i * 128:(i + 1) * 128] for i in range(3)] + [cat(a2 - a1, c2)]
            + [cat(a1, b2)])


def _pair_lhs(t1, t2):
    lo = _low_half(t1[0].shape[0])
    diff = t1[3] - t2[3]
    return (t1[:3] + [jnp.where(lo, t1[4], diff)]
            + t2[:3] + [jnp.where(lo, -diff, t2[4])]
            + [jnp.where(lo, t1[3], t2[3])])


def _pair_rhs(x):
    a, b, c = x[384:448], x[448:512], x[512:576]
    cat = lambda u, v: jnp.concatenate([u, v], axis=0)
    return [x[i * 128:(i + 1) * 128] for i in range(3)] + [cat(c, b), cat(a, c), x[384:512]]


def _pair_matmul(lhs, rhs):
    z = _dot(lhs(8), rhs[5])
    o1, o2 = z, z
    for i in range(4):
        o1 = o1 + _dot(lhs(i), rhs[i])
    for i in range(4):
        o2 = o2 + _dot(lhs(4 + i), rhs[i if i < 3 else 4])
    return o1, o2


def _kernel(xt_hbm, wqkv_hbm, wo_hbm, mem0_ref, wq_hbm, wk_hbm, wv_hbm, wot_hbm, gate_ref,
            out_hbm,
            xt_v, wqkv_v, wo_v, stg_qkv, stg_o, wt32, la, lo_a, kv_prev, oa_s,
            wb, wob, x32, ga_s, gm_s, h_s, b_s, out_v,
            sem_x, sem_wa, sem_wb, sem_out, *, seq, seg, mem):
    nt = seq // LANES
    rows = mem + seg
    spt = LANES // seg

    def cp_x(j):
        col = j * LANES if isinstance(j, int) else pl.multiple_of(j * LANES, LANES)
        return pltpu.make_async_copy(xt_hbm.at[:, pl.ds(col, LANES)], xt_v.at[j], sem_x.at[j])

    def cp_wqkv(k):
        r = pl.ds(k * 128, min(128, D - k * 128))
        return pltpu.make_async_copy(wqkv_hbm.at[r], wqkv_v.at[r], sem_wa.at[k])

    cp_wo = pltpu.make_async_copy(wo_hbm, wo_v, sem_wa.at[5])

    def cp_wb(i, p):
        if i == 3:
            return pltpu.make_async_copy(wot_hbm.at[pl.ds(2 * p, 2)], stg_o.at[pl.ds(2 * p, 2)],
                                         sem_wb.at[3, p])
        src = (wq_hbm, wk_hbm, wv_hbm)[i].bitcast(U32)
        return pltpu.make_async_copy(src.at[:, p, :], stg_qkv.at[i, p], sem_wb.at[i, p])

    def cp_out(j):
        col = j * LANES if isinstance(j, int) else pl.multiple_of(j * LANES, LANES)
        return pltpu.make_async_copy(out_v.at[j], out_hbm.at[:, pl.ds(col, LANES)], sem_out.at[j])

    for k in range(5):
        cp_wqkv(k).start()
    cp_x(0).start()
    cp_wo.start()
    for p in range(max(NP, nt)):
        if p + 1 < nt:
            cp_x(p + 1).start()
        if p < NP:
            for i in range(4):
                cp_wb(i, p).start()

    gate = jnp.broadcast_to(gate_ref[...].astype(F32).reshape(1, D), (8, D))
    gate_t = [gate[:, i * 128:(i + 1) * 128] for i in range(4)]
    gate_t.append(jnp.concatenate([gate[:, 512:], gate[:, 512:]], axis=1))

    for k in range(5):
        cp_wqkv(k).wait()
        if k < 4:
            blk = wqkv_v[k * 128:(k + 1) * 128, :]
        else:
            blk = jnp.concatenate([wqkv_v[512:D, :]] * 2, axis=0)
        wt32[k] = blk.T.astype(F32)

    for g in range(NG):
        for part in range(3):
            for dd in range(DA // 2):
                base = part * D + g * 8 * DA + 2 * dd
                t1 = [wt32[k, pl.ds(base, 8, stride=DA), :] for k in range(5)]
                t2 = [wt32[k, pl.ds(base + 1, 8, stride=DA), :] for k in range(5)]
                r0 = (part * (DA // 2) + dd) * 8
                for i, t in enumerate(_pair_lhs(t1, t2)):
                    la[g * 9 + i, r0:r0 + 8, :] = t
    for i, t in enumerate(_pair_lhs(gate_t, gate_t)):
        la[i, RA:RA + 8, :] = t

    cp_wo.wait()
    wo32 = wo_v[...].astype(F32)
    for n in range(4):
        wt32[n, 0:D, :] = wo32[:, n * 128:(n + 1) * 128]
    wt32[4, 0:D, :] = jnp.concatenate([wo32[:, 512:], wo32[:, 512:]], axis=1)
    perm = [jnp.concatenate([wt32[n, pl.ds(g * 8 * DA + d, 8, stride=DA), :]
                             for g in range(NG) for d in range(DA)], axis=0) for n in range(5)]
    tiles = []
    for k in range(5):
        if k < 4:
            pk = [pn[k * 128:(k + 1) * 128] for pn in perm]
        else:
            pk = [jnp.concatenate([pn[512:], pn[512:]], axis=0) for pn in perm]
        tiles.append(jnp.concatenate([t.T for t in pk[:4]] + [pk[4].T[:64]], axis=0))
    for i, t in enumerate(_pair_lhs([t[:D // 2] for t in tiles], [t[D // 2:] for t in tiles])):
        lo_a[i] = t

    def prep_pair(p):
        for i in range(4):
            cp_wb(i, p).wait()
        for i in range(3):
            u = stg_qkv[i, p]
            w1 = pltpu.bitcast(u << 16, F32)
            w2 = pltpu.bitcast((u >> 16) << 16, F32)
            for t, tile in enumerate(_pair_tiles(w1, w2)):
                wb[p, i, t] = pltpu.bitcast(tile.astype(BF16), U32)
        w1 = stg_o[2 * p].astype(F32)
        w2 = stg_o[2 * p + 1].astype(F32)
        for t, tile in enumerate(_pair_tiles(w1, w2)):
            wob[p, t] = pltpu.bitcast(tile.astype(BF16).T, U32)

    lane = lax.broadcasted_iota(jnp.int32, (8, LANES), 1)

    def shifted(prev, cur, w):
        if w == 0:
            return cur
        return pltpu.roll(jnp.where(lane >= LANES - DIL * w, prev, cur), DIL * w, 1)

    def a_tile(j, first):
        cp_x(j).wait()
        xt = xt_v[j]
        rhs = _pair_rhs(xt)
        t0 = j * LANES if isinstance(j, int) else pl.multiple_of(j * LANES, LANES)
        for i in range(6):
            x32[pl.ds(t0, LANES), i * 128:(i + 1) * 128] = rhs[i].T.astype(F32)
        gsig = None
        for g in range(NG):
            nr = RA + 8 if g == 0 else RA
            halves = _pair_matmul(lambda i: la[g * 9 + i, 0:nr, :], rhs)
            if g == 0:
                gsig = 1.0 / (1.0 + jnp.exp(-halves[0][RA:RA + 8]))

            def get(part, d):
                r0 = (part * (DA // 2) + d // 2) * 8
                return halves[d % 2][r0:r0 + 8]

            logit = [None] * WIN
            for d in range(DA):
                q, k = get(0, d), get(1, d)
                kp = k if first else kv_prev[g, 0, d]
                for w in range(WIN):
                    t = q * shifted(kp, k, w)
                    logit[w] = t if d == 0 else logit[w] + t
                kv_prev[g, 0, d] = k
            logit = [t * (DA ** -0.5) for t in logit]
            if first:
                logit = [jnp.where(lane >= DIL * w, t, NEG) for w, t in enumerate(logit)]
            mx = functools.reduce(jnp.maximum, logit)
            ex = [jnp.exp(t - mx) for t in logit]
            inv = 1.0 / functools.reduce(jnp.add, ex)
            prob = [e * inv for e in ex]
            for d in range(DA):
                v = get(2, d)
                vp = jnp.broadcast_to(v[:, 0:1], (8, LANES)) if first else kv_prev[g, 1, d]
                o = functools.reduce(jnp.add, [prob[w] * shifted(vp, v, w) for w in range(WIN)])
                kv_prev[g, 1, d] = v
                oa_s[(g * DA + d) * 8:(g * DA + d + 1) * 8, :] = o
        halves = _pair_matmul(lambda i: lo_a[i], _pair_rhs(oa_s[...].astype(BF16)))
        gs = jnp.concatenate([gsig] * (D // 16), axis=0)
        ga_s[j, 0:D // 2, :] = halves[0] * gs
        ga_s[j, D // 2:D, :] = halves[1] * gs
        gm_s[j] = 1.0 - gsig

    a_tile(0, True)

    def a_body(j, carry):
        prep_pair(j - 1)
        a_tile(j, False)
        return carry

    lax.fori_loop(1, nt, a_body, 0)
    for p in range(nt - 1, NP):
        prep_pair(p)

    def put_mem(t):
        lo = _low_half(mem)
        for i in range(3):
            h_s[0:mem, i * 128:(i + 1) * 128] = t[i]
        h_s[0:mem, 384:512] = jnp.where(lo, t[4], t[3])
        h_s[0:mem, 512:640] = jnp.where(lo, t[3], t[4])
        h_s[0:mem, 640:768] = t[3]

    m0 = mem0_ref[...].astype(F32)
    put_mem([m0[:, i * 128:(i + 1) * 128] for i in range(4)]
            + [jnp.concatenate([m0[:, 512:], m0[:, 512:]], axis=1)])
    b_s[...] = jnp.zeros(b_s.shape, F32)

    qi = lax.broadcasted_iota(jnp.int32, (rows, rows), 0)
    ki = lax.broadcasted_iota(jnp.int32, (rows, rows), 1)
    mask = (qi < mem) | (qi >= ki)

    def b_step(t0, r0):
        h_s[mem:rows, :] = x32[pl.ds(t0, seg), :]
        qkv, soft, outs = {}, {}, {}
        acc = [None] * 6

        def project(p, i):
            lhs = lambda c: h_s[:, c * 128:(c + 1) * 128]
            w = lambda t: pltpu.bitcast(wb[p, i, t], BF16)
            z = _dot(lhs(5), w(8))
            for hh in range(2):
                o = z
                for c in range(4):
                    o = o + _dot(lhs(c if c < 3 else 3 + hh), w(4 * hh + c))
                qkv[2 * p + hh, i] = o if i == 0 else o.astype(BF16)

        def scores(h):
            s = jnp.where(mask, _dot_nt(qkv[h, 0], qkv[h, 1]) * (DB ** -0.5), NEG)
            e = jnp.exp(s - jnp.max(s, axis=-1, keepdims=True))
            soft[h] = (e, jnp.sum(e, axis=-1, keepdims=True))

        def values(h):
            e, l = soft[h]
            outs[h] = _dot(e, qkv[h, 2]) * (1.0 / l)

        def out_proj(p):
            o1, o2 = outs[2 * p], outs[2 * p + 1]
            w = lambda t: pltpu.bitcast(wob[p, t], BF16)
            new = [_dot(o1, w(n)) + _dot(o2, w(4 + n)) for n in range(3)]
            new += [_dot(o1, w(3)), _dot(o2, w(7)), _dot(o1 + o2, w(8))]
            for n in range(6):
                acc[n] = new[n] if p == 0 else acc[n] + new[n]

        lag_o = 3
        for p in range(NP):
            project(p, 0)
            project(p, 1)
            if p >= 1:
                values(2 * p - 2)
                values(2 * p - 1)
            project(p, 2)
            if p >= lag_o:
                out_proj(p - lag_o)
            scores(2 * p)
            scores(2 * p + 1)
        out_proj(NP - 3)
        out_proj(NP - 2)
        values(HB - 2)
        values(HB - 1)
        out_proj(NP - 1)

        lo = _low_half(rows)
        ab = acc[5] + jnp.where(lo, acc[4], acc[3])
        y = jnp.where(lo, acc[3], acc[4])
        res = acc[:3] + [ab, y]
        ym = y[0:mem]
        put_mem([t[0:mem] for t in res[:4]] + [ym + pltpu.roll(ym, 64, 1)])
        for n in range(5):
            b_s[r0:r0 + seg, n * 128:(n + 1) * 128] = res[n][mem:rows]

    def emit_tile(j):
        gm = gm_s[j]
        for n in range(5):
            bt = b_s[:, n * 128:(n + 1) * 128].T
            if n == 4:
                bt = bt[0:64] + bt[64:128]
            nr = bt.shape[0]
            gmr = jnp.concatenate([gm] * (nr // 8), axis=0)
            out_v[j, n * 128:n * 128 + nr, :] = (
                ga_s[j, n * 128:n * 128 + nr, :] + gmr * bt).astype(out_v.dtype)

    def b_body(j, carry):
        emit_tile(jnp.maximum(j - 1, 0))
        for u in range(spt):
            b_step(pl.multiple_of(j * LANES + u * seg, seg), u * seg)

        @pl.when(j > 0)
        def _():
            cp_out(j - 1).start()

        return carry

    lax.fori_loop(0, nt, b_body, 0)
    emit_tile(nt - 1)
    cp_out(nt - 1).start()
    for j in range(nt):
        cp_out(j).wait()


@functools.partial(jax.jit, static_argnames=("B_seg_len",))
def pallas_gated_mix__sliding_local_dilated__memory_aug_recurrent_mem_tr__prompt_kernel(
    A_x: jax.Array,
    A_wqkv: jax.Array,
    A_wo: jax.Array,
    B_x: jax.Array,
    B_mem0: jax.Array,
    B_Wq: jax.Array,
    B_Wk: jax.Array,
    B_Wv: jax.Array,
    B_Wo: jax.Array,
    B_seg_len: int,
    gate_w: jax.Array,
):
    del B_x
    batch, seq, width = A_x.shape
    mem, seg = B_mem0.shape[1], int(B_seg_len)
    nt = seq // LANES
    assert batch == 1 and width == D and seq % LANES == 0 and nt <= NP + 1
    assert B_Wq.shape == (D, HB, DB) and mem % 8 == 0 and seg % 8 == 0 and LANES % seg == 0

    hbm = pl.BlockSpec(memory_space=pl.ANY)
    vmem = pl.BlockSpec(memory_space=pltpu.VMEM)
    out_t = pl.pallas_call(
        functools.partial(_kernel, seq=seq, seg=seg, mem=mem),
        out_shape=jax.ShapeDtypeStruct((D, seq), A_x.dtype),
        in_specs=[hbm, hbm, hbm, vmem, hbm, hbm, hbm, hbm, vmem],
        out_specs=hbm,
        scratch_shapes=[
            pltpu.VMEM((nt, D, LANES), BF16),
            pltpu.VMEM((D, 3 * D), BF16),
            pltpu.VMEM((D, D), BF16),
            pltpu.VMEM((3, NP, D, DB), U32),
            pltpu.VMEM((HB, D, DB), BF16),
            pltpu.VMEM((5, 3 * D, LANES), F32),
            pltpu.VMEM((NG * 9, RA + 8, LANES), F32),
            pltpu.VMEM((9, D // 2, LANES), F32),
            pltpu.VMEM((NG, 2, DA, 8, LANES), F32),
            pltpu.VMEM((D, LANES), F32),
            pltpu.VMEM((NP, 3, 9, 64, LANES), U32),
            pltpu.VMEM((NP, 9, 64, LANES), U32),
            pltpu.VMEM((seq, 6 * LANES), F32),
            pltpu.VMEM((nt, D, LANES), F32),
            pltpu.VMEM((nt, 8, LANES), F32),
            pltpu.VMEM((mem + seg, 6 * LANES), F32),
            pltpu.VMEM((LANES, 5 * LANES), F32),
            pltpu.VMEM((nt, D, LANES), A_x.dtype),
            pltpu.SemaphoreType.DMA((nt,)),
            pltpu.SemaphoreType.DMA((6,)),
            pltpu.SemaphoreType.DMA((4, NP)),
            pltpu.SemaphoreType.DMA((nt,)),
        ],
        compiler_params=pltpu.CompilerParams(vmem_limit_bytes=110 * 1024 * 1024),
        name="gated_mix_kernel",
    )(A_x[0].T, A_wqkv, A_wo, B_mem0[0], B_Wq, B_Wk, B_Wv, B_Wo.transpose(0, 2, 1), gate_w)
    return out_t.T[None]
```

```python
import functools

import jax
import jax.numpy as jnp
from jax import lax
import jax.experimental.pallas as pl
import jax.experimental.pallas.tpu as pltpu

F32, BF16, U32 = jnp.float32, jnp.bfloat16, jnp.uint32

D = 576
LANES = 128
HA, DA = 32, 18
WIN, DIL = 8, 2
HB, DB = 32, 128
NP = HB // 2
NEG = -1000000000.0
NG = HA // 8
RA = 3 * (DA // 2) * 8


def _dot(a, b):
    return lax.dot_general(a, b, (((1,), (0,)), ((), ())), preferred_element_type=F32)


def _dot_nt(a, b):
    return lax.dot_general(a, b, (((1,), (1,)), ((), ())), preferred_element_type=F32)


def _low_half(rows):
    return lax.broadcasted_iota(jnp.int32, (rows, LANES), 1) < 64


def _pair_tiles(w1, w2):
    a1, b1, c1 = w1[384:448], w1[448:512], w1[512:576]
    a2, b2, c2 = w2[384:448], w2[448:512], w2[512:576]
    cat = lambda u, v: jnp.concatenate([u, v], axis=0)
    sub = lambda u, v: (u.astype(F32) - v.astype(F32)).astype(u.dtype)
    return ([w1[i * 128:(i + 1) * 128] for i in range(3)] + [cat(c1, sub(b1, b2))]
            + [w2[i * 128:(i + 1) * 128] for i in range(3)] + [cat(sub(a2, a1), c2)]
            + [cat(a1, b2)])


def _pair_lhs(t1, t2):
    lo = _low_half(t1[0].shape[0])
    diff = t1[3] - t2[3]
    return (t1[:3] + [jnp.where(lo, t1[4], diff)]
            + t2[:3] + [jnp.where(lo, -diff, t2[4])]
            + [jnp.where(lo, t1[3], t2[3])])


def _pair_rhs(x):
    a, b, c = x[384:448], x[448:512], x[512:576]
    cat = lambda u, v: jnp.concatenate([u, v], axis=0)
    return [x[i * 128:(i + 1) * 128] for i in range(3)] + [cat(c, b), cat(a, c), x[384:512]]


def _pair_matmul(lhs, rhs):
    z = _dot(lhs(8), rhs[5])
    o1, o2 = z, z
    for i in range(4):
        o1 = o1 + _dot(lhs(i), rhs[i])
    for i in range(4):
        o2 = o2 + _dot(lhs(4 + i), rhs[i if i < 3 else 4])
    return o1, o2


def _kernel(xt_hbm, wqkv_hbm, wo_hbm, mem0_ref, wq_hbm, wk_hbm, wv_hbm, wot_hbm, gate_ref,
            out_hbm,
            xt_v, wqkv_v, wo_v, stg_qkv, stg_o, wt32, la, lo_a, kv_prev, oa_s,
            wb, wob, x32, ga_s, gm_s, h_s, b_s, out_v,
            sem_x, sem_wa, sem_wb, sem_out, *, seq, seg, mem):
    nt = seq // LANES
    rows = mem + seg
    spt = LANES // seg

    def cp_x(j):
        col = j * LANES if isinstance(j, int) else pl.multiple_of(j * LANES, LANES)
        return pltpu.make_async_copy(xt_hbm.at[:, pl.ds(col, LANES)], xt_v.at[j], sem_x.at[j])

    def cp_wqkv(k):
        r = pl.ds(k * 128, min(128, D - k * 128))
        return pltpu.make_async_copy(wqkv_hbm.at[r], wqkv_v.at[r], sem_wa.at[k])

    cp_wo = pltpu.make_async_copy(wo_hbm, wo_v, sem_wa.at[5])

    def cp_wb(i, p):
        if i == 3:
            return pltpu.make_async_copy(wot_hbm.at[pl.ds(2 * p, 2)], stg_o.at[pl.ds(2 * p, 2)],
                                         sem_wb.at[3, p])
        src = (wq_hbm, wk_hbm, wv_hbm)[i].bitcast(U32)
        return pltpu.make_async_copy(src.at[:, p, :], stg_qkv.at[i, p], sem_wb.at[i, p])

    def cp_out(j):
        col = j * LANES if isinstance(j, int) else pl.multiple_of(j * LANES, LANES)
        return pltpu.make_async_copy(out_v.at[j], out_hbm.at[:, pl.ds(col, LANES)], sem_out.at[j])

    for k in range(5):
        cp_wqkv(k).start()
    cp_x(0).start()
    cp_wo.start()
    for p in range(max(NP, nt)):
        if p + 1 < nt:
            cp_x(p + 1).start()
        if p < NP:
            for i in range(4):
                cp_wb(i, p).start()

    gate = jnp.broadcast_to(gate_ref[...].astype(F32).reshape(1, D), (8, D))
    gate_t = [gate[:, i * 128:(i + 1) * 128] for i in range(4)]
    gate_t.append(jnp.concatenate([gate[:, 512:], gate[:, 512:]], axis=1))

    for k in range(5):
        cp_wqkv(k).wait()
        if k < 4:
            blk = wqkv_v[k * 128:(k + 1) * 128, :]
        else:
            blk = jnp.concatenate([wqkv_v[512:D, :]] * 2, axis=0)
        wt32[k] = blk.T.astype(F32)

    for g in range(NG):
        for part in range(3):
            for dd in range(DA // 2):
                base = part * D + g * 8 * DA + 2 * dd
                t1 = [wt32[k, pl.ds(base, 8, stride=DA), :] for k in range(5)]
                t2 = [wt32[k, pl.ds(base + 1, 8, stride=DA), :] for k in range(5)]
                r0 = (part * (DA // 2) + dd) * 8
                for i, t in enumerate(_pair_lhs(t1, t2)):
                    la[g * 9 + i, r0:r0 + 8, :] = t
    for i, t in enumerate(_pair_lhs(gate_t, gate_t)):
        la[i, RA:RA + 8, :] = t

    cp_wo.wait()
    wo32 = wo_v[...].astype(F32)
    for n in range(4):
        wt32[n, 0:D, :] = wo32[:, n * 128:(n + 1) * 128]
    wt32[4, 0:D, :] = jnp.concatenate([wo32[:, 512:], wo32[:, 512:]], axis=1)
    perm = [jnp.concatenate([wt32[n, pl.ds(g * 8 * DA + d, 8, stride=DA), :]
                             for g in range(NG) for d in range(DA)], axis=0) for n in range(5)]
    tiles = []
    for k in range(5):
        if k < 4:
            pk = [pn[k * 128:(k + 1) * 128] for pn in perm]
        else:
            pk = [jnp.concatenate([pn[512:], pn[512:]], axis=0) for pn in perm]
        tiles.append(jnp.concatenate([t.T for t in pk[:4]] + [pk[4].T[:64]], axis=0))
    for i, t in enumerate(_pair_lhs([t[:D // 2] for t in tiles], [t[D // 2:] for t in tiles])):
        lo_a[i] = t

    def prep_pair(p):
        hi_mask = jnp.uint32(0xFFFF0000)
        low = lambda e, o: (e & ~hi_mask) | (o << 16)
        high = lambda e, o: (e >> 16) | (o & hi_mask)
        rnd = lambda t: pltpu.bitcast(t.astype(BF16).astype(F32), U32)
        w1 = lambda u: pltpu.bitcast(u << 16, F32)
        w2 = lambda u: pltpu.bitcast(u & hi_mask, F32)
        for i in range(3):
            for c in range(9):
                ev = stg_qkv[i, p, pl.ds(c * 64, 32, stride=2), :]
                od = stg_qkv[i, p, pl.ds(c * 64 + 1, 32, stride=2), :]
                half = pl.ds((c % 2) * 32, 32)
                if c < 6:
                    wb[p, i, c // 2, half, :] = low(ev, od)
                    wb[p, i, 4 + c // 2, half, :] = high(ev, od)
                elif c == 6:
                    wb[p, i, 8, 0:32, :] = low(ev, od)
                    wb[p, i, 7, 0:32, :] = high(rnd(w2(ev) - w1(ev)), rnd(w2(od) - w1(od)))
                elif c == 7:
                    wb[p, i, 8, 32:64, :] = high(ev, od)
                    wb[p, i, 3, 32:64, :] = high(rnd(w1(ev) - w2(ev)), rnd(w1(od) - w2(od)))
                else:
                    wb[p, i, 3, 0:32, :] = low(ev, od)
                    wb[p, i, 7, 32:64, :] = high(ev, od)
        for t, tile in enumerate(_pair_tiles(stg_o[2 * p], stg_o[2 * p + 1])):
            wob[p, t] = pltpu.bitcast(tile.T, U32)

    def wait_pair(p):
        for i in range(4):
            cp_wb(i, p).wait()

    lane = lax.broadcasted_iota(jnp.int32, (8, LANES), 1)

    def pack(even, odd):
        return pltpu.bitcast(jnp.concatenate([even, odd], axis=0).astype(BF16), U32)

    def shifted(prev, cur, w):
        if w > 0:
            cur = pltpu.roll(jnp.where(lane >= LANES - DIL * w, prev, cur), DIL * w, 1)
        both = pltpu.bitcast(cur, BF16).astype(F32)
        return both[0:8], both[8:16]

    def a_heads(j, first):
        rhs = _pair_rhs(xt_v[j])
        t0 = j * LANES if isinstance(j, int) else pl.multiple_of(j * LANES, LANES)
        for i in range(6):
            x32[pl.ds(t0, LANES), i * 128:(i + 1) * 128] = rhs[i].T.astype(F32)
        gsig, outs = None, []
        rp = RA // 3
        for g in range(NG):
            parts = []
            for part in range(3):
                nr = rp + 8 if (g, part) == (0, 2) else rp
                parts.append(_pair_matmul(
                    lambda i: la[g * 9 + i, part * rp:part * rp + nr, :], rhs))
            if g == 0:
                gsig = 1.0 / (1.0 + jnp.exp(-parts[2][0][rp:rp + 8]))
            get = lambda part, dd: [t[dd * 8:dd * 8 + 8] for t in parts[part]]

            logit = [None] * WIN
            for dd in range(DA // 2):
                q, k = get(0, dd), pack(*get(1, dd))
                kp = k if first else kv_prev[g, 0, dd]
                for w in range(WIN):
                    ks = shifted(kp, k, w)
                    t = q[0] * ks[0] + q[1] * ks[1]
                    logit[w] = t if dd == 0 else logit[w] + t
                kv_prev[g, 0, dd] = k
            logit = [t * (DA ** -0.5) for t in logit]
            if first:
                logit = [jnp.where(lane >= DIL * w, t, NEG) for w, t in enumerate(logit)]
            mx = functools.reduce(jnp.maximum, logit)
            ex = [jnp.exp(t - mx) for t in logit]
            inv = gsig / functools.reduce(jnp.add, ex)
            prob = [e * inv for e in ex]
            for dd in range(DA // 2):
                v = pack(*get(2, dd))
                vp = jnp.broadcast_to(v[:, 0:1], (8, LANES)) if first else kv_prev[g, 1, dd]
                o = [None, None]
                for w in range(WIN):
                    vs = shifted(vp, v, w)
                    o = [prob[w] * vs[i] if w == 0 else o[i] + prob[w] * vs[i] for i in range(2)]
                kv_prev[g, 1, dd] = v
                outs.append(pack(*o))
        gm_s[j] = 1.0 - gsig
        return jnp.concatenate(outs, axis=0)

    def a_out(j):
        rhs = _pair_rhs(pltpu.bitcast(oa_s[...], BF16))
        rp = D // 8
        for c in range(4):
            halves = _pair_matmul(lambda i: lo_a[i, c * rp:(c + 1) * rp, :], rhs)
            ga_s[j, c * rp:(c + 1) * rp, :] = halves[0]
            ga_s[j, D // 2 + c * rp:D // 2 + (c + 1) * rp, :] = halves[1]

    cp_x(0).wait()
    oa_s[...] = a_heads(0, True)

    def a_body(j, carry):
        cp_x(j).wait()
        wait_pair(j - 1)
        o = a_heads(j, False)
        a_out(j - 1)
        oa_s[...] = o
        prep_pair(j - 1)
        return carry

    lax.fori_loop(1, nt, a_body, 0)
    for p in range(nt - 1, NP):
        wait_pair(p)
    a_out(nt - 1)
    for p in range(nt - 1, NP):
        prep_pair(p)

    def put_mem(t):
        lo = _low_half(mem)
        for i in range(3):
            h_s[0:mem, i * 128:(i + 1) * 128] = t[i]
        h_s[0:mem, 384:512] = jnp.where(lo, t[4], t[3])
        h_s[0:mem, 512:640] = jnp.where(lo, t[3], t[4])
        h_s[0:mem, 640:768] = t[3]

    m0 = mem0_ref[...].astype(F32)
    put_mem([m0[:, i * 128:(i + 1) * 128] for i in range(4)]
            + [jnp.concatenate([m0[:, 512:], m0[:, 512:]], axis=1)])
    b_s[...] = jnp.zeros(b_s.shape, F32)

    qi = lax.broadcasted_iota(jnp.int32, (rows, rows), 0)
    ki = lax.broadcasted_iota(jnp.int32, (rows, rows), 1)
    mask = (qi < mem) | (qi >= ki)

    def b_step(t0, r0):
        h_s[mem:rows, :] = x32[pl.ds(t0, seg), :]
        qkv, soft, outs = {}, {}, {}
        acc = [None] * 6

        lhs = lambda c: h_s[:, c * 128:(c + 1) * 128]

        def project(p, *which):
            w = lambda i, t: pltpu.bitcast(wb[p, i, t], BF16)
            o = {}
            for i in which:
                z = _dot(lhs(5), w(i, 8))
                for hh in range(2):
                    o[i, hh] = z + _dot(lhs(3 + hh), w(i, 4 * hh + 3))
            for c in range(3):
                for i in which:
                    for hh in range(2):
                        o[i, hh] = o[i, hh] + _dot(lhs(c), w(i, 4 * hh + c))
            for (i, hh), t in o.items():
                qkv[2 * p + hh, i] = t if i == 0 else t.astype(BF16)

        def scores(p):
            for h in (2 * p, 2 * p + 1):
                s = jnp.where(mask, _dot_nt(qkv[h, 0], qkv[h, 1]) * (DB ** -0.5), NEG)
                e = jnp.exp(s - jnp.max(s, axis=-1, keepdims=True))
                soft[h] = (e, jnp.sum(e, axis=-1, keepdims=True))

        def values(p):
            for h in (2 * p, 2 * p + 1):
                e, l = soft[h]
                outs[h] = _dot(e, qkv[h, 2]) * (1.0 / l)

        def out_proj(pairs, cols=range(6)):
            for n in cols:
                tot = None
                for p in pairs:
                    o1, o2 = outs[2 * p], outs[2 * p + 1]
                    w = lambda t: pltpu.bitcast(wob[p, t], BF16)
                    if n < 3:
                        r = _dot(o1, w(n)) + _dot(o2, w(4 + n))
                    else:
                        r = _dot((o1, o2, o1 + o2)[n - 3], w((3, 7, 8)[n - 3]))
                    tot = r if tot is None else tot + r
                acc[n] = tot if acc[n] is None else acc[n] + tot

        lag, last = 8, 4
        project(0, 0, 1)
        project(0, 2)
        for p in range(1, NP):
            project(p, 0)
            project(p, 1)
            scores(p - 1)
            project(p, 2)
            if p >= 2:
                values(p - 2)
            if p >= lag:
                out_proj([p - lag])
        scores(NP - 1)
        out_proj([NP - lag])
        values(NP - 2)
        for p in range(NP - lag + 1, NP - last):
            out_proj([p])
        values(NP - 1)
        tail = list(range(NP - last, NP))
        out_proj(tail[:-1], [3, 4, 5, 0])
        out_proj(tail[-1:], [3, 4, 5, 0])
        out_proj(tail, [1, 2])

        lo = _low_half(rows)
        ab = acc[5] + jnp.where(lo, acc[4], acc[3])
        y = jnp.where(lo, acc[3], acc[4])
        res = acc[:3] + [ab, y]
        ym = y[0:mem]
        put_mem([t[0:mem] for t in res[:4]] + [ym + pltpu.roll(ym, 64, 1)])
        for n in range(5):
            b_s[r0:r0 + seg, n * 128:(n + 1) * 128] = res[n][mem:rows]

    def emit_tile(j):
        gm = gm_s[j]
        for n in range(5):
            bt = b_s[:, n * 128:(n + 1) * 128].T
            if n == 4:
                bt = bt[0:64] + bt[64:128]
            nr = bt.shape[0]
            gmr = jnp.concatenate([gm] * (nr // 8), axis=0)
            out_v[j, n * 128:n * 128 + nr, :] = (
                ga_s[j, n * 128:n * 128 + nr, :] + gmr * bt).astype(out_v.dtype)

    def b_body(j, carry):
        emit_tile(jnp.maximum(j - 1, 0))
        for u in range(spt):
            b_step(pl.multiple_of(j * LANES + u * seg, seg), u * seg)

        @pl.when(j > 0)
        def _():
            cp_out(j - 1).start()

        return carry

    lax.fori_loop(0, nt, b_body, 0)
    emit_tile(nt - 1)
    cp_out(nt - 1).start()
    for j in range(nt):
        cp_out(j).wait()


@functools.partial(jax.jit, static_argnames=("B_seg_len",))
def pallas_gated_mix__sliding_local_dilated__memory_aug_recurrent_mem_tr__prompt_kernel(
    A_x: jax.Array,
    A_wqkv: jax.Array,
    A_wo: jax.Array,
    B_x: jax.Array,
    B_mem0: jax.Array,
    B_Wq: jax.Array,
    B_Wk: jax.Array,
    B_Wv: jax.Array,
    B_Wo: jax.Array,
    B_seg_len: int,
    gate_w: jax.Array,
):
    del B_x
    batch, seq, width = A_x.shape
    mem, seg = B_mem0.shape[1], int(B_seg_len)
    nt = seq // LANES
    assert batch == 1 and width == D and seq % LANES == 0 and nt <= NP + 1
    assert B_Wq.shape == (D, HB, DB) and mem % 8 == 0 and seg % 8 == 0 and LANES % seg == 0

    hbm = pl.BlockSpec(memory_space=pl.ANY)
    vmem = pl.BlockSpec(memory_space=pltpu.VMEM)
    out_t = pl.pallas_call(
        functools.partial(_kernel, seq=seq, seg=seg, mem=mem),
        out_shape=jax.ShapeDtypeStruct((D, seq), A_x.dtype),
        in_specs=[hbm, hbm, hbm, vmem, hbm, hbm, hbm, hbm, vmem],
        out_specs=hbm,
        scratch_shapes=[
            pltpu.VMEM((nt, D, LANES), BF16),
            pltpu.VMEM((D, 3 * D), BF16),
            pltpu.VMEM((D, D), BF16),
            pltpu.VMEM((3, NP, D, DB), U32),
            pltpu.VMEM((HB, D, DB), BF16),
            pltpu.VMEM((5, 3 * D, LANES), F32),
            pltpu.VMEM((NG * 9, RA + 8, LANES), F32),
            pltpu.VMEM((9, D // 2, LANES), F32),
            pltpu.VMEM((NG, 2, DA // 2, 8, LANES), U32),
            pltpu.VMEM((D // 2, LANES), U32),
            pltpu.VMEM((NP, 3, 9, 64, LANES), U32),
            pltpu.VMEM((NP, 9, 64, LANES), U32),
            pltpu.VMEM((seq, 6 * LANES), F32),
            pltpu.VMEM((nt, D, LANES), F32),
            pltpu.VMEM((nt, 8, LANES), F32),
            pltpu.VMEM((mem + seg, 6 * LANES), F32),
            pltpu.VMEM((LANES, 5 * LANES), F32),
            pltpu.VMEM((nt, D, LANES), A_x.dtype),
            pltpu.SemaphoreType.DMA((nt,)),
            pltpu.SemaphoreType.DMA((6,)),
            pltpu.SemaphoreType.DMA((4, NP)),
            pltpu.SemaphoreType.DMA((nt,)),
        ],
        compiler_params=pltpu.CompilerParams(vmem_limit_bytes=110 * 1024 * 1024),
        name="gated_mix_kernel",
    )(A_x[0].T, A_wqkv, A_wo, B_mem0[0], B_Wq, B_Wk, B_Wv, B_Wo.transpose(0, 2, 1), gate_w)
    return out_t.T[None]
```

```python
import functools

import jax
import jax.numpy as jnp
from jax import lax
import jax.experimental.pallas as pl
import jax.experimental.pallas.tpu as pltpu

F32, BF16, U32 = jnp.float32, jnp.bfloat16, jnp.uint32

D = 576
LANES = 128
HA, DA = 32, 18
WIN, DIL = 8, 2
HB, DB = 32, 128
NP = HB // 2
NEG = -1000000000.0
NG = HA // 8
RA = 3 * (DA // 2) * 8


def _dot(a, b):
    return lax.dot_general(a, b, (((1,), (0,)), ((), ())), preferred_element_type=F32)


def _dot_nt(a, b):
    return lax.dot_general(a, b, (((1,), (1,)), ((), ())), preferred_element_type=F32)


def _low_half(rows):
    return lax.broadcasted_iota(jnp.int32, (rows, LANES), 1) < 64


def _pair_tiles(w1, w2):
    a1, b1, c1 = w1[384:448], w1[448:512], w1[512:576]
    a2, b2, c2 = w2[384:448], w2[448:512], w2[512:576]
    cat = lambda u, v: jnp.concatenate([u, v], axis=0)
    sub = lambda u, v: (u.astype(F32) - v.astype(F32)).astype(u.dtype)
    return ([w1[i * 128:(i + 1) * 128] for i in range(3)] + [cat(c1, sub(b1, b2))]
            + [w2[i * 128:(i + 1) * 128] for i in range(3)] + [cat(sub(a2, a1), c2)]
            + [cat(a1, b2)])


def _pair_lhs(t1, t2):
    lo = _low_half(t1[0].shape[0])
    diff = t1[3] - t2[3]
    return (t1[:3] + [jnp.where(lo, t1[4], diff)]
            + t2[:3] + [jnp.where(lo, -diff, t2[4])]
            + [jnp.where(lo, t1[3], t2[3])])


def _pair_rhs(x):
    a, b, c = x[384:448], x[448:512], x[512:576]
    cat = lambda u, v: jnp.concatenate([u, v], axis=0)
    return [x[i * 128:(i + 1) * 128] for i in range(3)] + [cat(c, b), cat(a, c), x[384:512]]


def _pair_matmul(lhs, rhs):
    z = _dot(lhs(8), rhs[5])
    o1, o2 = z, z
    for i in range(4):
        o1 = o1 + _dot(lhs(i), rhs[i])
    for i in range(4):
        o2 = o2 + _dot(lhs(4 + i), rhs[i if i < 3 else 4])
    return o1, o2


def _kernel(xt_hbm, wqkv_hbm, wo_hbm, mem0_ref, wq_hbm, wk_hbm, wv_hbm, wot_hbm, gate_ref,
            out_hbm,
            xt_v, wqkv_v, wo_v, stg_qkv, stg_o, wt32, la, lo_a, kv_prev, oa_s,
            wb, wob, x32, ga_s, gm_s, h_s, b_s, out_v,
            sem_x, sem_wa, sem_wb, sem_out, *, seq, seg, mem):
    nt = seq // LANES
    rows = mem + seg
    spt = LANES // seg

    def cp_x(j):
        col = j * LANES if isinstance(j, int) else pl.multiple_of(j * LANES, LANES)
        return pltpu.make_async_copy(xt_hbm.at[:, pl.ds(col, LANES)], xt_v.at[j], sem_x.at[j])

    def cp_wqkv(k):
        r = pl.ds(k * 128, min(128, D - k * 128))
        return pltpu.make_async_copy(wqkv_hbm.at[r], wqkv_v.at[r], sem_wa.at[k])

    cp_wo = pltpu.make_async_copy(wo_hbm, wo_v, sem_wa.at[5])

    def cp_wb(i, p):
        if i == 3:
            return pltpu.make_async_copy(wot_hbm.at[pl.ds(2 * p, 2)], stg_o.at[pl.ds(2 * p, 2)],
                                         sem_wb.at[3, p])
        src = (wq_hbm, wk_hbm, wv_hbm)[i].bitcast(U32)
        return pltpu.make_async_copy(src.at[:, p, :], stg_qkv.at[i, p], sem_wb.at[i, p])

    def cp_out(j):
        col = j * LANES if isinstance(j, int) else pl.multiple_of(j * LANES, LANES)
        return pltpu.make_async_copy(out_v.at[j], out_hbm.at[:, pl.ds(col, LANES)], sem_out.at[j])

    def start_pair(p):
        for i in range(4):
            cp_wb(i, p).start()

    for k in range(5):
        cp_wqkv(k).start()
    cp_x(0).start()
    cp_wo.start()

    gate = jnp.broadcast_to(gate_ref[...].astype(F32).reshape(1, D), (8, D))
    gate_t = [gate[:, i * 128:(i + 1) * 128] for i in range(4)]
    gate_t.append(jnp.concatenate([gate[:, 512:], gate[:, 512:]], axis=1))

    for k in range(5):
        cp_wqkv(k).wait()
        if k < 4:
            blk = wqkv_v[k * 128:(k + 1) * 128, :]
        else:
            blk = jnp.concatenate([wqkv_v[512:D, :]] * 2, axis=0)
        if k == 4:
            cp_x(1).start()
            start_pair(0)
            start_pair(1)
        wt32[k] = blk.T.astype(F32)

    for g in range(NG):
        for part in range(3):
            for dd in range(DA // 2):
                base = part * D + g * 8 * DA + 2 * dd
                t1 = [wt32[k, pl.ds(base, 8, stride=DA), :] for k in range(5)]
                t2 = [wt32[k, pl.ds(base + 1, 8, stride=DA), :] for k in range(5)]
                r0 = (part * (DA // 2) + dd) * 8
                for i, t in enumerate(_pair_lhs(t1, t2)):
                    la[g * 9 + i, r0:r0 + 8, :] = t
    for i, t in enumerate(_pair_lhs(gate_t, gate_t)):
        la[i, RA:RA + 8, :] = t

    cp_wo.wait()
    wo32 = wo_v[...].astype(F32)
    for n in range(4):
        wt32[n, 0:D, :] = wo32[:, n * 128:(n + 1) * 128]
    wt32[4, 0:D, :] = jnp.concatenate([wo32[:, 512:], wo32[:, 512:]], axis=1)
    perm = [jnp.concatenate([wt32[n, pl.ds(g * 8 * DA + d, 8, stride=DA), :]
                             for g in range(NG) for d in range(DA)], axis=0) for n in range(5)]
    tiles = []
    for k in range(5):
        if k < 4:
            pk = [pn[k * 128:(k + 1) * 128] for pn in perm]
        else:
            pk = [jnp.concatenate([pn[512:], pn[512:]], axis=0) for pn in perm]
        tiles.append(jnp.concatenate([t.T for t in pk[:4]] + [pk[4].T[:64]], axis=0))
    for i, t in enumerate(_pair_lhs([t[:D // 2] for t in tiles], [t[D // 2:] for t in tiles])):
        lo_a[i] = t

    def prep_pair(p):
        hi_mask = jnp.uint32(0xFFFF0000)
        low = lambda e, o: (e & ~hi_mask) | (o << 16)
        high = lambda e, o: (e >> 16) | (o & hi_mask)
        rnd = lambda t: pltpu.bitcast(t.astype(BF16).astype(F32), U32)
        w1 = lambda u: pltpu.bitcast(u << 16, F32)
        w2 = lambda u: pltpu.bitcast(u & hi_mask, F32)
        for i in range(3):
            for c in range(9):
                ev = stg_qkv[i, p, pl.ds(c * 64, 32, stride=2), :]
                od = stg_qkv[i, p, pl.ds(c * 64 + 1, 32, stride=2), :]
                half = pl.ds((c % 2) * 32, 32)
                if c < 6:
                    wb[p, i, c // 2, half, :] = low(ev, od)
                    wb[p, i, 4 + c // 2, half, :] = high(ev, od)
                elif c == 6:
                    wb[p, i, 8, 0:32, :] = low(ev, od)
                    wb[p, i, 7, 0:32, :] = high(rnd(w2(ev) - w1(ev)), rnd(w2(od) - w1(od)))
                elif c == 7:
                    wb[p, i, 8, 32:64, :] = high(ev, od)
                    wb[p, i, 3, 32:64, :] = high(rnd(w1(ev) - w2(ev)), rnd(w1(od) - w2(od)))
                else:
                    wb[p, i, 3, 0:32, :] = low(ev, od)
                    wb[p, i, 7, 32:64, :] = high(ev, od)
        for t, tile in enumerate(_pair_tiles(stg_o[2 * p], stg_o[2 * p + 1])):
            wob[p, t] = pltpu.bitcast(tile.T, U32)

    def wait_pair(p):
        for i in range(4):
            cp_wb(i, p).wait()

    lane = lax.broadcasted_iota(jnp.int32, (8, LANES), 1)

    def pack(even, odd):
        return pltpu.bitcast(jnp.concatenate([even, odd], axis=0).astype(BF16), U32)

    def shifted(prev, cur, w):
        if w > 0:
            cur = pltpu.roll(jnp.where(lane >= LANES - DIL * w, prev, cur), DIL * w, 1)
        both = pltpu.bitcast(cur, BF16).astype(F32)
        return both[0:8], both[8:16]

    def a_heads(j, first):
        rhs = _pair_rhs(xt_v[j])
        t0 = j * LANES if isinstance(j, int) else pl.multiple_of(j * LANES, LANES)
        for i in range(6):
            x32[pl.ds(t0, LANES), i * 128:(i + 1) * 128] = rhs[i].T.astype(F32)
        gsig, outs = None, []
        rp = RA // 3
        for g in range(NG):
            parts = []
            for part in range(3):
                nr = rp + 8 if (g, part) == (0, 2) else rp
                parts.append(_pair_matmul(
                    lambda i: la[g * 9 + i, part * rp:part * rp + nr, :], rhs))
            if g == 0:
                gsig = 1.0 / (1.0 + jnp.exp(-parts[2][0][rp:rp + 8]))
            get = lambda part, dd: [t[dd * 8:dd * 8 + 8] for t in parts[part]]

            logit = [None] * WIN
            for dd in range(DA // 2):
                q, k = get(0, dd), pack(*get(1, dd))
                kp = k if first else kv_prev[g, 0, dd]
                for w in range(WIN):
                    ks = shifted(kp, k, w)
                    t = q[0] * ks[0] + q[1] * ks[1]
                    logit[w] = t if dd == 0 else logit[w] + t
                kv_prev[g, 0, dd] = k
            logit = [t * (DA ** -0.5) for t in logit]
            if first:
                logit = [jnp.where(lane >= DIL * w, t, NEG) for w, t in enumerate(logit)]
            mx = functools.reduce(jnp.maximum, logit)
            ex = [jnp.exp(t - mx) for t in logit]
            inv = gsig / functools.reduce(jnp.add, ex)
            prob = [e * inv for e in ex]
            for dd in range(DA // 2):
                v = pack(*get(2, dd))
                vp = jnp.broadcast_to(v[:, 0:1], (8, LANES)) if first else kv_prev[g, 1, dd]
                o = [None, None]
                for w in range(WIN):
                    vs = shifted(vp, v, w)
                    o = [prob[w] * vs[i] if w == 0 else o[i] + prob[w] * vs[i] for i in range(2)]
                kv_prev[g, 1, dd] = v
                outs.append(pack(*o))
        gm_s[j] = 1.0 - gsig
        return jnp.concatenate(outs, axis=0)

    def a_out(j):
        rhs = _pair_rhs(pltpu.bitcast(oa_s[...], BF16))
        rp = D // 8
        for c in range(4):
            halves = _pair_matmul(lambda i: lo_a[i, c * rp:(c + 1) * rp, :], rhs)
            ga_s[j, c * rp:(c + 1) * rp, :] = halves[0]
            ga_s[j, D // 2 + c * rp:D // 2 + (c + 1) * rp, :] = halves[1]

    cp_x(0).wait()
    oa_s[...] = a_heads(0, True)

    def a_body(j, carry):
        @pl.when(j + 1 < nt)
        def _():
            cp_x(j + 1).start()
            start_pair(j + 1)

        cp_x(j).wait()
        wait_pair(j - 1)
        o = a_heads(j, False)
        a_out(j - 1)
        oa_s[...] = o
        prep_pair(j - 1)
        return carry

    lax.fori_loop(1, nt, a_body, 0)
    for p in range(nt - 1, NP):
        wait_pair(p)
    a_out(nt - 1)
    for p in range(nt - 1, NP):
        prep_pair(p)

    def put_mem(t):
        lo = _low_half(mem)
        for i in range(3):
            h_s[0:mem, i * 128:(i + 1) * 128] = t[i]
        h_s[0:mem, 384:512] = jnp.where(lo, t[4], t[3])
        h_s[0:mem, 512:640] = jnp.where(lo, t[3], t[4])
        h_s[0:mem, 640:768] = t[3]

    m0 = mem0_ref[...].astype(F32)
    put_mem([m0[:, i * 128:(i + 1) * 128] for i in range(4)]
            + [jnp.concatenate([m0[:, 512:], m0[:, 512:]], axis=1)])
    b_s[...] = jnp.zeros(b_s.shape, F32)

    qi = lax.broadcasted_iota(jnp.int32, (rows, rows), 0)
    ki = lax.broadcasted_iota(jnp.int32, (rows, rows), 1)
    mask = (qi < mem) | (qi >= ki)

    def b_step(t0, r0):
        h_s[mem:rows, :] = x32[pl.ds(t0, seg), :]
        qkv, soft, outs = {}, {}, {}
        acc = [None] * 6

        lhs = lambda c: h_s[:, c * 128:(c + 1) * 128]

        def project(p, *which):
            w = lambda i, t: pltpu.bitcast(wb[p, i, t], BF16)
            o = {}
            for i in which:
                z = _dot(lhs(5), w(i, 8))
                for hh in range(2):
                    o[i, hh] = z + _dot(lhs(3 + hh), w(i, 4 * hh + 3))
            for c in range(3):
                for i in which:
                    for hh in range(2):
                        o[i, hh] = o[i, hh] + _dot(lhs(c), w(i, 4 * hh + c))
            for (i, hh), t in o.items():
                qkv[2 * p + hh, i] = t if i == 0 else t.astype(BF16)

        def scores(p):
            for h in (2 * p, 2 * p + 1):
                s = jnp.where(mask, _dot_nt(qkv[h, 0], qkv[h, 1]) * (DB ** -0.5), NEG)
                e = jnp.exp(s - jnp.max(s, axis=-1, keepdims=True))
                soft[h] = (e, jnp.sum(e, axis=-1, keepdims=True))

        def values(p):
            for h in (2 * p, 2 * p + 1):
                e, l = soft[h]
                outs[h] = _dot(e, qkv[h, 2]) * (1.0 / l)

        def out_proj(pairs, cols=range(6)):
            for n in cols:
                tot = None
                for p in pairs:
                    o1, o2 = outs[2 * p], outs[2 * p + 1]
                    w = lambda t: pltpu.bitcast(wob[p, t], BF16)
                    if n < 3:
                        r = _dot(o1, w(n)) + _dot(o2, w(4 + n))
                    else:
                        r = _dot((o1, o2, o1 + o2)[n - 3], w((3, 7, 8)[n - 3]))
                    tot = r if tot is None else tot + r
                acc[n] = tot if acc[n] is None else acc[n] + tot

        lag, last = 8, 4
        project(0, 0, 1)
        project(0, 2)
        for p in range(1, NP):
            project(p, 0)
            project(p, 1)
            scores(p - 1)
            project(p, 2)
            if p >= 2:
                values(p - 2)
            if p >= lag:
                out_proj([p - lag])
        scores(NP - 1)
        out_proj([NP - lag])
        values(NP - 2)
        for p in range(NP - lag + 1, NP - last):
            out_proj([p])
        values(NP - 1)
        tail = list(range(NP - last, NP))
        out_proj(tail[:-1], [3, 4, 5, 0])
        out_proj(tail[-1:], [3, 4, 5, 0])
        out_proj(tail, [1, 2])

        lo = _low_half(rows)
        ab = acc[5] + jnp.where(lo, acc[4], acc[3])
        y = jnp.where(lo, acc[3], acc[4])
        res = acc[:3] + [ab, y]
        ym = y[0:mem]
        put_mem([t[0:mem] for t in res[:4]] + [ym + pltpu.roll(ym, 64, 1)])
        for n in range(5):
            b_s[r0:r0 + seg, n * 128:(n + 1) * 128] = res[n][mem:rows]

    def emit_tile(j):
        gm = gm_s[j]
        for n in range(5):
            bt = b_s[:, n * 128:(n + 1) * 128].T
            if n == 4:
                bt = bt[0:64] + bt[64:128]
            nr = bt.shape[0]
            gmr = jnp.concatenate([gm] * (nr // 8), axis=0)
            out_v[j, n * 128:n * 128 + nr, :] = (
                ga_s[j, n * 128:n * 128 + nr, :] + gmr * bt).astype(out_v.dtype)

    def b_body(j, carry):
        emit_tile(jnp.maximum(j - 1, 0))
        for u in range(spt):
            b_step(pl.multiple_of(j * LANES + u * seg, seg), u * seg)

        @pl.when(j > 0)
        def _():
            cp_out(j - 1).start()

        return carry

    lax.fori_loop(0, nt, b_body, 0)
    emit_tile(nt - 1)
    cp_out(nt - 1).start()
    for j in range(nt):
        cp_out(j).wait()


@functools.partial(jax.jit, static_argnames=("B_seg_len",))
def pallas_gated_mix__sliding_local_dilated__memory_aug_recurrent_mem_tr__prompt_kernel(
    A_x: jax.Array,
    A_wqkv: jax.Array,
    A_wo: jax.Array,
    B_x: jax.Array,
    B_mem0: jax.Array,
    B_Wq: jax.Array,
    B_Wk: jax.Array,
    B_Wv: jax.Array,
    B_Wo: jax.Array,
    B_seg_len: int,
    gate_w: jax.Array,
):
    del B_x
    batch, seq, width = A_x.shape
    mem, seg = B_mem0.shape[1], int(B_seg_len)
    nt = seq // LANES
    assert batch == 1 and width == D and seq == NP * LANES
    assert B_Wq.shape == (D, HB, DB) and mem % 8 == 0 and seg % 8 == 0 and LANES % seg == 0

    hbm = pl.BlockSpec(memory_space=pl.ANY)
    vmem = pl.BlockSpec(memory_space=pltpu.VMEM)
    out_t = pl.pallas_call(
        functools.partial(_kernel, seq=seq, seg=seg, mem=mem),
        out_shape=jax.ShapeDtypeStruct((D, seq), A_x.dtype),
        in_specs=[hbm, hbm, hbm, vmem, hbm, hbm, hbm, hbm, vmem],
        out_specs=hbm,
        scratch_shapes=[
            pltpu.VMEM((nt, D, LANES), BF16),
            pltpu.VMEM((D, 3 * D), BF16),
            pltpu.VMEM((D, D), BF16),
            pltpu.VMEM((3, NP, D, DB), U32),
            pltpu.VMEM((HB, D, DB), BF16),
            pltpu.VMEM((5, 3 * D, LANES), F32),
            pltpu.VMEM((NG * 9, RA + 8, LANES), F32),
            pltpu.VMEM((9, D // 2, LANES), F32),
            pltpu.VMEM((NG, 2, DA // 2, 8, LANES), U32),
            pltpu.VMEM((D // 2, LANES), U32),
            pltpu.VMEM((NP, 3, 9, 64, LANES), U32),
            pltpu.VMEM((NP, 9, 64, LANES), U32),
            pltpu.VMEM((seq, 6 * LANES), F32),
            pltpu.VMEM((nt, D, LANES), F32),
            pltpu.VMEM((nt, 8, LANES), F32),
            pltpu.VMEM((mem + seg, 6 * LANES), F32),
            pltpu.VMEM((LANES, 5 * LANES), F32),
            pltpu.VMEM((nt, D, LANES), A_x.dtype),
            pltpu.SemaphoreType.DMA((nt,)),
            pltpu.SemaphoreType.DMA((6,)),
            pltpu.SemaphoreType.DMA((4, NP)),
            pltpu.SemaphoreType.DMA((nt,)),
        ],
        compiler_params=pltpu.CompilerParams(vmem_limit_bytes=110 * 1024 * 1024),
        name="gated_mix_kernel",
    )(A_x[0].T, A_wqkv, A_wo, B_mem0[0], B_Wq, B_Wk, B_Wv, B_Wo.transpose(0, 2, 1), gate_w)
    return out_t.T[None]
```

```python
import functools

import jax
import jax.numpy as jnp
import numpy as np
from jax import lax
import jax.experimental.pallas as pl
import jax.experimental.pallas.tpu as pltpu

F32, BF16, U32 = jnp.float32, jnp.bfloat16, jnp.uint32

D = 576
LANES = 128
HA, DA = 32, 18
WIN, DIL = 8, 2
HB, DB = 32, 128
NP = HB // 2
NEG = -1000000000.0
LOG2E = 1.4426950408889634
NG = HA // 8
RA = 3 * (DA // 2) * 8

KB, GB, SUB = 4, 8, 16

_HK = (
    (".... +...", "+.-. -... .... ....", "+... +..."),
    ("+... -...", "+-.. .... -... ....", "+... ...."),
    (".+.. .-..", ".... +-.+ .+.. ....", ".... .+.."),
    (".+.. ....", ".-.. .+-. .... .-..", ".+.. .+.."),
    (".... ..+.", "...+ ..-. -.+- ....", ".... ..+."),
    ("..+. ....", "..-. .... .-+. +.-.", "..+. ...."),
    (".... ...+", "...- ...- .... +.-+", "...+ ...+"),
    ("...+ ...-", "...+ .... ...- --.+", "...+ ...."),
    (".... ++..", ".... +... .... ....", ".... ++.."),
    ("++.. ....", ".+.. .... .... ....", "++.. ...."),
    (".+.. +...", ".-.. +... .... ....", "+... .-.."),
    ("+.+. -.-.", "...+ .... -... ....", ".... +.+."),
    ("+.+. ....", "..+. .... .... -...", "+.+. +.+."),
    ("+.+. -...", "..-. .... +... ....", "+... +.+."),
    (".... .++.", ".... ..+. .... ....", ".++. .++."),
    (".++. .--.", ".... .... .+.. ....", ".++. ...."),
    (".+.. .--.", ".... ..+. .-.. ....", ".++. .+.."),
    (".... .+.+", ".... ...+ .... ....", ".... .+.+"),
    (".+.+ ....", ".... .... .... .+..", ".+.+ ...."),
    (".+.. ...+", ".... ...+ .... .-..", "...+ .-.."),
    ("..++ ..--", "...+ .... ...- ....", ".... ..++"),
    ("..++ ....", ".... .... .... -.+.", "..++ ..++"),
    ("..++ ...-", "...- .... ...+ +.-.", "...+ ..++"),
    (".... +.++", "...+ .... .... ....", ".... +.++"),
    ("+.++ ....", ".... .... .... +...", "+.++ ...."),
    ("+.+. ...+", "...+ .... .... -...", "...+ -.-."),
)
_U, _V, _C = (np.array([[["-.+".index(ch) - 1 for ch in row] for row in prod[i].split()]
                        for prod in _HK]) for i in range(3))
NR = len(_HK)
assert np.array_equal(np.einsum("rak,rln,rbm->akblnm", _U, _V, _C),
                      np.einsum("ab,kl,nm->akblnm", *(np.eye(n, dtype=int) for n in (2, KB, KB))))


def _phase(products):
    tiles = [max(r, ~r) for r in products]
    dual = np.rint(np.linalg.inv(_V[tiles].reshape(len(tiles), -1)).T).astype(int)
    slots = []
    for r, d in zip(products, dual.reshape(-1, KB, KB)):
        i, j = np.argwhere(d)[0]
        a, c = d[:, j] * d[i, j], d[i]
        assert np.array_equal(np.outer(a, c), d)
        slots.append(dict(r=max(r, ~r), tok=r >= 0, a=a.tolist(), c=c.tolist()))
    return slots


_PHASES = (_phase((18, 15, ~10, 7, 5, 25, 24, ~16, 12, 13, 0, 20, ~21, 17, 8, 2)),
           _phase((23, 11, ~13, 4, 22, 6, 21, ~18, 19, 14, 16, 3, ~25, 10, 9, 1)))
assert sorted(s["r"] for ph in _PHASES for s in ph if s["tok"]) == list(range(NR))


def _signed_sum(terms):
    terms = [(c, t) for c, t in terms if c]
    first = next((i for i, (c, _) in enumerate(terms) if c > 0), 0)
    c, acc = terms.pop(first)
    acc = acc if c > 0 else -acc
    for c, t in terms:
        acc = acc + t if c > 0 else acc - t
    return acc


class _Mixer:
    def __init__(self, block):
        self.block, self.known = block, {}

    def __call__(self, coef):
        want = {(i, k): int(c) for i, row in enumerate(coef) for k, c in enumerate(row) if c}
        key = tuple(sorted(want.items()))
        if key not in self.known:
            terms = []
            for have in sorted(self.known, key=lambda h: -len(h)):
                for sign in (1, -1):
                    if all(want.get(pos) == sign * c for pos, c in have):
                        terms.append((sign, self.known[have]))
                        want = {pos: c for pos, c in want.items() if pos not in dict(have)}
                        break
            for pos, c in sorted(want.items()):
                self.known[((pos, 1),)] = self.block(*pos)
                terms.append((c, self.known[((pos, 1),)]))
            self.known[key] = _signed_sum(terms)
        return self.known[key]


class _Carry:
    def __init__(self, ref):
        self.ref, self.val = ref, {}

    def __getitem__(self, key):
        return self.val[key] if key in self.val else self.ref[key]

    def __setitem__(self, key, value):
        self.val[key] = value

    def flush(self):
        for key, value in self.val.items():
            self.ref[key] = value
        self.val = {}


def _weave(passes, slots):
    keyed = []
    for tok in (True, False):
        some = [p for p in passes if slots[p[0]]["tok"] == tok]
        keyed += [((i + 0.5) / len(some), p) for i, p in enumerate(some)]
    return [p for _, p in sorted(keyed, key=lambda kp: kp[0])]


def _dot(a, b):
    return lax.dot_general(a, b, (((1,), (0,)), ((), ())), preferred_element_type=F32)


def _dot_nt(a, b):
    return lax.dot_general(a, b, (((1,), (1,)), ((), ())), preferred_element_type=F32)


def _low_half(rows):
    return lax.broadcasted_iota(jnp.int32, (rows, LANES), 1) < 64


def _pair_lhs(t1, t2):
    lo = _low_half(t1[0].shape[0])
    diff = t1[3] - t2[3]
    return (t1[:3] + [jnp.where(lo, t1[4], diff)]
            + t2[:3] + [jnp.where(lo, -diff, t2[4])]
            + [jnp.where(lo, t1[3], t2[3])])


def _pair_rhs(x):
    a, b, c = x[384:448], x[448:512], x[512:576]
    cat = lambda u, v: jnp.concatenate([u, v], axis=0)
    return [x[i * 128:(i + 1) * 128] for i in range(3)] + [cat(c, b), cat(a, c), x[384:512]]


def _pair_matmul(lhs, rhs):
    z = _dot(lhs(8), rhs[5])
    o1, o2 = z, z
    for i in range(4):
        o1 = o1 + _dot(lhs(i), rhs[i])
    for i in range(4):
        o2 = o2 + _dot(lhs(4 + i), rhs[i if i < 3 else 4])
    return o1, o2


def _kernel(xt_hbm, wqkv_hbm, wo_hbm, mem0_ref, wq_hbm, wk_hbm, wv_hbm, wot_hbm, gate_ref,
            out_hbm,
            xt_v, wqkv_v, wo_v, stg_qkv, stg_o, wt32, la, lo_a, kv_prev, oa_s,
            z_s, wb, wob, x32, ga_s, gm_s, mem_s, zero_s, part_s, zpart_s, o_s, opart_s, b_s, out_v,
            sem_x, sem_wa, sem_wb, sem_out, *, seq, seg, mem):
    nt = seq // LANES
    rows = mem + seg

    def cp_x(j):
        col = j * LANES if isinstance(j, int) else pl.multiple_of(j * LANES, LANES)
        return pltpu.make_async_copy(xt_hbm.at[:, pl.ds(col, LANES)], xt_v.at[j], sem_x.at[j % 2])

    def cp_wqkv(k):
        r = pl.ds(k * 128, min(128, D - k * 128))
        return pltpu.make_async_copy(wqkv_hbm.at[r], wqkv_v.at[r], sem_wa.at[k])

    cp_wo = pltpu.make_async_copy(wo_hbm, wo_v, sem_wa.at[5])

    def cp_wb(i, third):
        r0 = third * (D // 3)
        r = pl.ds(r0 if isinstance(third, int) else pl.multiple_of(r0, D // 3), D // 3)
        if i == 3:
            return [pltpu.make_async_copy(wot_hbm.at[:, r, :], stg_o.at[:, r, :], sem_wb.at[third])]
        src = (wq_hbm, wk_hbm, wv_hbm)[i].bitcast(U32)
        return [pltpu.make_async_copy(src.at[r, p, :], stg_qkv.at[i, p, r, :], sem_wb.at[third])
                for p in range(NP)]

    def each_wb(chunk, act):
        for i in range(4):
            @pl.when((chunk >= 3 * i) & (chunk < 3 * i + 3))
            def _():
                for c in cp_wb(i, chunk - 3 * i):
                    act(c)

    def cp_out(j):
        col = j * LANES if isinstance(j, int) else pl.multiple_of(j * LANES, LANES)
        return pltpu.make_async_copy(out_v.at[j], out_hbm.at[:, pl.ds(col, LANES)], sem_out)

    for k in range(5):
        cp_wqkv(k).start()
    cp_x(0).start()
    cp_wo.start()

    gate = jnp.broadcast_to(gate_ref[...].astype(F32).reshape(1, D), (8, D))
    gate_t = [gate[:, i * 128:(i + 1) * 128] for i in range(4)]
    gate_t.append(jnp.concatenate([gate[:, 512:], gate[:, 512:]], axis=1))

    for k in range(5):
        cp_wqkv(k).wait()
        if k < 4:
            blk = wqkv_v[k * 128:(k + 1) * 128, :]
        else:
            blk = jnp.concatenate([wqkv_v[512:D, :]] * 2, axis=0)
        if k == 4:
            cp_x(1).start()
            for c in cp_wb(0, 0) + cp_wb(0, 1):
                c.start()
        wt32[k] = blk.T.astype(F32)

    for g in range(NG):
        for part in range(3):
            for dd in range(DA // 2):
                base = part * D + g * 8 * DA + 2 * dd
                t1 = [wt32[k, pl.ds(base, 8, stride=DA), :] for k in range(5)]
                t2 = [wt32[k, pl.ds(base + 1, 8, stride=DA), :] for k in range(5)]
                r0 = (part * (DA // 2) + dd) * 8
                for i, t in enumerate(_pair_lhs(t1, t2)):
                    la[g * 9 + i, r0:r0 + 8, :] = t
    for i, t in enumerate(_pair_lhs(gate_t, gate_t)):
        la[i, RA:RA + 8, :] = t

    cp_wo.wait()
    wo32 = wo_v[...].astype(F32)
    for n in range(4):
        wt32[n, 0:D, :] = wo32[:, n * 128:(n + 1) * 128]
    wt32[4, 0:D, :] = jnp.concatenate([wo32[:, 512:], wo32[:, 512:]], axis=1)
    perm = [jnp.concatenate([wt32[n, pl.ds(g * 8 * DA + d, 8, stride=DA), :]
                             for g in range(NG) for d in range(DA)], axis=0) for n in range(5)]
    tiles = []
    for k in range(5):
        if k < 4:
            pk = [pn[k * 128:(k + 1) * 128] for pn in perm]
        else:
            pk = [jnp.concatenate([pn[512:], pn[512:]], axis=0) for pn in perm]
        tiles.append(jnp.concatenate([t.T for t in pk[:4]] + [pk[4].T[:64]], axis=0))
    for i, t in enumerate(_pair_lhs([t[:D // 2] for t in tiles], [t[D // 2:] for t in tiles])):
        lo_a[i] = t

    by_size = sorted(range(NR), key=lambda r: int(np.abs(_V[r]).sum()))

    def prep_qkv(i, j, slot):
        inner = j < GB
        for e in range(GB):
            g = (j + e) % GB

            def block(kk, nu):
                u = stg_qkv[i, 2 * g + nu // 2, pl.ds(pl.multiple_of(64 * j + SUB * kk, SUB), SUB), :]
                return pltpu.bitcast(u & jnp.uint32(0xFFFF0000) if nu % 2 else u << 16, F32)

            mix = _Mixer(block)
            tile = jnp.where(inner, 0, 1 + g) if e == 0 else 1 + g
            at = pl.ds(pl.multiple_of(jnp.where(inner, j, g) * 8, 8), 8)
            for r in by_size:
                if e == 0:
                    w = mix(_V[r]).astype(BF16)
                    z_s[slot, r] = jnp.where(inner, w.astype(F32), 0.0)
                else:
                    w = (mix(_V[r]) - z_s[slot, r]).astype(BF16)
                wb[i, r, tile, at, :] = pltpu.bitcast(w, U32)

    def prep_out():
        def source(group_of, sub_of):
            return {(kk, nu): jnp.concatenate(
                [stg_o[KB * group_of(j) + kk, pl.ds(SUB * (KB * sub_of(j) + nu), SUB), :]
                 for j in range(GB)], axis=0).T for kk in range(KB) for nu in range(KB)}

        lane_sub = lax.broadcasted_iota(jnp.int32, (8, LANES), 1) // SUB
        for g in range(-1, GB):
            if g < 0:
                src = source(lambda j: j, lambda j: j)
            else:
                src = source(lambda j: g, lambda j: GB if j == g else j)
            for e in range(DB // 16):
                mix = _Mixer(lambda kk, nu: src[kk, nu][16 * e:16 * e + 16].astype(F32))
                for r in by_size:
                    w = mix(_V[r])
                    if g >= 0:
                        z = jnp.where(lane_sub == g, jnp.uint32(0), wob[r, 0, 8 * e:8 * e + 8, :])
                        w = w - pltpu.bitcast(z, BF16).astype(F32)
                    wob[r, 1 + g, 8 * e:8 * e + 8, :] = pltpu.bitcast(w.astype(BF16), U32)

    lane = lax.broadcasted_iota(jnp.int32, (8, LANES), 1)

    def pack(even, odd):
        return pltpu.bitcast(jnp.concatenate([even, odd], axis=0).astype(BF16), U32)

    def shifted(prev, cur, w):
        if w > 0:
            cur = pltpu.roll(jnp.where(lane >= LANES - DIL * w, prev, cur), DIL * w, 1)
        both = pltpu.bitcast(cur, BF16).astype(F32)
        return both[0:8], both[8:16]

    def a_heads(j, first):
        xt = xt_v[j]
        rhs = _pair_rhs(xt)
        t0 = j * LANES if isinstance(j, int) else pl.multiple_of(j * LANES, LANES)
        for c in range(2):
            for kk in range(KB):
                subs = [SUB * (KB * (GB if c else e) + kk) for e in range(GB)]
                tile = jnp.concatenate([xt[r0:r0 + SUB] for r0 in subs], axis=0)
                x32[c, kk, pl.ds(t0, LANES), :] = tile.T.astype(F32)
        gsig, outs = None, []
        rp = RA // 3
        for g in range(NG):
            parts = []
            for part in range(3):
                nr = rp + 8 if (g, part) == (0, 2) else rp
                parts.append(_pair_matmul(
                    lambda i: la[g * 9 + i, part * rp:part * rp + nr, :], rhs))
            if g == 0:
                gsig = 1.0 / (1.0 + jnp.exp(-parts[2][0][rp:rp + 8]))
            get = lambda part, dd: [t[dd * 8:dd * 8 + 8] for t in parts[part]]

            logit = [None] * WIN
            for dd in range(DA // 2):
                q, k = get(0, dd), pack(*get(1, dd))
                kp = k if first else kv_prev[g, 0, dd]
                for w in range(WIN):
                    ks = shifted(kp, k, w)
                    t = q[0] * ks[0] + q[1] * ks[1]
                    logit[w] = t if dd == 0 else logit[w] + t
                kv_prev[g, 0, dd] = k
            logit = [t * (DA ** -0.5) for t in logit]
            if first:
                logit = [jnp.where(lane >= DIL * w, t, NEG) for w, t in enumerate(logit)]
            mx = functools.reduce(jnp.maximum, logit)
            ex = [jnp.exp(t - mx) for t in logit]
            inv = gsig / functools.reduce(jnp.add, ex)
            prob = [e * inv for e in ex]
            for dd in range(DA // 2):
                v = pack(*get(2, dd))
                vp = jnp.broadcast_to(v[:, 0:1], (8, LANES)) if first else kv_prev[g, 1, dd]
                o = [None, None]
                for w in range(WIN):
                    vs = shifted(vp, v, w)
                    o = [prob[w] * vs[i] if w == 0 else o[i] + prob[w] * vs[i] for i in range(2)]
                kv_prev[g, 1, dd] = v
                outs.append(pack(*o))
        gm_s[j] = 1.0 - gsig
        return jnp.concatenate(outs, axis=0)

    def a_out(j):
        rhs = _pair_rhs(pltpu.bitcast(oa_s[...], BF16))
        rp = D // 8
        for c in range(4):
            halves = _pair_matmul(lambda i: lo_a[i, c * rp:(c + 1) * rp, :], rhs)
            ga_s[j, c * rp:(c + 1) * rp, :] = halves[0]
            ga_s[j, D // 2 + c * rp:D // 2 + (c + 1) * rp, :] = halves[1]

    cp_x(0).wait()
    oa_s[...] = a_heads(0, True)

    def a_body(j, carry):
        cp_x(j).wait()

        @pl.when(j + 1 < nt)
        def _():
            cp_x(j + 1).start()

        each_wb(j - 1, lambda c: c.wait())
        each_wb(j + 1, lambda c: c.start())
        o = a_heads(j, False)
        a_out(j - 1)
        oa_s[...] = o
        for slot in range(2):
            unit = jnp.minimum(2 * (j - 1) + slot, 26)
            prep_qkv(unit // 9, unit % 9, slot)
        return carry

    lax.fori_loop(1, nt, a_body, 0)
    a_out(nt - 1)
    prep_out()

    m0 = mem0_ref[...].astype(F32)
    for c in range(2):
        for kk in range(KB):
            subs = [SUB * (KB * (GB if c else e) + kk) for e in range(GB)]
            mem_s[c, kk] = jnp.concatenate([m0[:, f0:f0 + SUB] for f0 in subs], axis=1)
    for ref in (o_s, opart_s, b_s):
        ref[...] = jnp.zeros(ref.shape, F32)
    lane_sub = lax.broadcasted_iota(jnp.int32, (8, LANES), 1) // SUB
    for i in range(3):
        zero_s[i] = lane_sub

    qi = lax.broadcasted_iota(jnp.int32, (rows, rows), 0)
    ki = lax.broadcasted_iota(jnp.int32, (rows, rows), 1)
    mask = (qi >= seg) | (ki >= seg) | (qi >= ki)
    part, zpart, o_prev, opart, b_rows = (_Carry(r) for r in (part_s, zpart_s, o_s, opart_s, b_s))
    ahead = {}

    def stack(*parts):
        parts = [t for t in parts if t is not None]
        return parts[0] if len(parts) == 1 else jnp.concatenate(parts, axis=0)

    def b_step(u, t0, memv, project_only=False, output_only=False):
        odd = u % 2
        keep = lambda slots: [s for s in slots if s["tok"] or memv is not None]
        qs, os_ = keep(_PHASES[odd]), keep(_PHASES[1 - odd])
        z_tok, z_mem, qkv, soft, o_mem, o_sum, o_diag, o_mix = {}, {}, {}, {}, {}, {}, {}, {}

        def tok_terms(slots, res, mu, nu, at):
            return [(_C[s["r"]][mu][nu], r[at]) for s, r in zip(slots, res) if s["tok"]]

        def mem_terms(slots, res, nu, at):
            return [(s["c"][nu], r[at]) for s, r in zip(slots, res)]

        if not output_only:
            x_mix = [_Mixer(functools.partial(
                lambda c, mu, kk: x32[c, kk, pl.ds(t0 + mu * seg, seg), :], c)) for c in range(2)]
            m_mix = [_Mixer(functools.partial(lambda c, _, kk: memv[c, kk], c)) for c in range(2)]
            lhs = [[stack(x_mix[c](_U[s["r"]]) if s["tok"] else None,
                          m_mix[c]([s["a"]]) if memv else None) for c in range(2)] for s in qs]

        def shared():
            ready = [max(e for e, s in enumerate(_PHASES[odd]) if s["c"][nu]) for nu in range(KB)]
            order = sorted(range(len(qs)),
                           key=lambda e: max(ready[kk] for kk in range(KB) if qs[e]["a"][kk]))
            z = {(e, i): _dot(lhs[e][0], pltpu.bitcast(wb[i, qs[e]["r"], 0], BF16))
                 for e, i in _weave([(e, i) for e in order for i in range(3)], qs)}
            for i in range(3):
                slots, res = [qs[e] for e in order], [z[e, i] for e in order]
                for nu in range(KB):
                    if memv:
                        z_mem[i, nu] = _signed_sum(mem_terms(slots, res, nu, slice(-mem, None)))
                    for mu in range(2):
                        terms = tok_terms(slots, res, mu, nu, slice(0, seg))
                        if odd:
                            zpart[i, mu, nu] = _signed_sum(terms)
                        else:
                            z_tok[i, mu, nu] = _signed_sum([(1, zpart[i, mu, nu])] + terms)

        def project(i, g, extra):
            pick = zero_s[i] == g
            res = []
            for e, (s, t) in enumerate(zip(qs, lhs)):
                for fn, h in extra.get(e, ()):
                    fn(h)
                sel = jnp.concatenate([jnp.where(pick, t[1][r0:r0 + 8], t[0][r0:r0 + 8])
                                       for r0 in range(0, t[0].shape[0], 8)], axis=0)
                res.append(_dot(sel, pltpu.bitcast(wb[i, s["r"], 1 + g], BF16)))
            for nu in range(KB):
                h = g * KB + nu
                terms = [tok_terms(qs, res, mu, nu, slice(0, seg)) for mu in range(2)]
                if odd:
                    cur = ahead.get((i, h))
                    for mu in range(2):
                        part[i, h, mu] = _signed_sum(terms[mu])
                else:
                    cur, ahead[i, h] = (
                        _signed_sum(terms[mu] + [(1, part[i, h, mu]), (1, z_tok[i, mu, nu])])
                        for mu in range(2))
                if memv:
                    t = stack(cur, _signed_sum(mem_terms(qs, res, nu, slice(-mem, None))
                                               + [(1, z_mem[i, nu])]))
                    qkv[h, i] = t if i == 0 else t.astype(BF16)

        def scores(h):
            s = jnp.where(mask, _dot_nt(qkv[h, 0], qkv[h, 1]), NEG * DB ** 0.5)
            e = jnp.exp2((s - jnp.max(s, axis=-1, keepdims=True)) * (DB ** -0.5 * LOG2E))
            total = jnp.sum(e, axis=-1, keepdims=True)
            inv = pltpu.reciprocal(total, approx=True)
            soft[h] = e * (inv * (2.0 - total * inv))

        def values(h):
            o = _dot(soft[h], qkv[h, 2])
            o_mem[h] = o[seg:]
            if odd:
                o_prev[0, h], o_prev[1, h] = ahead["o", h], o[:seg]
            else:
                ahead["o", h] = o[:seg]

        def out_pass(e, g):
            s = os_[e]
            if g not in o_mix:
                groups = range(GB) if g < 0 else (g,)
                over = lambda f, mu, kk: functools.reduce(
                    jnp.add, [f(mu, gg * KB + kk) for gg in groups])
                o_mix[g] = (_Mixer(functools.partial(over, lambda _, h: o_mem[h])),
                            _Mixer(functools.partial(over, lambda mu, h: o_prev[mu, h])))
            p = _dot(stack(o_mix[g][0]([s["a"]]) if memv else None,
                           o_mix[g][1](_U[s["r"]]) if s["tok"] else None),
                     pltpu.bitcast(wob[s["r"], 1 + g], BF16))
            o_sum[e] = o_sum[e] + p if e in o_sum else p
            if g >= 0:
                pick = jnp.concatenate([lane_sub] * (p.shape[0] // 8), axis=0) == g
                o_diag[e] = jnp.where(pick, p, o_diag[e]) if e in o_diag else p

        lag = 10
        if not output_only:
            shared()
            for g in range(GB):
                extra = {}
                for e in range(KB if memv else 0):
                    if g >= 1:
                        extra.setdefault(6 + 12 * e, []).append((scores, KB * (g - 1) + e))
                    if KB * g + e >= lag:
                        extra.setdefault(12 * e, []).append((values, KB * g + e - lag))
                for i in range(3):
                    project(i, g, {pos - 16 * i: fns for pos, fns in extra.items()})
        if project_only:
            return None
        extra = {}
        if memv:
            extra.update({3 + 5 * e: (scores, HB - KB + e) for e in range(KB)})
            extra.update({1 + 8 * e // 5 * 5: (values, HB - lag + e) for e in range(lag - KB)})
            extra.update({70 + 5 * e: (values, HB - KB + e) for e in range(KB)})
        passes = [p for groups in ((0, 1, 2, 3), (4, 5, 6), (7, -1))
                  for p in _weave([(e, g) for e in range(len(os_)) for g in groups], os_)]
        for n, p in enumerate(passes):
            if n in extra:
                extra[n][0](extra[n][1])
            out_pass(*p)

        new = {}
        for c in range(2):
            res = [o_diag[e] if c else o_sum[e] - o_diag[e] for e in range(len(os_))]
            for nu in range(KB):
                if memv:
                    t = _signed_sum(mem_terms(os_, res, nu, slice(0, mem)))
                    turns = [pltpu.roll(t, e * SUB, 1) for e in range(1, GB)] if c else []
                    new[c, nu] = functools.reduce(jnp.add, turns, t)
                for mu in range(2):
                    terms = tok_terms(os_, res, mu, nu, slice(-seg, None))
                    if odd:
                        opart[c, nu, mu] = _signed_sum(terms)
                    else:
                        b_rows[c, nu, (u - 2) % 4 + mu] = _signed_sum(
                            [(1, opart[c, nu, mu])] + terms)
        return new

    def emit_tile(j):
        gm = jnp.concatenate([gm_s[j]] * 2, axis=0)
        for c in range(2):
            for nu in range(KB):
                bt = jnp.concatenate([b_s[c, nu, 0], b_s[c, nu, 1], b_rows.val.pop((c, nu, 2)),
                                      b_rows.val.pop((c, nu, 3))], axis=0).T
                subs = [bt[e * SUB:(e + 1) * SUB] for e in range(GB)]
                for e, t in ((GB, functools.reduce(jnp.add, subs)),) if c else enumerate(subs):
                    at = pl.ds(SUB * (KB * e + nu), SUB)
                    out_v[j, at, :] = (ga_s[j, at, :] + gm * t).astype(out_v.dtype)

    b_step(3, 0, None, project_only=True)
    part.flush()
    zpart.flush()

    def b_body(j, carry):
        memv = {(c, kk): mem_s[c, kk] for c in range(2) for kk in range(KB)}
        for u in range(4):
            t0 = jnp.minimum(j * LANES + (u + 1) // 2 * 2 * seg, seq - 2 * seg)
            memv = b_step(u, pl.multiple_of(t0, seg), memv)
            if u == 0:
                emit_tile(jnp.maximum(j - 1, 0))
        for key, t in memv.items():
            mem_s[key] = t
        for c in (part, zpart, o_prev, opart, b_rows):
            c.flush()

        @pl.when(j > 0)
        def _():
            cp_out(j - 1).start()

        return carry

    lax.fori_loop(0, nt, b_body, 0)
    b_step(0, None, None, output_only=True)
    emit_tile(nt - 1)
    cp_out(nt - 1).start()
    for j in range(nt):
        cp_out(j).wait()


@functools.partial(jax.jit, static_argnames=("B_seg_len",))
def pallas_gated_mix__sliding_local_dilated__memory_aug_recurrent_mem_tr__prompt_kernel(
    A_x: jax.Array,
    A_wqkv: jax.Array,
    A_wo: jax.Array,
    B_x: jax.Array,
    B_mem0: jax.Array,
    B_Wq: jax.Array,
    B_Wk: jax.Array,
    B_Wv: jax.Array,
    B_Wo: jax.Array,
    B_seg_len: int,
    gate_w: jax.Array,
):
    del B_x
    batch, seq, width = A_x.shape
    mem, seg = B_mem0.shape[1], int(B_seg_len)
    nt = seq // LANES
    assert batch == 1 and width == D and seq == NP * LANES
    assert B_Wq.shape == (D, HB, DB) and mem == 8 and 4 * seg == LANES

    hbm = pl.BlockSpec(memory_space=pl.ANY)
    vmem = pl.BlockSpec(memory_space=pltpu.VMEM)
    out_t = pl.pallas_call(
        functools.partial(_kernel, seq=seq, seg=seg, mem=mem),
        out_shape=jax.ShapeDtypeStruct((D, seq), A_x.dtype),
        in_specs=[hbm, hbm, hbm, vmem, hbm, hbm, hbm, hbm, vmem],
        out_specs=hbm,
        scratch_shapes=[
            pltpu.VMEM((nt, D, LANES), BF16),
            pltpu.VMEM((D, 3 * D), BF16),
            pltpu.VMEM((D, D), BF16),
            pltpu.VMEM((3, NP, D, DB), U32),
            pltpu.VMEM((HB, D, DB), BF16),
            pltpu.VMEM((5, 3 * D, LANES), F32),
            pltpu.VMEM((NG * 9, RA + 8, LANES), F32),
            pltpu.VMEM((9, D // 2, LANES), F32),
            pltpu.VMEM((NG, 2, DA // 2, 8, LANES), U32),
            pltpu.VMEM((D // 2, LANES), U32),
            pltpu.VMEM((2, NR, SUB, LANES), F32),
            pltpu.VMEM((3, NR, 9, 64, LANES), U32),
            pltpu.VMEM((NR, 9, 64, LANES), U32),
            pltpu.VMEM((2, KB, seq, LANES), F32),
            pltpu.VMEM((nt, D, LANES), F32),
            pltpu.VMEM((nt, 8, LANES), F32),
            pltpu.VMEM((2, KB, mem, LANES), F32),
            pltpu.VMEM((3, 8, LANES), jnp.int32),
            pltpu.VMEM((3, HB, 2, seg, LANES), F32),
            pltpu.VMEM((3, 2, KB, seg, LANES), F32),
            pltpu.VMEM((2, HB, seg, LANES), F32),
            pltpu.VMEM((2, KB, 2, seg, LANES), F32),
            pltpu.VMEM((2, KB, 2, seg, LANES), F32),
            pltpu.VMEM((nt, D, LANES), A_x.dtype),
            pltpu.SemaphoreType.DMA((2,)),
            pltpu.SemaphoreType.DMA((6,)),
            pltpu.SemaphoreType.DMA((3,)),
            pltpu.SemaphoreType.DMA(()),
        ],
        compiler_params=pltpu.CompilerParams(vmem_limit_bytes=110 * 1024 * 1024),
        name="gated_mix_kernel",
    )(A_x[0].T, A_wqkv, A_wo, B_mem0[0], B_Wq, B_Wk, B_Wv, B_Wo.transpose(0, 2, 1), gate_w)
    return out_t.T[None]
```

```python
import functools
import itertools

import jax
import jax.numpy as jnp
import numpy as np
from jax import lax
import jax.experimental.pallas as pl
import jax.experimental.pallas.tpu as pltpu

F32, BF16, U32 = jnp.float32, jnp.bfloat16, jnp.uint32

D = 576
LANES = 128
HA, DA = 32, 18
WIN, DIL = 8, 2
HB, DB = 32, 128
NEG = -1000000000.0
LOG2E = 1.4426950408889634
NG = HA // 8
RA = 3 * (DA // 2) * 8

KB = 4
GP = HB // (2 * KB)

_HK = (
    (".... +...", "+.-. -... .... -...", "+... +..."),
    ("+... -...", "+-.- .... -... ....", "+... ...."),
    (".+.. .-..", ".... +-.. .+.. ....", ".... .+.."),
    (".+.. ....", ".-.. .+-. .... ....", ".+.. .+.."),
    (".... ..+.", ".... ..-. -.+. .+-.", ".... ..+."),
    ("..+. ....", "..-. ...+ .-+- ....", "..+. ...."),
    ("...+ ...-", ".... ...- ...+ ++.-", ".... ...+"),
    ("...+ ....", "...- ...- .... .+-+", "...+ ...+"),
    (".... ++..", ".... +... .... ....", ".... ++.."),
    ("++.. ....", ".+.. .... .... ....", "++.. ...."),
    (".+.. +...", ".-.. +... .... ....", "+... .-.."),
    ("+.+. -.-.", ".... .... -... ....", ".... +.+."),
    ("+.+. ....", "..+. .... .... ....", "+.+. +.+."),
    ("+.+. -...", "..-. .... +... ....", "+... +.+."),
    (".... +..+", ".... .... .... +...", ".... +..+"),
    ("+..+ ....", "...+ .... .... ....", "+..+ ...."),
    ("...+ +...", "...- .... .... +...", "+... ...-"),
    (".... .++.", ".... ..+. .... .-..", ".++. .++."),
    (".++. .--.", ".... ...- .+.. ....", ".++. ...."),
    (".+.. .--.", ".... ..+. .-.. ....", ".++. .+.."),
    (".... ..++", ".... .... .... .-+.", "..++ ..++"),
    ("..++ ..--", ".... ...- ...+ ....", "..++ ...."),
    ("...+ ..--", ".... ...+ ...- .-+.", "..++ ...+"),
    (".... .+++", ".... .... .... .+..", ".... .+++"),
    (".+++ ....", ".... ...+ .... ....", ".+++ ...."),
    ("...+ .++.", ".... ...- .... .+..", ".++. ...-"),
)
_U, _V, _C = (np.array([[["-.+".index(ch) - 1 for ch in row] for row in prod[i].split()]
                        for prod in _HK]) for i in range(3))
NR = len(_HK)
assert np.array_equal(np.einsum("rak,rln,rbm->akblnm", _U, _V, _C),
                      np.einsum("ab,kl,nm->akblnm", *(np.eye(n, dtype=int) for n in (2, KB, KB))))


def _phase(products):
    tiles = [max(r, ~r) for r in products]
    dual = np.rint(np.linalg.inv(_V[tiles].reshape(len(tiles), -1)).T).astype(int)
    slots = []
    for r, d in zip(products, dual.reshape(-1, KB, KB)):
        i, j = np.argwhere(d)[0]
        a, c = d[:, j] * d[i, j], d[i]
        assert np.array_equal(np.outer(a, c), d)
        slots.append(dict(r=max(r, ~r), tok=r >= 0, a=a.tolist(), c=c.tolist()))
    return slots


_PHASES = (_phase((11, 8, ~9, 4, 2, 23, 17, ~13, 25, 20, 22, 7, ~19, 16, 15, 1)),
           _phase((24, 21, ~16, 18, 19, 3, 10, ~22, 9, 5, 12, 13, ~25, 0, 14, 6)))
assert sorted(s["r"] for ph in _PHASES for s in ph if s["tok"]) == list(range(NR))

NH = 2 * KB
assert all(sorted(s["r"] // 2 for s in ph if s["r"] < NH) == list(range(KB)) for ph in _PHASES)
assert all(np.abs(s[k]).tolist() == np.eye(KB)[s["r"] // 2].tolist()
           for ph in _PHASES for s in ph if s["r"] < NH for k in "ac")
_TAIL_IN, _TAIL_OUT = (
    np.concatenate([np.rint(np.linalg.inv(t[2 * n:2 * n + 2, :, n]).T).astype(int)
                    for n in range(KB)]) for t in (_C, _U))


CHUNKS, S0, LAG, SPAN, HEAD, M0 = ((0, 1), (2, 3)), 78, 48, (11.25, 2), 36, 6
MO = (366, 386, 406, 426, 446, 466)


D0, DS, TS, Q = 0, (0, 0, 0), ((0, 1),), 1


AHEAD = 0
QA, BA = (8, 11, 14, 17, 20, 40, 54, 68, 82, 96, 110, 132, 136, 140), 20
QB = range(20, 144, 14)


def _signed_sum(terms):
    terms = [(c, t) for c, t in terms if c]
    first = next((i for i, (c, _) in enumerate(terms) if c > 0), 0)
    c, acc = terms.pop(first)
    acc = acc if c > 0 else -acc
    for c, t in terms:
        acc = acc + t if c > 0 else acc - t
    return acc


class _Mixer:
    def __init__(self, block):
        self.block, self.known = block, {}

    def __call__(self, coef):
        want = {(i, k): int(c) for i, row in enumerate(coef) for k, c in enumerate(row) if c}
        key = tuple(sorted(want.items()))
        if key not in self.known:
            terms = []
            for have in sorted(self.known, key=lambda h: -len(h)):
                for sign in (1, -1):
                    if all(want.get(pos) == sign * c for pos, c in have):
                        terms.append((sign, self.known[have]))
                        want = {pos: c for pos, c in want.items() if pos not in dict(have)}
                        break
            for pos, c in sorted(want.items()):
                self.known[((pos, 1),)] = self.block(*pos)
                terms.append((c, self.known[((pos, 1),)]))
            self.known[key] = _signed_sum(terms)
        return self.known[key]


class _Sums:
    def __init__(self, done):
        self.done, self.acc = done, {}

    def add(self, key, sign, value, expected):
        if not sign:
            return
        count, neg, tot = self.acc.pop(key, (0, sign < 0, value))
        if count and neg == (sign < 0):
            tot = tot + value
        elif count:
            tot, neg = (value - tot if neg else tot - value), False
        if count + 1 == expected:
            self.done(key, -tot if neg else tot)
        else:
            self.acc[key] = (count + 1, neg, tot)


class _Carry:
    def __init__(self, ref):
        self.ref, self.val = ref, {}

    def __getitem__(self, key):
        return self.val[key] if key in self.val else self.ref[key]

    def __setitem__(self, key, value):
        self.val[key] = value

    def flush(self):
        for key, value in self.val.items():
            self.ref[key] = value
        self.val = {}


def _dot(a, b):
    return lax.dot_general(a, b, (((1,), (0,)), ((), ())), preferred_element_type=F32)


def _dot_nt(a, b):
    return lax.dot_general(a, b, (((1,), (1,)), ((), ())), preferred_element_type=F32)


def _tile(ref, *idx):
    return pltpu.bitcast(ref.bitcast(U32)[idx], BF16)


def stack(*parts):
    parts = [t for t in parts if t is not None]
    return parts[0] if len(parts) == 1 else jnp.concatenate(parts, axis=0)


def _low_half(rows):
    return lax.broadcasted_iota(jnp.int32, (rows, LANES), 1) < 64


def _pair_lhs(t1, t2):
    lo = _low_half(t1[0].shape[0])
    diff = t1[3] - t2[3]
    return (t1[:3] + [jnp.where(lo, t1[4], diff)]
            + t2[:3] + [jnp.where(lo, -diff, t2[4])]
            + [jnp.where(lo, t1[3], t2[3])])


def _pair_rhs(x):
    a, b, c = x[384:448], x[448:512], x[512:576]
    cat = lambda u, v: jnp.concatenate([u, v], axis=0)
    return [x[i * 128:(i + 1) * 128] for i in range(3)] + [cat(c, b), cat(a, c), x[384:512]]


def _pair_matmul(lhs, rhs, dot):
    out = [dot(lhs(8), rhs[5])] * 2
    for i in range(8):
        out[i // 4] = out[i // 4] + dot(lhs(i), rhs[i % 4 if i < 7 else 4])
    return out


def _kernel(xt_hbm, wqkv_hbm, wo_hbm, mem0_ref, wq_hbm, wk_hbm, wv_hbm, wot_hbm, gate_ref,
            out_hbm,
            xt_v, wqkv_v, wo_v, stg_qkv, stg_o, wo_t, wt32, la, lo_a, kv_prev, oa_s,
            wb, x32, ga_s, gm_s, mem_s, part_s, o_s, opart_s, b_s, out_v,
            sem_x, sem_wa, sem_wb, sem_out, *, seq, seg, mem):
    nt = seq // LANES
    rows = mem + seg

    def cp_x(j):
        col = j * LANES if isinstance(j, int) else pl.multiple_of(j * LANES, LANES)
        return pltpu.make_async_copy(xt_hbm.at[:, pl.ds(col, LANES)], xt_v.at[j], sem_x.at[j % 2])

    def cp_wqkv(k):
        r = pl.ds(k * 128, min(128, D - k * 128))
        return pltpu.make_async_copy(wqkv_hbm.at[r], wqkv_v.at[r], sem_wa.at[k])

    cp_wo = pltpu.make_async_copy(wo_hbm, wo_v, sem_wa.at[5])

    def cp_unit(unit):
        i, gp = divmod(unit, GP)
        sem = sem_wb.at[unit % 3]
        if i == 3:
            heads = pl.ds(2 * KB * gp, 2 * KB)
            return [pltpu.make_async_copy(wot_hbm.at[heads], stg_o.at[heads], sem)]
        src = (wq_hbm, wk_hbm, wv_hbm)[i].bitcast(U32)
        return [pltpu.make_async_copy(src.at[:, KB * gp + p, :], stg_qkv.at[unit, p], sem)
                for p in range(KB)]

    def start_unit(unit):
        for c in cp_unit(unit):
            c.start()

    def wait_unit(unit):
        for c in cp_unit(unit):
            c.wait()

    def cp_out(j):
        col = j * LANES if isinstance(j, int) else pl.multiple_of(j * LANES, LANES)
        return pltpu.make_async_copy(out_v.at[j], out_hbm.at[:, pl.ds(col, LANES)], sem_out)

    for k in range(5):
        cp_wqkv(k).start()
    cp_x(0).start()
    cp_wo.start()

    m0 = mem0_ref[...].astype(F32)
    for kk in range(KB):
        mem_s[kk] = m0[:, kk * LANES:(kk + 1) * LANES]
    mem_s[KB] = jnp.concatenate([m0[:, KB * LANES:]] * 2, axis=1)
    for ref in (o_s, opart_s, b_s):
        ref[...] = jnp.zeros(ref.shape, ref.dtype)
    wb[4 * GP, 0, 0:16, :] = jnp.zeros((16, LANES), BF16)
    wo_t[GP, 0, 0, 0:8, :] = jnp.zeros((8, LANES), U32)

    gate = jnp.broadcast_to(gate_ref[...].astype(F32).reshape(1, D), (8, D))
    gate_t = [gate[:, i * 128:(i + 1) * 128] for i in range(4)]
    gate_t.append(jnp.concatenate([gate[:, 512:], gate[:, 512:]], axis=1))

    for k in range(5):
        cp_wqkv(k).wait()
        if k < 4:
            blk = wqkv_v[k * 128:(k + 1) * 128, :]
        else:
            blk = jnp.concatenate([wqkv_v[512:D, :]] * 2, axis=0)
        if k == 4:
            cp_x(1).start()
            start_unit(0)
            start_unit(1)
        wt32[k] = blk.T.astype(F32)

    for g in range(NG):
        for part in range(3):
            for dd in range(DA // 2):
                base = part * D + g * 8 * DA + 2 * dd
                t1 = [wt32[k, pl.ds(base, 8, stride=DA), :] for k in range(5)]
                t2 = [wt32[k, pl.ds(base + 1, 8, stride=DA), :] for k in range(5)]
                r0 = (part * (DA // 2) + dd) * 8
                for i, t in enumerate(_pair_lhs(t1, t2)):
                    la[g * 9 + i, r0:r0 + 8, :] = t
    for i, t in enumerate(_pair_lhs(gate_t, gate_t)):
        la[i, RA:RA + 8, :] = t

    cp_wo.wait()
    wo32 = wo_v[...].astype(F32)
    for n in range(4):
        wt32[n, 0:D, :] = wo32[:, n * 128:(n + 1) * 128]
    wt32[4, 0:D, :] = jnp.concatenate([wo32[:, 512:], wo32[:, 512:]], axis=1)
    perm = [jnp.concatenate([wt32[n, pl.ds(g * 8 * DA + d, 8, stride=DA), :]
                             for g in range(NG) for d in range(DA)], axis=0) for n in range(5)]
    tiles = []
    for k in range(5):
        if k < 4:
            pk = [pn[k * 128:(k + 1) * 128] for pn in perm]
        else:
            pk = [jnp.concatenate([pn[512:], pn[512:]], axis=0) for pn in perm]
        tiles.append(jnp.concatenate([t.T for t in pk[:4]] + [pk[4].T[:64]], axis=0))
    for i, t in enumerate(_pair_lhs([t[:D // 2] for t in tiles], [t[D // 2:] for t in tiles])):
        lo_a[i] = t

    by_size = sorted(range(NR), key=lambda r: int(np.abs(_V[r]).sum()))

    def prep_qkv(unit):
        src, dst = stg_qkv.at[unit], wb.at[unit]

        def rows(g, r0, nu):
            u = src[2 * g + nu // 2, r0:r0 + 16, :]
            return pltpu.bitcast(u & jnp.uint32(0xFFFF0000) if nu % 2 else u << 16, F32)

        for e in range(8):
            at, own, shared = pl.ds(16 * e, 16), e // 4, {}
            for g in (own, 1 - own):
                mix = _Mixer(lambda kk, nu: rows(g, kk * LANES + 16 * e, nu))
                for r in by_size:
                    w = mix(_V[r])
                    if r < NH and g == own:
                        shared[r] = w.astype(BF16)
                        dst[2 * NR + r, at, :] = shared[r]
                        w = rows(g, KB * LANES + 16 * (e % 4), r // 2)
                    elif r < NH:
                        w = w - shared[r].astype(F32)
                    dst[g * NR + r, at, :] = w.astype(BF16)
                yield

    def turn_out(gp):
        words = lambda head, r0, n: _tile(stg_o, 2 * KB * gp + head, pl.ds(r0 // 2, n // 2))
        for head in range(2 * KB + 1):
            for nu in range(KB):
                if head < 2 * KB:
                    tile = words(head, nu * LANES, LANES)
                else:
                    tile = stack(*(words(g * KB + nu, KB * LANES, 64) for g in range(2)))
                wo_t[gp, head, nu] = pltpu.bitcast(tile.T, U32)
            yield

    def prep_out(gp):
        dst, lo = wb.at[3 * GP + gp], _low_half(16)
        for e in range(8):
            at, first = pl.ds(16 * e, 16), {}
            rows = lambda head, nu: pltpu.bitcast(
                wo_t[gp, head, nu, 8 * e:8 * e + 8, :], BF16).astype(F32)
            for g in range(2):
                mix = _Mixer(lambda kk, nu: rows(g * KB + kk, nu))
                for r in by_size:
                    w = mix(_V[r])
                    if r >= NH:
                        dst[g * NR + r, at, :] = w.astype(BF16)
                    elif g == 0:
                        first[r] = w
                    else:
                        z, t = jnp.where(lo, first[r], w).astype(BF16), rows(2 * KB, r // 2)
                        dst[2 * NR + r, at, :] = z
                        dst[r, at, :] = jnp.where(lo, t, first[r] - z.astype(F32)).astype(BF16)
                        dst[NR + r, at, :] = jnp.where(lo, w - z.astype(F32), t).astype(BF16)
            yield

    lane = lax.broadcasted_iota(jnp.int32, (8, LANES), 1)

    def exchange(idx, pair, first):
        at = pl.ds(8 * idx, 8)
        prev = None if first else kv_prev.bitcast(U32)[at, :]
        kv_prev[16 * idx:16 * idx + 16, :] = jnp.concatenate(pair, axis=0).astype(BF16)
        cur = kv_prev.bitcast(U32)[at, :]
        return (jnp.broadcast_to(cur[:, 0:1], (8, LANES)) if first else prev), cur

    def to_rows(j):
        t0 = j * LANES if isinstance(j, int) else pl.multiple_of(j * LANES, LANES)
        xt = _tile(xt_v, j)
        tiles = [xt[kk * LANES:(kk + 1) * LANES].T for kk in range(KB)]
        tiles.append(jnp.concatenate([xt[KB * LANES:]] * 2, axis=0).T)
        for kk, t in enumerate(tiles):
            for r0 in range(0, LANES, 32):
                x32[kk, pl.ds(t0 + r0, 32), :] = t[r0:r0 + 32].astype(F32)
                yield

    def attend(j, first, parts, outs):
        get = lambda g, part, dd: [t[dd * 8:dd * 8 + 8] for t in parts[g, part]]
        items = [(g, part, dd) for g in range(NG) for part in (1, 2) for dd in range(DA // 2)]

        def shifts(g, part, dd):
            prev, cur = exchange((2 * g + part - 1) * (DA // 2) + dd, get(g, part, dd), first)
            return [cur] + [pltpu.roll(jnp.where(lane >= LANES - DIL * w, prev, cur), DIL * w, 1)
                            for w in range(1, WIN)]

        gsig = 1.0 / (1.0 + jnp.exp(-parts[0, 1][0][RA // 3:]))
        gm_s[j] = 1.0 - gsig
        early = []
        for n, (g, part, dd) in enumerate(items):
            if n + AHEAD < len(items):
                early.append(shifts(*items[n + AHEAD]))
            both = [pltpu.bitcast(t, BF16).astype(F32) for t in early.pop(0)]
            if part == 1:
                q = get(g, 0, dd)
                terms = [q[0] * t[0:8] + q[1] * t[8:16] for t in both]
                logit = terms if dd == 0 else [a + b for a, b in zip(logit, terms)]
            else:
                outs.append(functools.reduce(jnp.add, [
                    jnp.concatenate([p] * 2, axis=0) * t for p, t in zip(prob, both)]))
            if (part, dd) == (1, DA // 2 - 1):
                logit = [t * (DA ** -0.5) for t in logit]
                if first:
                    logit = [jnp.where(lane >= DIL * w, t, NEG) for w, t in enumerate(logit)]
                top = functools.reduce(jnp.maximum, logit)
                ex = [jnp.exp(t - top) for t in logit]
                inv = gsig / functools.reduce(jnp.add, ex)
                prob = [e * inv for e in ex]
            yield

    def paced(job, src, dst, when, back):
        results = []

        def dot(left, right):
            if len(results) in when:
                if src is not None and len(results) >= back:
                    src[...] = pltpu.bitcast(results[-back][0:8], U32)
                next(job, None)
                left = stack(left[:-8], left[-8:] + pltpu.bitcast(dst[...], F32))
            results.append(_dot(left, right))
            return results[-1]

        return dot

    spare_qkv, spare_t = stg_qkv.at[3 * GP, 0, 0:8], wo_t.at[GP, 0, 1, 0:8]
    zero_t, zero_w = wo_t.at[GP, 0, 0, 0:8], wb.bitcast(U32).at[4 * GP, 0, 0:8]

    def a_out(j, dot):
        rhs = _pair_rhs(_tile(oa_s, slice(None)))
        rp = D // 8
        for c in range(4):
            halves = _pair_matmul(lambda i: lo_a[i, c * rp:(c + 1) * rp, :], rhs, dot)
            ga_s[j, c * rp:(c + 1) * rp, :] = halves[0]
            ga_s[j, D // 2 + c * rp:D // 2 + (c + 1) * rp, :] = halves[1]

    def a_tile(j, first, dot):
        parts, outs = {}, []
        window = attend(j, first, parts, outs)
        list(to_rows(j))
        rhs, rp = _pair_rhs(_tile(xt_v, j)), RA // 3
        for g in range(NG):
            for part in (1, 0, 2):
                def left(i):
                    w = la[g * 9 + i, part * rp:(part + 1) * rp, :]
                    return stack(w, la[i, RA:RA + 8, :]) if (g, part) == (0, 1) else w

                parts[g, part] = _pair_matmul(left, rhs, dot)
                if part != 1:
                    list(itertools.islice(window, DA // 2))
        if not first:
            a_out(j - 1, dot)
        oa_s[...] = jnp.concatenate(outs, axis=0).astype(BF16)

    cp_x(0).wait()
    start_unit(2)
    a_tile(0, True, _dot)

    def a_loop(units, work, *pacing):
        def body(j, carry):
            cp_x(j).wait()
            pl.when(j + 1 < nt)(lambda: cp_x(j + 1).start())
            for unit in units:
                pl.when(j == unit + 1)(functools.partial(wait_unit, unit))
            job = work(j - 1 - units[0])
            a_tile(j, False, paced(job, *pacing))
            list(job)
            for unit in units:
                if unit + 3 < 4 * GP:
                    pl.when(j == unit + 1)(functools.partial(start_unit, unit + 3))
            return carry

        lax.fori_loop(units[0] + 1, units[-1] + 2, body, 0)

    a_loop(range(3 * GP), prep_qkv, spare_qkv, zero_w, QA, BA)
    a_loop(range(3 * GP, nt - 1), turn_out, None, zero_t, QB, 0)
    wait_unit(4 * GP - 1)

    qi = lax.broadcasted_iota(jnp.int32, (rows, rows), 0)
    ki = lax.broadcasted_iota(jnp.int32, (rows, rows), 1)
    mask = (qi >= seg) | (ki >= seg) | (qi >= ki)
    part, o_prev, opart, b_rows = (_Carry(r) for r in (part_s, o_s, opart_s, b_s))
    ahead = {}

    def b_step(u, t0, memv, project_only=False, output_only=False):
        odd = u % 2
        keep = lambda slots: [s for s in slots if s["tok"] or memv]
        qs, os_ = keep(_PHASES[odd]), keep(_PHASES[1 - odd])
        lhs, shared, tok, mrow, full, soft, o_mem, o_mix, o_left, o_host, new = ({} for _ in range(11))
        clock, queue = [0], {}

        def later(delay, fn, *args):
            queue.setdefault(clock[0] + delay, []).append((fn, args))

        def tick():
            for fn, args in queue.pop(clock[0], ()):
                fn(*args)
            clock[0] += 1

        def spread(sums, key, slots, s, tok_rows, mem_rows):
            for nu in range(KB):
                if memv:
                    sums.add(key + (nu, 2), s["c"][nu], mem_rows, sum(abs(o["c"][nu]) for o in slots))
                for mu in range(2 if s["tok"] else 0):
                    sums.add(key + (nu, mu), _C[s["r"]][mu][nu], tok_rows,
                             sum(abs(_C[o["r"]][mu][nu]) for o in slots if o["tok"]))

        x_mix = _Mixer(lambda mu, kk: x32[kk, pl.ds(t0 + mu * seg, seg), :])
        c_mix = _Mixer(lambda mu, _: x32[KB, pl.ds(t0 + mu * seg, seg), :])
        m_mix = _Mixer(lambda _, kk: memv[kk])

        def q_left(e, t):
            s = qs[e]
            if (e, t) not in lhs:
                left = stack(x_mix(_U[s["r"]]) if s["tok"] else None,
                             m_mix([s["a"]]) if memv else None)
                if s["r"] < NH and t < 2:
                    c = stack(c_mix(_TAIL_IN[s["r"]][:, None]),
                              _signed_sum([(sum(s["c"]), memv[KB])]) if memv else None)
                    left = jnp.where(_low_half(c.shape[0]), *((c, left), (left, c))[t])
                lhs[e, t] = left
            return lhs[e, t]

        def q_total(key, value):
            i, g, nu, mu = key
            h = g * KB + nu
            if mu == 2:
                mrow[i, h] = value
            elif odd:
                part[i, h, mu] = value
            elif mu == 0:
                tok[i, h] = value + part[i, h, mu]
            else:
                ahead[i, h] = (value + part[i, h, mu]).astype(BF16 if i else F32)
            cur = (ahead if odd else tok).get((i, h))
            if (i, h) in mrow and cur is not None and (i, h) not in full:
                full[i, h] = stack(cur.astype(BF16 if i else F32),
                                   mrow[i, h].astype(BF16 if i else F32))

        q_sums = _Sums(q_total)

        def q_pass(e, i, gp, t):
            s = qs[e]
            p = _dot(q_left(e, t), _tile(wb, i * GP + gp, t * NR + s["r"]))
            if t == 2:
                shared[e, i, gp] = p
                return

            def use():
                r = p + shared[e, i, gp] if s["r"] < NH else p
                spread(q_sums, (i, 2 * gp + t), qs, s, r[:seg], r[-mem:])

            later(D0, use)

        def scores(h):
            def stages():
                raw = _dot_nt(full[0, h], full[1, h])
                yield
                s = jnp.where(mask, raw, NEG * DB ** 0.5)
                top = jnp.max(s, axis=-1, keepdims=True)
                yield
                e = jnp.exp2((s - top) * (DB ** -0.5 * LOG2E))
                total = jnp.sum(e, axis=-1, keepdims=True)
                yield
                inv = pltpu.reciprocal(total, approx=True)
                soft[h] = e * (inv * (2.0 - total * inv))
                yield

            run = stages()
            next(run)
            for delay in DS:
                later(delay, next, run)

        def values(h):
            o = _dot(soft[h], full[2, h])
            o_mem[h] = o[seg:]
            if odd:
                o_prev[0, h], o_prev[1, h] = ahead["o", h], o[:seg]
            else:
                ahead["o", h] = o[:seg]

        def o_rows(e, gp, t):
            s = os_[e]
            if (e, gp, t) not in o_left:
                g = 2 * gp + t
                if t == 2:
                    o_left[e, gp, t] = o_rows(e, gp, 0) + o_rows(e, gp, 1)
                    return o_left[e, gp, t]
                if g not in o_mix:
                    o_mix[g] = (_Mixer(lambda _, kk: o_mem[g * KB + kk]),
                                _Mixer(lambda mu, kk: o_prev[mu, g * KB + kk]))
                o_left[e, gp, t] = stack(o_mix[g][0]([s["a"]]) if memv else None,
                                         o_mix[g][1](_U[s["r"]]) if s["tok"] else None)
            return o_left[e, gp, t]

        def o_total(key, value):
            nu, mu = key
            if mu == 2:
                new[nu] = value if nu < KB else value + pltpu.roll(value, 64, 1)
            elif odd:
                opart[nu, mu] = value
            else:
                b_rows[nu, (u - 2) % 4 + mu] = value + opart[nu, mu]

        out_sums = _Sums(o_total)

        def o_product(key, value):
            e, t = key
            s = os_[e]
            if s["r"] < NH:
                o_host[key] = value
                if any((e, t_) not in o_host for t_ in range(3)):
                    return
                lo = _low_half(value.shape[0])
                value = o_host[e, 2] + jnp.where(lo, o_host[e, 1], o_host[e, 0])
                y = jnp.where(lo, o_host[e, 0], o_host[e, 1])
                if memv:
                    out_sums.add((KB, 2), sum(s["a"]), y[:mem], KB)
                for mu in range(2):
                    out_sums.add((KB, mu), _TAIL_OUT[s["r"]][mu], y[-seg:],
                                 sum(abs(_TAIL_OUT[o["r"]][mu]) for o in os_ if o["r"] < NH))
            spread(out_sums, (), os_, s, value[-seg:], value[:mem])

        o_sums = _Sums(o_product)

        def o_pass(e, gp, t):
            host = os_[e]["r"] < NH
            p = _dot(o_rows(e, gp, t), _tile(wb, 3 * GP + gp, t * NR + os_[e]["r"]))
            later(D0, o_sums.add, (e, t if host else 0), 1, p, GP if host else 2 * GP)

        todo = []
        tiles = lambda s, ts: (2,) + ts if s["r"] < NH and 0 in ts else ts
        if not output_only:
            units = [(i, gp, t) for gp in range(GP) for i in range(3) for t in TS]
            todo = [(s["tok"], q_pass, e, i, gp, t_) for i, gp, t in units
                    for e, s in enumerate(qs) for t_ in tiles(s, t)]
            last = [max(e for e, s in enumerate(_PHASES[odd]) if s["tok"] and s["c"][nu])
                    for nu in range(KB)]
            ready = lambda e, t: 99 if qs[e]["r"] < NH and t < 2 else max(
                last[kk] for kk in range(KB) if qs[e]["a"][kk])
            todo[:HEAD] = sorted(todo[:HEAD], key=lambda p: ready(p[2], p[5]))
        if not project_only:
            todo += [(s["tok"], o_pass, e, gp, t) for pairs in CHUNKS for e, s in enumerate(os_)
                     for gp in pairs for t in tiles(s, (0, 1))]
        long_, short = ([p[1:] for p in todo if p[0] == tok] for tok in (True, False))
        extra = {}
        for h in range(HB if memv else 0):
            gp, n = divmod(h, 2 * KB)
            at = (90 * gp + S0 + int(SPAN[gp == GP - 1] * (n // Q * Q))) // Q * Q
            extra.setdefault(at, []).append((scores, h))
            extra.setdefault(at + LAG, []).append((values, h))
        issued = 0
        for n, p in enumerate(long_):
            for fn, *args in extra.get(n, []) + [p]:
                if issued % 4 == 0 and short and n >= (480 + M0 - 5 * len(short) if len(short) > 24 else MO[6 - len(short) // 4]):
                    for fn_s, *args_s in short[:4]:
                        fn_s(*args_s)
                        tick()
                    del short[:4]
                fn(*args)
                tick()
                issued += 1
        assert not short
        while queue:
            tick()
        return new

    def emit_tile(j):
        for nu in range(KB + 1):
            bt = jnp.concatenate([b_s[nu, 0], b_s[nu, 1], b_rows.val.pop((nu, 2)),
                                  b_rows.val.pop((nu, 3))], axis=0).T
            bt = bt if nu < KB else bt[:64] + bt[64:]
            at = pl.ds(nu * LANES, bt.shape[0])
            gm = jnp.concatenate([gm_s[j]] * (bt.shape[0] // 8), axis=0)
            out_v[j, at, :] = (ga_s[j, at, :] + gm * bt).astype(out_v.dtype)

    list(turn_out(GP - 1))
    a_out(nt - 1, _dot)
    b_step(3, 0, None, project_only=True)
    part.flush()
    for gp in range(2):
        list(prep_out(gp))

    @pl.loop(2, GP)
    def _(gp):
        list(prep_out(gp))

    def b_body(j, carry):
        memv = {kk: mem_s[kk] for kk in range(KB + 1)}
        for u in range(4):
            t0 = jnp.minimum(j * LANES + (u + 1) // 2 * 2 * seg, seq - 2 * seg)
            memv = b_step(u, pl.multiple_of(t0, seg), memv)
            if u == 0:
                emit_tile(jnp.maximum(j - 1, 0))
        for kk, t in memv.items():
            mem_s[kk] = t
        for c in (part, o_prev, opart, b_rows):
            c.flush()
        pl.when(j > 0)(lambda: cp_out(j - 1).start())
        return carry

    lax.fori_loop(0, nt, b_body, 0)
    b_step(0, None, None, output_only=True)
    emit_tile(nt - 1)
    cp_out(nt - 1).start()
    for j in range(nt):
        cp_out(j).wait()


@functools.partial(jax.jit, static_argnames=("B_seg_len",))
def pallas_gated_mix__sliding_local_dilated__memory_aug_recurrent_mem_tr__prompt_kernel(
    A_x: jax.Array,
    A_wqkv: jax.Array,
    A_wo: jax.Array,
    B_x: jax.Array,
    B_mem0: jax.Array,
    B_Wq: jax.Array,
    B_Wk: jax.Array,
    B_Wv: jax.Array,
    B_Wo: jax.Array,
    B_seg_len: int,
    gate_w: jax.Array,
):
    del B_x
    batch, seq, width = A_x.shape
    mem, seg = B_mem0.shape[1], int(B_seg_len)
    nt = seq // LANES
    assert batch == 1 and width == D and nt == 4 * GP and seq % LANES == 0
    assert B_Wq.shape == (D, HB, DB) and mem == 8 and 4 * seg == LANES

    hbm = pl.BlockSpec(memory_space=pl.ANY)
    vmem = pl.BlockSpec(memory_space=pltpu.VMEM)
    out_t = pl.pallas_call(
        functools.partial(_kernel, seq=seq, seg=seg, mem=mem),
        out_shape=jax.ShapeDtypeStruct((D, seq), A_x.dtype),
        in_specs=[hbm, hbm, hbm, vmem, hbm, hbm, hbm, hbm, vmem],
        out_specs=hbm,
        scratch_shapes=[
            pltpu.VMEM((nt, D, LANES), BF16),
            pltpu.VMEM((D, 3 * D), BF16),
            pltpu.VMEM((D, D), BF16),
            pltpu.VMEM((3 * GP + 1, KB, D, DB), U32),
            pltpu.VMEM((HB, D, DB), BF16),
            pltpu.VMEM((GP + 1, 2 * KB + 1, KB, 64, LANES), U32),
            pltpu.VMEM((5, 3 * D, LANES), F32),
            pltpu.VMEM((NG * 9, RA + 8, LANES), F32),
            pltpu.VMEM((9, D // 2, LANES), F32),
            pltpu.VMEM((2 * D, LANES), BF16),
            pltpu.VMEM((D, LANES), BF16),
            pltpu.VMEM((4 * GP + 1, 2 * NR + NH, LANES, LANES), BF16),
            pltpu.VMEM((KB + 1, seq, LANES), F32),
            pltpu.VMEM((nt, D, LANES), F32),
            pltpu.VMEM((nt, 8, LANES), F32),
            pltpu.VMEM((KB + 1, mem, LANES), F32),
            pltpu.VMEM((3, HB, 2, seg, LANES), F32),
            pltpu.VMEM((2, HB, seg, LANES), F32),
            pltpu.VMEM((KB + 1, 2, seg, LANES), F32),
            pltpu.VMEM((KB + 1, 2, seg, LANES), F32),
            pltpu.VMEM((nt, D, LANES), A_x.dtype),
            pltpu.SemaphoreType.DMA((2,)),
            pltpu.SemaphoreType.DMA((6,)),
            pltpu.SemaphoreType.DMA((3,)),
            pltpu.SemaphoreType.DMA(()),
        ],
        compiler_params=pltpu.CompilerParams(vmem_limit_bytes=110 * 1024 * 1024),
        name="gated_mix_kernel",
    )(A_x[0].T, A_wqkv, A_wo, B_mem0[0], B_Wq, B_Wk, B_Wv, B_Wo.transpose(0, 2, 1), gate_w)
    return out_t.T[None]
```

```python
import functools
import itertools

import jax
import jax.numpy as jnp
import numpy as np
from jax import lax
import jax.experimental.pallas as pl
import jax.experimental.pallas.tpu as pltpu

F32, BF16, U32 = jnp.float32, jnp.bfloat16, jnp.uint32

D = 576
LANES = 128
HA, DA = 32, 18
WIN, DIL = 8, 2
HB, DB = 32, 128
NEG = -1000000000.0
LOG2E = 1.4426950408889634
NG = HA // 8

KB = 4
GP = HB // (2 * KB)

_HK = (
    (".... +...", "+.-. -... .... -...", "+... +..."),
    ("+... -...", "+-.- .... -... ....", "+... ...."),
    (".+.. .-..", ".... +-.. .+.. ....", ".... .+.."),
    (".+.. ....", ".-.. .+-. .... ....", ".+.. .+.."),
    (".... ..+.", ".... ..-. -.+. .+-.", ".... ..+."),
    ("..+. ....", "..-. ...+ .-+- ....", "..+. ...."),
    ("...+ ...-", ".... ...- ...+ ++.-", ".... ...+"),
    ("...+ ....", "...- ...- .... .+-+", "...+ ...+"),
    (".... ++..", ".... +... .... ....", ".... ++.."),
    ("++.. ....", ".+.. .... .... ....", "++.. ...."),
    (".+.. +...", ".-.. +... .... ....", "+... .-.."),
    ("+.+. -.-.", ".... .... -... ....", ".... +.+."),
    ("+.+. ....", "..+. .... .... ....", "+.+. +.+."),
    ("+.+. -...", "..-. .... +... ....", "+... +.+."),
    (".... +..+", ".... .... .... +...", ".... +..+"),
    ("+..+ ....", "...+ .... .... ....", "+..+ ...."),
    ("...+ +...", "...- .... .... +...", "+... ...-"),
    (".... .++.", ".... ..+. .... .-..", ".++. .++."),
    (".++. .--.", ".... ...- .+.. ....", ".++. ...."),
    (".+.. .--.", ".... ..+. .-.. ....", ".++. .+.."),
    (".... ..++", ".... .... .... .-+.", "..++ ..++"),
    ("..++ ..--", ".... ...- ...+ ....", "..++ ...."),
    ("...+ ..--", ".... ...+ ...- .-+.", "..++ ...+"),
    (".... .+++", ".... .... .... .+..", ".... .+++"),
    (".+++ ....", ".... ...+ .... ....", ".+++ ...."),
    ("...+ .++.", ".... ...- .... .+..", ".++. ...-"),
)
_U, _V, _C = (np.array([[["-.+".index(ch) - 1 for ch in row] for row in prod[i].split()]
                        for prod in _HK]) for i in range(3))
NR = len(_HK)
assert np.array_equal(np.einsum("rak,rln,rbm->akblnm", _U, _V, _C),
                      np.einsum("ab,kl,nm->akblnm", *(np.eye(n, dtype=int) for n in (2, KB, KB))))


def _phase(products):
    tiles = [max(r, ~r) for r in products]
    dual = np.rint(np.linalg.inv(_V[tiles].reshape(len(tiles), -1)).T).astype(int)
    slots = []
    for r, d in zip(products, dual.reshape(-1, KB, KB)):
        i, j = np.argwhere(d)[0]
        a, c = d[:, j] * d[i, j], d[i]
        assert np.array_equal(np.outer(a, c), d)
        slots.append(dict(r=max(r, ~r), tok=r >= 0, a=a.tolist(), c=c.tolist()))
    return slots


_PHASES = (_phase((11, 8, ~9, 4, 2, 23, 17, ~13, 25, 20, 22, 7, ~19, 16, 15, 1)),
           _phase((24, 21, ~16, 18, 19, 3, 10, ~22, 9, 5, 12, 13, ~25, 0, 14, 6)))
assert sorted(s["r"] for ph in _PHASES for s in ph if s["tok"]) == list(range(NR))

NH = 2 * KB
assert all(sorted(s["r"] // 2 for s in ph if s["r"] < NH) == list(range(KB)) for ph in _PHASES)
assert all(np.abs(s[k]).tolist() == np.eye(KB)[s["r"] // 2].tolist()
           for ph in _PHASES for s in ph if s["r"] < NH for k in "ac")
_TAIL_IN, _TAIL_OUT = (
    np.concatenate([np.rint(np.linalg.inv(t[2 * n:2 * n + 2, :, n]).T).astype(int)
                    for n in range(KB)]) for t in (_C, _U))


CHUNKS, S0, LAG, SPAN, HEAD, M0 = ((0, 1), (2, 3)), 72, 40, (11.25, 1), 72, 6
PO = (1, 0, 2)
MO = (364, 385, 410, 426, 444, 463)


D0, DS, TS, Q = 0, (0, 0, 0), ((0, 1),), 2


AHEAD = 0
QA, BA = (8, 11, 14, 17, 20, 40, 54, 68, 82, 96, 110, 132, 136, 140), 20
QB = range(20, 144, 14)


def _signed_sum(terms):
    terms = [(c, t) for c, t in terms if c]
    first = next((i for i, (c, _) in enumerate(terms) if c > 0), 0)
    c, acc = terms.pop(first)
    acc = acc if c > 0 else -acc
    for c, t in terms:
        acc = acc + t if c > 0 else acc - t
    return acc


class _Mixer:
    def __init__(self, block):
        self.block, self.known = block, {}

    def __call__(self, coef):
        want = {(i, k): int(c) for i, row in enumerate(coef) for k, c in enumerate(row) if c}
        key = tuple(sorted(want.items()))
        if key not in self.known:
            terms = []
            for have in sorted(self.known, key=lambda h: -len(h)):
                for sign in (1, -1):
                    if all(want.get(pos) == sign * c for pos, c in have):
                        terms.append((sign, self.known[have]))
                        want = {pos: c for pos, c in want.items() if pos not in dict(have)}
                        break
            for pos, c in sorted(want.items()):
                self.known[((pos, 1),)] = self.block(*pos)
                terms.append((c, self.known[((pos, 1),)]))
            self.known[key] = _signed_sum(terms)
        return self.known[key]


class _Sums:
    def __init__(self, done):
        self.done, self.acc = done, {}

    def add(self, key, sign, value, expected):
        if not sign:
            return
        count, neg, tot = self.acc.pop(key, (0, sign < 0, value))
        if count and neg == (sign < 0):
            tot = tot + value
        elif count:
            tot, neg = (value - tot if neg else tot - value), False
        if count + 1 == expected:
            self.done(key, -tot if neg else tot)
        else:
            self.acc[key] = (count + 1, neg, tot)


class _Carry:
    def __init__(self, ref):
        self.ref, self.val = ref, {}

    def __getitem__(self, key):
        return self.val[key] if key in self.val else self.ref[key]

    def __setitem__(self, key, value):
        self.val[key] = value

    def flush(self):
        for key, value in self.val.items():
            self.ref[key] = value
        self.val = {}


def _dot(a, b):
    return lax.dot_general(a, b, (((1,), (0,)), ((), ())), preferred_element_type=F32)


def _dot_nt(a, b):
    return lax.dot_general(a, b, (((1,), (1,)), ((), ())), preferred_element_type=F32)


def _tile(ref, *idx):
    return pltpu.bitcast(ref.bitcast(U32)[idx], BF16)


def stack(*parts):
    parts = [t for t in parts if t is not None]
    return parts[0] if len(parts) == 1 else jnp.concatenate(parts, axis=0)


def _low_half(rows):
    return lax.broadcasted_iota(jnp.int32, (rows, LANES), 1) < 64


def _pair_lhs(t1, t2):
    lo = _low_half(t1[3].shape[0])
    diff = t1[3] - t2[3]
    return (t1[:3] + [jnp.where(lo, t1[4], diff)]
            + t2[:3] + [jnp.where(lo, -diff, t2[4])]
            + [jnp.where(lo, t1[3], t2[3])])


def _pair_rhs(x):
    a, b, c = x[384:448], x[448:512], x[512:576]
    cat = lambda u, v: jnp.concatenate([u, v], axis=0)
    return [x[i * 128:(i + 1) * 128] for i in range(3)] + [cat(c, b), cat(a, c), x[384:512]]


def _pair_matmul(lhs, rhs, dot):
    out = [dot(lhs(8), rhs[5])] * 2
    for i in range(8):
        out[i // 4] = out[i // 4] + dot(lhs(i), rhs[i % 4 if i < 7 else 4])
    return out


def _kernel(xt_hbm, wqkv_hbm, wo_hbm, mem0_ref, wq_hbm, wk_hbm, wv_hbm, wot_hbm, gate_ref,
            out_hbm,
            xt_v, wqkv_v, wo_v, stg_qkv, stg_o, wo_t, wt32, wo32_s, la, gate_s, lo_a, kv_prev, oa_s,
            wb, x32, ga_s, gm_s, mem_s, part_s, o_s, opart_s, b_s, out_v,
            sem_x, sem_wa, sem_wb, sem_out, *, seq, seg, mem):
    nt = seq // LANES
    rows = mem + seg

    def cp_x(j):
        col = j * LANES if isinstance(j, int) else pl.multiple_of(j * LANES, LANES)
        return pltpu.make_async_copy(xt_hbm.at[:, pl.ds(col, LANES)], xt_v.at[j], sem_x.at[j % 3])

    def cp_wqkv(k):
        r = pl.ds(k * 128, min(128, D - k * 128))
        return pltpu.make_async_copy(wqkv_hbm.at[r], wqkv_v.at[r], sem_wa.at[k])

    cp_wo = pltpu.make_async_copy(wo_hbm, wo_v, sem_wa.at[5])

    def cp_unit(unit):
        i, gp = divmod(unit, GP)
        sem = sem_wb.at[unit % 3]
        if i == 3:
            heads = pl.ds(2 * KB * gp, 2 * KB)
            return [pltpu.make_async_copy(wot_hbm.at[heads], stg_o.at[heads], sem)]
        src = (wq_hbm, wk_hbm, wv_hbm)[i].bitcast(U32)
        return [pltpu.make_async_copy(src.at[:, KB * gp + p, :], stg_qkv.at[unit, p], sem)
                for p in range(KB)]

    def start_unit(unit):
        for c in cp_unit(unit):
            c.start()

    def wait_unit(unit):
        for c in cp_unit(unit):
            c.wait()

    def cp_out(j):
        col = j * LANES if isinstance(j, int) else pl.multiple_of(j * LANES, LANES)
        return pltpu.make_async_copy(out_v.at[j], out_hbm.at[:, pl.ds(col, LANES)], sem_out)

    for c in [cp_wqkv(k) for k in (3, 4, 0, 1, 2)] + [cp_x(0), cp_wo, cp_x(1), cp_x(2)]:
        c.start()

    m0 = mem0_ref[...].astype(F32)
    for kk in range(KB):
        mem_s[kk] = m0[:, kk * LANES:(kk + 1) * LANES]
    mem_s[KB] = jnp.concatenate([m0[:, KB * LANES:]] * 2, axis=1)
    for ref in (o_s, opart_s, b_s):
        ref[...] = jnp.zeros(ref.shape, ref.dtype)
    wb[4 * GP, 0, 0:16, :] = jnp.zeros((16, LANES), BF16)
    wo_t[GP, 0, 0, 0:8, :] = jnp.zeros((8, LANES), U32)

    gate = jnp.broadcast_to(gate_ref[...].astype(F32).reshape(1, D), (8, D))
    gate_t = [gate[:, i * 128:(i + 1) * 128] for i in range(4)]
    gate_t.append(jnp.concatenate([gate[:, 512:], gate[:, 512:]], axis=1))

    for i, t in enumerate(_pair_lhs(gate_t, gate_t)):
        gate_s[i] = t
    rp = 8 * DA // 2

    def head_rows(k, g, part, e):
        base = part * D + g * 8 * DA + e
        return stack(*(wt32[k, pl.ds(base + 2 * n, 8, stride=DA), :] for n in range(DA // 2)))

    for k in (3, 4, 0, 1, 2):
        cp_wqkv(k).wait()
        if k == 2:
            start_unit(0)
        rows_k = wqkv_v[k * LANES:min(D, (k + 1) * LANES), :]
        wt32[k] = (rows_k if k < 4 else stack(rows_k, rows_k)).T.astype(F32)
        for g in range(NG if k in (4, 0, 1) else 0):
            part = (4, 0, 1).index(k)
            halves = [[None] * 3 + [head_rows(kk, g, part, e) for kk in (3, 4)] for e in range(2)]
            for n, i in enumerate((3, 7, 8)):
                la[part, g, n] = _pair_lhs(*halves)[i]

    def prep_wo():
        wo32 = wo_v[...].astype(F32)
        for n in range(4):
            wo32_s[n] = wo32[:, n * LANES:(n + 1) * LANES]
        wo32_s[4] = jnp.concatenate([wo32[:, 4 * LANES:]] * 2, axis=1)
        turned = []
        for n in range(5):
            perm = stack(*(wo32_s[n, pl.ds(g * 8 * DA + d, 8, stride=DA), :]
                           for g in range(NG) for d in range(DA))).astype(BF16)
            turned.append([perm[k * LANES:(k + 1) * LANES].T for k in range(4)]
                          + [stack(perm[4 * LANES:], perm[4 * LANES:]).T])
        tiles = [stack(*(t[k] for t in turned))[:D].astype(F32) for k in range(5)]
        for i, t in enumerate(_pair_lhs([t[:D // 2] for t in tiles], [t[D // 2:] for t in tiles])):
            lo_a[i] = t

    by_size = sorted(range(NR), key=lambda r: int(np.abs(_V[r]).sum()))

    def prep_qkv(unit):
        src, dst = stg_qkv.at[unit], wb.at[unit]

        def rows(g, r0, nu):
            u = src[2 * g + nu // 2, r0:r0 + 16, :]
            return pltpu.bitcast(u & jnp.uint32(0xFFFF0000) if nu % 2 else u << 16, F32)

        for e in range(8):
            at, own, shared = pl.ds(16 * e, 16), e // 4, {}
            for g in (own, 1 - own):
                mix = _Mixer(lambda kk, nu: rows(g, kk * LANES + 16 * e, nu))
                for r in by_size:
                    w = mix(_V[r])
                    if r < NH and g == own:
                        shared[r] = w.astype(BF16)
                        dst[2 * NR + r, at, :] = shared[r]
                        w = rows(g, KB * LANES + 16 * (e % 4), r // 2)
                    elif r < NH:
                        w = w - shared[r].astype(F32)
                    dst[g * NR + r, at, :] = w.astype(BF16)
                yield

    def turn_out(gp):
        words = lambda head, r0, n: _tile(stg_o, 2 * KB * gp + head, pl.ds(r0 // 2, n // 2))
        for head in range(2 * KB + 1):
            for nu in range(KB):
                if head < 2 * KB:
                    tile = words(head, nu * LANES, LANES)
                else:
                    tile = stack(*(words(g * KB + nu, KB * LANES, 64) for g in range(2)))
                wo_t[gp, head, nu] = pltpu.bitcast(tile.T, U32)
            yield

    def prep_out(gp):
        dst, lo = wb.at[3 * GP + gp], _low_half(16)
        for e in range(8):
            at, first = pl.ds(16 * e, 16), {}
            rows = lambda head, nu: pltpu.bitcast(
                wo_t[gp, head, nu, 8 * e:8 * e + 8, :], BF16).astype(F32)
            for g in range(2):
                mix = _Mixer(lambda kk, nu: rows(g * KB + kk, nu))
                for r in by_size:
                    w = mix(_V[r])
                    if r >= NH:
                        dst[g * NR + r, at, :] = w.astype(BF16)
                    elif g == 0:
                        first[r] = w
                    else:
                        z, t = jnp.where(lo, first[r], w).astype(BF16), rows(2 * KB, r // 2)
                        dst[2 * NR + r, at, :] = z
                        dst[r, at, :] = jnp.where(lo, t, first[r] - z.astype(F32)).astype(BF16)
                        dst[NR + r, at, :] = jnp.where(lo, w - z.astype(F32), t).astype(BF16)
            yield

    lane = lax.broadcasted_iota(jnp.int32, (8, LANES), 1)

    def exchange(idx, pair, first):
        at = pl.ds(8 * idx, 8)
        prev = None if first else kv_prev.bitcast(U32)[at, :]
        kv_prev[16 * idx:16 * idx + 16, :] = jnp.concatenate(pair, axis=0).astype(BF16)
        cur = kv_prev.bitcast(U32)[at, :]
        return (jnp.broadcast_to(cur[:, 0:1], (8, LANES)) if first else prev), cur

    def to_rows(j):
        t0 = j * LANES if isinstance(j, int) else pl.multiple_of(j * LANES, LANES)
        xt = _tile(xt_v, j)
        tiles = [xt[kk * LANES:(kk + 1) * LANES].T for kk in range(KB)]
        tiles.append(jnp.concatenate([xt[KB * LANES:]] * 2, axis=0).T)
        for kk, t in enumerate(tiles):
            for r0 in range(0, LANES, 32):
                x32[kk, pl.ds(t0 + r0, 32), :] = t[r0:r0 + 32].astype(F32)
                yield

    def attend(j, first, parts, outs):
        get = lambda g, part, dd: [t[dd * 8:dd * 8 + 8] for t in parts[g, part]]
        items = [(g, part, dd) for g in range(NG) for part in (1, 2) for dd in range(DA // 2)]

        def shifts(g, part, dd):
            prev, cur = exchange((2 * g + part - 1) * (DA // 2) + dd, get(g, part, dd), first)
            return [cur] + [pltpu.roll(jnp.where(lane >= LANES - DIL * w, prev, cur), DIL * w, 1)
                            for w in range(1, WIN)]

        gsig = 1.0 / (1.0 + jnp.exp(-parts[0, 1][0][rp:]))
        gm_s[j] = 1.0 - gsig
        early = []
        for n, (g, part, dd) in enumerate(items):
            if n + AHEAD < len(items):
                early.append(shifts(*items[n + AHEAD]))
            both = [pltpu.bitcast(t, BF16).astype(F32) for t in early.pop(0)]
            if part == 1:
                q = get(g, 0, dd)
                terms = [q[0] * t[0:8] + q[1] * t[8:16] for t in both]
                logit = terms if dd == 0 else [a + b for a, b in zip(logit, terms)]
            else:
                outs.append(functools.reduce(jnp.add, [
                    jnp.concatenate([p] * 2, axis=0) * t for p, t in zip(prob, both)]))
            if (part, dd) == (1, DA // 2 - 1):
                logit = [t * (DA ** -0.5) for t in logit]
                if first:
                    logit = [jnp.where(lane >= DIL * w, t, NEG) for w, t in enumerate(logit)]
                top = functools.reduce(jnp.maximum, logit)
                ex = [jnp.exp(t - top) for t in logit]
                inv = gsig / functools.reduce(jnp.add, ex)
                prob = [e * inv for e in ex]
            yield

    def paced(job, src, dst, when, back):
        results = []

        def dot(left, right):
            if len(results) in when:
                if src is not None and len(results) >= back:
                    src[...] = pltpu.bitcast(results[-back][0:8], U32)
                next(job, None)
                left = stack(left[:-8], left[-8:] + pltpu.bitcast(dst[...], F32))
            results.append(_dot(left, right))
            return results[-1]

        return dot

    spare_qkv, spare_t = stg_qkv.at[3 * GP, 0, 0:8], wo_t.at[GP, 0, 1, 0:8]
    zero_t, zero_w = wo_t.at[GP, 0, 0, 0:8], wb.bitcast(U32).at[4 * GP, 0, 0:8]

    def a_out(j, dot):
        rhs = _pair_rhs(_tile(oa_s, slice(None)))
        for c in range(4):
            halves = _pair_matmul(lambda i: lo_a[i, c * rp:(c + 1) * rp, :], rhs, dot)
            ga_s[j, c * rp:(c + 1) * rp, :] = halves[0]
            ga_s[j, D // 2 + c * rp:D // 2 + (c + 1) * rp, :] = halves[1]

    def a_tile(j, first, dot):
        parts, outs = {}, []
        window = attend(j, first, parts, outs)
        list(to_rows(j))
        rhs = _pair_rhs(_tile(xt_v, j))
        for g in range(NG):
            for part in (1, 0, 2):
                def left(i):
                    if i in (3, 7, 8):
                        w = la[part, g, (3, 7, 8).index(i)]
                    else:
                        w = head_rows(i % 4, g, part, i // 4)
                    return stack(w, gate_s[i]) if (g, part) == (0, 1) else w

                parts[g, part] = _pair_matmul(left, rhs, dot)
                if part != 1:
                    list(itertools.islice(window, DA // 2))
        if not first:
            a_out(j - 1, dot)
        oa_s[...] = jnp.concatenate(outs, axis=0).astype(BF16)

    cp_x(0).wait()
    a_tile(0, True, _dot)
    cp_wo.wait()
    start_unit(1)
    prep_wo()
    start_unit(2)

    def a_loop(units, work, *pacing):
        def body(j, carry):
            cp_x(j).wait()
            pl.when(j + 2 < nt)(lambda: cp_x(j + 2).start())
            for unit in units:
                pl.when(j == unit + 1)(functools.partial(wait_unit, unit))
            job = work(j - 1 - units[0])
            a_tile(j, False, paced(job, *pacing))
            list(job)
            for unit in units:
                if unit + 3 < 4 * GP:
                    pl.when(j == unit + 1)(functools.partial(start_unit, unit + 3))
            return carry

        lax.fori_loop(units[0] + 1, units[-1] + 2, body, 0)

    a_loop(range(3 * GP), prep_qkv, spare_qkv, zero_w, QA, BA)
    a_loop(range(3 * GP, nt - 1), turn_out, None, zero_t, QB, 0)
    wait_unit(4 * GP - 1)

    qi = lax.broadcasted_iota(jnp.int32, (rows, rows), 0)
    ki = lax.broadcasted_iota(jnp.int32, (rows, rows), 1)
    mask = (qi >= seg) | (ki >= seg) | (qi >= ki)
    part, o_prev, opart, b_rows = (_Carry(r) for r in (part_s, o_s, opart_s, b_s))
    ahead = {}

    def b_step(u, t0, memv, project_only=False, output_only=False):
        odd = u % 2
        keep = lambda slots: [s for s in slots if s["tok"] or memv]
        qs, os_ = keep(_PHASES[odd]), keep(_PHASES[1 - odd])
        lhs, shared, tok, mrow, full, soft, o_mem, o_mix, o_left, o_host, new = ({} for _ in range(11))
        clock, queue = [0], {}

        def later(delay, fn, *args):
            queue.setdefault(clock[0] + delay, []).append((fn, args))

        def tick():
            for fn, args in queue.pop(clock[0], ()):
                fn(*args)
            clock[0] += 1

        def spread(sums, key, slots, s, tok_rows, mem_rows):
            for nu in range(KB):
                if memv:
                    sums.add(key + (nu, 2), s["c"][nu], mem_rows, sum(abs(o["c"][nu]) for o in slots))
                for mu in range(2 if s["tok"] else 0):
                    sums.add(key + (nu, mu), _C[s["r"]][mu][nu], tok_rows,
                             sum(abs(_C[o["r"]][mu][nu]) for o in slots if o["tok"]))

        x_mix = _Mixer(lambda mu, kk: x32[kk, pl.ds(t0 + mu * seg, seg), :])
        c_mix = _Mixer(lambda mu, _: x32[KB, pl.ds(t0 + mu * seg, seg), :])
        m_mix = _Mixer(lambda _, kk: memv[kk])

        def q_left(e, t):
            s = qs[e]
            if (e, t) not in lhs:
                left = stack(x_mix(_U[s["r"]]) if s["tok"] else None,
                             m_mix([s["a"]]) if memv else None)
                if s["r"] < NH and t < 2:
                    c = stack(c_mix(_TAIL_IN[s["r"]][:, None]),
                              _signed_sum([(sum(s["c"]), memv[KB])]) if memv else None)
                    left = jnp.where(_low_half(c.shape[0]), *((c, left), (left, c))[t])
                lhs[e, t] = left
            return lhs[e, t]

        def q_total(key, value):
            i, g, nu, mu = key
            h = g * KB + nu
            if mu == 2:
                mrow[i, h] = value
            elif odd:
                part[i, h, mu] = value
            elif mu == 0:
                tok[i, h] = value + part[i, h, mu]
            else:
                ahead[i, h] = (value + part[i, h, mu]).astype(BF16 if i else F32)
            cur = (ahead if odd else tok).get((i, h))
            if (i, h) in mrow and cur is not None and (i, h) not in full:
                full[i, h] = stack(cur.astype(BF16 if i else F32),
                                   mrow[i, h].astype(BF16 if i else F32))

        q_sums = _Sums(q_total)

        def q_pass(e, i, gp, t):
            s = qs[e]
            p = _dot(q_left(e, t), _tile(wb, i * GP + gp, t * NR + s["r"]))
            if t == 2:
                shared[e, i, gp] = p
                return

            def use():
                r = p + shared[e, i, gp] if s["r"] < NH else p
                spread(q_sums, (i, 2 * gp + t), qs, s, r[:seg], r[-mem:])

            later(D0, use)

        def scores(h):
            def stages():
                raw = _dot_nt(full[0, h], full[1, h])
                yield
                s = jnp.where(mask, raw, NEG * DB ** 0.5)
                top = jnp.max(s, axis=-1, keepdims=True)
                yield
                e = jnp.exp2((s - top) * (DB ** -0.5 * LOG2E))
                total = jnp.sum(e, axis=-1, keepdims=True)
                yield
                inv = pltpu.reciprocal(total, approx=True)
                soft[h] = e * (inv * (2.0 - total * inv))
                yield

            run = stages()
            next(run)
            for delay in DS:
                later(delay, next, run)

        def values(h):
            o = _dot(soft[h], full[2, h])
            o_mem[h] = o[seg:]
            if odd:
                o_prev[0, h], o_prev[1, h] = ahead["o", h], o[:seg]
            else:
                ahead["o", h] = o[:seg]

        def o_rows(e, gp, t):
            s = os_[e]
            if (e, gp, t) not in o_left:
                g = 2 * gp + t
                if t == 2:
                    o_left[e, gp, t] = o_rows(e, gp, 0) + o_rows(e, gp, 1)
                    return o_left[e, gp, t]
                if g not in o_mix:
                    o_mix[g] = (_Mixer(lambda _, kk: o_mem[g * KB + kk]),
                                _Mixer(lambda mu, kk: o_prev[mu, g * KB + kk]))
                o_left[e, gp, t] = stack(o_mix[g][0]([s["a"]]) if memv else None,
                                         o_mix[g][1](_U[s["r"]]) if s["tok"] else None)
            return o_left[e, gp, t]

        def o_total(key, value):
            nu, mu = key
            if mu == 2:
                new[nu] = value if nu < KB else value + pltpu.roll(value, 64, 1)
            elif odd:
                opart[nu, mu] = value
            else:
                b_rows[nu, (u - 2) % 4 + mu] = value + opart[nu, mu]

        out_sums = _Sums(o_total)

        def o_product(key, value):
            e, t = key
            s = os_[e]
            if s["r"] < NH:
                o_host[key] = value
                if any((e, t_) not in o_host for t_ in range(3)):
                    return
                lo = _low_half(value.shape[0])
                value = o_host[e, 2] + jnp.where(lo, o_host[e, 1], o_host[e, 0])
                y = jnp.where(lo, o_host[e, 0], o_host[e, 1])
                if memv:
                    out_sums.add((KB, 2), sum(s["a"]), y[:mem], KB)
                for mu in range(2):
                    out_sums.add((KB, mu), _TAIL_OUT[s["r"]][mu], y[-seg:],
                                 sum(abs(_TAIL_OUT[o["r"]][mu]) for o in os_ if o["r"] < NH))
            spread(out_sums, (), os_, s, value[-seg:], value[:mem])

        o_sums = _Sums(o_product)

        def o_pass(e, gp, t):
            host = os_[e]["r"] < NH
            p = _dot(o_rows(e, gp, t), _tile(wb, 3 * GP + gp, t * NR + os_[e]["r"]))
            later(D0, o_sums.add, (e, t if host else 0), 1, p, GP if host else 2 * GP)

        todo = []
        tiles = lambda s, ts: (2,) + ts if s["r"] < NH and 0 in ts else ts
        if not output_only:
            units = [(i, gp, t) for gp in range(GP) for i in PO for t in TS]
            todo = [(s["tok"], q_pass, e, i, gp, t_) for i, gp, t in units
                    for e, s in enumerate(qs) for t_ in tiles(s, t)]
            last = [max(e for e, s in enumerate(_PHASES[odd]) if s["tok"] and s["c"][nu])
                    for nu in range(KB)]
            ready = lambda e, t: 99 if qs[e]["r"] < NH and t < 2 else max(
                last[kk] for kk in range(KB) if qs[e]["a"][kk])
            todo[:HEAD] = sorted(todo[:HEAD], key=lambda p: ready(p[2], p[5]))
        if not project_only:
            todo += [(s["tok"], o_pass, e, gp, t) for pairs in CHUNKS for e, s in enumerate(os_)
                     for gp in pairs for t in tiles(s, (0, 1))]
        long_, short = ([p[1:] for p in todo if p[0] == tok] for tok in (True, False))
        extra = {}
        for h in range(HB if memv else 0):
            gp, n = divmod(h, 2 * KB)
            at = (90 * gp + S0 + int(SPAN[gp == GP - 1] * (n // Q * Q))) // Q * Q
            extra.setdefault(at, []).append((scores, h))
            extra.setdefault(at + LAG, []).append((values, h))
        issued = 0
        for n, p in enumerate(long_):
            for fn, *args in extra.get(n, []) + [p]:
                if issued % 4 == 0 and short and n >= (480 + M0 - 5 * len(short) if len(short) > 24 else MO[6 - len(short) // 4]):
                    for fn_s, *args_s in short[:4]:
                        fn_s(*args_s)
                        tick()
                    del short[:4]
                fn(*args)
                tick()
                issued += 1
        assert not short
        while queue:
            tick()
        return new

    def emit_tile(j):
        for nu in range(KB + 1):
            bt = jnp.concatenate([b_s[nu, 0], b_s[nu, 1], b_rows.val.pop((nu, 2)),
                                  b_rows.val.pop((nu, 3))], axis=0).T
            bt = bt if nu < KB else bt[:64] + bt[64:]
            at = pl.ds(nu * LANES, bt.shape[0])
            gm = jnp.concatenate([gm_s[j]] * (bt.shape[0] // 8), axis=0)
            out_v[j, at, :] = (ga_s[j, at, :] + gm * bt).astype(out_v.dtype)

    list(turn_out(GP - 1))
    a_out(nt - 1, _dot)
    b_step(3, 0, None, project_only=True)
    part.flush()
    for gp in range(2):
        list(prep_out(gp))

    @pl.loop(2, GP)
    def _(gp):
        list(prep_out(gp))

    def b_body(j, carry):
        memv = {kk: mem_s[kk] for kk in range(KB + 1)}
        for u in range(4):
            t0 = jnp.minimum(j * LANES + (u + 1) // 2 * 2 * seg, seq - 2 * seg)
            memv = b_step(u, pl.multiple_of(t0, seg), memv)
            if u == 0:
                emit_tile(jnp.maximum(j - 1, 0))
        for kk, t in memv.items():
            mem_s[kk] = t
        for c in (part, o_prev, opart, b_rows):
            c.flush()
        pl.when(j > 0)(lambda: cp_out(j - 1).start())
        return carry

    lax.fori_loop(0, nt, b_body, 0)
    b_step(0, None, None, output_only=True)
    emit_tile(nt - 1)
    cp_out(nt - 1).start()
    for j in range(nt):
        cp_out(j).wait()


@functools.partial(jax.jit, static_argnames=("B_seg_len",))
def pallas_gated_mix__sliding_local_dilated__memory_aug_recurrent_mem_tr__prompt_kernel(
    A_x: jax.Array,
    A_wqkv: jax.Array,
    A_wo: jax.Array,
    B_x: jax.Array,
    B_mem0: jax.Array,
    B_Wq: jax.Array,
    B_Wk: jax.Array,
    B_Wv: jax.Array,
    B_Wo: jax.Array,
    B_seg_len: int,
    gate_w: jax.Array,
):
    del B_x
    batch, seq, width = A_x.shape
    mem, seg = B_mem0.shape[1], int(B_seg_len)
    nt = seq // LANES
    assert batch == 1 and width == D and nt == 4 * GP and seq % LANES == 0
    assert B_Wq.shape == (D, HB, DB) and mem == 8 and 4 * seg == LANES

    hbm = pl.BlockSpec(memory_space=pl.ANY)
    vmem = pl.BlockSpec(memory_space=pltpu.VMEM)
    out_t = pl.pallas_call(
        functools.partial(_kernel, seq=seq, seg=seg, mem=mem),
        out_shape=jax.ShapeDtypeStruct((D, seq), A_x.dtype),
        in_specs=[hbm, hbm, hbm, vmem, hbm, hbm, hbm, hbm, vmem],
        out_specs=hbm,
        scratch_shapes=[
            pltpu.VMEM((nt, D, LANES), BF16),
            pltpu.VMEM((D, 3 * D), BF16),
            pltpu.VMEM((D, D), BF16),
            pltpu.VMEM((3 * GP + 1, KB, D, DB), U32),
            pltpu.VMEM((HB, D, DB), BF16),
            pltpu.VMEM((GP + 1, 2 * KB + 1, KB, 64, LANES), U32),
            pltpu.VMEM((5, 3 * D, LANES), F32),
            pltpu.VMEM((5, D, LANES), F32),
            pltpu.VMEM((3, NG, 3, 8 * DA // 2, LANES), F32),
            pltpu.VMEM((12, 8, LANES), F32),
            pltpu.VMEM((9, D // 2, LANES), F32),
            pltpu.VMEM((2 * D, LANES), BF16),
            pltpu.VMEM((D, LANES), BF16),
            pltpu.VMEM((4 * GP + 1, 2 * NR + NH, LANES, LANES), BF16),
            pltpu.VMEM((KB + 1, seq, LANES), F32),
            pltpu.VMEM((nt, D, LANES), F32),
            pltpu.VMEM((nt, 8, LANES), F32),
            pltpu.VMEM((2 * KB, mem, LANES), F32),
            pltpu.VMEM((3, HB, 2, seg, LANES), F32),
            pltpu.VMEM((2, HB, seg, LANES), F32),
            pltpu.VMEM((KB + 1, 2, seg, LANES), F32),
            pltpu.VMEM((KB + 1, 2, seg, LANES), F32),
            pltpu.VMEM((nt, D, LANES), A_x.dtype),
            pltpu.SemaphoreType.DMA((3,)),
            pltpu.SemaphoreType.DMA((6,)),
            pltpu.SemaphoreType.DMA((3,)),
            pltpu.SemaphoreType.DMA(()),
        ],
        compiler_params=pltpu.CompilerParams(vmem_limit_bytes=110 * 1024 * 1024),
        name="gated_mix_kernel",
    )(A_x[0].T, A_wqkv, A_wo, B_mem0[0], B_Wq, B_Wk, B_Wv, B_Wo.transpose(0, 2, 1), gate_w)
    return out_t.T[None]
```

```python
import functools
import itertools

import jax
import jax.numpy as jnp
import numpy as np
from jax import lax
import jax.experimental.pallas as pl
import jax.experimental.pallas.tpu as pltpu

F32, BF16, U32 = jnp.float32, jnp.bfloat16, jnp.uint32

D = 576
LANES = 128
HA, DA = 32, 18
WIN, DIL = 8, 2
HB, DB = 32, 128
NEG = -1000000000.0
LOG2E = 1.4426950408889634
NG = HA // 8

KB = 4
GP = HB // (2 * KB)

_HK = (
    (".... +...", "+.-. -... .... -...", "+... +..."),
    ("+... -...", "+-.- .... -... ....", "+... ...."),
    (".+.. .-..", ".... +-.. .+.. ....", ".... .+.."),
    (".+.. ....", ".-.. .+-. .... ....", ".+.. .+.."),
    (".... ..+.", ".... ..-. -.+. .+-.", ".... ..+."),
    ("..+. ....", "..-. ...+ .-+- ....", "..+. ...."),
    ("...+ ...-", ".... ...- ...+ ++.-", ".... ...+"),
    ("...+ ....", "...- ...- .... .+-+", "...+ ...+"),
    (".... ++..", ".... +... .... ....", ".... ++.."),
    ("++.. ....", ".+.. .... .... ....", "++.. ...."),
    (".+.. +...", ".-.. +... .... ....", "+... .-.."),
    ("+.+. -.-.", ".... .... -... ....", ".... +.+."),
    ("+.+. ....", "..+. .... .... ....", "+.+. +.+."),
    ("+.+. -...", "..-. .... +... ....", "+... +.+."),
    (".... +..+", ".... .... .... +...", ".... +..+"),
    ("+..+ ....", "...+ .... .... ....", "+..+ ...."),
    ("...+ +...", "...- .... .... +...", "+... ...-"),
    (".... .++.", ".... ..+. .... .-..", ".++. .++."),
    (".++. .--.", ".... ...- .+.. ....", ".++. ...."),
    (".+.. .--.", ".... ..+. .-.. ....", ".++. .+.."),
    (".... ..++", ".... .... .... .-+.", "..++ ..++"),
    ("..++ ..--", ".... ...- ...+ ....", "..++ ...."),
    ("...+ ..--", ".... ...+ ...- .-+.", "..++ ...+"),
    (".... .+++", ".... .... .... .+..", ".... .+++"),
    (".+++ ....", ".... ...+ .... ....", ".+++ ...."),
    ("...+ .++.", ".... ...- .... .+..", ".++. ...-"),
)
_U, _V, _C = (np.array([[["-.+".index(ch) - 1 for ch in row] for row in prod[i].split()]
                        for prod in _HK]) for i in range(3))
NR = len(_HK)
assert np.array_equal(np.einsum("rak,rln,rbm->akblnm", _U, _V, _C),
                      np.einsum("ab,kl,nm->akblnm", *(np.eye(n, dtype=int) for n in (2, KB, KB))))


def _phase(products):
    tiles = [max(r, ~r) for r in products]
    dual = np.rint(np.linalg.inv(_V[tiles].reshape(len(tiles), -1)).T).astype(int)
    slots = []
    for r, d in zip(products, dual.reshape(-1, KB, KB)):
        i, j = np.argwhere(d)[0]
        a, c = d[:, j] * d[i, j], d[i]
        assert np.array_equal(np.outer(a, c), d)
        slots.append(dict(r=max(r, ~r), tok=r >= 0, a=a.tolist(), c=c.tolist()))
    return slots


_PHASES = (_phase((11, 8, ~9, 4, 2, 23, 17, ~13, 25, 20, 22, 7, ~19, 16, 15, 1)),
           _phase((24, 21, ~16, 18, 19, 3, 10, ~22, 9, 5, 12, 13, ~25, 0, 14, 6)))
assert sorted(s["r"] for ph in _PHASES for s in ph if s["tok"]) == list(range(NR))

NH = 2 * KB
assert all(sorted(s["r"] // 2 for s in ph if s["r"] < NH) == list(range(KB)) for ph in _PHASES)
assert all(np.abs(s[k]).tolist() == np.eye(KB)[s["r"] // 2].tolist()
           for ph in _PHASES for s in ph if s["r"] < NH for k in "ac")
_TAIL_IN, _TAIL_OUT = (
    np.concatenate([np.rint(np.linalg.inv(t[2 * n:2 * n + 2, :, n]).T).astype(int)
                    for n in range(KB)]) for t in (_C, _U))


CHUNKS, S0, LAG, SPAN, HEAD, M0 = ((0, 1), (2, 3)), 72, 40, (11.25, 1), 72, 6
PO = (1, 0, 2)
MO = (364, 385, 410, 426, 444, 463)


D0, DS, TS, Q = 0, (0, 0, 0), ((0, 1),), 2


SEQ, RE, RO = 0, 8, 48
ORD = (9, 8, 10, 19, 2, 3, 23, 24, 25, 17, 18, 20, 21, 22, 12, 11, 13, 4, 5, 15, 14, 16, 6, 7, 0, 1)
CUT = (1,)
QA = ((10, 16, 30, 45, 61, 77, 92, 108, 124, 152, 159, 166, 173), 20)
QB = ((10, 16, 22, 42, 58, 75, 91, 108, 146, 150, 155, 160, 165, 170, 175), 24)
QC = (range(8, 54, 4), 16)


def _signed_sum(terms):
    terms = [(c, t) for c, t in terms if c]
    first = next((i for i, (c, _) in enumerate(terms) if c > 0), 0)
    c, acc = terms.pop(first)
    acc = acc if c > 0 else -acc
    for c, t in terms:
        acc = acc + t if c > 0 else acc - t
    return acc


class _Mixer:
    def __init__(self, block):
        self.block, self.known = block, {}

    def __call__(self, coef):
        want = {(i, k): int(c) for i, row in enumerate(coef) for k, c in enumerate(row) if c}
        key = tuple(sorted(want.items()))
        if key not in self.known:
            terms = []
            for have in sorted(self.known, key=lambda h: -len(h)):
                for sign in (1, -1):
                    if all(want.get(pos) == sign * c for pos, c in have):
                        terms.append((sign, self.known[have]))
                        want = {pos: c for pos, c in want.items() if pos not in dict(have)}
                        break
            for pos, c in sorted(want.items()):
                self.known[((pos, 1),)] = self.block(*pos)
                terms.append((c, self.known[((pos, 1),)]))
            self.known[key] = _signed_sum(terms)
        return self.known[key]


class _Sums:
    def __init__(self, done):
        self.done, self.acc = done, {}

    def add(self, key, sign, value, expected):
        if not sign:
            return
        count, neg, tot = self.acc.pop(key, (0, sign < 0, value))
        if count and neg == (sign < 0):
            tot = tot + value
        elif count:
            tot, neg = (value - tot if neg else tot - value), False
        if count + 1 == expected:
            self.done(key, -tot if neg else tot)
        else:
            self.acc[key] = (count + 1, neg, tot)


class _Carry:
    def __init__(self, ref):
        self.ref, self.val = ref, {}

    def __getitem__(self, key):
        return self.val[key] if key in self.val else self.ref[key]

    def __setitem__(self, key, value):
        self.val[key] = value

    def flush(self):
        for key, value in self.val.items():
            self.ref[key] = value
        self.val = {}


def _dot(a, b):
    return lax.dot_general(a, b, (((1,), (0,)), ((), ())), preferred_element_type=F32)


def _dot_nt(a, b):
    return lax.dot_general(a, b, (((1,), (1,)), ((), ())), preferred_element_type=F32)


def _tile(ref, *idx):
    return pltpu.bitcast(ref.bitcast(U32)[idx], BF16)


def stack(*parts):
    parts = [t for t in parts if t is not None and t.shape[0]]
    return parts[0] if len(parts) == 1 else jnp.concatenate(parts, axis=0)


def _low_half(rows):
    return lax.broadcasted_iota(jnp.int32, (rows, LANES), 1) < 64


def _pair_lhs(t1, t2):
    lo = _low_half(t1[3].shape[0])
    diff = t1[3] - t2[3]
    return (t1[:3] + [jnp.where(lo, t1[4], diff)]
            + t2[:3] + [jnp.where(lo, -diff, t2[4])]
            + [jnp.where(lo, t1[3], t2[3])])


def _pair_rhs(x):
    a, b, c = x[384:448], x[448:512], x[512:576]
    cat = lambda u, v: jnp.concatenate([u, v], axis=0)
    return [x[i * 128:(i + 1) * 128] for i in range(3)] + [cat(c, b), cat(a, c), x[384:512]]


def _pair_matmul(lhs, rhs, dot):
    out = [dot(lhs(8), rhs[5])] * 2
    for i in range(8):
        out[i // 4] = out[i // 4] + dot(lhs(i), rhs[i % 4 if i < 7 else 4])
    return out


def _kernel(xt_hbm, wqkv_hbm, wo_hbm, mem0_ref, wq_hbm, wk_hbm, wv_hbm, wot_hbm, gate_ref,
            out_hbm,
            xt_v, wqkv_v, wo_v, stg_qkv, stg_o, wo_t, wt32, wo32_s, la, lo_a, kv_prev, oa_s,
            wb, x32, ga_s, gm_s, mem_s, part_s, o_s, opart_s, b_s, out_v,
            sem_x, sem_wa, sem_wb, sem_out, *, seq, seg, mem):
    nt = seq // LANES
    rows = mem + seg

    def cp_x(j):
        col = j * LANES if isinstance(j, int) else pl.multiple_of(j * LANES, LANES)
        return pltpu.make_async_copy(xt_hbm.at[:, pl.ds(col, LANES)], xt_v.at[j], sem_x.at[j & 3])

    def cp_wqkv(k):
        r = pl.ds(k * 128, min(128, D - k * 128))
        return pltpu.make_async_copy(wqkv_hbm.at[r], wqkv_v.at[r], sem_wa.at[k])

    cp_wo = pltpu.make_async_copy(wo_hbm, wo_v, sem_wa.at[5])

    def start_unit(unit):
        i, gp = divmod(unit, GP)
        src = (wq_hbm, wk_hbm, wv_hbm)[i].bitcast(U32)
        for p in range(KB):
            pltpu.make_async_copy(src.at[:, KB * gp + p, :], stg_qkv.at[unit, p],
                                  sem_wb.at[unit & 3]).start()

    def start_more(j):
        if j + 2 < 3 * GP:
            start_unit(j + 2)
        h0, h1 = (2 * t if t < 10 else min(HB, 7 * t - 45) for t in (j - 1, j))
        if h1 > h0:
            pltpu.make_async_copy(wot_hbm.at[h0:h1], stg_o.at[h0:h1], sem_wa.at[6]).start()

    def cp_out(j):
        col = j * LANES if isinstance(j, int) else pl.multiple_of(j * LANES, LANES)
        return pltpu.make_async_copy(out_v.at[j], out_hbm.at[:, pl.ds(col, LANES)], sem_out)

    for c in [cp_wqkv(k) for k in (3, 4, 0, 1, 2)] + [cp_x(0)]:
        c.start()

    m0 = mem0_ref[...].astype(F32)
    for kk in range(KB):
        mem_s[kk] = m0[:, kk * LANES:(kk + 1) * LANES]
    mem_s[KB] = jnp.concatenate([m0[:, KB * LANES:]] * 2, axis=1)
    for ref in (o_s, opart_s, b_s):
        ref[...] = jnp.zeros(ref.shape, ref.dtype)
    wb[4 * GP, 0, 0:16, :] = jnp.zeros((16, LANES), BF16)

    gate = jnp.broadcast_to(gate_ref[...].astype(F32).reshape(1, D), (8, D))
    gate_t = [gate[:, i * 128:(i + 1) * 128] for i in range(4)]
    gate_t.append(jnp.concatenate([gate[:, 512:], gate[:, 512:]], axis=1))

    entries = [None] * 2 + [(g - part // 2, part, n) for g in range(NG + 1) for n in range(DA // 2)
                            for part in (1, 0, 2) if 0 <= g - part // 2 < NG]
    if SEQ:
        entries = [None] * 2 + [(g, part, n) for g in range(NG) for parts in ((1, 0), (2,))
                                for n in range(DA // 2) for part in parts]

    def feature_rows(k, e):
        return stack(*(gate_t[k] if ent is None else
                       wt32[k, pl.ds(ent[1] * D + ent[0] * 8 * DA + 2 * ent[2] + e, 8, stride=DA), :]
                       for ent in entries))

    for k in (3, 4, 0, 1, 2):
        cp_wqkv(k).wait()
        if k == 2:
            for c in (cp_wo, cp_x(1)):
                c.start()
            start_unit(0)
        rows_k = wqkv_v[k * LANES:min(D, (k + 1) * LANES), :]
        wt32[k] = (rows_k if k < 4 else stack(rows_k, rows_k)).T.astype(F32)
        for e in range(2 if k < 3 else 0):
            la[4 * e + k] = feature_rows(k, e).astype(BF16)
        if k == 4:
            mixed = _pair_lhs(*([None] * 3 + [feature_rows(3, e), feature_rows(4, e)]
                                for e in range(2)))
            for i in (3, 7, 8):
                la[i] = mixed[i].astype(BF16)

    def prep_wo():
        wo32 = wo_v[...].astype(F32)
        for n in range(4):
            wo32_s[n] = wo32[:, n * LANES:(n + 1) * LANES]
        wo32_s[4] = jnp.concatenate([wo32[:, 4 * LANES:]] * 2, axis=1)
        turned = []
        for n in range(5):
            perm = stack(*(wo32_s[n, pl.ds(g * 8 * DA + d, 8, stride=DA), :]
                           for g in range(NG) for d in range(DA))).astype(BF16)
            turned.append([perm[k * LANES:(k + 1) * LANES].T for k in range(4)]
                          + [stack(perm[4 * LANES:], perm[4 * LANES:]).T])
        tiles = [stack(*(t[k] for t in turned))[:D].astype(F32) for k in range(5)]
        for i, t in enumerate(_pair_lhs([t[:D // 2] for t in tiles], [t[D // 2:] for t in tiles])):
            lo_a[i] = t.astype(BF16)

    by_size = ORD

    def prep_qkv(unit):
        src, dst = stg_qkv.at[unit], wb.at[unit]

        def rows(g, r0, nu):
            u = src[2 * g + nu // 2, r0:r0 + 16, :]
            return pltpu.bitcast(u & jnp.uint32(0xFFFF0000) if nu % 2 else u << 16, F32)

        for e in range(8):
            at, own, shared = pl.ds(16 * e, 16), e // 4, {}
            for g in (own, 1 - own):
                mix = _Mixer(lambda kk, nu: rows(g, kk * LANES + 16 * e, nu))
                for r in by_size:
                    w = mix(_V[r])
                    if r < NH and g == own:
                        shared[r] = w.astype(BF16)
                        dst[2 * NR + r, at, :] = shared[r]
                        w = rows(g, KB * LANES + 16 * (e % 4), r // 2)
                    elif r < NH:
                        w = w - shared[r].astype(F32)
                    dst[g * NR + r, at, :] = w.astype(BF16)
                    if r in CUT:
                        yield

    def turn_out(gp):
        words = lambda head, r0, n: _tile(stg_o, 2 * KB * gp + head, pl.ds(r0 // 2, n // 2))
        for head in range(2 * KB + 1):
            for nu in range(KB):
                if head < 2 * KB:
                    tile = words(head, nu * LANES, LANES)
                else:
                    tile = stack(*(words(g * KB + nu, KB * LANES, 64) for g in range(2)))
                wo_t[gp, head, nu] = pltpu.bitcast(tile.T, U32)

    def prep_out(gp):
        dst, lo = wb.at[3 * GP + gp], _low_half(16)
        for e in range(8):
            at, first = pl.ds(16 * e, 16), {}
            rows = lambda head, nu: pltpu.bitcast(
                wo_t[gp, head, nu, 8 * e:8 * e + 8, :], BF16).astype(F32)
            for g in range(2):
                mix = _Mixer(lambda kk, nu: rows(g * KB + kk, nu))
                for r in by_size:
                    w = mix(_V[r])
                    if r >= NH:
                        dst[g * NR + r, at, :] = w.astype(BF16)
                    elif g == 0:
                        first[r] = w
                    else:
                        z, t = jnp.where(lo, first[r], w).astype(BF16), rows(2 * KB, r // 2)
                        dst[2 * NR + r, at, :] = z
                        dst[r, at, :] = jnp.where(lo, t, first[r] - z.astype(F32)).astype(BF16)
                        dst[NR + r, at, :] = jnp.where(lo, w - z.astype(F32), t).astype(BF16)
                    if r in CUT:
                        yield

    lane = lax.broadcasted_iota(jnp.int32, (8, LANES), 1)

    def exchange(idx, pair, first):
        at = pl.ds(8 * idx, 8)
        prev = None if first else kv_prev.bitcast(U32)[at, :]
        kv_prev[16 * idx:16 * idx + 16, :] = jnp.concatenate(pair, axis=0).astype(BF16)
        cur = kv_prev.bitcast(U32)[at, :]
        return (jnp.broadcast_to(cur[:, 0:1], (8, LANES)) if first else prev), cur

    def to_rows(j):
        t0 = j * LANES if isinstance(j, int) else pl.multiple_of(j * LANES, LANES)
        xt = _tile(xt_v, j)
        for kk in range(KB + 1):
            tile = xt[kk * LANES:(kk + 1) * LANES]
            x32[kk, pl.ds(t0, LANES), :] = (tile if kk < KB else stack(tile, tile)).T.astype(F32)

    def paced(job, src, dst, when, back):
        results = []

        def dot(left, right):
            if len(results) in when:
                if src is not None and len(results) >= back:
                    src[...] = pltpu.bitcast(results[-back][0:8], U32)
                next(job, None)
                left = stack(left[:-8] if len(left) > 8 else None, left[-8:] | dst[...])
            results.append(_dot(pltpu.bitcast(left, BF16), right))
            return results[-1]

        return dot

    spare_qkv, spare_t = stg_qkv.at[3 * GP, 0, 0:8], wo_t.at[GP, 0, 1, 0:8]
    zero_w = wb.bitcast(U32).at[4 * GP, 0, 0:8]

    def a_out(j, dot):
        rhs = _pair_rhs(_tile(oa_s, slice(None)))
        for r0 in range(0, D // 2, RO):
            halves = _pair_matmul(lambda i: lo_a.bitcast(U32)[i, r0 // 2:(r0 + RO) // 2, :], rhs, dot)
            for e in range(2):
                ga_s[j, pl.ds(e * D // 2 + r0, RO), :] = halves[e]

    def a_tile(j, first, dot):
        rhs = _pair_rhs(_tile(xt_v, j))
        logit, prob, outs = {}, {}, {}
        for e0 in range(0, len(entries), RE):
            some = entries[e0:e0 + RE]
            halves = _pair_matmul(
                lambda i: la.bitcast(U32)[i, 4 * e0:4 * (e0 + len(some)), :], rhs, dot)
            for ent, r0 in zip(some, range(0, 8 * RE, 8)):
                pair = [t[r0:r0 + 8] for t in halves]
                if ent is None:
                    gsig = 1.0 / (1.0 + jnp.exp(-halves[0][0:8]))
                    continue
                g, part, n = ent
                if part:
                    prev, cur = exchange((2 * g + part - 1) * (DA // 2) + n, pair, first)
                    back = [cur] + [
                        pltpu.roll(jnp.where(lane >= LANES - DIL * w, prev, cur), DIL * w, 1)
                        for w in range(1, WIN)]
                    back = [pltpu.bitcast(t, BF16).astype(F32) for t in back]
                if part == 2:
                    outs[g, n] = functools.reduce(
                        jnp.add, [stack(p, p) * t for p, t in zip(prob[g], back)]).astype(BF16)
                elif part == 0:
                    terms = [pair[0] * t[0:8] + pair[1] * t[8:16] for t in back]
                    logit[g] = terms if n == 0 else [a + t for a, t in zip(logit[g], terms)]
                if (part, n) == (0, DA // 2 - 1):
                    s = [t * (DA ** -0.5) for t in logit[g]]
                    if first:
                        s = [jnp.where(lane >= DIL * w, t, NEG) for w, t in enumerate(s)]
                    top = functools.reduce(jnp.maximum, s)
                    ex = [jnp.exp(t - top) for t in s]
                    inv = gsig / functools.reduce(jnp.add, ex)
                    prob[g] = [t * inv for t in ex]
        gm_s[j] = 1.0 - gsig
        if not first:
            a_out(j - 1, dot)
        oa_s[...] = stack(*(outs[key] for key in sorted(outs)))

    plain = lambda left, right: _dot(pltpu.bitcast(left, BF16), right)
    cp_x(0).wait()
    to_rows(0)
    a_tile(0, True, plain)
    cp_wo.wait()
    cp_x(2).start()
    cp_x(3).start()
    start_unit(1)
    prep_wo()
    start_unit(2)

    def a_loop(first, count, work, spare, loading):
        def body(j, carry):
            if loading:
                cp_x(j).wait()
                whole = stg_qkv.at[j - first]
                pltpu.make_async_copy(whole, whole, sem_wb.at[(j - first) & 3]).wait()
                to_rows(j)
            job = work(j - first)
            a_tile(j, False, paced(job, spare, zero_w, *(QA if loading else QB)))
            list(job)
            if loading:
                cp_x(j + 3).start()
                for t in range(first, first + count):
                    pl.when(j == t)(functools.partial(start_more, t))
            return carry

        lax.fori_loop(first, first + count, body, 0)

    a_loop(1, 3 * GP, prep_qkv, spare_qkv, True)

    qi = lax.broadcasted_iota(jnp.int32, (rows, rows), 0)
    ki = lax.broadcasted_iota(jnp.int32, (rows, rows), 1)
    mask = (qi >= seg) | (ki >= seg) | (qi >= ki)
    part, o_prev, opart, b_rows = (_Carry(r) for r in (part_s, o_s, opart_s, b_s))
    ahead = {}

    def b_step(u, t0, memv, project_only=False, output_only=False):
        odd = u % 2
        keep = lambda slots: [s for s in slots if s["tok"] or memv]
        qs, os_ = keep(_PHASES[odd]), keep(_PHASES[1 - odd])
        lhs, shared, tok, mrow, full, soft, o_mem, o_mix, o_left, o_host, new = ({} for _ in range(11))
        clock, queue = [0], {}

        def later(delay, fn, *args):
            queue.setdefault(clock[0] + delay, []).append((fn, args))

        def tick():
            for fn, args in queue.pop(clock[0], ()):
                fn(*args)
            clock[0] += 1

        def spread(sums, key, slots, s, tok_rows, mem_rows):
            for nu in range(KB):
                if memv:
                    sums.add(key + (nu, 2), s["c"][nu], mem_rows, sum(abs(o["c"][nu]) for o in slots))
                for mu in range(2 if s["tok"] else 0):
                    sums.add(key + (nu, mu), _C[s["r"]][mu][nu], tok_rows,
                             sum(abs(_C[o["r"]][mu][nu]) for o in slots if o["tok"]))

        x_mix = _Mixer(lambda mu, kk: x32[kk, pl.ds(t0 + mu * seg, seg), :])
        c_mix = _Mixer(lambda mu, _: x32[KB, pl.ds(t0 + mu * seg, seg), :])
        m_mix = _Mixer(lambda _, kk: memv[kk])

        def q_left(e, t):
            s = qs[e]
            if (e, t) not in lhs:
                left = stack(x_mix(_U[s["r"]]) if s["tok"] else None,
                             m_mix([s["a"]]) if memv else None)
                if s["r"] < NH and t < 2:
                    c = stack(c_mix(_TAIL_IN[s["r"]][:, None]),
                              _signed_sum([(sum(s["c"]), memv[KB])]) if memv else None)
                    left = jnp.where(_low_half(c.shape[0]), *((c, left), (left, c))[t])
                lhs[e, t] = left
            return lhs[e, t]

        def q_total(key, value):
            i, g, nu, mu = key
            h = g * KB + nu
            if mu == 2:
                mrow[i, h] = value
            elif odd:
                part[i, h, mu] = value
            elif mu == 0:
                tok[i, h] = value + part[i, h, mu]
            else:
                ahead[i, h] = (value + part[i, h, mu]).astype(BF16 if i else F32)
            cur = (ahead if odd else tok).get((i, h))
            if (i, h) in mrow and cur is not None and (i, h) not in full:
                full[i, h] = stack(cur.astype(BF16 if i else F32),
                                   mrow[i, h].astype(BF16 if i else F32))

        q_sums = _Sums(q_total)

        def q_pass(e, i, gp, t):
            s = qs[e]
            p = _dot(q_left(e, t), _tile(wb, i * GP + gp, t * NR + s["r"]))
            if t == 2:
                shared[e, i, gp] = p
                return

            def use():
                r = p + shared[e, i, gp] if s["r"] < NH else p
                spread(q_sums, (i, 2 * gp + t), qs, s, r[:seg], r[-mem:])

            later(D0, use)

        def scores(h):
            def stages():
                raw = _dot_nt(full[0, h], full[1, h])
                yield
                s = jnp.where(mask, raw, NEG * DB ** 0.5)
                top = jnp.max(s, axis=-1, keepdims=True)
                yield
                e = jnp.exp2((s - top) * (DB ** -0.5 * LOG2E))
                total = jnp.sum(e, axis=-1, keepdims=True)
                yield
                inv = pltpu.reciprocal(total, approx=True)
                soft[h] = e * (inv * (2.0 - total * inv))
                yield

            run = stages()
            next(run)
            for delay in DS:
                later(delay, next, run)

        def values(h):
            o = _dot(soft[h], full[2, h])
            o_mem[h] = o[seg:]
            if odd:
                o_prev[0, h], o_prev[1, h] = ahead["o", h], o[:seg]
            else:
                ahead["o", h] = o[:seg]

        def o_rows(e, gp, t):
            s = os_[e]
            if (e, gp, t) not in o_left:
                g = 2 * gp + t
                if t == 2:
                    o_left[e, gp, t] = o_rows(e, gp, 0) + o_rows(e, gp, 1)
                    return o_left[e, gp, t]
                if g not in o_mix:
                    o_mix[g] = (_Mixer(lambda _, kk: o_mem[g * KB + kk]),
                                _Mixer(lambda mu, kk: o_prev[mu, g * KB + kk]))
                o_left[e, gp, t] = stack(o_mix[g][0]([s["a"]]) if memv else None,
                                         o_mix[g][1](_U[s["r"]]) if s["tok"] else None)
            return o_left[e, gp, t]

        def o_total(key, value):
            nu, mu = key
            if mu == 2:
                new[nu] = value if nu < KB else value + pltpu.roll(value, 64, 1)
            elif odd:
                opart[nu, mu] = value
            else:
                b_rows[nu, (u - 2) % 4 + mu] = value + opart[nu, mu]

        out_sums = _Sums(o_total)

        def o_product(key, value):
            e, t = key
            s = os_[e]
            if s["r"] < NH:
                o_host[key] = value
                if any((e, t_) not in o_host for t_ in range(3)):
                    return
                lo = _low_half(value.shape[0])
                value = o_host[e, 2] + jnp.where(lo, o_host[e, 1], o_host[e, 0])
                y = jnp.where(lo, o_host[e, 0], o_host[e, 1])
                if memv:
                    out_sums.add((KB, 2), sum(s["a"]), y[:mem], KB)
                for mu in range(2):
                    out_sums.add((KB, mu), _TAIL_OUT[s["r"]][mu], y[-seg:],
                                 sum(abs(_TAIL_OUT[o["r"]][mu]) for o in os_ if o["r"] < NH))
            spread(out_sums, (), os_, s, value[-seg:], value[:mem])

        o_sums = _Sums(o_product)

        def o_pass(e, gp, t):
            host = os_[e]["r"] < NH
            p = _dot(o_rows(e, gp, t), _tile(wb, 3 * GP + gp, t * NR + os_[e]["r"]))
            later(D0, o_sums.add, (e, t if host else 0), 1, p, GP if host else 2 * GP)

        todo = []
        tiles = lambda s, ts: (2,) + ts if s["r"] < NH and 0 in ts else ts
        if not output_only:
            units = [(i, gp, t) for gp in range(GP) for i in PO for t in TS]
            todo = [(s["tok"], q_pass, e, i, gp, t_) for i, gp, t in units
                    for e, s in enumerate(qs) for t_ in tiles(s, t)]
            last = [max(e for e, s in enumerate(_PHASES[odd]) if s["tok"] and s["c"][nu])
                    for nu in range(KB)]
            ready = lambda e, t: 99 if qs[e]["r"] < NH and t < 2 else max(
                last[kk] for kk in range(KB) if qs[e]["a"][kk])
            todo[:HEAD] = sorted(todo[:HEAD], key=lambda p: ready(p[2], p[5]))
        if not project_only:
            todo += [(s["tok"], o_pass, e, gp, t) for pairs in CHUNKS for e, s in enumerate(os_)
                     for gp in pairs for t in tiles(s, (0, 1))]
        long_, short = ([p[1:] for p in todo if p[0] == tok] for tok in (True, False))
        extra = {}
        for h in range(HB if memv else 0):
            gp, n = divmod(h, 2 * KB)
            at = (90 * gp + S0 + int(SPAN[gp == GP - 1] * (n // Q * Q))) // Q * Q
            extra.setdefault(at, []).append((scores, h))
            extra.setdefault(at + LAG, []).append((values, h))
        issued = 0
        for n, p in enumerate(long_):
            for fn, *args in extra.get(n, []) + [p]:
                if issued % 4 == 0 and short and n >= (480 + M0 - 5 * len(short) if len(short) > 24 else MO[6 - len(short) // 4]):
                    for fn_s, *args_s in short[:4]:
                        fn_s(*args_s)
                        tick()
                    del short[:4]
                fn(*args)
                tick()
                issued += 1
        assert not short
        while queue:
            tick()
        return new

    def emit_tile(j):
        for nu in range(KB + 1):
            bt = jnp.concatenate([b_s[nu, 0], b_s[nu, 1], b_rows.val.pop((nu, 2)),
                                  b_rows.val.pop((nu, 3))], axis=0).T
            bt = bt if nu < KB else bt[:64] + bt[64:]
            at = pl.ds(nu * LANES, bt.shape[0])
            gm = jnp.concatenate([gm_s[j]] * (bt.shape[0] // 8), axis=0)
            out_v[j, at, :] = (ga_s[j, at, :] + gm * bt).astype(out_v.dtype)

    pltpu.make_async_copy(stg_o, stg_o, sem_wa.at[6]).wait()
    for j in range(3 * GP + 1, nt):
        cp_x(j).wait()
    for gp in range(GP):
        turn_out(gp)
    b_step(3, 0, None, project_only=True)
    part.flush()
    for j in range(3 * GP + 1, nt):
        to_rows(j)
    a_loop(3 * GP + 1, GP - 1, prep_out, spare_t, False)
    job = prep_out(GP - 1)
    a_out(nt - 1, paced(job, spare_t, zero_w, *QC))
    list(job)

    def b_body(j, carry):
        memv = {kk: mem_s[kk] for kk in range(KB + 1)}
        for u in range(4):
            t0 = jnp.minimum(j * LANES + (u + 1) // 2 * 2 * seg, seq - 2 * seg)
            memv = b_step(u, pl.multiple_of(t0, seg), memv)
            if u == 0:
                emit_tile(jnp.maximum(j - 1, 0))
        for kk, t in memv.items():
            mem_s[kk] = t
        for c in (part, o_prev, opart, b_rows):
            c.flush()
        pl.when(j > 0)(lambda: cp_out(j - 1).start())
        return carry

    lax.fori_loop(0, nt, b_body, 0)
    b_step(0, None, None, output_only=True)
    emit_tile(nt - 1)
    cp_out(nt - 1).start()
    for j in range(nt):
        cp_out(j).wait()


@functools.partial(jax.jit, static_argnames=("B_seg_len",))
def pallas_gated_mix__sliding_local_dilated__memory_aug_recurrent_mem_tr__prompt_kernel(
    A_x: jax.Array,
    A_wqkv: jax.Array,
    A_wo: jax.Array,
    B_x: jax.Array,
    B_mem0: jax.Array,
    B_Wq: jax.Array,
    B_Wk: jax.Array,
    B_Wv: jax.Array,
    B_Wo: jax.Array,
    B_seg_len: int,
    gate_w: jax.Array,
):
    del B_x
    batch, seq, width = A_x.shape
    mem, seg = B_mem0.shape[1], int(B_seg_len)
    nt = seq // LANES
    assert batch == 1 and width == D and nt == 4 * GP and seq % LANES == 0
    assert B_Wq.shape == (D, HB, DB) and mem == 8 and 4 * seg == LANES

    hbm = pl.BlockSpec(memory_space=pl.ANY)
    vmem = pl.BlockSpec(memory_space=pltpu.VMEM)
    out_t = pl.pallas_call(
        functools.partial(_kernel, seq=seq, seg=seg, mem=mem),
        out_shape=jax.ShapeDtypeStruct((D, seq), A_x.dtype),
        in_specs=[hbm, hbm, hbm, vmem, hbm, hbm, hbm, hbm, vmem],
        out_specs=hbm,
        scratch_shapes=[
            pltpu.VMEM((nt, D, LANES), BF16),
            pltpu.VMEM((D, 3 * D), BF16),
            pltpu.VMEM((D, D), BF16),
            pltpu.VMEM((3 * GP + 1, KB, D, DB), U32),
            pltpu.VMEM((HB, D, DB), BF16),
            pltpu.VMEM((GP + 1, 2 * KB + 1, KB, 64, LANES), U32),
            pltpu.VMEM((5, 3 * D, LANES), F32),
            pltpu.VMEM((5, D, LANES), F32),
            pltpu.VMEM((12, 3 * D // 2 + 16, LANES), BF16),
            pltpu.VMEM((12, D // 2, LANES), BF16),
            pltpu.VMEM((2 * D, LANES), BF16),
            pltpu.VMEM((D, LANES), BF16),
            pltpu.VMEM((4 * GP + 1, 2 * NR + NH, LANES, LANES), BF16),
            pltpu.VMEM((KB + 1, seq, LANES), F32),
            pltpu.VMEM((nt, D, LANES), F32),
            pltpu.VMEM((nt, 8, LANES), F32),
            pltpu.VMEM((2 * KB, mem, LANES), F32),
            pltpu.VMEM((3, HB, 2, seg, LANES), F32),
            pltpu.VMEM((2, HB, seg, LANES), F32),
            pltpu.VMEM((KB + 1, 2, seg, LANES), F32),
            pltpu.VMEM((KB + 1, 2, seg, LANES), F32),
            pltpu.VMEM((nt, D, LANES), A_x.dtype),
            pltpu.SemaphoreType.DMA((4,)),
            pltpu.SemaphoreType.DMA((7,)),
            pltpu.SemaphoreType.DMA((4,)),
            pltpu.SemaphoreType.DMA(()),
        ],
        compiler_params=pltpu.CompilerParams(vmem_limit_bytes=110 * 1024 * 1024),
        name="gated_mix_kernel",
    )(A_x[0].T, A_wqkv, A_wo, B_mem0[0], B_Wq, B_Wk, B_Wv, B_Wo.transpose(0, 2, 1), gate_w)
    return out_t.T[None]
```

```python
import functools
import itertools

import jax
import jax.numpy as jnp
import numpy as np
from jax import lax
import jax.experimental.pallas as pl
import jax.experimental.pallas.tpu as pltpu

F32, BF16, U32 = jnp.float32, jnp.bfloat16, jnp.uint32

D = 576
LANES = 128
HA, DA = 32, 18
WIN, DIL = 8, 2
HB, DB = 32, 128
NEG = -1000000000.0
LOG2E = 1.4426950408889634
NG = HA // 8

KB = 4
GP = HB // (2 * KB)

_HK = (
    (".... +...", "+.-. -... .... -...", "+... +..."),
    ("+... -...", "+-.- .... -... ....", "+... ...."),
    (".+.. .-..", ".... +-.. .+.. ....", ".... .+.."),
    (".+.. ....", ".-.. .+-. .... ....", ".+.. .+.."),
    (".... ..+.", ".... ..-. -.+. .+-.", ".... ..+."),
    ("..+. ....", "..-. ...+ .-+- ....", "..+. ...."),
    ("...+ ...-", ".... ...- ...+ ++.-", ".... ...+"),
    ("...+ ....", "...- ...- .... .+-+", "...+ ...+"),
    (".... ++..", ".... +... .... ....", ".... ++.."),
    ("++.. ....", ".+.. .... .... ....", "++.. ...."),
    (".+.. +...", ".-.. +... .... ....", "+... .-.."),
    ("+.+. -.-.", ".... .... -... ....", ".... +.+."),
    ("+.+. ....", "..+. .... .... ....", "+.+. +.+."),
    ("+.+. -...", "..-. .... +... ....", "+... +.+."),
    (".... +..+", ".... .... .... +...", ".... +..+"),
    ("+..+ ....", "...+ .... .... ....", "+..+ ...."),
    ("...+ +...", "...- .... .... +...", "+... ...-"),
    (".... .++.", ".... ..+. .... .-..", ".++. .++."),
    (".++. .--.", ".... ...- .+.. ....", ".++. ...."),
    (".+.. .--.", ".... ..+. .-.. ....", ".++. .+.."),
    (".... ..++", ".... .... .... .-+.", "..++ ..++"),
    ("..++ ..--", ".... ...- ...+ ....", "..++ ...."),
    ("...+ ..--", ".... ...+ ...- .-+.", "..++ ...+"),
    (".... .+++", ".... .... .... .+..", ".... .+++"),
    (".+++ ....", ".... ...+ .... ....", ".+++ ...."),
    ("...+ .++.", ".... ...- .... .+..", ".++. ...-"),
)
_U, _V, _C = (np.array([[["-.+".index(ch) - 1 for ch in row] for row in prod[i].split()]
                        for prod in _HK]) for i in range(3))
NR = len(_HK)
assert np.array_equal(np.einsum("rak,rln,rbm->akblnm", _U, _V, _C),
                      np.einsum("ab,kl,nm->akblnm", *(np.eye(n, dtype=int) for n in (2, KB, KB))))


def _phase(products):
    tiles = [max(r, ~r) for r in products]
    dual = np.rint(np.linalg.inv(_V[tiles].reshape(len(tiles), -1)).T).astype(int)
    slots = []
    for r, d in zip(products, dual.reshape(-1, KB, KB)):
        i, j = np.argwhere(d)[0]
        a, c = d[:, j] * d[i, j], d[i]
        assert np.array_equal(np.outer(a, c), d)
        slots.append(dict(r=max(r, ~r), tok=r >= 0, a=a.tolist(), c=c.tolist()))
    return slots


_PHASES = (_phase((11, 8, ~9, 4, 2, 23, 17, ~13, 25, 20, 22, 7, ~19, 16, 15, 1)),
           _phase((24, 21, ~16, 18, 19, 3, 10, ~22, 9, 5, 12, 13, ~25, 0, 14, 6)))
assert sorted(s["r"] for ph in _PHASES for s in ph if s["tok"]) == list(range(NR))

NH = 2 * KB
assert all(sorted(s["r"] // 2 for s in ph if s["r"] < NH) == list(range(KB)) for ph in _PHASES)
assert all(np.abs(s[k]).tolist() == np.eye(KB)[s["r"] // 2].tolist()
           for ph in _PHASES for s in ph if s["r"] < NH for k in "ac")
_TAIL_IN, _TAIL_OUT = (
    np.concatenate([np.rint(np.linalg.inv(t[2 * n:2 * n + 2, :, n]).T).astype(int)
                    for n in range(KB)]) for t in (_C, _U))


CHUNKS, S0, LAG, SPAN, HEAD, M0 = ((0, 1), (2, 3)), 72, 40, (11.25, 1), 72, 6
PO = (1, 0, 2)
MO = (364, 385, 410, 426, 444, 463)


D0, DS, TS, Q = 0, (0, 0, 0), ((0, 1),), 2


SEQ, RE, RO = 0, 8, 48
ORD = (9, 8, 10, 19, 2, 3, 23, 24, 25, 17, 18, 20, 21, 22, 12, 11, 13, 4, 5, 15, 14, 16, 6, 7, 0, 1)
CUT = (1,)
QA = ((10, 16, 30, 45, 61, 77, 92, 108, 124, 152, 159, 166, 173), 20)
QB = ((10, 16, 22, 42, 58, 75, 91, 108, 146, 150, 155, 160, 165, 170, 175), 24)
QC = (range(8, 54, 4), 16)


def _signed_sum(terms):
    terms = [(c, t) for c, t in terms if c]
    first = next((i for i, (c, _) in enumerate(terms) if c > 0), 0)
    c, acc = terms.pop(first)
    acc = acc if c > 0 else -acc
    for c, t in terms:
        acc = acc + t if c > 0 else acc - t
    return acc


class _Mixer:
    def __init__(self, block):
        self.block, self.known = block, {}

    def __call__(self, coef):
        want = {(i, k): int(c) for i, row in enumerate(coef) for k, c in enumerate(row) if c}
        key = tuple(sorted(want.items()))
        if key not in self.known:
            terms = []
            for have in sorted(self.known, key=lambda h: -len(h)):
                for sign in (1, -1):
                    if all(want.get(pos) == sign * c for pos, c in have):
                        terms.append((sign, self.known[have]))
                        want = {pos: c for pos, c in want.items() if pos not in dict(have)}
                        break
            for pos, c in sorted(want.items()):
                self.known[((pos, 1),)] = self.block(*pos)
                terms.append((c, self.known[((pos, 1),)]))
            self.known[key] = _signed_sum(terms)
        return self.known[key]


class _Sums:
    def __init__(self, done):
        self.done, self.acc = done, {}

    def add(self, key, sign, value, expected):
        if not sign:
            return
        count, neg, tot = self.acc.pop(key, (0, sign < 0, value))
        if count and neg == (sign < 0):
            tot = tot + value
        elif count:
            tot, neg = (value - tot if neg else tot - value), False
        if count + 1 == expected:
            self.done(key, -tot if neg else tot)
        else:
            self.acc[key] = (count + 1, neg, tot)


class _Carry:
    def __init__(self, ref):
        self.ref, self.val = ref, {}

    def __getitem__(self, key):
        return self.val[key] if key in self.val else self.ref[key]

    def __setitem__(self, key, value):
        self.val[key] = value

    def flush(self):
        for key, value in self.val.items():
            self.ref[key] = value
        self.val = {}


def _dot(a, b):
    return lax.dot_general(a, b, (((1,), (0,)), ((), ())), preferred_element_type=F32)


def _dot_nt(a, b):
    return lax.dot_general(a, b, (((1,), (1,)), ((), ())), preferred_element_type=F32)


def _tile(ref, *idx):
    return pltpu.bitcast(ref.bitcast(U32)[idx], BF16)


def stack(*parts):
    parts = [t for t in parts if t is not None and t.shape[0]]
    return parts[0] if len(parts) == 1 else jnp.concatenate(parts, axis=0)


def _low_half(rows):
    return lax.broadcasted_iota(jnp.int32, (rows, LANES), 1) < 64


def _pair_lhs(t1, t2):
    lo = _low_half(t1[3].shape[0])
    diff = t1[3] - t2[3]
    return (t1[:3] + [jnp.where(lo, t1[4], diff)]
            + t2[:3] + [jnp.where(lo, -diff, t2[4])]
            + [jnp.where(lo, t1[3], t2[3])])


def _pair_rhs(x):
    a, b, c = x[384:448], x[448:512], x[512:576]
    cat = lambda u, v: jnp.concatenate([u, v], axis=0)
    return [x[i * 128:(i + 1) * 128] for i in range(3)] + [cat(c, b), cat(a, c), x[384:512]]


def _pair_matmul(lhs, rhs, dot):
    out = [dot(lhs(8), rhs[5])] * 2
    for i in range(8):
        out[i // 4] = out[i // 4] + dot(lhs(i), rhs[i % 4 if i < 7 else 4])
    return out


def _kernel(xt_hbm, wqkv_hbm, wo_hbm, mem0_ref, wq_hbm, wk_hbm, wv_hbm, wot_hbm, gate_ref,
            out_hbm,
            xt_v, wqkv_v, wo_v, stg_qkv, stg_o, wo_t, wt32, wo32_s, la, lo_a, kv_prev, oa_s,
            wb, x32, ga_s, gm_s, mem_s, part_s, o_s, opart_s, b_s, out_v,
            sem_x, sem_wa, sem_out, *, seq, seg, mem):
    nt = seq // LANES
    rows = mem + seg

    def cp_x(j):
        col = j * LANES if isinstance(j, int) else pl.multiple_of(j * LANES, LANES)
        return pltpu.make_async_copy(xt_hbm.at[:, pl.ds(col, LANES)], xt_v.at[j], sem_x.at[jnp.minimum(j, 3 * GP + 1)])

    def cp_wqkv(k):
        r = pl.ds(k * 128, min(128, D - k * 128))
        return pltpu.make_async_copy(wqkv_hbm.at[r], wqkv_v.at[r], sem_wa.at[k])

    cp_wo = pltpu.make_async_copy(wo_hbm, wo_v, sem_wa.at[5])

    def start_unit(unit):
        i, gp = divmod(unit, GP)
        src = (wq_hbm, wk_hbm, wv_hbm)[i].bitcast(U32)
        cp_x(unit + 1).start(priority=1)
        for p in range(KB):
            pltpu.make_async_copy(src.at[:, KB * gp + p, :], stg_qkv.at[unit, p],
                                  sem_x.at[unit + 1]).start(priority=1)

    cp_wot = [pltpu.make_async_copy(wot_hbm.at[h0:h1], stg_o.at[h0:h1], sem_wa.at[6 + n])
              for n, (h0, h1) in enumerate(((0, HB - 2 * KB), (HB - 2 * KB, HB)))]

    def cp_out(j):
        col = j * LANES if isinstance(j, int) else pl.multiple_of(j * LANES, LANES)
        return pltpu.make_async_copy(out_v.at[j], out_hbm.at[:, pl.ds(col, LANES)], sem_out)

    for c in [cp_wqkv(k) for k in (3, 4, 0, 1, 2)] + [cp_x(0)]:
        c.start()

    m0 = mem0_ref[...].astype(F32)
    for kk in range(KB):
        mem_s[kk] = m0[:, kk * LANES:(kk + 1) * LANES]
    mem_s[KB] = jnp.concatenate([m0[:, KB * LANES:]] * 2, axis=1)
    for ref in (o_s, opart_s, b_s):
        ref[...] = jnp.zeros(ref.shape, ref.dtype)
    wb[4 * GP, 0, 0:16, :] = jnp.zeros((16, LANES), BF16)

    gate = jnp.broadcast_to(gate_ref[...].astype(F32).reshape(1, D), (8, D))
    gate_t = [gate[:, i * 128:(i + 1) * 128] for i in range(4)]
    gate_t.append(jnp.concatenate([gate[:, 512:], gate[:, 512:]], axis=1))

    entries = [None] * 2 + [(g - part // 2, part, n) for g in range(NG + 1) for n in range(DA // 2)
                            for part in (1, 0, 2) if 0 <= g - part // 2 < NG]
    if SEQ:
        entries = [None] * 2 + [(g, part, n) for g in range(NG) for parts in ((1, 0), (2,))
                                for n in range(DA // 2) for part in parts]

    def feature_rows(k, e):
        return stack(*(gate_t[k] if ent is None else
                       wt32[k, pl.ds(ent[1] * D + ent[0] * 8 * DA + 2 * ent[2] + e, 8, stride=DA), :]
                       for ent in entries))

    for k in (3, 4, 0, 1, 2):
        cp_wqkv(k).wait()
        if k == 2:
            cp_wo.start()
        if k == 1:
            start_unit(0)
        rows_k = wqkv_v[k * LANES:min(D, (k + 1) * LANES), :]
        wt32[k] = (rows_k if k < 4 else stack(rows_k, rows_k)).T.astype(F32)
        for e in range(2 if k < 3 else 0):
            la[4 * e + k] = feature_rows(k, e).astype(BF16)
        if k == 4:
            mixed = _pair_lhs(*([None] * 3 + [feature_rows(3, e), feature_rows(4, e)]
                                for e in range(2)))
            for i in (3, 7, 8):
                la[i] = mixed[i].astype(BF16)

    def prep_wo():
        wo32 = wo_v[...].astype(F32)
        for n in range(4):
            wo32_s[n] = wo32[:, n * LANES:(n + 1) * LANES]
        wo32_s[4] = jnp.concatenate([wo32[:, 4 * LANES:]] * 2, axis=1)
        turned = []
        for n in range(5):
            perm = stack(*(wo32_s[n, pl.ds(g * 8 * DA + d, 8, stride=DA), :]
                           for g in range(NG) for d in range(DA))).astype(BF16)
            turned.append([perm[k * LANES:(k + 1) * LANES].T for k in range(4)]
                          + [stack(perm[4 * LANES:], perm[4 * LANES:]).T])
        tiles = [stack(*(t[k] for t in turned))[:D].astype(F32) for k in range(5)]
        for i, t in enumerate(_pair_lhs([t[:D // 2] for t in tiles], [t[D // 2:] for t in tiles])):
            lo_a[i] = t.astype(BF16)

    by_size = ORD

    def prep_qkv(unit):
        src, dst = stg_qkv.at[unit], wb.at[unit]

        def rows(g, r0, nu):
            u = src[2 * g + nu // 2, r0:r0 + 16, :]
            return pltpu.bitcast(u & jnp.uint32(0xFFFF0000) if nu % 2 else u << 16, F32)

        for e in range(8):
            at, own, shared = pl.ds(16 * e, 16), e // 4, {}
            for g in (own, 1 - own):
                mix = _Mixer(lambda kk, nu: rows(g, kk * LANES + 16 * e, nu))
                for r in by_size:
                    w = mix(_V[r])
                    if r < NH and g == own:
                        shared[r] = w.astype(BF16)
                        dst[2 * NR + r, at, :] = shared[r]
                        w = rows(g, KB * LANES + 16 * (e % 4), r // 2)
                    elif r < NH:
                        w = w - shared[r].astype(F32)
                    dst[g * NR + r, at, :] = w.astype(BF16)
                    if r in CUT:
                        yield

    def turn_out(gp):
        words = lambda head, r0, n: _tile(stg_o, 2 * KB * gp + head, pl.ds(r0 // 2, n // 2))
        for head in range(2 * KB + 1):
            for nu in range(KB):
                if head < 2 * KB:
                    tile = words(head, nu * LANES, LANES)
                else:
                    tile = stack(*(words(g * KB + nu, KB * LANES, 64) for g in range(2)))
                wo_t[gp, head, nu] = pltpu.bitcast(tile.T, U32)

    def prep_out(gp):
        dst, lo = wb.at[3 * GP + gp], _low_half(16)
        for e in range(8):
            at, first = pl.ds(16 * e, 16), {}
            rows = lambda head, nu: pltpu.bitcast(
                wo_t[gp, head, nu, 8 * e:8 * e + 8, :], BF16).astype(F32)
            for g in range(2):
                mix = _Mixer(lambda kk, nu: rows(g * KB + kk, nu))
                for r in by_size:
                    w = mix(_V[r])
                    if r >= NH:
                        dst[g * NR + r, at, :] = w.astype(BF16)
                    elif g == 0:
                        first[r] = w
                    else:
                        z, t = jnp.where(lo, first[r], w).astype(BF16), rows(2 * KB, r // 2)
                        dst[2 * NR + r, at, :] = z
                        dst[r, at, :] = jnp.where(lo, t, first[r] - z.astype(F32)).astype(BF16)
                        dst[NR + r, at, :] = jnp.where(lo, w - z.astype(F32), t).astype(BF16)
                    if r in CUT:
                        yield

    lane = lax.broadcasted_iota(jnp.int32, (8, LANES), 1)

    def exchange(idx, pair, first):
        at = pl.ds(8 * idx, 8)
        prev = None if first else kv_prev.bitcast(U32)[at, :]
        kv_prev[16 * idx:16 * idx + 16, :] = jnp.concatenate(pair, axis=0).astype(BF16)
        cur = kv_prev.bitcast(U32)[at, :]
        return (jnp.broadcast_to(cur[:, 0:1], (8, LANES)) if first else prev), cur

    def to_rows(j):
        t0 = j * LANES if isinstance(j, int) else pl.multiple_of(j * LANES, LANES)
        xt = _tile(xt_v, j)
        for kk in range(KB + 1):
            tile = xt[kk * LANES:(kk + 1) * LANES]
            x32[kk, pl.ds(t0, LANES), :] = (tile if kk < KB else stack(tile, tile)).T.astype(F32)

    def paced(job, src, dst, when, back):
        results = []

        def dot(left, right):
            if len(results) in when:
                if src is not None and len(results) >= back:
                    src[...] = pltpu.bitcast(results[-back][0:8], U32)
                next(job, None)
                left = stack(left[:-8] if len(left) > 8 else None, left[-8:] | dst[...])
            results.append(_dot(pltpu.bitcast(left, BF16), right))
            return results[-1]

        return dot

    spare_qkv, spare_t = stg_qkv.at[3 * GP, 0, 0:8], wo_t.at[GP, 0, 1, 0:8]
    zero_w = wb.bitcast(U32).at[4 * GP, 0, 0:8]

    def a_out(j, dot):
        rhs = _pair_rhs(_tile(oa_s, slice(None)))
        for r0 in range(0, D // 2, RO):
            halves = _pair_matmul(lambda i: lo_a.bitcast(U32)[i, r0 // 2:(r0 + RO) // 2, :], rhs, dot)
            for e in range(2):
                ga_s[j, pl.ds(e * D // 2 + r0, RO), :] = halves[e]

    def a_tile(j, first, dot):
        rhs = _pair_rhs(_tile(xt_v, j))
        logit, prob, outs = {}, {}, {}
        for e0 in range(0, len(entries), RE):
            some = entries[e0:e0 + RE]
            halves = _pair_matmul(
                lambda i: la.bitcast(U32)[i, 4 * e0:4 * (e0 + len(some)), :], rhs, dot)
            for ent, r0 in zip(some, range(0, 8 * RE, 8)):
                pair = [t[r0:r0 + 8] for t in halves]
                if ent is None:
                    gsig = 1.0 / (1.0 + jnp.exp(-halves[0][0:8]))
                    continue
                g, part, n = ent
                if part:
                    prev, cur = exchange((2 * g + part - 1) * (DA // 2) + n, pair, first)
                    back = [cur] + [
                        pltpu.roll(jnp.where(lane >= LANES - DIL * w, prev, cur), DIL * w, 1)
                        for w in range(1, WIN)]
                    back = [pltpu.bitcast(t, BF16).astype(F32) for t in back]
                if part == 2:
                    outs[g, n] = functools.reduce(
                        jnp.add, [stack(p, p) * t for p, t in zip(prob[g], back)]).astype(BF16)
                elif part == 0:
                    terms = [pair[0] * t[0:8] + pair[1] * t[8:16] for t in back]
                    logit[g] = terms if n == 0 else [a + t for a, t in zip(logit[g], terms)]
                if (part, n) == (0, DA // 2 - 1):
                    s = [t * (DA ** -0.5) for t in logit[g]]
                    if first:
                        s = [jnp.where(lane >= DIL * w, t, NEG) for w, t in enumerate(s)]
                    top = functools.reduce(jnp.maximum, s)
                    ex = [jnp.exp(t - top) for t in s]
                    inv = gsig / functools.reduce(jnp.add, ex)
                    prob[g] = [t * inv for t in ex]
        gm_s[j] = 1.0 - gsig
        if not first:
            a_out(j - 1, dot)
        oa_s[...] = stack(*(outs[key] for key in sorted(outs)))

    plain = lambda left, right: _dot(pltpu.bitcast(left, BF16), right)
    cp_x(0).wait()
    start_unit(1)
    to_rows(0)
    a_tile(0, True, plain)
    cp_wo.wait()
    for unit in range(2, 3 * GP):
        start_unit(unit)
    for c in [cp_x(j) for j in range(3 * GP + 1, nt)] + cp_wot:
        c.start(priority=1)
    prep_wo()

    def a_loop(first, count, work, spare, loading):
        def body(j, carry):
            if loading:
                cp_x(j).wait()
                whole = stg_qkv.at[j - first]
                pltpu.make_async_copy(whole, whole, sem_x.at[j]).wait()
                to_rows(j)
            job = work(j - first)
            a_tile(j, False, paced(job, spare, zero_w, *(QA if loading else QB)))
            list(job)
            return carry

        lax.fori_loop(first, first + count, body, 0)

    a_loop(1, 3 * GP, prep_qkv, spare_qkv, True)

    qi = lax.broadcasted_iota(jnp.int32, (rows, rows), 0)
    ki = lax.broadcasted_iota(jnp.int32, (rows, rows), 1)
    mask = (qi >= seg) | (ki >= seg) | (qi >= ki)
    part, o_prev, opart, b_rows = (_Carry(r) for r in (part_s, o_s, opart_s, b_s))
    ahead = {}

    def b_step(u, t0, memv, project_only=False, output_only=False):
        odd = u % 2
        keep = lambda slots: [s for s in slots if s["tok"] or memv]
        qs, os_ = keep(_PHASES[odd]), keep(_PHASES[1 - odd])
        lhs, shared, tok, mrow, full, soft, o_mem, o_mix, o_left, o_host, new = ({} for _ in range(11))
        clock, queue = [0], {}

        def later(delay, fn, *args):
            queue.setdefault(clock[0] + delay, []).append((fn, args))

        def tick():
            for fn, args in queue.pop(clock[0], ()):
                fn(*args)
            clock[0] += 1

        def spread(sums, key, slots, s, tok_rows, mem_rows):
            for nu in range(KB):
                if memv:
                    sums.add(key + (nu, 2), s["c"][nu], mem_rows, sum(abs(o["c"][nu]) for o in slots))
                for mu in range(2 if s["tok"] else 0):
                    sums.add(key + (nu, mu), _C[s["r"]][mu][nu], tok_rows,
                             sum(abs(_C[o["r"]][mu][nu]) for o in slots if o["tok"]))

        x_mix = _Mixer(lambda mu, kk: x32[kk, pl.ds(t0 + mu * seg, seg), :])
        c_mix = _Mixer(lambda mu, _: x32[KB, pl.ds(t0 + mu * seg, seg), :])
        m_mix = _Mixer(lambda _, kk: memv[kk])

        def q_left(e, t):
            s = qs[e]
            if (e, t) not in lhs:
                left = stack(x_mix(_U[s["r"]]) if s["tok"] else None,
                             m_mix([s["a"]]) if memv else None)
                if s["r"] < NH and t < 2:
                    c = stack(c_mix(_TAIL_IN[s["r"]][:, None]),
                              _signed_sum([(sum(s["c"]), memv[KB])]) if memv else None)
                    left = jnp.where(_low_half(c.shape[0]), *((c, left), (left, c))[t])
                lhs[e, t] = left
            return lhs[e, t]

        def q_total(key, value):
            i, g, nu, mu = key
            h = g * KB + nu
            if mu == 2:
                mrow[i, h] = value
            elif odd:
                part[i, h, mu] = value
            elif mu == 0:
                tok[i, h] = value + part[i, h, mu]
            else:
                ahead[i, h] = (value + part[i, h, mu]).astype(BF16 if i else F32)
            cur = (ahead if odd else tok).get((i, h))
            if (i, h) in mrow and cur is not None and (i, h) not in full:
                full[i, h] = stack(cur.astype(BF16 if i else F32),
                                   mrow[i, h].astype(BF16 if i else F32))

        q_sums = _Sums(q_total)

        def q_pass(e, i, gp, t):
            s = qs[e]
            p = _dot(q_left(e, t), _tile(wb, i * GP + gp, t * NR + s["r"]))
            if t == 2:
                shared[e, i, gp] = p
                return

            def use():
                r = p + shared[e, i, gp] if s["r"] < NH else p
                spread(q_sums, (i, 2 * gp + t), qs, s, r[:seg], r[-mem:])

            later(D0, use)

        def scores(h):
            def stages():
                raw = _dot_nt(full[0, h], full[1, h])
                yield
                s = jnp.where(mask, raw, NEG * DB ** 0.5)
                top = jnp.max(s, axis=-1, keepdims=True)
                yield
                e = jnp.exp2((s - top) * (DB ** -0.5 * LOG2E))
                total = jnp.sum(e, axis=-1, keepdims=True)
                yield
                inv = pltpu.reciprocal(total, approx=True)
                soft[h] = e * (inv * (2.0 - total * inv))
                yield

            run = stages()
            next(run)
            for delay in DS:
                later(delay, next, run)

        def values(h):
            o = _dot(soft[h], full[2, h])
            o_mem[h] = o[seg:]
            if odd:
                o_prev[0, h], o_prev[1, h] = ahead["o", h], o[:seg]
            else:
                ahead["o", h] = o[:seg]

        def o_rows(e, gp, t):
            s = os_[e]
            if (e, gp, t) not in o_left:
                g = 2 * gp + t
                if t == 2:
                    o_left[e, gp, t] = o_rows(e, gp, 0) + o_rows(e, gp, 1)
                    return o_left[e, gp, t]
                if g not in o_mix:
                    o_mix[g] = (_Mixer(lambda _, kk: o_mem[g * KB + kk]),
                                _Mixer(lambda mu, kk: o_prev[mu, g * KB + kk]))
                o_left[e, gp, t] = stack(o_mix[g][0]([s["a"]]) if memv else None,
                                         o_mix[g][1](_U[s["r"]]) if s["tok"] else None)
            return o_left[e, gp, t]

        def o_total(key, value):
            nu, mu = key
            if mu == 2:
                new[nu] = value if nu < KB else value + pltpu.roll(value, 64, 1)
            elif odd:
                opart[nu, mu] = value
            else:
                b_rows[nu, (u - 2) % 4 + mu] = value + opart[nu, mu]

        out_sums = _Sums(o_total)

        def o_product(key, value):
            e, t = key
            s = os_[e]
            if s["r"] < NH:
                o_host[key] = value
                if any((e, t_) not in o_host for t_ in range(3)):
                    return
                lo = _low_half(value.shape[0])
                value = o_host[e, 2] + jnp.where(lo, o_host[e, 1], o_host[e, 0])
                y = jnp.where(lo, o_host[e, 0], o_host[e, 1])
                if memv:
                    out_sums.add((KB, 2), sum(s["a"]), y[:mem], KB)
                for mu in range(2):
                    out_sums.add((KB, mu), _TAIL_OUT[s["r"]][mu], y[-seg:],
                                 sum(abs(_TAIL_OUT[o["r"]][mu]) for o in os_ if o["r"] < NH))
            spread(out_sums, (), os_, s, value[-seg:], value[:mem])

        o_sums = _Sums(o_product)

        def o_pass(e, gp, t):
            host = os_[e]["r"] < NH
            p = _dot(o_rows(e, gp, t), _tile(wb, 3 * GP + gp, t * NR + os_[e]["r"]))
            later(D0, o_sums.add, (e, t if host else 0), 1, p, GP if host else 2 * GP)

        todo = []
        tiles = lambda s, ts: (2,) + ts if s["r"] < NH and 0 in ts else ts
        if not output_only:
            units = [(i, gp, t) for gp in range(GP) for i in PO for t in TS]
            todo = [(s["tok"], q_pass, e, i, gp, t_) for i, gp, t in units
                    for e, s in enumerate(qs) for t_ in tiles(s, t)]
            last = [max(e for e, s in enumerate(_PHASES[odd]) if s["tok"] and s["c"][nu])
                    for nu in range(KB)]
            ready = lambda e, t: 99 if qs[e]["r"] < NH and t < 2 else max(
                last[kk] for kk in range(KB) if qs[e]["a"][kk])
            todo[:HEAD] = sorted(todo[:HEAD], key=lambda p: ready(p[2], p[5]))
        if not project_only:
            todo += [(s["tok"], o_pass, e, gp, t) for pairs in CHUNKS for e, s in enumerate(os_)
                     for gp in pairs for t in tiles(s, (0, 1))]
        long_, short = ([p[1:] for p in todo if p[0] == tok] for tok in (True, False))
        extra = {}
        for h in range(HB if memv else 0):
            gp, n = divmod(h, 2 * KB)
            at = (90 * gp + S0 + int(SPAN[gp == GP - 1] * (n // Q * Q))) // Q * Q
            extra.setdefault(at, []).append((scores, h))
            extra.setdefault(at + LAG, []).append((values, h))
        issued = 0
        for n, p in enumerate(long_):
            for fn, *args in extra.get(n, []) + [p]:
                if issued % 4 == 0 and short and n >= (480 + M0 - 5 * len(short) if len(short) > 24 else MO[6 - len(short) // 4]):
                    for fn_s, *args_s in short[:4]:
                        fn_s(*args_s)
                        tick()
                    del short[:4]
                fn(*args)
                tick()
                issued += 1
        assert not short
        while queue:
            tick()
        return new

    def emit_tile(j):
        for nu in range(KB + 1):
            bt = jnp.concatenate([b_s[nu, 0], b_s[nu, 1], b_rows.val.pop((nu, 2)),
                                  b_rows.val.pop((nu, 3))], axis=0).T
            bt = bt if nu < KB else bt[:64] + bt[64:]
            at = pl.ds(nu * LANES, bt.shape[0])
            gm = jnp.concatenate([gm_s[j]] * (bt.shape[0] // 8), axis=0)
            out_v[j, at, :] = (ga_s[j, at, :] + gm * bt).astype(out_v.dtype)

    cp_wot[0].wait()
    for j in range(3 * GP + 1, nt):
        cp_x(j).wait()
    for gp in range(GP - 1):
        turn_out(gp)
    b_step(3, 0, None, project_only=True)
    part.flush()
    for j in range(3 * GP + 1, nt):
        to_rows(j)
    cp_wot[1].wait()
    turn_out(GP - 1)
    a_loop(3 * GP + 1, GP - 1, prep_out, spare_t, False)
    job = prep_out(GP - 1)
    a_out(nt - 1, paced(job, spare_t, zero_w, *QC))
    list(job)

    def b_body(j, carry):
        memv = {kk: mem_s[kk] for kk in range(KB + 1)}
        for u in range(4):
            t0 = jnp.minimum(j * LANES + (u + 1) // 2 * 2 * seg, seq - 2 * seg)
            memv = b_step(u, pl.multiple_of(t0, seg), memv)
            if u == 0:
                emit_tile(jnp.maximum(j - 1, 0))
        for kk, t in memv.items():
            mem_s[kk] = t
        for c in (part, o_prev, opart, b_rows):
            c.flush()
        pl.when(j > 0)(lambda: cp_out(j - 1).start())
        return carry

    lax.fori_loop(0, nt, b_body, 0)
    b_step(0, None, None, output_only=True)
    emit_tile(nt - 1)
    cp_out(nt - 1).start()
    for j in range(nt):
        cp_out(j).wait()


@functools.partial(jax.jit, static_argnames=("B_seg_len",))
def pallas_gated_mix__sliding_local_dilated__memory_aug_recurrent_mem_tr__prompt_kernel(
    A_x: jax.Array,
    A_wqkv: jax.Array,
    A_wo: jax.Array,
    B_x: jax.Array,
    B_mem0: jax.Array,
    B_Wq: jax.Array,
    B_Wk: jax.Array,
    B_Wv: jax.Array,
    B_Wo: jax.Array,
    B_seg_len: int,
    gate_w: jax.Array,
):
    del B_x
    batch, seq, width = A_x.shape
    mem, seg = B_mem0.shape[1], int(B_seg_len)
    nt = seq // LANES
    assert batch == 1 and width == D and nt == 4 * GP and seq % LANES == 0
    assert B_Wq.shape == (D, HB, DB) and mem == 8 and 4 * seg == LANES

    hbm = pl.BlockSpec(memory_space=pl.ANY)
    vmem = pl.BlockSpec(memory_space=pltpu.VMEM)
    out_t = pl.pallas_call(
        functools.partial(_kernel, seq=seq, seg=seg, mem=mem),
        out_shape=jax.ShapeDtypeStruct((D, seq), A_x.dtype),
        in_specs=[hbm, hbm, hbm, vmem, hbm, hbm, hbm, hbm, vmem],
        out_specs=hbm,
        scratch_shapes=[
            pltpu.VMEM((nt, D, LANES), BF16),
            pltpu.VMEM((D, 3 * D), BF16),
            pltpu.VMEM((D, D), BF16),
            pltpu.VMEM((3 * GP + 1, KB, D, DB), U32),
            pltpu.VMEM((HB, D, DB), BF16),
            pltpu.VMEM((GP + 1, 2 * KB + 1, KB, 64, LANES), U32),
            pltpu.VMEM((5, 3 * D, LANES), F32),
            pltpu.VMEM((5, D, LANES), F32),
            pltpu.VMEM((12, 3 * D // 2 + 16, LANES), BF16),
            pltpu.VMEM((12, D // 2, LANES), BF16),
            pltpu.VMEM((2 * D, LANES), BF16),
            pltpu.VMEM((D, LANES), BF16),
            pltpu.VMEM((4 * GP + 1, 2 * NR + NH, LANES, LANES), BF16),
            pltpu.VMEM((KB + 1, seq, LANES), F32),
            pltpu.VMEM((nt, D, LANES), F32),
            pltpu.VMEM((nt, 8, LANES), F32),
            pltpu.VMEM((2 * KB, mem, LANES), F32),
            pltpu.VMEM((3, HB, 2, seg, LANES), F32),
            pltpu.VMEM((2, HB, seg, LANES), F32),
            pltpu.VMEM((KB + 1, 2, seg, LANES), F32),
            pltpu.VMEM((KB + 1, 2, seg, LANES), F32),
            pltpu.VMEM((nt, D, LANES), A_x.dtype),
            pltpu.SemaphoreType.DMA((3 * GP + 2,)),
            pltpu.SemaphoreType.DMA((8,)),
            pltpu.SemaphoreType.DMA(()),
        ],
        compiler_params=pltpu.CompilerParams(vmem_limit_bytes=110 * 1024 * 1024),
        name="gated_mix_kernel",
    )(A_x[0].T, A_wqkv, A_wo, B_mem0[0], B_Wq, B_Wk, B_Wv, B_Wo.transpose(0, 2, 1), gate_w)
    return out_t.T[None]
```

```python
import functools
import itertools

import jax
import jax.numpy as jnp
import numpy as np
from jax import lax
import jax.experimental.pallas as pl
import jax.experimental.pallas.tpu as pltpu

F32, BF16, U32 = jnp.float32, jnp.bfloat16, jnp.uint32

D = 576
LANES = 128
HA, DA = 32, 18
WIN, DIL = 8, 2
HB, DB = 32, 128
NEG = -1000000000.0
LOG2E = 1.4426950408889634
NG = HA // 8

KB = 4
GP = HB // (2 * KB)

_HK = (
    (".... +...", "+.-. -... .... -...", "+... +..."),
    ("+... -...", "+-.- .... -... ....", "+... ...."),
    (".+.. .-..", ".... +-.. .+.. ....", ".... .+.."),
    (".+.. ....", ".-.. .+-. .... ....", ".+.. .+.."),
    (".... ..+.", ".... ..-. -.+. .+-.", ".... ..+."),
    ("..+. ....", "..-. ...+ .-+- ....", "..+. ...."),
    ("...+ ...-", ".... ...- ...+ ++.-", ".... ...+"),
    ("...+ ....", "...- ...- .... .+-+", "...+ ...+"),
    (".... ++..", ".... +... .... ....", ".... ++.."),
    ("++.. ....", ".+.. .... .... ....", "++.. ...."),
    (".+.. +...", ".-.. +... .... ....", "+... .-.."),
    ("+.+. -.-.", ".... .... -... ....", ".... +.+."),
    ("+.+. ....", "..+. .... .... ....", "+.+. +.+."),
    ("+.+. -...", "..-. .... +... ....", "+... +.+."),
    (".... +..+", ".... .... .... +...", ".... +..+"),
    ("+..+ ....", "...+ .... .... ....", "+..+ ...."),
    ("...+ +...", "...- .... .... +...", "+... ...-"),
    (".... .++.", ".... ..+. .... .-..", ".++. .++."),
    (".++. .--.", ".... ...- .+.. ....", ".++. ...."),
    (".+.. .--.", ".... ..+. .-.. ....", ".++. .+.."),
    (".... ..++", ".... .... .... .-+.", "..++ ..++"),
    ("..++ ..--", ".... ...- ...+ ....", "..++ ...."),
    ("...+ ..--", ".... ...+ ...- .-+.", "..++ ...+"),
    (".... .+++", ".... .... .... .+..", ".... .+++"),
    (".+++ ....", ".... ...+ .... ....", ".+++ ...."),
    ("...+ .++.", ".... ...- .... .+..", ".++. ...-"),
)
_U, _V, _C = (np.array([[["-.+".index(ch) - 1 for ch in row] for row in prod[i].split()]
                        for prod in _HK]) for i in range(3))
NR = len(_HK)
assert np.array_equal(np.einsum("rak,rln,rbm->akblnm", _U, _V, _C),
                      np.einsum("ab,kl,nm->akblnm", *(np.eye(n, dtype=int) for n in (2, KB, KB))))


def _phase(products):
    tiles = [max(r, ~r) for r in products]
    dual = np.rint(np.linalg.inv(_V[tiles].reshape(len(tiles), -1)).T).astype(int)
    slots = []
    for r, d in zip(products, dual.reshape(-1, KB, KB)):
        i, j = np.argwhere(d)[0]
        a, c = d[:, j] * d[i, j], d[i]
        assert np.array_equal(np.outer(a, c), d)
        slots.append(dict(r=max(r, ~r), tok=r >= 0, a=a.tolist(), c=c.tolist()))
    return slots


_PHASES = (_phase((11, 8, ~9, 4, 2, 23, 17, ~13, 25, 20, 22, 7, ~19, 16, 15, 1)),
           _phase((24, 21, ~16, 18, 19, 3, 10, ~22, 9, 5, 12, 13, ~25, 0, 14, 6)))
assert sorted(s["r"] for ph in _PHASES for s in ph if s["tok"]) == list(range(NR))

NH = 2 * KB
assert all(sorted(s["r"] // 2 for s in ph if s["r"] < NH) == list(range(KB)) for ph in _PHASES)
assert all(np.abs(s[k]).tolist() == np.eye(KB)[s["r"] // 2].tolist()
           for ph in _PHASES for s in ph if s["r"] < NH for k in "ac")
_TAIL_IN, _TAIL_OUT = (
    np.concatenate([np.rint(np.linalg.inv(t[2 * n:2 * n + 2, :, n]).T).astype(int)
                    for n in range(KB)]) for t in (_C, _U))


CHUNKS, S0, LAG, SPAN, HEAD, M0 = ((0, 1), (2, 3)), 72, 40, (11.25, 1), 72, 6
PO = (1, 0, 2)
MO = (364, 385, 410, 426, 444, 463)


Q = 2


XCUT = (0, 1, 3, 8)
RE, RO = 8, 48
ORD = (9, 8, 10, 19, 2, 3, 23, 24, 25, 17, 18, 20, 21, 22, 12, 11, 13, 4, 5, 15, 14, 16, 6, 7, 0, 1)
CUT = (1,)
QA = ((10, 16, 30, 45, 61, 77, 92, 108, 124, 152, 159, 166, 173), 20)
QB = ((10, 16, 22, 42, 58, 75, 91, 108, 146, 150, 155, 160, 165, 170, 175), 24)
QC = (range(8, 54, 4), 16)


def _signed_sum(terms):
    terms = [(c, t) for c, t in terms if c]
    first = next((i for i, (c, _) in enumerate(terms) if c > 0), 0)
    c, acc = terms.pop(first)
    acc = acc if c > 0 else -acc
    for c, t in terms:
        acc = acc + t if c > 0 else acc - t
    return acc


class _Mixer:
    def __init__(self, block):
        self.block, self.known = block, {}

    def __call__(self, coef):
        want = {(i, k): int(c) for i, row in enumerate(coef) for k, c in enumerate(row) if c}
        key = tuple(sorted(want.items()))
        if key not in self.known:
            terms = []
            for have in sorted(self.known, key=lambda h: -len(h)):
                for sign in (1, -1):
                    if all(want.get(pos) == sign * c for pos, c in have):
                        terms.append((sign, self.known[have]))
                        want = {pos: c for pos, c in want.items() if pos not in dict(have)}
                        break
            for pos, c in sorted(want.items()):
                self.known[((pos, 1),)] = self.block(*pos)
                terms.append((c, self.known[((pos, 1),)]))
            self.known[key] = _signed_sum(terms)
        return self.known[key]


class _Sums:
    def __init__(self, done):
        self.done, self.acc = done, {}

    def add(self, key, sign, value, expected):
        if not sign:
            return
        count, neg, tot = self.acc.pop(key, (0, sign < 0, value))
        if count and neg == (sign < 0):
            tot = tot + value
        elif count:
            tot, neg = (value - tot if neg else tot - value), False
        if count + 1 == expected:
            self.done(key, -tot if neg else tot)
        else:
            self.acc[key] = (count + 1, neg, tot)


class _Carry:
    def __init__(self, ref):
        self.ref, self.val = ref, {}

    def __getitem__(self, key):
        return self.val[key] if key in self.val else self.ref[key]

    def __setitem__(self, key, value):
        self.val[key] = value

    def flush(self):
        for key, value in self.val.items():
            self.ref[key] = value
        self.val = {}


def _dot(a, b):
    return lax.dot_general(a, b, (((1,), (0,)), ((), ())), preferred_element_type=F32)


def _dot_nt(a, b):
    return lax.dot_general(a, b, (((1,), (1,)), ((), ())), preferred_element_type=F32)


def _tile(ref, *idx):
    return pltpu.bitcast(ref.bitcast(U32)[idx], BF16)


def stack(*parts):
    parts = [t for t in parts if t is not None]
    return parts[0] if len(parts) == 1 else jnp.concatenate(parts, axis=0)


def _low_half(rows):
    return lax.broadcasted_iota(jnp.int32, (rows, LANES), 1) < 64


def _pair_lhs(t1, t2):
    lo = _low_half(t1[3].shape[0])
    diff = t1[3] - t2[3]
    return (t1[:3] + [jnp.where(lo, t1[4], diff)]
            + t2[:3] + [jnp.where(lo, -diff, t2[4])]
            + [jnp.where(lo, t1[3], t2[3])])


def _pair_rhs(x):
    a, b, c = x[384:448], x[448:512], x[512:576]
    cat = lambda u, v: jnp.concatenate([u, v], axis=0)
    return [x[i * 128:(i + 1) * 128] for i in range(3)] + [cat(c, b), cat(a, c), x[384:512]]


def _pair_matmul(lhs, rhs, dot):
    out = [dot(lhs(8), rhs[5])] * 2
    for i in range(8):
        out[i // 4] = out[i // 4] + dot(lhs(i), rhs[i % 4 if i < 7 else 4])
    return out


def _kernel(xt_hbm, wqkv_hbm, wo_hbm, mem0_ref, wq_hbm, wk_hbm, wv_hbm, wot_hbm, gate_ref,
            out_hbm,
            xt_v, wqkv_v, wo_v, stg_qkv, stg_o, wo_t, wt32, wo32_s, la, lo_a, kv_prev, oa_s,
            wb, x32, ga_s, gm_s, mem_s, part_s, o_s, opart_s, b_s, out_v,
            sem_in, sem_out, *, seq, seg, mem):
    nt = seq // LANES
    rows = mem + seg

    sems = (sem_in.at[n] for n in itertools.count(3 * GP))
    copy = pltpu.make_async_copy
    cp_wqkv = {k: copy(wqkv_hbm.at[k * LANES:min(D, (k + 1) * LANES)],
                       wqkv_v.at[k * LANES:min(D, (k + 1) * LANES)], next(sems))
               for k in (3, 4, 0, 1, 2)}
    cp_wo = copy(wo_hbm, wo_v, next(sems))
    cp_x = {j0: [copy(xt_hbm.at[:, j * LANES:(j + 1) * LANES], xt_v.at[j], sem)
                 for j in range(j0, j1)] for j0, j1, sem in zip(XCUT, XCUT[1:] + (nt,), sems)}
    cp_wot = [copy(wot_hbm.at[h0:h1], stg_o.at[h0:h1], next(sems))
              for h0, h1 in ((0, HB - 2 * KB), (HB - 2 * KB, HB))]
    queue = list(cp_wqkv.values()) + cp_x[0] + [cp_wo]
    for unit in range(3 * GP):
        src = (wq_hbm, wk_hbm, wv_hbm)[unit // GP].bitcast(U32)
        queue += cp_x.get(unit + 1, []) + [
            copy(src.at[:, KB * (unit % GP) + p, :], stg_qkv.at[unit, p], sem_in.at[unit])
            for p in range(KB)]
    for c in queue + cp_wot:
        c.start()

    def wait_all(copies):
        for c in copies:
            c.wait()

    def cp_out(j):
        col = j * LANES if isinstance(j, int) else pl.multiple_of(j * LANES, LANES)
        return copy(out_v.at[j], out_hbm.at[:, pl.ds(col, LANES)], sem_out)

    m0 = mem0_ref[...].astype(F32)
    for kk in range(KB):
        mem_s[kk] = m0[:, kk * LANES:(kk + 1) * LANES]
    mem_s[KB] = jnp.concatenate([m0[:, KB * LANES:]] * 2, axis=1)
    for ref in (o_s, opart_s, b_s):
        ref[...] = jnp.zeros(ref.shape, ref.dtype)
    wb[4 * GP, 0, 0:16, :] = jnp.zeros((16, LANES), BF16)

    gate = jnp.broadcast_to(gate_ref[...].astype(F32).reshape(1, D), (8, D))
    gate_t = [gate[:, i * 128:(i + 1) * 128] for i in range(4)]
    gate_t.append(jnp.concatenate([gate[:, 512:], gate[:, 512:]], axis=1))

    entries = [None] * 2 + [(g - part // 2, part, n) for g in range(NG + 1) for n in range(DA // 2)
                            for part in (1, 0, 2) if 0 <= g - part // 2 < NG]

    def feature_rows(k, e):
        return stack(*(gate_t[k] if ent is None else
                       wt32[k, pl.ds(ent[1] * D + ent[0] * 8 * DA + 2 * ent[2] + e, 8, stride=DA), :]
                       for ent in entries))

    for k in cp_wqkv:
        cp_wqkv[k].wait()
        rows_k = wqkv_v[k * LANES:min(D, (k + 1) * LANES), :]
        wt32[k, 0:3 * D] = (rows_k if k < 4 else stack(rows_k, rows_k)).T.astype(F32)
        for e in range(2 if k < 3 else 0):
            la[4 * e + k] = feature_rows(k, e).astype(BF16)
        if k == 4:
            mixed = _pair_lhs(*([None] * 3 + [feature_rows(3, e), feature_rows(4, e)]
                                for e in range(2)))
            for i in (3, 7, 8):
                la[i] = mixed[i].astype(BF16)

    def prep_wo():
        wo32 = wo_v[...].astype(F32)
        for n in range(4):
            wo32_s[n, 0:D] = wo32[:, n * LANES:(n + 1) * LANES]
        wo32_s[4, 0:D] = jnp.concatenate([wo32[:, 4 * LANES:]] * 2, axis=1)
        turned = []
        for n in range(5):
            perm = stack(*(wo32_s[n, pl.ds(g * 8 * DA + d, 8, stride=DA), :]
                           for g in range(NG) for d in range(DA))).astype(BF16)
            turned.append([perm[k * LANES:(k + 1) * LANES].T for k in range(4)]
                          + [stack(perm[4 * LANES:], perm[4 * LANES:]).T])
        tiles = [stack(*(t[k] for t in turned))[:D].astype(F32) for k in range(5)]
        for i, t in enumerate(_pair_lhs([t[:D // 2] for t in tiles], [t[D // 2:] for t in tiles])):
            lo_a[i] = t.astype(BF16)

    by_size = ORD

    def prep_qkv(unit):
        src, dst = stg_qkv.at[unit], wb.at[unit]

        def rows(g, r0, nu):
            u = src[2 * g + nu // 2, r0:r0 + 16, :]
            return pltpu.bitcast(u & jnp.uint32(0xFFFF0000) if nu % 2 else u << 16, F32)

        for e in range(8):
            at, own, shared = pl.ds(16 * e, 16), e // 4, {}
            for g in (own, 1 - own):
                mix = _Mixer(lambda kk, nu: rows(g, kk * LANES + 16 * e, nu))
                for r in by_size:
                    w = mix(_V[r])
                    if r < NH and g == own:
                        shared[r] = w.astype(BF16)
                        dst[2 * NR + r, at, :] = shared[r]
                        w = rows(g, KB * LANES + 16 * (e % 4), r // 2)
                    elif r < NH:
                        w = w - shared[r].astype(F32)
                    dst[g * NR + r, at, :] = w.astype(BF16)
                    if r in CUT:
                        yield

    def turn_out(gp):
        words = lambda head, r0, n: _tile(stg_o, 2 * KB * gp + head, pl.ds(r0 // 2, n // 2))
        for head in range(2 * KB + 1):
            for nu in range(KB):
                if head < 2 * KB:
                    tile = words(head, nu * LANES, LANES)
                else:
                    tile = stack(*(words(g * KB + nu, KB * LANES, 64) for g in range(2)))
                wo_t[gp, head, nu] = pltpu.bitcast(tile.T, U32)

    def prep_out(gp):
        dst, lo = wb.at[3 * GP + gp], _low_half(16)
        for e in range(8):
            at, first = pl.ds(16 * e, 16), {}
            rows = lambda head, nu: pltpu.bitcast(
                wo_t[gp, head, nu, 8 * e:8 * e + 8, :], BF16).astype(F32)
            for g in range(2):
                mix = _Mixer(lambda kk, nu: rows(g * KB + kk, nu))
                for r in by_size:
                    w = mix(_V[r])
                    if r >= NH:
                        dst[g * NR + r, at, :] = w.astype(BF16)
                    elif g == 0:
                        first[r] = w
                    else:
                        z, t = jnp.where(lo, first[r], w).astype(BF16), rows(2 * KB, r // 2)
                        dst[2 * NR + r, at, :] = z
                        dst[r, at, :] = jnp.where(lo, t, first[r] - z.astype(F32)).astype(BF16)
                        dst[NR + r, at, :] = jnp.where(lo, w - z.astype(F32), t).astype(BF16)
                    if r in CUT:
                        yield

    lane = lax.broadcasted_iota(jnp.int32, (8, LANES), 1)

    def exchange(idx, pair, first):
        at = pl.ds(8 * idx, 8)
        prev = None if first else kv_prev.bitcast(U32)[at, :]
        kv_prev[16 * idx:16 * idx + 16, :] = jnp.concatenate(pair, axis=0).astype(BF16)
        cur = kv_prev.bitcast(U32)[at, :]
        return (jnp.broadcast_to(cur[:, 0:1], (8, LANES)) if first else prev), cur

    def to_rows(j):
        t0 = j * LANES if isinstance(j, int) else pl.multiple_of(j * LANES, LANES)
        xt = _tile(xt_v, j)
        for kk in range(KB + 1):
            tile = xt[kk * LANES:(kk + 1) * LANES]
            x32[kk, pl.ds(t0, LANES), :] = (tile if kk < KB else stack(tile, tile)).T.astype(F32)

    def paced(job, src, dst, when, back):
        results = []

        def dot(left, right):
            if len(results) in when:
                if src is not None and len(results) >= back:
                    src[...] = pltpu.bitcast(results[-back][0:8], U32)
                next(job, None)
                left = stack(left[:-8] if len(left) > 8 else None, left[-8:] | dst[...])
            results.append(_dot(pltpu.bitcast(left, BF16), right))
            return results[-1]

        return dot

    spare_qkv, spare_t = stg_qkv.at[3 * GP, 0, 0:8], wo_t.at[GP, 0, 1, 0:8]
    zero_w = wb.bitcast(U32).at[4 * GP, 0, 0:8]

    def a_out(j, dot):
        rhs = _pair_rhs(_tile(oa_s, slice(None)))
        for r0 in range(0, D // 2, RO):
            halves = _pair_matmul(lambda i: lo_a.bitcast(U32)[i, r0 // 2:(r0 + RO) // 2, :], rhs, dot)
            for e in range(2):
                ga_s[j, pl.ds(e * D // 2 + r0, RO), :] = halves[e]

    def a_tile(j, first, dot):
        rhs = _pair_rhs(_tile(xt_v, j))
        logit, prob, outs = {}, {}, {}
        for e0 in range(0, len(entries), RE):
            some = entries[e0:e0 + RE]
            halves = _pair_matmul(
                lambda i: la.bitcast(U32)[i, 4 * e0:4 * (e0 + len(some)), :], rhs, dot)
            for ent, r0 in zip(some, range(0, 8 * RE, 8)):
                pair = [t[r0:r0 + 8] for t in halves]
                if ent is None:
                    gsig = 1.0 / (1.0 + jnp.exp(-halves[0][0:8]))
                    continue
                g, part, n = ent
                if part:
                    prev, cur = exchange((2 * g + part - 1) * (DA // 2) + n, pair, first)
                    back = [cur] + [
                        pltpu.roll(jnp.where(lane >= LANES - DIL * w, prev, cur), DIL * w, 1)
                        for w in range(1, WIN)]
                    back = [pltpu.bitcast(t, BF16).astype(F32) for t in back]
                if part == 2:
                    outs[g, n] = functools.reduce(
                        jnp.add, [stack(p, p) * t for p, t in zip(prob[g], back)]).astype(BF16)
                elif part == 0:
                    terms = [pair[0] * t[0:8] + pair[1] * t[8:16] for t in back]
                    logit[g] = terms if n == 0 else [a + t for a, t in zip(logit[g], terms)]
                if (part, n) == (0, DA // 2 - 1):
                    s = [t * (DA ** -0.5) for t in logit[g]]
                    if first:
                        s = [jnp.where(lane >= DIL * w, t, NEG) for w, t in enumerate(s)]
                    top = functools.reduce(jnp.maximum, s)
                    ex = [jnp.exp(t - top) for t in s]
                    inv = gsig / functools.reduce(jnp.add, ex)
                    prob[g] = [t * inv for t in ex]
        gm_s[j] = 1.0 - gsig
        if not first:
            a_out(j - 1, dot)
        oa_s[...] = stack(*(outs[key] for key in sorted(outs)))

    plain = lambda left, right: _dot(pltpu.bitcast(left, BF16), right)
    wait_all(cp_x[0])
    to_rows(0)
    a_tile(0, True, plain)
    cp_wo.wait()
    prep_wo()

    def a_loop(first, count, work, spare, loading):
        def body(j, carry):
            if loading:
                for j0 in XCUT[1:]:
                    pl.when(j == j0)(functools.partial(wait_all, cp_x[j0]))
                copy(stg_qkv.at[j - first], stg_qkv.at[j - first], sem_in.at[j - first]).wait()
                to_rows(j)
            job = work(j - first)
            a_tile(j, False, paced(job, spare, zero_w, *(QA if loading else QB)))
            list(job)
            return carry

        lax.fori_loop(first, first + count, body, 0)

    a_loop(1, 3 * GP, prep_qkv, spare_qkv, True)

    qi = lax.broadcasted_iota(jnp.int32, (rows, rows), 0)
    ki = lax.broadcasted_iota(jnp.int32, (rows, rows), 1)
    mask = (qi >= seg) | (ki >= seg) | (qi >= ki)
    part, o_prev, opart, b_rows = (_Carry(r) for r in (part_s, o_s, opart_s, b_s))
    ahead = {}

    def b_step(u, t0, memv, project_only=False, output_only=False):
        odd = u % 2
        keep = lambda slots: [s for s in slots if s["tok"] or memv]
        qs, os_ = keep(_PHASES[odd]), keep(_PHASES[1 - odd])
        lhs, shared, tok, mrow, full, soft, o_mem, o_mix, o_left, o_host, new = ({} for _ in range(11))

        def spread(sums, key, slots, s, tok_rows, mem_rows):
            for nu in range(KB):
                if memv:
                    sums.add(key + (nu, 2), s["c"][nu], mem_rows, sum(abs(o["c"][nu]) for o in slots))
                for mu in range(2 if s["tok"] else 0):
                    sums.add(key + (nu, mu), _C[s["r"]][mu][nu], tok_rows,
                             sum(abs(_C[o["r"]][mu][nu]) for o in slots if o["tok"]))

        x_mix = _Mixer(lambda mu, kk: x32[kk, pl.ds(t0 + mu * seg, seg), :])
        c_mix = _Mixer(lambda mu, _: x32[KB, pl.ds(t0 + mu * seg, seg), :])
        m_mix = _Mixer(lambda _, kk: memv[kk])

        def q_left(e, t):
            s = qs[e]
            if (e, t) not in lhs:
                left = stack(x_mix(_U[s["r"]]) if s["tok"] else None,
                             m_mix([s["a"]]) if memv else None)
                if s["r"] < NH and t < 2:
                    c = stack(c_mix(_TAIL_IN[s["r"]][:, None]),
                              _signed_sum([(sum(s["c"]), memv[KB])]) if memv else None)
                    left = jnp.where(_low_half(c.shape[0]), *((c, left), (left, c))[t])
                lhs[e, t] = left
            return lhs[e, t]

        def q_total(key, value):
            i, g, nu, mu = key
            h = g * KB + nu
            if mu == 2:
                mrow[i, h] = value
            elif odd:
                part[i, h, mu] = value
            elif mu == 0:
                tok[i, h] = value + part[i, h, mu]
            else:
                ahead[i, h] = value + part[i, h, mu]
            cur = (ahead if odd else tok).get((i, h))
            if (i, h) in mrow and cur is not None and (i, h) not in full:
                full[i, h] = stack(cur, mrow[i, h]).astype(BF16 if i else F32)

        q_sums = _Sums(q_total)

        def q_pass(e, i, gp, t):
            s = qs[e]
            p = _dot(q_left(e, t), _tile(wb, i * GP + gp, t * NR + s["r"]))
            if t == 2:
                shared[e, i, gp] = p
                return
            if s["r"] < NH:
                p = p + shared[e, i, gp]
            spread(q_sums, (i, 2 * gp + t), qs, s, p[:seg], p[-mem:])

        def scores(h):
            s = jnp.where(mask, _dot_nt(full[0, h], full[1, h]), NEG * DB ** 0.5)
            e = jnp.exp2((s - jnp.max(s, axis=-1, keepdims=True)) * (DB ** -0.5 * LOG2E))
            total = jnp.sum(e, axis=-1, keepdims=True)
            inv = pltpu.reciprocal(total, approx=True)
            soft[h] = e * (inv * (2.0 - total * inv))

        def values(h):
            o = _dot(soft[h], full[2, h])
            o_mem[h] = o[seg:]
            if odd:
                o_prev[0, h], o_prev[1, h] = ahead["o", h], o[:seg]
            else:
                ahead["o", h] = o[:seg]

        def o_rows(e, gp, t):
            s = os_[e]
            if (e, gp, t) not in o_left:
                g = 2 * gp + t
                if t == 2:
                    o_left[e, gp, t] = o_rows(e, gp, 0) + o_rows(e, gp, 1)
                    return o_left[e, gp, t]
                if g not in o_mix:
                    o_mix[g] = (_Mixer(lambda _, kk: o_mem[g * KB + kk]),
                                _Mixer(lambda mu, kk: o_prev[mu, g * KB + kk]))
                o_left[e, gp, t] = stack(o_mix[g][0]([s["a"]]) if memv else None,
                                         o_mix[g][1](_U[s["r"]]) if s["tok"] else None)
            return o_left[e, gp, t]

        def o_total(key, value):
            nu, mu = key
            if mu == 2:
                new[nu] = value if nu < KB else value + pltpu.roll(value, 64, 1)
            elif odd:
                opart[nu, mu] = value
            else:
                b_rows[nu, (u - 2) % 4 + mu] = value + opart[nu, mu]

        out_sums = _Sums(o_total)

        def o_product(key, value):
            e, t = key
            s = os_[e]
            if s["r"] < NH:
                o_host[key] = value
                if any((e, t_) not in o_host for t_ in range(3)):
                    return
                lo = _low_half(value.shape[0])
                value = o_host[e, 2] + jnp.where(lo, o_host[e, 1], o_host[e, 0])
                y = jnp.where(lo, o_host[e, 0], o_host[e, 1])
                if memv:
                    out_sums.add((KB, 2), sum(s["a"]), y[:mem], KB)
                for mu in range(2):
                    out_sums.add((KB, mu), _TAIL_OUT[s["r"]][mu], y[-seg:],
                                 sum(abs(_TAIL_OUT[o["r"]][mu]) for o in os_ if o["r"] < NH))
            spread(out_sums, (), os_, s, value[-seg:], value[:mem])

        o_sums = _Sums(o_product)

        def o_pass(e, gp, t):
            host = os_[e]["r"] < NH
            p = _dot(o_rows(e, gp, t), _tile(wb, 3 * GP + gp, t * NR + os_[e]["r"]))
            o_sums.add((e, t if host else 0), 1, p, GP if host else 2 * GP)

        todo = []
        tiles = lambda s: (2, 0, 1) if s["r"] < NH else (0, 1)
        if not output_only:
            todo = [(s["tok"], q_pass, e, i, gp, t) for gp in range(GP) for i in PO
                    for e, s in enumerate(qs) for t in tiles(s)]
            last = [max(e for e, s in enumerate(_PHASES[odd]) if s["tok"] and s["c"][nu])
                    for nu in range(KB)]
            ready = lambda e, t: 99 if qs[e]["r"] < NH and t < 2 else max(
                last[kk] for kk in range(KB) if qs[e]["a"][kk])
            todo[:HEAD] = sorted(todo[:HEAD], key=lambda p: ready(p[2], p[5]))
        if not project_only:
            todo += [(s["tok"], o_pass, e, gp, t) for pairs in CHUNKS for e, s in enumerate(os_)
                     for gp in pairs for t in tiles(s)]
        long_, short = ([p[1:] for p in todo if p[0] == tok] for tok in (True, False))
        extra = {}
        for h in range(HB if memv else 0):
            gp, n = divmod(h, 2 * KB)
            at = (90 * gp + S0 + int(SPAN[gp == GP - 1] * (n // Q * Q))) // Q * Q
            extra.setdefault(at, []).append((scores, h))
            extra.setdefault(at + LAG, []).append((values, h))
        issued = 0
        for n, p in enumerate(long_):
            for fn, *args in extra.get(n, []) + [p]:
                if issued % 4 == 0 and short and n >= (480 + M0 - 5 * len(short) if len(short) > 24 else MO[6 - len(short) // 4]):
                    for fn_s, *args_s in short[:4]:
                        fn_s(*args_s)
                    del short[:4]
                fn(*args)
                issued += 1
        assert not short
        return new

    def emit_tile(j):
        for nu in range(KB + 1):
            bt = jnp.concatenate([b_s[nu, 0], b_s[nu, 1], b_rows.val.pop((nu, 2)),
                                  b_rows.val.pop((nu, 3))], axis=0).T
            bt = bt if nu < KB else bt[:64] + bt[64:]
            at = pl.ds(nu * LANES, bt.shape[0])
            gm = jnp.concatenate([gm_s[j]] * (bt.shape[0] // 8), axis=0)
            out_v[j, at, :] = (ga_s[j, at, :] + gm * bt).astype(out_v.dtype)

    cp_wot[0].wait()
    for gp in range(GP - 1):
        turn_out(gp)
    b_step(3, 0, None, project_only=True)
    part.flush()
    for j in range(3 * GP + 1, nt):
        to_rows(j)
    cp_wot[1].wait()
    turn_out(GP - 1)
    a_loop(3 * GP + 1, GP - 1, prep_out, spare_t, False)
    job = prep_out(GP - 1)
    a_out(nt - 1, paced(job, spare_t, zero_w, *QC))
    list(job)

    def b_body(j, carry):
        memv = {kk: mem_s[kk] for kk in range(KB + 1)}
        for u in range(4):
            t0 = jnp.minimum(j * LANES + (u + 1) // 2 * 2 * seg, seq - 2 * seg)
            memv = b_step(u, pl.multiple_of(t0, seg), memv)
            if u == 0:
                emit_tile(jnp.maximum(j - 1, 0))
        for kk, t in memv.items():
            mem_s[kk] = t
        for c in (part, o_prev, opart, b_rows):
            c.flush()
        pl.when(j > 0)(lambda: cp_out(j - 1).start())
        return carry

    lax.fori_loop(0, nt, b_body, 0)
    b_step(0, None, None, output_only=True)
    emit_tile(nt - 1)
    cp_out(nt - 1).start()
    for j in range(nt):
        cp_out(j).wait()


@functools.partial(jax.jit, static_argnames=("B_seg_len",))
def pallas_gated_mix__sliding_local_dilated__memory_aug_recurrent_mem_tr__prompt_kernel(
    A_x: jax.Array,
    A_wqkv: jax.Array,
    A_wo: jax.Array,
    B_x: jax.Array,
    B_mem0: jax.Array,
    B_Wq: jax.Array,
    B_Wk: jax.Array,
    B_Wv: jax.Array,
    B_Wo: jax.Array,
    B_seg_len: int,
    gate_w: jax.Array,
):
    del B_x
    batch, seq, width = A_x.shape
    mem, seg = B_mem0.shape[1], int(B_seg_len)
    nt = seq // LANES
    assert batch == 1 and width == D and nt == 4 * GP and seq % LANES == 0
    assert B_Wq.shape == (D, HB, DB) and mem == 8 and 4 * seg == LANES

    hbm = pl.BlockSpec(memory_space=pl.ANY)
    vmem = pl.BlockSpec(memory_space=pltpu.VMEM)
    out_t = pl.pallas_call(
        functools.partial(_kernel, seq=seq, seg=seg, mem=mem),
        out_shape=jax.ShapeDtypeStruct((D, seq), A_x.dtype),
        in_specs=[hbm, hbm, hbm, vmem, hbm, hbm, hbm, hbm, vmem],
        out_specs=hbm,
        scratch_shapes=[
            pltpu.VMEM((nt, D, LANES), BF16),
            pltpu.VMEM((D, 3 * D), BF16),
            pltpu.VMEM((D, D), BF16),
            pltpu.VMEM((3 * GP + 1, KB, D, DB), U32),
            pltpu.VMEM((HB, D, DB), BF16),
            pltpu.VMEM((GP + 1, 2 * KB + 1, KB, 64, LANES), U32),
            pltpu.VMEM((5, 3 * D + 32, LANES), F32),
            pltpu.VMEM((5, D + 32, LANES), F32),
            pltpu.VMEM((12, 3 * D // 2 + 16, LANES), BF16),
            pltpu.VMEM((12, D // 2, LANES), BF16),
            pltpu.VMEM((2 * D, LANES), BF16),
            pltpu.VMEM((D, LANES), BF16),
            pltpu.VMEM((4 * GP + 1, 2 * NR + NH, LANES, LANES), BF16),
            pltpu.VMEM((KB + 1, seq, LANES), F32),
            pltpu.VMEM((nt, D, LANES), F32),
            pltpu.VMEM((nt, 8, LANES), F32),
            pltpu.VMEM((2 * KB, mem, LANES), F32),
            pltpu.VMEM((3, HB, 2, seg, LANES), F32),
            pltpu.VMEM((2, HB, seg, LANES), F32),
            pltpu.VMEM((KB + 1, 2, seg, LANES), F32),
            pltpu.VMEM((KB + 1, 2, seg, LANES), F32),
            pltpu.VMEM((nt, D, LANES), A_x.dtype),
            pltpu.SemaphoreType.DMA((3 * GP + 8 + len(XCUT),)),
            pltpu.SemaphoreType.DMA(()),
        ],
        compiler_params=pltpu.CompilerParams(vmem_limit_bytes=110 * 1024 * 1024),
        name="gated_mix_kernel",
    )(A_x.reshape(seq, D).T, A_wqkv, A_wo, B_mem0.reshape(mem, D), B_Wq, B_Wk, B_Wv,
      B_Wo.transpose(0, 2, 1), gate_w)
    return out_t.T.reshape(batch, seq, D)
```

```python
import functools
import itertools

import jax
import jax.numpy as jnp
import numpy as np
from jax import lax
import jax.experimental.pallas as pl
import jax.experimental.pallas.tpu as pltpu

F32, BF16, U32 = jnp.float32, jnp.bfloat16, jnp.uint32

D = 576
LANES = 128
HA, DA = 32, 18
WIN, DIL = 8, 2
HB, DB = 32, 128
NEG = -1000000000.0
LOG2E = 1.4426950408889634
NG = HA // 8

KB = 4
GP = HB // (2 * KB)

_HK = (
    (".... +...", "+.-. -... .... -...", "+... +..."),
    ("+... -...", "+-.- .... -... ....", "+... ...."),
    (".+.. .-..", ".... +-.. .+.. ....", ".... .+.."),
    (".+.. ....", ".-.. .+-. .... ....", ".+.. .+.."),
    (".... ..+.", ".... ..-. -.+. .+-.", ".... ..+."),
    ("..+. ....", "..-. ...+ .-+- ....", "..+. ...."),
    ("...+ ...-", ".... ...- ...+ ++.-", ".... ...+"),
    ("...+ ....", "...- ...- .... .+-+", "...+ ...+"),
    (".... ++..", ".... +... .... ....", ".... ++.."),
    ("++.. ....", ".+.. .... .... ....", "++.. ...."),
    (".+.. +...", ".-.. +... .... ....", "+... .-.."),
    ("+.+. -.-.", ".... .... -... ....", ".... +.+."),
    ("+.+. ....", "..+. .... .... ....", "+.+. +.+."),
    ("+.+. -...", "..-. .... +... ....", "+... +.+."),
    (".... +..+", ".... .... .... +...", ".... +..+"),
    ("+..+ ....", "...+ .... .... ....", "+..+ ...."),
    ("...+ +...", "...- .... .... +...", "+... ...-"),
    (".... .++.", ".... ..+. .... .-..", ".++. .++."),
    (".++. .--.", ".... ...- .+.. ....", ".++. ...."),
    (".+.. .--.", ".... ..+. .-.. ....", ".++. .+.."),
    (".... ..++", ".... .... .... .-+.", "..++ ..++"),
    ("..++ ..--", ".... ...- ...+ ....", "..++ ...."),
    ("...+ ..--", ".... ...+ ...- .-+.", "..++ ...+"),
    (".... .+++", ".... .... .... .+..", ".... .+++"),
    (".+++ ....", ".... ...+ .... ....", ".+++ ...."),
    ("...+ .++.", ".... ...- .... .+..", ".++. ...-"),
)
_U, _V, _C = (np.array([[["-.+".index(ch) - 1 for ch in row] for row in prod[i].split()]
                        for prod in _HK]) for i in range(3))
NR = len(_HK)
assert np.array_equal(np.einsum("rak,rln,rbm->akblnm", _U, _V, _C),
                      np.einsum("ab,kl,nm->akblnm", *(np.eye(n, dtype=int) for n in (2, KB, KB))))


def _phase(products):
    tiles = [max(r, ~r) for r in products]
    dual = np.rint(np.linalg.inv(_V[tiles].reshape(len(tiles), -1)).T).astype(int)
    slots = []
    for r, d in zip(products, dual.reshape(-1, KB, KB)):
        i, j = np.argwhere(d)[0]
        a, c = d[:, j] * d[i, j], d[i]
        assert np.array_equal(np.outer(a, c), d)
        slots.append(dict(r=max(r, ~r), tok=r >= 0, a=a.tolist(), c=c.tolist()))
    return slots


_PHASES = (_phase((11, 8, ~9, 4, 2, 23, 17, ~13, 25, 20, 22, 7, ~19, 16, 15, 1)),
           _phase((24, 21, ~16, 18, 19, 3, 10, ~22, 9, 5, 12, 13, ~25, 0, 14, 6)))
assert sorted(s["r"] for ph in _PHASES for s in ph if s["tok"]) == list(range(NR))

NH = 2 * KB
assert all(sorted(s["r"] // 2 for s in ph if s["r"] < NH) == list(range(KB)) for ph in _PHASES)
assert all(np.abs(s[k]).tolist() == np.eye(KB)[s["r"] // 2].tolist()
           for ph in _PHASES for s in ph if s["r"] < NH for k in "ac")
_TAIL_IN, _TAIL_OUT = (
    np.concatenate([np.rint(np.linalg.inv(t[2 * n:2 * n + 2, :, n]).T).astype(int)
                    for n in range(KB)]) for t in (_C, _U))


CHUNKS, S0, LAG, SPAN, HEAD, M0 = ((0, 1), (2, 3)), 72, 40, (11.25, 1), 72, 6
PO = (1, 0, 2)
MO = (364, 385, 410, 426, 444, 463)


Q = 2


XCUT = (0, 1, 3, 8)
RE, RO = 8, 48
ORD = (9, 8, 10, 19, 2, 3, 23, 24, 25, 17, 18, 20, 21, 22, 12, 11, 13, 4, 5, 15, 14, 16, 6, 7, 0, 1)
CUT = (1,)
QA = ((4, 10, 22, 27, 39, 42, 63, 83, 94, 150, 158, 161, 165, 166, 172), 24)
QB = ((11, 13, 22, 42, 58, 73, 90, 108, 146, 155, 161, 166, 171, 176, 179), 32)
QC = ((4, 5, 8, 14, 16, 21, 24, 28, 32, 35, 40, 44, 48, 53), 12)
RQ, RP = (1, 1), (1, 1)


def _signed_sum(terms):
    terms = [(c, t) for c, t in terms if c]
    first = next((i for i, (c, _) in enumerate(terms) if c > 0), 0)
    c, acc = terms.pop(first)
    acc = acc if c > 0 else -acc
    for c, t in terms:
        acc = acc + t if c > 0 else acc - t
    return acc


class _Mixer:
    def __init__(self, block):
        self.block, self.known = block, {}

    def __call__(self, coef):
        want = {(i, k): int(c) for i, row in enumerate(coef) for k, c in enumerate(row) if c}
        key = tuple(sorted(want.items()))
        if key not in self.known:
            terms = []
            for have in sorted(self.known, key=lambda h: -len(h)):
                for sign in (1, -1):
                    if all(want.get(pos) == sign * c for pos, c in have):
                        terms.append((sign, self.known[have]))
                        want = {pos: c for pos, c in want.items() if pos not in dict(have)}
                        break
            for pos, c in sorted(want.items()):
                self.known[((pos, 1),)] = self.block(*pos)
                terms.append((c, self.known[((pos, 1),)]))
            self.known[key] = _signed_sum(terms)
        return self.known[key]


class _Sums:
    def __init__(self, done):
        self.done, self.acc = done, {}

    def add(self, key, sign, value, expected):
        if not sign:
            return
        count, neg, tot = self.acc.pop(key, (0, sign < 0, value))
        if count and neg == (sign < 0):
            tot = tot + value
        elif count:
            tot, neg = (value - tot if neg else tot - value), False
        if count + 1 == expected:
            self.done(key, -tot if neg else tot)
        else:
            self.acc[key] = (count + 1, neg, tot)


class _Carry:
    def __init__(self, ref):
        self.ref, self.val = ref, {}

    def __getitem__(self, key):
        return self.val[key] if key in self.val else self.ref[key]

    def __setitem__(self, key, value):
        self.val[key] = value

    def flush(self):
        for key, value in self.val.items():
            self.ref[key] = value
        self.val = {}


def _dot(a, b):
    return lax.dot_general(a, b, (((1,), (0,)), ((), ())), preferred_element_type=F32)


def _dot_nt(a, b):
    return lax.dot_general(a, b, (((1,), (1,)), ((), ())), preferred_element_type=F32)


def _tile(ref, *idx):
    return pltpu.bitcast(ref.bitcast(U32)[idx], BF16)


def stack(*parts):
    parts = [t for t in parts if t is not None]
    return parts[0] if len(parts) == 1 else jnp.concatenate(parts, axis=0)


def _low_half(rows):
    return lax.broadcasted_iota(jnp.int32, (rows, LANES), 1) < 64


def _pair_lhs(t1, t2):
    lo = _low_half(t1[3].shape[0])
    diff = t1[3] - t2[3]
    return (t1[:3] + [jnp.where(lo, t1[4], diff)]
            + t2[:3] + [jnp.where(lo, -diff, t2[4])]
            + [jnp.where(lo, t1[3], t2[3])])


def _pair_rhs(x):
    a, b, c = x[384:448], x[448:512], x[512:576]
    cat = lambda u, v: jnp.concatenate([u, v], axis=0)
    return [x[i * 128:(i + 1) * 128] for i in range(3)] + [cat(c, b), cat(a, c), x[384:512]]


def _pair_matmul(lhs, rhs, dot):
    out = [dot(lhs(8), rhs[5])] * 2
    for i in range(8):
        out[i // 4] = out[i // 4] + dot(lhs(i), rhs[i % 4 if i < 7 else 4])
    return out


def _kernel(xt_hbm, wqkv_hbm, wo_hbm, mem0_hbm, wq_hbm, wk_hbm, wv_hbm, wot_hbm, gate_hbm,
            out_hbm,
            xt_v, wqkv_v, wo_v, stg_qkv, stg_o, wo_t, wt32, wo32_s, la, lo_a, kv_prev, oa_s,
            wb, x32, ga_s, gm_s, mem_s, part_s, o_s, opart_s, b_s, out_v, mem0_v, gate_v,
            sem_in, sem_out, *, seq, seg, mem):
    nt = seq // LANES
    rows = mem + seg

    sems = (sem_in.at[n] for n in itertools.count(3 * GP))
    copy = pltpu.make_async_copy
    cp_wqkv = {k: copy(wqkv_hbm.at[k * LANES:min(D, (k + 1) * LANES)],
                       wqkv_v.at[k * LANES:min(D, (k + 1) * LANES)], next(sems))
               for k in (3, 4, 0, 1, 2)}
    cp_wo = copy(wo_hbm, wo_v, next(sems))
    cp_x = {j0: [copy(xt_hbm.at[:, j * LANES:(j + 1) * LANES], xt_v.at[j], sem)
                 for j in range(j0, j1)] for j0, j1, sem in zip(XCUT, XCUT[1:] + (nt,), sems)}
    cp_wot = [copy(wot_hbm.at[h0:h1], stg_o.at[h0:h1], next(sems))
              for h0, h1 in ((0, HB - 2 * KB), (HB - 2 * KB, HB))]
    cp_small = [copy(mem0_hbm, mem0_v, next(sems)), copy(gate_hbm, gate_v, next(sems))]
    queue = cp_small + list(cp_wqkv.values()) + cp_x[0] + [cp_wo]
    for unit in range(3 * GP):
        src = (wq_hbm, wk_hbm, wv_hbm)[unit // GP].bitcast(U32)
        queue += cp_x.get(unit + 1, []) + [
            copy(src.at[:, KB * (unit % GP) + p, :], stg_qkv.at[unit, p], sem_in.at[unit])
            for p in range(KB)]
    for c in queue + cp_wot:
        c.start()

    def wait_all(copies):
        for c in copies:
            c.wait()

    def cp_out(j):
        col = j * LANES if isinstance(j, int) else pl.multiple_of(j * LANES, LANES)
        return copy(out_v.at[j], out_hbm.at[:, pl.ds(col, LANES)], sem_out)

    for ref in (o_s, opart_s, b_s):
        ref[...] = jnp.zeros(ref.shape, ref.dtype)
    wait_all(cp_small)
    m0 = mem0_v[...].astype(F32)
    for kk in range(KB):
        mem_s[kk] = m0[:, kk * LANES:(kk + 1) * LANES]
    mem_s[KB] = jnp.concatenate([m0[:, KB * LANES:], jnp.zeros((mem, 64), F32)], axis=1)
    wb[4 * GP, 0, 0:16, :] = jnp.zeros((16, LANES), BF16)

    gate = jnp.broadcast_to(gate_v[...].astype(F32).reshape(1, D), (8, D))
    gate_t = [gate[:, i * 128:(i + 1) * 128] for i in range(4)]
    gate_t.append(jnp.concatenate([gate[:, 512:], gate[:, 512:]], axis=1))

    entries = [None] * 2 + [(g - part // 2, part, n) for g in range(NG + 1) for n in range(DA // 2)
                            for part in (1, 0, 2) if 0 <= g - part // 2 < NG]

    def feature_rows(k, e):
        return stack(*(gate_t[k] if ent is None else
                       wt32[k, pl.ds(ent[1] * D + ent[0] * 8 * DA + 2 * ent[2] + e, 8, stride=DA), :]
                       for ent in entries))

    for k in cp_wqkv:
        cp_wqkv[k].wait()
        rows_k = wqkv_v[k * LANES:min(D, (k + 1) * LANES), :]
        wt32[k, 0:3 * D] = (rows_k if k < 4 else stack(rows_k, rows_k)).T.astype(F32)
        for e in range(2 if k < 3 else 0):
            la[4 * e + k] = feature_rows(k, e).astype(BF16)
        if k == 4:
            mixed = _pair_lhs(*([None] * 3 + [feature_rows(3, e), feature_rows(4, e)]
                                for e in range(2)))
            for i in (3, 7, 8):
                la[i] = mixed[i].astype(BF16)

    def prep_wo():
        wo32 = wo_v[...].astype(F32)
        for n in range(4):
            wo32_s[n, 0:D] = wo32[:, n * LANES:(n + 1) * LANES]
        wo32_s[4, 0:D] = jnp.concatenate([wo32[:, 4 * LANES:]] * 2, axis=1)
        turned = []
        for n in range(5):
            perm = stack(*(wo32_s[n, pl.ds(g * 8 * DA + d, 8, stride=DA), :]
                           for g in range(NG) for d in range(DA))).astype(BF16)
            turned.append([perm[k * LANES:(k + 1) * LANES].T for k in range(4)]
                          + [stack(perm[4 * LANES:], perm[4 * LANES:]).T])
        tiles = [stack(*(t[k] for t in turned))[:D].astype(F32) for k in range(5)]
        for i, t in enumerate(_pair_lhs([t[:D // 2] for t in tiles], [t[D // 2:] for t in tiles])):
            lo_a[i] = t.astype(BF16)

    by_size = ORD

    def prep_qkv(unit):
        src, dst = stg_qkv.at[unit], wb.at[unit]

        def rows(g, r0, nu):
            u = src[2 * g + nu // 2, r0:r0 + 16, :]
            return pltpu.bitcast(u & jnp.uint32(0xFFFF0000) if nu % 2 else u << 16, F32)

        for e in range(8):
            at, own, shared = pl.ds(16 * e, 16), e // 4, {}
            for g in (own, 1 - own):
                mix = _Mixer(lambda kk, nu: rows(g, kk * LANES + 16 * e, nu))
                for r in by_size:
                    w = mix(_V[r])
                    if r < NH and g == own:
                        shared[r] = w.astype(BF16)
                        dst[2 * NR + r, at, :] = shared[r]
                        w = rows(g, KB * LANES + 16 * (e % 4), r // 2)
                    elif r < NH:
                        w = w - shared[r].astype(F32)
                    dst[g * NR + r, at, :] = w.astype(BF16)
                    if r in CUT:
                        yield

    def turn_out(gp):
        words = lambda head, r0, n: _tile(stg_o, 2 * KB * gp + head, pl.ds(r0 // 2, n // 2))
        for head in range(2 * KB + 1):
            for nu in range(KB):
                if head < 2 * KB:
                    tile = words(head, nu * LANES, LANES)
                else:
                    tile = stack(*(words(g * KB + nu, KB * LANES, 64) for g in range(2)))
                wo_t[gp, head, nu] = pltpu.bitcast(tile.T, U32)

    def prep_out(gp):
        dst, lo = wb.at[3 * GP + gp], _low_half(16)
        for e in range(8):
            at, first = pl.ds(16 * e, 16), {}
            rows = lambda head, nu: pltpu.bitcast(
                wo_t[gp, head, nu, 8 * e:8 * e + 8, :], BF16).astype(F32)
            for g in range(2):
                mix = _Mixer(lambda kk, nu: rows(g * KB + kk, nu))
                for r in by_size:
                    w = mix(_V[r])
                    if r >= NH:
                        dst[g * NR + r, at, :] = w.astype(BF16)
                    elif g == 0:
                        first[r] = w
                    else:
                        z, t = jnp.where(lo, first[r], w).astype(BF16), rows(2 * KB, r // 2)
                        dst[2 * NR + r, at, :] = z
                        dst[r, at, :] = jnp.where(lo, t, first[r] - z.astype(F32)).astype(BF16)
                        dst[NR + r, at, :] = jnp.where(lo, w - z.astype(F32), t).astype(BF16)
                    if r in CUT:
                        yield

    lane = lax.broadcasted_iota(jnp.int32, (8, LANES), 1)

    def exchange(idx, pair, first):
        at = pl.ds(8 * idx, 8)
        prev = None if first else kv_prev.bitcast(U32)[at, :]
        kv_prev[16 * idx:16 * idx + 16, :] = jnp.concatenate(pair, axis=0).astype(BF16)
        cur = kv_prev.bitcast(U32)[at, :]
        return (jnp.broadcast_to(cur[:, 0:1], (8, LANES)) if first else prev), cur

    def to_rows(j):
        t0 = j * LANES if isinstance(j, int) else pl.multiple_of(j * LANES, LANES)
        xt = _tile(xt_v, j)
        for kk in range(KB + 1):
            tile = xt[kk * LANES:(kk + 1) * LANES]
            x32[kk, pl.ds(t0, LANES), :] = (tile if kk < KB else stack(tile, tile)).T.astype(F32)

    def paced(job, src, dst, when, back):
        results = []

        def dot(left, right):
            if len(results) in when:
                if src is not None and len(results) >= back:
                    src[...] = pltpu.bitcast(results[-back][0:8], U32)
                next(job, None)
                left = stack(left[:-8] if len(left) > 8 else None, left[-8:] | dst[...])
            results.append(_dot(pltpu.bitcast(left, BF16), right))
            return results[-1]

        return dot

    spare_qkv, spare_t = stg_qkv.at[3 * GP, 0, 0:8], wo_t.at[GP, 0, 1, 0:8]
    zero_w = wb.bitcast(U32).at[4 * GP, 0, 0:8]

    def a_out(j, dot):
        rhs = _pair_rhs(_tile(oa_s, slice(None)))
        for r0 in range(0, D // 2, RO):
            halves = _pair_matmul(lambda i: lo_a.bitcast(U32)[i, r0 // 2:(r0 + RO) // 2, :], rhs, dot)
            for e in range(2):
                ga_s[j, pl.ds(e * D // 2 + r0, RO), :] = halves[e]

    def a_tile(j, first, dot):
        rhs = _pair_rhs(_tile(xt_v, j))
        logit, prob, outs = {}, {}, {}
        for e0 in range(0, len(entries), RE):
            some = entries[e0:e0 + RE]
            halves = _pair_matmul(
                lambda i: la.bitcast(U32)[i, 4 * e0:4 * (e0 + len(some)), :], rhs, dot)
            for ent, r0 in zip(some, range(0, 8 * RE, 8)):
                pair = [t[r0:r0 + 8] for t in halves]
                if ent is None:
                    gsig = 1.0 / (1.0 + jnp.exp(-halves[0][0:8]))
                    continue
                g, part, n = ent
                if part:
                    prev, cur = exchange((2 * g + part - 1) * (DA // 2) + n, pair, first)
                    back = [cur] + [
                        pltpu.roll(jnp.where(lane >= LANES - DIL * w, prev, cur), DIL * w, 1)
                        for w in range(1, WIN)]
                    back = [pltpu.bitcast(t, BF16).astype(F32) for t in back]
                if part == 2:
                    outs[g, n] = functools.reduce(
                        jnp.add, [stack(p, p) * t for p, t in zip(prob[g], back)]).astype(BF16)
                elif part == 0:
                    terms = [pair[0] * t[0:8] + pair[1] * t[8:16] for t in back]
                    logit[g] = terms if n == 0 else [a + t for a, t in zip(logit[g], terms)]
                if (part, n) == (0, DA // 2 - 1):
                    s = [t * (DA ** -0.5) for t in logit[g]]
                    if first:
                        s = [jnp.where(lane >= DIL * w, t, NEG) for w, t in enumerate(s)]
                    top = functools.reduce(jnp.maximum, s)
                    ex = [jnp.exp(t - top) for t in s]
                    inv = gsig / functools.reduce(jnp.add, ex)
                    prob[g] = [t * inv for t in ex]
        gm_s[j] = 1.0 - gsig
        if not first:
            a_out(j - 1, dot)
        oa_s[...] = stack(*(outs[key] for key in sorted(outs)))

    plain = lambda left, right: _dot(pltpu.bitcast(left, BF16), right)
    wait_all(cp_x[0])
    to_rows(0)
    a_tile(0, True, plain)
    cp_wo.wait()
    prep_wo()

    def a_loop(first, count, work, spare, loading):
        def body(j, carry):
            if loading:
                for j0 in XCUT[1:]:
                    pl.when(j == j0)(functools.partial(wait_all, cp_x[j0]))
                copy(stg_qkv.at[j - first], stg_qkv.at[j - first], sem_in.at[j - first]).wait()
                to_rows(j)
            job = work(j - first)
            a_tile(j, False, paced(job, spare, zero_w, *(QA if loading else QB)))
            list(job)
            return carry

        lax.fori_loop(first, first + count, body, 0)

    a_loop(1, 3 * GP, prep_qkv, spare_qkv, True)

    qi = lax.broadcasted_iota(jnp.int32, (rows, rows), 0)
    ki = lax.broadcasted_iota(jnp.int32, (rows, rows), 1)
    mask = (qi >= seg) | (ki >= seg) | (qi >= ki)
    part, o_prev, opart, b_rows = (_Carry(r) for r in (part_s, o_s, opart_s, b_s))
    ahead = {}

    def b_step(u, t0, memv, project_only=False, output_only=False):
        odd = u % 2
        keep = lambda slots: [s for s in slots if s["tok"] or memv]
        qs, os_ = keep(_PHASES[odd][::RQ[odd]]), keep(_PHASES[1 - odd][::RP[1 - odd]])
        lhs, shared, tok, mrow, full, soft, o_mem, o_mix, o_left, o_host, new = ({} for _ in range(11))

        def spread(sums, key, slots, s, tok_rows, mem_rows):
            for nu in range(KB):
                if memv:
                    sums.add(key + (nu, 2), s["c"][nu], mem_rows, sum(abs(o["c"][nu]) for o in slots))
                for mu in range(2 if s["tok"] else 0):
                    sums.add(key + (nu, mu), _C[s["r"]][mu][nu], tok_rows,
                             sum(abs(_C[o["r"]][mu][nu]) for o in slots if o["tok"]))

        x_mix = _Mixer(lambda mu, kk: x32[kk, pl.ds(t0 + mu * seg, seg), :])
        c_mix = _Mixer(lambda mu, _: x32[KB, pl.ds(t0 + mu * seg, seg), :])
        m_mix = _Mixer(lambda _, kk: memv[kk])
        m_tail = memv[KB] + pltpu.roll(memv[KB], 64, 1) if memv else None

        def q_left(e, t):
            s = qs[e]
            if (e, t) not in lhs:
                left = stack(x_mix(_U[s["r"]]) if s["tok"] else None,
                             m_mix([s["a"]]) if memv else None)
                if s["r"] < NH and t < 2:
                    c = stack(c_mix(_TAIL_IN[s["r"]][:, None]),
                              _signed_sum([(sum(s["c"]), m_tail)]) if memv else None)
                    left = jnp.where(_low_half(c.shape[0]), *((c, left), (left, c))[t])
                lhs[e, t] = left
            return lhs[e, t]

        def q_total(key, value):
            i, g, nu, mu = key
            h = g * KB + nu
            if mu == 2:
                mrow[i, h] = value
            elif odd:
                part[i, h, mu] = value
            elif mu == 0:
                tok[i, h] = value + part[i, h, mu]
            else:
                ahead[i, h] = value + part[i, h, mu]
            cur = (ahead if odd else tok).get((i, h))
            if (i, h) in mrow and cur is not None and (i, h) not in full:
                full[i, h] = stack(cur, mrow[i, h]).astype(BF16 if i else F32)

        q_sums = _Sums(q_total)

        def q_pass(e, i, gp, t):
            s = qs[e]
            p = _dot(q_left(e, t), _tile(wb, i * GP + gp, t * NR + s["r"]))
            if t == 2:
                shared[e, i, gp] = p
                return
            if s["r"] < NH:
                p = p + shared[e, i, gp]
            spread(q_sums, (i, 2 * gp + t), qs, s, p[:seg], p[-mem:])

        def scores(h):
            s = jnp.where(mask, _dot_nt(full[0, h], full[1, h]), NEG * DB ** 0.5)
            e = jnp.exp2((s - jnp.max(s, axis=-1, keepdims=True)) * (DB ** -0.5 * LOG2E))
            total = jnp.sum(e, axis=-1, keepdims=True)
            inv = pltpu.reciprocal(total, approx=True)
            soft[h] = e * (inv * (2.0 - total * inv))

        def values(h):
            o = _dot(soft[h], full[2, h])
            o_mem[h] = o[seg:]
            if odd:
                o_prev[0, h], o_prev[1, h] = ahead["o", h], o[:seg]
            else:
                ahead["o", h] = o[:seg]

        def o_rows(e, gp, t):
            s = os_[e]
            if (e, gp, t) not in o_left:
                g = 2 * gp + t
                if t == 2:
                    o_left[e, gp, t] = o_rows(e, gp, 0) + o_rows(e, gp, 1)
                    return o_left[e, gp, t]
                if g not in o_mix:
                    o_mix[g] = (_Mixer(lambda _, kk: o_mem[g * KB + kk]),
                                _Mixer(lambda mu, kk: o_prev[mu, g * KB + kk]))
                o_left[e, gp, t] = stack(o_mix[g][0]([s["a"]]) if memv else None,
                                         o_mix[g][1](_U[s["r"]]) if s["tok"] else None)
            return o_left[e, gp, t]

        def o_total(key, value):
            nu, mu = key
            if mu == 2:
                new[nu] = value
            elif odd:
                opart[nu, mu] = value
            else:
                b_rows[nu, (u - 2) % 4 + mu] = value + opart[nu, mu]

        out_sums = _Sums(o_total)

        def o_product(key, value):
            e, t = key
            s = os_[e]
            if s["r"] < NH:
                o_host[key] = value
                if any((e, t_) not in o_host for t_ in range(3)):
                    return
                lo = _low_half(value.shape[0])
                value = o_host[e, 2] + jnp.where(lo, o_host[e, 1], o_host[e, 0])
                y = jnp.where(lo, o_host[e, 0], o_host[e, 1])
                if memv:
                    out_sums.add((KB, 2), sum(s["a"]), y[:mem], KB)
                for mu in range(2):
                    out_sums.add((KB, mu), _TAIL_OUT[s["r"]][mu], y[-seg:],
                                 sum(abs(_TAIL_OUT[o["r"]][mu]) for o in os_ if o["r"] < NH))
            spread(out_sums, (), os_, s, value[-seg:], value[:mem])

        o_sums = _Sums(o_product)

        def o_pass(e, gp, t):
            host = os_[e]["r"] < NH
            p = _dot(o_rows(e, gp, t), _tile(wb, 3 * GP + gp, t * NR + os_[e]["r"]))
            o_sums.add((e, t if host else 0), 1, p, GP if host else 2 * GP)

        todo = []
        tiles = lambda s: (2, 0, 1) if s["r"] < NH else (0, 1)
        if not output_only:
            todo = [(s["tok"], q_pass, e, i, gp, t) for gp in range(GP) for i in PO
                    for e, s in enumerate(qs) for t in tiles(s)]
            last = [max(e for e, s in enumerate(_PHASES[odd][::RP[odd]]) if s["tok"] and s["c"][nu])
                    for nu in range(KB)]
            ready = lambda e, t: 99 if qs[e]["r"] < NH and t < 2 else max(
                last[kk] for kk in range(KB) if qs[e]["a"][kk])
            todo[:HEAD] = sorted(todo[:HEAD], key=lambda p: ready(p[2], p[5]))
        if not project_only:
            todo += [(s["tok"], o_pass, e, gp, t) for pairs in CHUNKS for e, s in enumerate(os_)
                     for gp in pairs for t in tiles(s)]
        long_, short = ([p[1:] for p in todo if p[0] == tok] for tok in (True, False))
        extra = {}
        for h in range(HB if memv else 0):
            gp, n = divmod(h, 2 * KB)
            at = (90 * gp + S0 + int(SPAN[gp == GP - 1] * (n // Q * Q))) // Q * Q
            extra.setdefault(at, []).append((scores, h))
            extra.setdefault(at + LAG, []).append((values, h))
        issued = 0
        for n, p in enumerate(long_):
            for fn, *args in extra.get(n, []) + [p]:
                if issued % 4 == 0 and short and n >= (480 + M0 - 5 * len(short) if len(short) > 24 else MO[6 - len(short) // 4]):
                    for fn_s, *args_s in short[:4]:
                        fn_s(*args_s)
                    del short[:4]
                fn(*args)
                issued += 1
        assert not short
        return new

    def emit_tile(j):
        for nu in range(KB + 1):
            bt = jnp.concatenate([b_s[nu, 0], b_s[nu, 1], b_rows.val.pop((nu, 2)),
                                  b_rows.val.pop((nu, 3))], axis=0).T
            bt = bt if nu < KB else bt[:64] + bt[64:]
            at = pl.ds(nu * LANES, bt.shape[0])
            gm = jnp.concatenate([gm_s[j]] * (bt.shape[0] // 8), axis=0)
            out_v[j, at, :] = (ga_s[j, at, :] + gm * bt).astype(out_v.dtype)

    cp_wot[0].wait()
    for gp in range(GP - 1):
        turn_out(gp)
    b_step(3, 0, None, project_only=True)
    part.flush()
    for j in range(3 * GP + 1, nt):
        to_rows(j)
    cp_wot[1].wait()
    turn_out(GP - 1)
    a_loop(3 * GP + 1, GP - 1, prep_out, spare_t, False)
    job = prep_out(GP - 1)
    a_out(nt - 1, paced(job, spare_t, zero_w, *QC))
    list(job)

    def b_body(j, carry):
        memv = {kk: mem_s[kk] for kk in range(KB + 1)}
        for u in range(4):
            t0 = jnp.minimum(j * LANES + (u + 1) // 2 * 2 * seg, seq - 2 * seg)
            memv = b_step(u, pl.multiple_of(t0, seg), memv)
            if u == 0:
                emit_tile(jnp.maximum(j - 1, 0))
        for kk, t in memv.items():
            mem_s[kk] = t
        for c in (part, o_prev, opart, b_rows):
            c.flush()
        pl.when(j > 0)(lambda: cp_out(j - 1).start())
        return carry

    lax.fori_loop(0, nt, b_body, 0)
    b_step(0, None, None, output_only=True)
    emit_tile(nt - 1)
    cp_out(nt - 1).start()
    for j in range(nt):
        cp_out(j).wait()


@functools.partial(jax.jit, static_argnames=("B_seg_len",))
def pallas_gated_mix__sliding_local_dilated__memory_aug_recurrent_mem_tr__prompt_kernel(
    A_x: jax.Array,
    A_wqkv: jax.Array,
    A_wo: jax.Array,
    B_x: jax.Array,
    B_mem0: jax.Array,
    B_Wq: jax.Array,
    B_Wk: jax.Array,
    B_Wv: jax.Array,
    B_Wo: jax.Array,
    B_seg_len: int,
    gate_w: jax.Array,
):
    del B_x
    batch, seq, width = A_x.shape
    mem, seg = B_mem0.shape[1], int(B_seg_len)
    nt = seq // LANES
    assert batch == 1 and width == D and nt == 4 * GP and seq % LANES == 0
    assert B_Wq.shape == (D, HB, DB) and mem == 8 and 4 * seg == LANES

    hbm = pl.BlockSpec(memory_space=pl.ANY)
    out_t = pl.pallas_call(
        functools.partial(_kernel, seq=seq, seg=seg, mem=mem),
        out_shape=jax.ShapeDtypeStruct((D, seq), A_x.dtype),
        in_specs=[hbm] * 9,
        out_specs=hbm,
        scratch_shapes=[
            pltpu.VMEM((nt, D, LANES), BF16),
            pltpu.VMEM((D, 3 * D), BF16),
            pltpu.VMEM((D, D), BF16),
            pltpu.VMEM((3 * GP + 1, KB, D, DB), U32),
            pltpu.VMEM((HB, D, DB), BF16),
            pltpu.VMEM((GP + 1, 2 * KB + 1, KB, 64, LANES), U32),
            pltpu.VMEM((5, 3 * D + 32, LANES), F32),
            pltpu.VMEM((5, D + 32, LANES), F32),
            pltpu.VMEM((12, 3 * D // 2 + 16, LANES), BF16),
            pltpu.VMEM((12, D // 2, LANES), BF16),
            pltpu.VMEM((2 * D, LANES), BF16),
            pltpu.VMEM((D, LANES), BF16),
            pltpu.VMEM((4 * GP + 1, 2 * NR + NH, LANES, LANES), BF16),
            pltpu.VMEM((KB + 1, seq, LANES), F32),
            pltpu.VMEM((nt, D, LANES), F32),
            pltpu.VMEM((nt, 8, LANES), F32),
            pltpu.VMEM((2 * KB, mem, LANES), F32),
            pltpu.VMEM((3, HB, 2, seg, LANES), F32),
            pltpu.VMEM((2, HB, seg, LANES), F32),
            pltpu.VMEM((KB + 1, 2, seg, LANES), F32),
            pltpu.VMEM((KB + 1, 2, seg, LANES), F32),
            pltpu.VMEM((nt, D, LANES), A_x.dtype),
            pltpu.VMEM((mem, D), BF16),
            pltpu.VMEM((D,), BF16),
            pltpu.SemaphoreType.DMA((3 * GP + 10 + len(XCUT),)),
            pltpu.SemaphoreType.DMA(()),
        ],
        compiler_params=pltpu.CompilerParams(vmem_limit_bytes=110 * 1024 * 1024),
        name="gated_mix_kernel",
    )(A_x.reshape(seq, D).T, A_wqkv, A_wo, B_mem0.reshape(mem, D), B_Wq, B_Wk, B_Wv,
      B_Wo.transpose(0, 2, 1), gate_w)
    return out_t.T.reshape(batch, seq, D)
```

```python
import functools
import itertools

import jax
import jax.numpy as jnp
import numpy as np
from jax import lax
import jax.experimental.pallas as pl
import jax.experimental.pallas.tpu as pltpu

F32, BF16, U32 = jnp.float32, jnp.bfloat16, jnp.uint32

D = 576
LANES = 128
HA, DA = 32, 18
WIN, DIL = 8, 2
HB, DB = 32, 128
NEG = -1000000000.0
LOG2E = 1.4426950408889634
NG = HA // 8

KB = 4
GP = HB // (2 * KB)

_HK = (
    (".... +...", "+.-. -... .... -...", "+... +..."),
    ("+... -...", "+-.- .... -... ....", "+... ...."),
    (".+.. .-..", ".... +-.. .+.. ....", ".... .+.."),
    (".+.. ....", ".-.. .+-. .... ....", ".+.. .+.."),
    (".... ..+.", ".... ..-. -.+. .+-.", ".... ..+."),
    ("..+. ....", "..-. ...+ .-+- ....", "..+. ...."),
    ("...+ ...-", ".... ...- ...+ ++.-", ".... ...+"),
    ("...+ ....", "...- ...- .... .+-+", "...+ ...+"),
    (".... ++..", ".... +... .... ....", ".... ++.."),
    ("++.. ....", ".+.. .... .... ....", "++.. ...."),
    (".+.. +...", ".-.. +... .... ....", "+... .-.."),
    ("+.+. -.-.", ".... .... -... ....", ".... +.+."),
    ("+.+. ....", "..+. .... .... ....", "+.+. +.+."),
    ("+.+. -...", "..-. .... +... ....", "+... +.+."),
    (".... +..+", ".... .... .... +...", ".... +..+"),
    ("+..+ ....", "...+ .... .... ....", "+..+ ...."),
    ("...+ +...", "...- .... .... +...", "+... ...-"),
    (".... .++.", ".... ..+. .... .-..", ".++. .++."),
    (".++. .--.", ".... ...- .+.. ....", ".++. ...."),
    (".+.. .--.", ".... ..+. .-.. ....", ".++. .+.."),
    (".... ..++", ".... .... .... .-+.", "..++ ..++"),
    ("..++ ..--", ".... ...- ...+ ....", "..++ ...."),
    ("...+ ..--", ".... ...+ ...- .-+.", "..++ ...+"),
    (".... .+++", ".... .... .... .+..", ".... .+++"),
    (".+++ ....", ".... ...+ .... ....", ".+++ ...."),
    ("...+ .++.", ".... ...- .... .+..", ".++. ...-"),
)
_U, _V, _C = (np.array([[["-.+".index(ch) - 1 for ch in row] for row in prod[i].split()]
                        for prod in _HK]) for i in range(3))
NR = len(_HK)
assert np.array_equal(np.einsum("rak,rln,rbm->akblnm", _U, _V, _C),
                      np.einsum("ab,kl,nm->akblnm", *(np.eye(n, dtype=int) for n in (2, KB, KB))))


def _phase(products):
    tiles = [max(r, ~r) for r in products]
    dual = np.rint(np.linalg.inv(_V[tiles].reshape(len(tiles), -1)).T).astype(int)
    slots = []
    for r, d in zip(products, dual.reshape(-1, KB, KB)):
        i, j = np.argwhere(d)[0]
        a, c = d[:, j] * d[i, j], d[i]
        assert np.array_equal(np.outer(a, c), d)
        slots.append(dict(r=max(r, ~r), tok=r >= 0, a=a.tolist(), c=c.tolist()))
    return slots


_PHASES = (_phase((11, 8, ~9, 4, 2, 23, 17, ~13, 25, 20, 22, 7, ~19, 16, 15, 1)),
           _phase((24, 21, ~16, 18, 19, 3, 10, ~22, 9, 5, 12, 13, ~25, 0, 14, 6)))
assert sorted(s["r"] for ph in _PHASES for s in ph if s["tok"]) == list(range(NR))

NH = 2 * KB
assert all(sorted(s["r"] // 2 for s in ph if s["r"] < NH) == list(range(KB)) for ph in _PHASES)
assert all(np.abs(s[k]).tolist() == np.eye(KB)[s["r"] // 2].tolist()
           for ph in _PHASES for s in ph if s["r"] < NH for k in "ac")
_TAIL_IN, _TAIL_OUT = (
    np.concatenate([np.rint(np.linalg.inv(t[2 * n:2 * n + 2, :, n]).T).astype(int)
                    for n in range(KB)]) for t in (_C, _U))


CHUNKS, S0, LAG, SPAN, HEAD, M0 = ((0, 1), (2, 3)), 72, 40, (11.25, 1), 72, 6
PO = (1, 0, 2)
MO = (364, 385, 410, 426, 444, 463)


Q = 2


XCUT = (0, 1, 3, 8)
RE, RO = 8, 48
ORD = (9, 8, 10, 19, 2, 3, 23, 24, 25, 17, 18, 20, 21, 22, 12, 11, 13, 4, 5, 15, 14, 16, 6, 7, 0, 1)
CUT = (1,)
QA = ((4, 10, 22, 27, 39, 42, 63, 83, 94, 150, 158, 161, 165, 166, 172), 24)
QB = ((11, 13, 22, 42, 58, 73, 90, 108, 146, 155, 161, 166, 171, 176, 179), 32)
QC = ((4, 5, 8, 14, 16, 21, 24, 28, 32, 35, 40, 44, 48, 53), 12)
RQ, RP = (1, 1), (1, 1)


def _signed_sum(terms):
    terms = [(c, t) for c, t in terms if c]
    first = next((i for i, (c, _) in enumerate(terms) if c > 0), 0)
    c, acc = terms.pop(first)
    acc = acc if c > 0 else -acc
    for c, t in terms:
        acc = acc + t if c > 0 else acc - t
    return acc


class _Mixer:
    def __init__(self, block):
        self.block, self.known = block, {}

    def __call__(self, coef):
        want = {(i, k): int(c) for i, row in enumerate(coef) for k, c in enumerate(row) if c}
        key = tuple(sorted(want.items()))
        if key not in self.known:
            terms = []
            for have in sorted(self.known, key=lambda h: -len(h)):
                for sign in (1, -1):
                    if all(want.get(pos) == sign * c for pos, c in have):
                        terms.append((sign, self.known[have]))
                        want = {pos: c for pos, c in want.items() if pos not in dict(have)}
                        break
            for pos, c in sorted(want.items()):
                self.known[((pos, 1),)] = self.block(*pos)
                terms.append((c, self.known[((pos, 1),)]))
            self.known[key] = _signed_sum(terms)
        return self.known[key]


class _Sums:
    def __init__(self, done):
        self.done, self.acc = done, {}

    def add(self, key, sign, value, expected):
        if not sign:
            return
        count, neg, tot = self.acc.pop(key, (0, sign < 0, value))
        if count and neg == (sign < 0):
            tot = tot + value
        elif count:
            tot, neg = (value - tot if neg else tot - value), False
        if count + 1 == expected:
            self.done(key, -tot if neg else tot)
        else:
            self.acc[key] = (count + 1, neg, tot)


class _Carry:
    def __init__(self, ref):
        self.ref, self.val = ref, {}

    def __getitem__(self, key):
        return self.val[key] if key in self.val else self.ref[key]

    def __setitem__(self, key, value):
        self.val[key] = value

    def flush(self):
        for key, value in self.val.items():
            self.ref[key] = value
        self.val = {}


def _dot(a, b):
    return lax.dot_general(a, b, (((1,), (0,)), ((), ())), preferred_element_type=F32)


def _dot_nt(a, b):
    return lax.dot_general(a, b, (((1,), (1,)), ((), ())), preferred_element_type=F32)


def _tile(ref, *idx):
    return pltpu.bitcast(ref.bitcast(U32)[idx], BF16)


def stack(*parts):
    parts = [t for t in parts if t is not None]
    return parts[0] if len(parts) == 1 else jnp.concatenate(parts, axis=0)


def _low_half(rows):
    return lax.broadcasted_iota(jnp.int32, (rows, LANES), 1) < 64


def _pair_lhs(t1, t2):
    lo = _low_half(t1[3].shape[0])
    diff = t1[3] - t2[3]
    return (t1[:3] + [jnp.where(lo, t1[4], diff)]
            + t2[:3] + [jnp.where(lo, -diff, t2[4])]
            + [jnp.where(lo, t1[3], t2[3])])


def _pair_rhs(x):
    a, b, c = x[384:448], x[448:512], x[512:576]
    cat = lambda u, v: jnp.concatenate([u, v], axis=0)
    return [x[i * 128:(i + 1) * 128] for i in range(3)] + [cat(c, b), cat(a, c), x[384:512]]


def _pair_matmul(lhs, rhs, dot):
    out = [dot(lhs(8), rhs[5])] * 2
    for i in range(8):
        out[i // 4] = out[i // 4] + dot(lhs(i), rhs[i % 4 if i < 7 else 4])
    return out


def _kernel(xt_hbm, wqkv_hbm, wo_hbm, mem0_hbm, wq_hbm, wk_hbm, wv_hbm, wot_hbm, gate_hbm,
            out_hbm,
            xt_v, wqkv_v, wo_v, stg_qkv, stg_o, wo_t, wt32, wo32_s, la, lo_a, kv_prev, oa_s,
            wb, x32, ga_s, gm_s, mem_s, part_s, o_s, opart_s, b_s, out_v, mem0_v, gate_v,
            sem_in, sem_out, *, seq, seg, mem):
    nt = seq // LANES
    rows = mem + seg

    sems = (sem_in.at[n] for n in itertools.count(3 * GP))
    copy = pltpu.make_async_copy
    cp_wqkv = {k: copy(wqkv_hbm.at[k * LANES:min(D, (k + 1) * LANES)],
                       wqkv_v.at[k * LANES:min(D, (k + 1) * LANES)], next(sems))
               for k in (3, 4, 0, 1, 2)}
    cp_wo = copy(wo_hbm, wo_v, next(sems))
    cp_x = {j0: [copy(xt_hbm.at[:, j * LANES:(j + 1) * LANES], xt_v.at[j], sem)
                 for j in range(j0, j1)] for j0, j1, sem in zip(XCUT, XCUT[1:] + (nt,), sems)}
    cp_wot = copy(wot_hbm, stg_o, next(sems))
    cp_small = [copy(mem0_hbm, mem0_v, next(sems)), copy(gate_hbm, gate_v, next(sems))]
    queue = cp_small + list(cp_wqkv.values()) + cp_x[0] + [cp_wo]
    for unit in range(3 * GP):
        src = (wq_hbm, wk_hbm, wv_hbm)[unit // GP].bitcast(U32)
        queue += cp_x.get(unit + 1, []) + [
            copy(src.at[:, KB * (unit % GP) + p, :], stg_qkv.at[unit, p], sem_in.at[unit])
            for p in range(KB)]
    for c in queue + [cp_wot]:
        c.start()

    def wait_all(copies):
        for c in copies:
            c.wait()

    def cp_out(j):
        col = j * LANES if isinstance(j, int) else pl.multiple_of(j * LANES, LANES)
        return copy(out_v.at[j], out_hbm.at[:, pl.ds(col, LANES)], sem_out)

    for ref in (o_s, opart_s, b_s):
        ref[...] = jnp.zeros(ref.shape, ref.dtype)
    wait_all(cp_small)
    m0 = mem0_v[...].astype(F32)
    for kk in range(KB):
        mem_s[kk] = m0[:, kk * LANES:(kk + 1) * LANES]
    mem_s[KB] = jnp.concatenate([m0[:, KB * LANES:], jnp.zeros((mem, 64), F32)], axis=1)
    wb[4 * GP, 0, 0:16, :] = jnp.zeros((16, LANES), BF16)

    gate = jnp.broadcast_to(gate_v[...].astype(F32).reshape(1, D), (8, D))
    gate_t = [gate[:, i * 128:(i + 1) * 128] for i in range(4)]
    gate_t.append(jnp.concatenate([gate[:, 512:], gate[:, 512:]], axis=1))

    entries = [None] * 2 + [(g - part // 2, part, n) for g in range(NG + 1) for n in range(DA // 2)
                            for part in (1, 0, 2) if 0 <= g - part // 2 < NG]

    def feature_rows(k, e):
        return stack(*(gate_t[k] if ent is None else
                       wt32[k, pl.ds(ent[1] * D + ent[0] * 8 * DA + 2 * ent[2] + e, 8, stride=DA), :]
                       for ent in entries))

    for k in cp_wqkv:
        cp_wqkv[k].wait()
        rows_k = wqkv_v[k * LANES:min(D, (k + 1) * LANES), :]
        wt32[k, 0:3 * D] = (rows_k if k < 4 else stack(rows_k, rows_k)).T.astype(F32)
        for e in range(2 if k < 3 else 0):
            la[4 * e + k] = feature_rows(k, e).astype(BF16)
        if k == 4:
            mixed = _pair_lhs(*([None] * 3 + [feature_rows(3, e), feature_rows(4, e)]
                                for e in range(2)))
            for i in (3, 7, 8):
                la[i] = mixed[i].astype(BF16)

    def prep_wo():
        wo32 = wo_v[...].astype(F32)
        for n in range(4):
            wo32_s[n, 0:D] = wo32[:, n * LANES:(n + 1) * LANES]
        wo32_s[4, 0:D] = jnp.concatenate([wo32[:, 4 * LANES:]] * 2, axis=1)
        turned = []
        for n in range(5):
            perm = stack(*(wo32_s[n, pl.ds(g * 8 * DA + d, 8, stride=DA), :]
                           for g in range(NG) for d in range(DA))).astype(BF16)
            turned.append([perm[k * LANES:(k + 1) * LANES].T for k in range(4)]
                          + [stack(perm[4 * LANES:], perm[4 * LANES:]).T])
        tiles = [stack(*(t[k] for t in turned))[:D].astype(F32) for k in range(5)]
        for i, t in enumerate(_pair_lhs([t[:D // 2] for t in tiles], [t[D // 2:] for t in tiles])):
            lo_a[i] = t.astype(BF16)

    by_size = ORD

    def prep_qkv(unit):
        src, dst = stg_qkv.at[unit], wb.at[unit]

        def rows(g, r0, nu):
            u = src[2 * g + nu // 2, r0:r0 + 16, :]
            return pltpu.bitcast(u & jnp.uint32(0xFFFF0000) if nu % 2 else u << 16, F32)

        for e in range(8):
            at, own, shared = pl.ds(16 * e, 16), e // 4, {}
            for g in (own, 1 - own):
                mix = _Mixer(lambda kk, nu: rows(g, kk * LANES + 16 * e, nu))
                for r in by_size:
                    w = mix(_V[r])
                    if r < NH and g == own:
                        shared[r] = w.astype(BF16)
                        dst[2 * NR + r, at, :] = shared[r]
                        w = rows(g, KB * LANES + 16 * (e % 4), r // 2)
                    elif r < NH:
                        w = w - shared[r].astype(F32)
                    dst[g * NR + r, at, :] = w.astype(BF16)
                    if r in CUT:
                        yield

    def turn_out(gp):
        words = lambda head, r0, n: _tile(stg_o, 2 * KB * gp + head, pl.ds(r0 // 2, n // 2))
        for head in range(2 * KB + 1):
            for nu in range(KB):
                if head < 2 * KB:
                    tile = words(head, nu * LANES, LANES)
                else:
                    tile = stack(*(words(g * KB + nu, KB * LANES, 64) for g in range(2)))
                wo_t[gp, head, nu] = pltpu.bitcast(tile.T, U32)

    def prep_out(gp):
        dst, lo = wb.at[3 * GP + gp], _low_half(16)
        for e in range(8):
            at, first = pl.ds(16 * e, 16), {}
            rows = lambda head, nu: pltpu.bitcast(
                wo_t[gp, head, nu, 8 * e:8 * e + 8, :], BF16).astype(F32)
            for g in range(2):
                mix = _Mixer(lambda kk, nu: rows(g * KB + kk, nu))
                for r in by_size:
                    w = mix(_V[r])
                    if r >= NH:
                        dst[g * NR + r, at, :] = w.astype(BF16)
                    elif g == 0:
                        first[r] = w
                    else:
                        z, t = jnp.where(lo, first[r], w).astype(BF16), rows(2 * KB, r // 2)
                        dst[2 * NR + r, at, :] = z
                        dst[r, at, :] = jnp.where(lo, t, first[r] - z.astype(F32)).astype(BF16)
                        dst[NR + r, at, :] = jnp.where(lo, w - z.astype(F32), t).astype(BF16)
                    if r in CUT:
                        yield

    lane = lax.broadcasted_iota(jnp.int32, (8, LANES), 1)

    def exchange(idx, pair, first):
        at = pl.ds(8 * idx, 8)
        prev = None if first else kv_prev.bitcast(U32)[at, :]
        kv_prev[16 * idx:16 * idx + 16, :] = jnp.concatenate(pair, axis=0).astype(BF16)
        cur = kv_prev.bitcast(U32)[at, :]
        return (jnp.broadcast_to(cur[:, 0:1], (8, LANES)) if first else prev), cur

    def to_rows(j):
        t0 = j * LANES if isinstance(j, int) else pl.multiple_of(j * LANES, LANES)
        xt = _tile(xt_v, j)
        for kk in range(KB + 1):
            tile = xt[kk * LANES:(kk + 1) * LANES]
            x32[kk, pl.ds(t0, LANES), :] = (tile if kk < KB else stack(tile, tile)).T.astype(F32)

    def paced(job, src, dst, when, back):
        results = []

        def dot(left, right):
            if len(results) in when:
                if src is not None and len(results) >= back:
                    src[...] = pltpu.bitcast(results[-back][0:8], U32)
                next(job, None)
                left = stack(left[:-8] if len(left) > 8 else None, left[-8:] | dst[...])
            results.append(_dot(pltpu.bitcast(left, BF16), right))
            return results[-1]

        return dot

    spare_qkv, spare_t = stg_qkv.at[3 * GP, 0, 0:8], wo_t.at[GP, 0, 1, 0:8]
    zero_w = wb.bitcast(U32).at[4 * GP, 0, 0:8]

    def a_out(j, dot):
        rhs = _pair_rhs(_tile(oa_s, slice(None)))
        for r0 in range(0, D // 2, RO):
            halves = _pair_matmul(lambda i: lo_a.bitcast(U32)[i, r0 // 2:(r0 + RO) // 2, :], rhs, dot)
            for e in range(2):
                ga_s[j, pl.ds(e * D // 2 + r0, RO), :] = halves[e]

    def a_tile(j, first, dot):
        rhs = _pair_rhs(_tile(xt_v, j))
        logit, prob, outs = {}, {}, {}
        for e0 in range(0, len(entries), RE):
            some = entries[e0:e0 + RE]
            halves = _pair_matmul(
                lambda i: la.bitcast(U32)[i, 4 * e0:4 * (e0 + len(some)), :], rhs, dot)
            for ent, r0 in zip(some, range(0, 8 * RE, 8)):
                pair = [t[r0:r0 + 8] for t in halves]
                if ent is None:
                    gsig = 1.0 / (1.0 + jnp.exp(-halves[0][0:8]))
                    continue
                g, part, n = ent
                if part:
                    prev, cur = exchange((2 * g + part - 1) * (DA // 2) + n, pair, first)
                    back = [cur] + [
                        pltpu.roll(jnp.where(lane >= LANES - DIL * w, prev, cur), DIL * w, 1)
                        for w in range(1, WIN)]
                    back = [pltpu.bitcast(t, BF16).astype(F32) for t in back]
                if part == 2:
                    outs[g, n] = functools.reduce(
                        jnp.add, [stack(p, p) * t for p, t in zip(prob[g], back)]).astype(BF16)
                elif part == 0:
                    terms = [pair[0] * t[0:8] + pair[1] * t[8:16] for t in back]
                    logit[g] = terms if n == 0 else [a + t for a, t in zip(logit[g], terms)]
                if (part, n) == (0, DA // 2 - 1):
                    s = [t * (DA ** -0.5) for t in logit[g]]
                    if first:
                        s = [jnp.where(lane >= DIL * w, t, NEG) for w, t in enumerate(s)]
                    top = functools.reduce(jnp.maximum, s)
                    ex = [jnp.exp(t - top) for t in s]
                    inv = gsig / functools.reduce(jnp.add, ex)
                    prob[g] = [t * inv for t in ex]
        gm_s[j] = 1.0 - gsig
        if not first:
            a_out(j - 1, dot)
        oa_s[...] = stack(*(outs[key] for key in sorted(outs)))

    plain = lambda left, right: _dot(pltpu.bitcast(left, BF16), right)
    wait_all(cp_x[0])
    to_rows(0)
    a_tile(0, True, plain)
    cp_wo.wait()
    wait_all(cp_x[1])
    prep_wo()
    a_tile(1, False, plain)
    to_rows(1)

    def a_loop(first, count, work, spare, loading):
        def body(j, carry):
            if loading:
                for j0 in XCUT[2:]:
                    pl.when(j == j0)(functools.partial(wait_all, cp_x[j0]))
                copy(stg_qkv.at[j - first], stg_qkv.at[j - first], sem_in.at[j - first]).wait()
                to_rows(j)
            job = work(j - first)
            a_tile(j, False, paced(job, spare, zero_w, *(QA if loading else QB)))
            list(job)
            return carry

        lax.fori_loop(first, first + count, body, 0)

    a_loop(2, 3 * GP, prep_qkv, spare_qkv, True)

    qi = lax.broadcasted_iota(jnp.int32, (rows, rows), 0)
    ki = lax.broadcasted_iota(jnp.int32, (rows, rows), 1)
    mask = (qi >= seg) | (ki >= seg) | (qi >= ki)
    part, o_prev, opart, b_rows = (_Carry(r) for r in (part_s, o_s, opart_s, b_s))
    ahead = {}

    def b_step(u, t0, memv, project_only=False, output_only=False):
        odd = u % 2
        keep = lambda slots: [s for s in slots if s["tok"] or memv]
        qs, os_ = keep(_PHASES[odd][::RQ[odd]]), keep(_PHASES[1 - odd][::RP[1 - odd]])
        lhs, shared, tok, mrow, full, soft, o_mem, o_mix, o_left, o_host, new = ({} for _ in range(11))

        def spread(sums, key, slots, s, tok_rows, mem_rows):
            for nu in range(KB):
                if memv:
                    sums.add(key + (nu, 2), s["c"][nu], mem_rows, sum(abs(o["c"][nu]) for o in slots))
                for mu in range(2 if s["tok"] else 0):
                    sums.add(key + (nu, mu), _C[s["r"]][mu][nu], tok_rows,
                             sum(abs(_C[o["r"]][mu][nu]) for o in slots if o["tok"]))

        x_mix = _Mixer(lambda mu, kk: x32[kk, pl.ds(t0 + mu * seg, seg), :])
        c_mix = _Mixer(lambda mu, _: x32[KB, pl.ds(t0 + mu * seg, seg), :])
        m_mix = _Mixer(lambda _, kk: memv[kk])
        m_tail = memv[KB] + pltpu.roll(memv[KB], 64, 1) if memv else None

        def q_left(e, t):
            s = qs[e]
            if (e, t) not in lhs:
                left = stack(x_mix(_U[s["r"]]) if s["tok"] else None,
                             m_mix([s["a"]]) if memv else None)
                if s["r"] < NH and t < 2:
                    c = stack(c_mix(_TAIL_IN[s["r"]][:, None]),
                              _signed_sum([(sum(s["c"]), m_tail)]) if memv else None)
                    left = jnp.where(_low_half(c.shape[0]), *((c, left), (left, c))[t])
                lhs[e, t] = left
            return lhs[e, t]

        def q_total(key, value):
            i, g, nu, mu = key
            h = g * KB + nu
            if mu == 2:
                mrow[i, h] = value
            elif odd:
                part[i, h, mu] = value
            elif mu == 0:
                tok[i, h] = value + part[i, h, mu]
            else:
                ahead[i, h] = value + part[i, h, mu]
            cur = (ahead if odd else tok).get((i, h))
            if (i, h) in mrow and cur is not None and (i, h) not in full:
                full[i, h] = stack(cur, mrow[i, h]).astype(BF16 if i else F32)

        q_sums = _Sums(q_total)

        def q_pass(e, i, gp, t):
            s = qs[e]
            p = _dot(q_left(e, t), _tile(wb, i * GP + gp, t * NR + s["r"]))
            if t == 2:
                shared[e, i, gp] = p
                return
            if s["r"] < NH:
                p = p + shared[e, i, gp]
            spread(q_sums, (i, 2 * gp + t), qs, s, p[:seg], p[-mem:])

        def scores(h):
            s = jnp.where(mask, _dot_nt(full[0, h], full[1, h]), NEG * DB ** 0.5)
            e = jnp.exp2((s - jnp.max(s, axis=-1, keepdims=True)) * (DB ** -0.5 * LOG2E))
            total = jnp.sum(e, axis=-1, keepdims=True)
            inv = pltpu.reciprocal(total, approx=True)
            soft[h] = e * (inv * (2.0 - total * inv))

        def values(h):
            o = _dot(soft[h], full[2, h])
            o_mem[h] = o[seg:]
            if odd:
                o_prev[0, h], o_prev[1, h] = ahead["o", h], o[:seg]
            else:
                ahead["o", h] = o[:seg]

        def o_rows(e, gp, t):
            s = os_[e]
            if (e, gp, t) not in o_left:
                g = 2 * gp + t
                if t == 2:
                    o_left[e, gp, t] = o_rows(e, gp, 0) + o_rows(e, gp, 1)
                    return o_left[e, gp, t]
                if g not in o_mix:
                    o_mix[g] = (_Mixer(lambda _, kk: o_mem[g * KB + kk]),
                                _Mixer(lambda mu, kk: o_prev[mu, g * KB + kk]))
                o_left[e, gp, t] = stack(o_mix[g][0]([s["a"]]) if memv else None,
                                         o_mix[g][1](_U[s["r"]]) if s["tok"] else None)
            return o_left[e, gp, t]

        def o_total(key, value):
            nu, mu = key
            if mu == 2:
                new[nu] = value
            elif odd:
                opart[nu, mu] = value
            else:
                b_rows[nu, (u - 2) % 4 + mu] = value + opart[nu, mu]

        out_sums = _Sums(o_total)

        def o_product(key, value):
            e, t = key
            s = os_[e]
            if s["r"] < NH:
                o_host[key] = value
                if any((e, t_) not in o_host for t_ in range(3)):
                    return
                lo = _low_half(value.shape[0])
                value = o_host[e, 2] + jnp.where(lo, o_host[e, 1], o_host[e, 0])
                y = jnp.where(lo, o_host[e, 0], o_host[e, 1])
                if memv:
                    out_sums.add((KB, 2), sum(s["a"]), y[:mem], KB)
                for mu in range(2):
                    out_sums.add((KB, mu), _TAIL_OUT[s["r"]][mu], y[-seg:],
                                 sum(abs(_TAIL_OUT[o["r"]][mu]) for o in os_ if o["r"] < NH))
            spread(out_sums, (), os_, s, value[-seg:], value[:mem])

        o_sums = _Sums(o_product)

        def o_pass(e, gp, t):
            host = os_[e]["r"] < NH
            p = _dot(o_rows(e, gp, t), _tile(wb, 3 * GP + gp, t * NR + os_[e]["r"]))
            o_sums.add((e, t if host else 0), 1, p, GP if host else 2 * GP)

        todo = []
        tiles = lambda s: (2, 0, 1) if s["r"] < NH else (0, 1)
        if not output_only:
            todo = [(s["tok"], q_pass, e, i, gp, t) for gp in range(GP) for i in PO
                    for e, s in enumerate(qs) for t in tiles(s)]
            last = [max(e for e, s in enumerate(_PHASES[odd][::RP[odd]]) if s["tok"] and s["c"][nu])
                    for nu in range(KB)]
            ready = lambda e, t: 99 if qs[e]["r"] < NH and t < 2 else max(
                last[kk] for kk in range(KB) if qs[e]["a"][kk])
            todo[:HEAD] = sorted(todo[:HEAD], key=lambda p: ready(p[2], p[5]))
        if not project_only:
            todo += [(s["tok"], o_pass, e, gp, t) for pairs in CHUNKS for e, s in enumerate(os_)
                     for gp in pairs for t in tiles(s)]
        long_, short = ([p[1:] for p in todo if p[0] == tok] for tok in (True, False))
        extra = {}
        for h in range(HB if memv else 0):
            gp, n = divmod(h, 2 * KB)
            at = (90 * gp + S0 + int(SPAN[gp == GP - 1] * (n // Q * Q))) // Q * Q
            extra.setdefault(at, []).append((scores, h))
            extra.setdefault(at + LAG, []).append((values, h))
        issued = 0
        for n, p in enumerate(long_):
            for fn, *args in extra.get(n, []) + [p]:
                if issued % 4 == 0 and short and n >= (480 + M0 - 5 * len(short) if len(short) > 24 else MO[6 - len(short) // 4]):
                    for fn_s, *args_s in short[:4]:
                        fn_s(*args_s)
                    del short[:4]
                fn(*args)
                issued += 1
        assert not short
        return new

    def emit_tile(j):
        for nu in range(KB + 1):
            bt = jnp.concatenate([b_s[nu, 0], b_s[nu, 1], b_rows.val.pop((nu, 2)),
                                  b_rows.val.pop((nu, 3))], axis=0).T
            bt = bt if nu < KB else bt[:64] + bt[64:]
            at = pl.ds(nu * LANES, bt.shape[0])
            gm = jnp.concatenate([gm_s[j]] * (bt.shape[0] // 8), axis=0)
            out_v[j, at, :] = (ga_s[j, at, :] + gm * bt).astype(out_v.dtype)

    cp_wot.wait()
    for gp in range(GP):
        turn_out(gp)
    b_step(3, 0, None, project_only=True)
    part.flush()
    for j in range(3 * GP + 2, nt):
        to_rows(j)
    a_loop(3 * GP + 2, GP - 2, prep_out, spare_t, False)
    job = itertools.chain(prep_out(GP - 2), prep_out(GP - 1))
    a_out(nt - 1, paced(job, spare_t, zero_w, *QC))
    list(job)

    def b_body(j, carry):
        memv = {kk: mem_s[kk] for kk in range(KB + 1)}
        for u in range(4):
            t0 = jnp.minimum(j * LANES + (u + 1) // 2 * 2 * seg, seq - 2 * seg)
            memv = b_step(u, pl.multiple_of(t0, seg), memv)
            if u == 0:
                emit_tile(jnp.maximum(j - 1, 0))
        for kk, t in memv.items():
            mem_s[kk] = t
        for c in (part, o_prev, opart, b_rows):
            c.flush()
        pl.when(j > 0)(lambda: cp_out(j - 1).start())
        return carry

    lax.fori_loop(0, nt, b_body, 0)
    b_step(0, None, None, output_only=True)
    emit_tile(nt - 1)
    cp_out(nt - 1).start()
    for j in range(nt):
        cp_out(j).wait()


@functools.partial(jax.jit, static_argnames=("B_seg_len",))
def pallas_gated_mix__sliding_local_dilated__memory_aug_recurrent_mem_tr__prompt_kernel(
    A_x: jax.Array,
    A_wqkv: jax.Array,
    A_wo: jax.Array,
    B_x: jax.Array,
    B_mem0: jax.Array,
    B_Wq: jax.Array,
    B_Wk: jax.Array,
    B_Wv: jax.Array,
    B_Wo: jax.Array,
    B_seg_len: int,
    gate_w: jax.Array,
):
    del B_x
    batch, seq, width = A_x.shape
    mem, seg = B_mem0.shape[1], int(B_seg_len)
    nt = seq // LANES
    assert batch == 1 and width == D and nt == 4 * GP and seq % LANES == 0
    assert B_Wq.shape == (D, HB, DB) and mem == 8 and 4 * seg == LANES

    hbm = pl.BlockSpec(memory_space=pl.ANY)
    out_t = pl.pallas_call(
        functools.partial(_kernel, seq=seq, seg=seg, mem=mem),
        out_shape=jax.ShapeDtypeStruct((D, seq), A_x.dtype),
        in_specs=[hbm] * 9,
        out_specs=hbm,
        scratch_shapes=[
            pltpu.VMEM((nt, D, LANES), BF16),
            pltpu.VMEM((D, 3 * D), BF16),
            pltpu.VMEM((D, D), BF16),
            pltpu.VMEM((3 * GP + 1, KB, D, DB), U32),
            pltpu.VMEM((HB, D, DB), BF16),
            pltpu.VMEM((GP + 1, 2 * KB + 1, KB, 64, LANES), U32),
            pltpu.VMEM((5, 3 * D + 32, LANES), F32),
            pltpu.VMEM((5, D + 32, LANES), F32),
            pltpu.VMEM((12, 3 * D // 2 + 16, LANES), BF16),
            pltpu.VMEM((12, D // 2, LANES), BF16),
            pltpu.VMEM((2 * D, LANES), BF16),
            pltpu.VMEM((D, LANES), BF16),
            pltpu.VMEM((4 * GP + 1, 2 * NR + NH, LANES, LANES), BF16),
            pltpu.VMEM((KB + 1, seq, LANES), F32),
            pltpu.VMEM((nt, D, LANES), F32),
            pltpu.VMEM((nt, 8, LANES), F32),
            pltpu.VMEM((2 * KB, mem, LANES), F32),
            pltpu.VMEM((3, HB, 2, seg, LANES), F32),
            pltpu.VMEM((2, HB, seg, LANES), F32),
            pltpu.VMEM((KB + 1, 2, seg, LANES), F32),
            pltpu.VMEM((KB + 1, 2, seg, LANES), F32),
            pltpu.VMEM((nt, D, LANES), A_x.dtype),
            pltpu.VMEM((mem, D), BF16),
            pltpu.VMEM((D,), BF16),
            pltpu.SemaphoreType.DMA((3 * GP + 9 + len(XCUT),)),
            pltpu.SemaphoreType.DMA(()),
        ],
        compiler_params=pltpu.CompilerParams(vmem_limit_bytes=110 * 1024 * 1024),
        name="gated_mix_kernel",
    )(A_x.reshape(seq, D).T, A_wqkv, A_wo, B_mem0.reshape(mem, D), B_Wq, B_Wk, B_Wv,
      B_Wo.transpose(0, 2, 1), gate_w)
    return out_t.T.reshape(batch, seq, D)
```

```python
import functools
import itertools

import jax
import jax.numpy as jnp
import numpy as np
from jax import lax
import jax.experimental.pallas as pl
import jax.experimental.pallas.tpu as pltpu

F32, BF16, U32 = jnp.float32, jnp.bfloat16, jnp.uint32

D = 576
LANES = 128
HA, DA = 32, 18
WIN, DIL = 8, 2
HB, DB = 32, 128
NEG = -1000000000.0
LOG2E = 1.4426950408889634
NG = HA // 8

KB = 4
GP = HB // (2 * KB)

_HK = (
    (".... +...", "+.-. -... .... -...", "+... +..."),
    ("+... -...", "+-.- .... -... ....", "+... ...."),
    (".+.. .-..", ".... +-.. .+.. ....", ".... .+.."),
    (".+.. ....", ".-.. .+-. .... ....", ".+.. .+.."),
    (".... ..+.", ".... ..-. -.+. .+-.", ".... ..+."),
    ("..+. ....", "..-. ...+ .-+- ....", "..+. ...."),
    ("...+ ...-", ".... ...- ...+ ++.-", ".... ...+"),
    ("...+ ....", "...- ...- .... .+-+", "...+ ...+"),
    (".... ++..", ".... +... .... ....", ".... ++.."),
    ("++.. ....", ".+.. .... .... ....", "++.. ...."),
    (".+.. +...", ".-.. +... .... ....", "+... .-.."),
    ("+.+. -.-.", ".... .... -... ....", ".... +.+."),
    ("+.+. ....", "..+. .... .... ....", "+.+. +.+."),
    ("+.+. -...", "..-. .... +... ....", "+... +.+."),
    (".... +..+", ".... .... .... +...", ".... +..+"),
    ("+..+ ....", "...+ .... .... ....", "+..+ ...."),
    ("...+ +...", "...- .... .... +...", "+... ...-"),
    (".... .++.", ".... ..+. .... .-..", ".++. .++."),
    (".++. .--.", ".... ...- .+.. ....", ".++. ...."),
    (".+.. .--.", ".... ..+. .-.. ....", ".++. .+.."),
    (".... ..++", ".... .... .... .-+.", "..++ ..++"),
    ("..++ ..--", ".... ...- ...+ ....", "..++ ...."),
    ("...+ ..--", ".... ...+ ...- .-+.", "..++ ...+"),
    (".... .+++", ".... .... .... .+..", ".... .+++"),
    (".+++ ....", ".... ...+ .... ....", ".+++ ...."),
    ("...+ .++.", ".... ...- .... .+..", ".++. ...-"),
)
_U, _V, _C = (np.array([[["-.+".index(ch) - 1 for ch in row] for row in prod[i].split()]
                        for prod in _HK]) for i in range(3))
NR = len(_HK)
assert np.array_equal(np.einsum("rak,rln,rbm->akblnm", _U, _V, _C),
                      np.einsum("ab,kl,nm->akblnm", *(np.eye(n, dtype=int) for n in (2, KB, KB))))


def _phase(products):
    tiles = [max(r, ~r) for r in products]
    dual = np.rint(np.linalg.inv(_V[tiles].reshape(len(tiles), -1)).T).astype(int)
    slots = []
    for r, d in zip(products, dual.reshape(-1, KB, KB)):
        i, j = np.argwhere(d)[0]
        a, c = d[:, j] * d[i, j], d[i]
        assert np.array_equal(np.outer(a, c), d)
        slots.append(dict(r=max(r, ~r), tok=r >= 0, a=a.tolist(), c=c.tolist()))
    return slots


_PHASES = (_phase((11, 8, ~9, 4, 2, 23, 17, ~13, 25, 20, 22, 7, ~19, 16, 15, 1)),
           _phase((24, 21, ~16, 18, 19, 3, 10, ~22, 9, 5, 12, 13, ~25, 0, 14, 6)))
assert sorted(s["r"] for ph in _PHASES for s in ph if s["tok"]) == list(range(NR))

NH = 2 * KB
assert all(sorted(s["r"] // 2 for s in ph if s["r"] < NH) == list(range(KB)) for ph in _PHASES)
assert all(np.abs(s[k]).tolist() == np.eye(KB)[s["r"] // 2].tolist()
           for ph in _PHASES for s in ph if s["r"] < NH for k in "ac")
_TAIL_IN, _TAIL_OUT = (
    np.concatenate([np.rint(np.linalg.inv(t[2 * n:2 * n + 2, :, n]).T).astype(int)
                    for n in range(KB)]) for t in (_C, _U))


SCORE_AT = ((76, 94, 116, 138, 162, 184, 206, 228,
             252, 274, 296, 318, 342, 344, 346, 348),
            (72, 94, 116, 138, 162, 184, 206, 228,
             252, 274, 296, 318, 342, 344, 346, 348))
VALUE_AT = ((112, 134, 156, 182, 202, 224, 252, 268,
             294, 314, 336, 358, 382, 384, 386, 388),
            (112, 134, 156, 182, 202, 224, 246, 268,
             292, 310, 336, 356, 382, 384, 386, 388))
SHORT_AT = ((6, 26, 46, 66, 86, 106, 126, 146, 166, 186, 206, 226,
             246, 266, 286, 306, 326, 346, 364, 385, 410, 426, 444, 463),
            (6, 26, 46, 66, 86, 106, 126, 146, 170, 186, 206, 226,
             246, 266, 286, 306, 326, 346, 360, 385, 410, 426, 440, 463))
HEAD = (72, 66)
XCUT = (0, 1, 3, 8)
RE, RO = 8, 48
ORD = (9, 8, 10, 19, 2, 3, 23, 24, 25, 17, 18, 20, 21, 22, 12, 11, 13, 4, 5, 15, 14, 16, 6, 7, 0, 1)
CUT = (1,)
QA = ((4, 10, 22, 26, 39, 42, 63, 80, 94, 149, 158, 162, 165, 169, 172), 24)
QB = ((10, 13, 22, 42, 52, 73, 90, 109, 146, 155, 160, 166, 171, 176, 179), 32)
QC = ((4, 5, 7, 11, 14, 16, 21, 24, 28, 32, 35, 37, 41, 44, 48, 52), 12)


def _signed_sum(terms):
    terms = [(c, t) for c, t in terms if c]
    first = next((i for i, (c, _) in enumerate(terms) if c > 0), 0)
    c, acc = terms.pop(first)
    acc = acc if c > 0 else -acc
    for c, t in terms:
        acc = acc + t if c > 0 else acc - t
    return acc


class _Mixer:
    def __init__(self, block):
        self.block, self.known = block, {}

    def __call__(self, coef):
        want = {(i, k): int(c) for i, row in enumerate(coef) for k, c in enumerate(row) if c}
        key = tuple(sorted(want.items()))
        if key not in self.known:
            terms = []
            for have in sorted(self.known, key=lambda h: -len(h)):
                for sign in (1, -1):
                    if all(want.get(pos) == sign * c for pos, c in have):
                        terms.append((sign, self.known[have]))
                        want = {pos: c for pos, c in want.items() if pos not in dict(have)}
                        break
            for pos, c in sorted(want.items()):
                self.known[((pos, 1),)] = self.block(*pos)
                terms.append((c, self.known[((pos, 1),)]))
            self.known[key] = _signed_sum(terms)
        return self.known[key]


class _Sums:
    def __init__(self, done):
        self.done, self.acc = done, {}

    def add(self, key, sign, value, expected):
        if not sign:
            return
        count, neg, tot = self.acc.pop(key, (0, sign < 0, value))
        if count and neg == (sign < 0):
            tot = tot + value
        elif count:
            tot, neg = (value - tot if neg else tot - value), False
        if count + 1 == expected:
            self.done(key, -tot if neg else tot)
        else:
            self.acc[key] = (count + 1, neg, tot)


class _Carry:
    def __init__(self, ref):
        self.ref, self.val = ref, {}

    def __getitem__(self, key):
        return self.val[key] if key in self.val else self.ref[key]

    def __setitem__(self, key, value):
        self.val[key] = value

    def flush(self):
        for key, value in self.val.items():
            self.ref[key] = value
        self.val = {}


def _dot(a, b):
    return lax.dot_general(a, b, (((1,), (0,)), ((), ())), preferred_element_type=F32)


def _dot_nt(a, b):
    return lax.dot_general(a, b, (((1,), (1,)), ((), ())), preferred_element_type=F32)


def _tile(ref, *idx):
    return pltpu.bitcast(ref.bitcast(U32)[idx], BF16)


def stack(*parts):
    parts = [t for t in parts if t is not None]
    return parts[0] if len(parts) == 1 else jnp.concatenate(parts, axis=0)


def _low_half(rows):
    return lax.broadcasted_iota(jnp.int32, (rows, LANES), 1) < 64


def _pair_lhs(t1, t2):
    lo = _low_half(t1[3].shape[0])
    diff = t1[3] - t2[3]
    return (t1[:3] + [jnp.where(lo, t1[4], diff)]
            + t2[:3] + [jnp.where(lo, -diff, t2[4])]
            + [jnp.where(lo, t1[3], t2[3])])


def _pair_rhs(x):
    a, b, c = x[384:448], x[448:512], x[512:576]
    cat = lambda u, v: jnp.concatenate([u, v], axis=0)
    return [x[i * 128:(i + 1) * 128] for i in range(3)] + [cat(c, b), cat(a, c), x[384:512]]


def _pair_matmul(lhs, rhs, dot):
    out = [dot(lhs(8), rhs[5])] * 2
    for i in range(8):
        out[i // 4] = out[i // 4] + dot(lhs(i), rhs[i % 4 if i < 7 else 4])
    return out


def _kernel(xt_hbm, wqkv_hbm, wo_hbm, mem0_hbm, wq_hbm, wk_hbm, wv_hbm, wot_hbm, gate_hbm,
            out_hbm,
            xt_v, wqkv_v, wo_v, stg_qkv, stg_o, wo_t, wt32, wo32_s, la, lo_a, kv_prev, oa_s,
            wb, x32, ga_s, gm_s, mem_s, part_s, o_s, opart_s, b_s, out_v, mem0_v, gate_v,
            sem_in, sem_out, *, seq, seg, mem):
    nt = seq // LANES
    rows = mem + seg

    sems = (sem_in.at[n] for n in itertools.count(3 * GP))
    copy = pltpu.make_async_copy
    cp_wqkv = {k: copy(wqkv_hbm.at[k * LANES:min(D, (k + 1) * LANES)],
                       wqkv_v.at[k * LANES:min(D, (k + 1) * LANES)], next(sems))
               for k in (3, 4, 0, 1, 2)}
    cp_wo = copy(wo_hbm, wo_v, next(sems))
    cp_x = {j0: [copy(xt_hbm.at[:, j * LANES:(j + 1) * LANES], xt_v.at[j], sem)
                 for j in range(j0, j1)] for j0, j1, sem in zip(XCUT, XCUT[1:] + (nt,), sems)}
    cp_wot = copy(wot_hbm, stg_o, next(sems))
    cp_small = [copy(mem0_hbm, mem0_v, next(sems)), copy(gate_hbm, gate_v, next(sems))]
    queue = cp_small + list(cp_wqkv.values()) + cp_x[0] + [cp_wo]
    for unit in range(3 * GP):
        src = (wq_hbm, wk_hbm, wv_hbm)[unit // GP].bitcast(U32)
        queue += cp_x.get(unit + 1, []) + [
            copy(src.at[:, KB * (unit % GP) + p, :], stg_qkv.at[unit, p], sem_in.at[unit])
            for p in range(KB)]
    for c in queue + [cp_wot]:
        c.start()

    def wait_all(copies):
        for c in copies:
            c.wait()

    def cp_out(j):
        col = j * LANES if isinstance(j, int) else pl.multiple_of(j * LANES, LANES)
        return copy(out_v.at[j], out_hbm.at[:, pl.ds(col, LANES)], sem_out)

    for ref in (o_s, opart_s, b_s):
        ref[...] = jnp.zeros(ref.shape, ref.dtype)
    wait_all(cp_small)
    m0 = mem0_v[...].astype(F32)
    for kk in range(KB):
        mem_s[kk] = m0[:, kk * LANES:(kk + 1) * LANES]
    mem_s[KB] = jnp.concatenate([m0[:, KB * LANES:], jnp.zeros((mem, 64), F32)], axis=1)
    wb[4 * GP, 0, 0:16, :] = jnp.zeros((16, LANES), BF16)

    gate = jnp.broadcast_to(gate_v[...].astype(F32).reshape(1, D), (8, D))
    gate_t = [gate[:, i * 128:(i + 1) * 128] for i in range(4)]
    gate_t.append(jnp.concatenate([gate[:, 512:], gate[:, 512:]], axis=1))

    entries = [None] * 2 + [(g - part // 2, part, n) for g in range(NG + 1) for n in range(DA // 2)
                            for part in (1, 0, 2) if 0 <= g - part // 2 < NG]

    def feature_rows(k, e):
        return stack(*(gate_t[k] if ent is None else
                       wt32[k, pl.ds(ent[1] * D + ent[0] * 8 * DA + 2 * ent[2] + e, 8, stride=DA), :]
                       for ent in entries))

    for k in cp_wqkv:
        cp_wqkv[k].wait()
        rows_k = wqkv_v[k * LANES:min(D, (k + 1) * LANES), :]
        wt32[k, 0:3 * D] = (rows_k if k < 4 else stack(rows_k, rows_k)).T.astype(F32)
        for e in range(2 if k < 3 else 0):
            la[4 * e + k] = feature_rows(k, e).astype(BF16)
        if k == 4:
            mixed = _pair_lhs(*([None] * 3 + [feature_rows(3, e), feature_rows(4, e)]
                                for e in range(2)))
            for i in (3, 7, 8):
                la[i] = mixed[i].astype(BF16)

    def prep_wo():
        wo32 = wo_v[...].astype(F32)
        for n in range(4):
            wo32_s[n, 0:D] = wo32[:, n * LANES:(n + 1) * LANES]
        wo32_s[4, 0:D] = jnp.concatenate([wo32[:, 4 * LANES:]] * 2, axis=1)
        turned = []
        for n in range(5):
            perm = stack(*(wo32_s[n, pl.ds(g * 8 * DA + d, 8, stride=DA), :]
                           for g in range(NG) for d in range(DA))).astype(BF16)
            turned.append([perm[k * LANES:(k + 1) * LANES].T for k in range(4)]
                          + [stack(perm[4 * LANES:], perm[4 * LANES:]).T])
        tiles = [stack(*(t[k] for t in turned))[:D].astype(F32) for k in range(5)]
        for i, t in enumerate(_pair_lhs([t[:D // 2] for t in tiles], [t[D // 2:] for t in tiles])):
            lo_a[i] = t.astype(BF16)

    by_size = ORD

    def prep_qkv(unit):
        src, dst = stg_qkv.at[unit], wb.at[unit]

        def rows(g, r0, nu):
            u = src[2 * g + nu // 2, r0:r0 + 16, :]
            return pltpu.bitcast(u & jnp.uint32(0xFFFF0000) if nu % 2 else u << 16, F32)

        for e in range(8):
            at, own, shared = pl.ds(16 * e, 16), e // 4, {}
            for g in (own, 1 - own):
                mix = _Mixer(lambda kk, nu: rows(g, kk * LANES + 16 * e, nu))
                for r in by_size:
                    w = mix(_V[r])
                    if r < NH and g == own:
                        shared[r] = w.astype(BF16)
                        dst[2 * NR + r, at, :] = shared[r]
                        w = rows(g, KB * LANES + 16 * (e % 4), r // 2)
                    elif r < NH:
                        w = w - shared[r].astype(F32)
                    dst[g * NR + r, at, :] = w.astype(BF16)
                    if r in CUT:
                        yield

    def turn_out(gp):
        words = lambda head, r0, n: _tile(stg_o, 2 * KB * gp + head, pl.ds(r0 // 2, n // 2))
        for head in range(2 * KB + 1):
            for nu in range(KB):
                if head < 2 * KB:
                    tile = words(head, nu * LANES, LANES)
                else:
                    tile = stack(*(words(g * KB + nu, KB * LANES, 64) for g in range(2)))
                wo_t[gp, head, nu] = pltpu.bitcast(tile.T, U32)

    def prep_out(gp):
        dst, lo = wb.at[3 * GP + gp], _low_half(16)
        for e in range(8):
            at, first = pl.ds(16 * e, 16), {}
            rows = lambda head, nu: pltpu.bitcast(
                wo_t[gp, head, nu, 8 * e:8 * e + 8, :], BF16).astype(F32)
            for g in range(2):
                mix = _Mixer(lambda kk, nu: rows(g * KB + kk, nu))
                for r in by_size:
                    w = mix(_V[r])
                    if r >= NH:
                        dst[g * NR + r, at, :] = w.astype(BF16)
                    elif g == 0:
                        first[r] = w
                    else:
                        z, t = jnp.where(lo, first[r], w).astype(BF16), rows(2 * KB, r // 2)
                        dst[2 * NR + r, at, :] = z
                        dst[r, at, :] = jnp.where(lo, t, first[r] - z.astype(F32)).astype(BF16)
                        dst[NR + r, at, :] = jnp.where(lo, w - z.astype(F32), t).astype(BF16)
                    if r in CUT:
                        yield

    lane = lax.broadcasted_iota(jnp.int32, (8, LANES), 1)

    def exchange(idx, pair, first):
        at = pl.ds(8 * idx, 8)
        prev = None if first else kv_prev.bitcast(U32)[at, :]
        kv_prev[16 * idx:16 * idx + 16, :] = jnp.concatenate(pair, axis=0).astype(BF16)
        cur = kv_prev.bitcast(U32)[at, :]
        return (jnp.broadcast_to(cur[:, 0:1], (8, LANES)) if first else prev), cur

    def to_rows(j):
        t0 = j * LANES if isinstance(j, int) else pl.multiple_of(j * LANES, LANES)
        xt = _tile(xt_v, j)
        for kk in range(KB + 1):
            tile = xt[kk * LANES:(kk + 1) * LANES]
            x32[kk, pl.ds(t0, LANES), :] = (tile if kk < KB else stack(tile, tile)).T.astype(F32)

    def paced(job, src, dst, when, back):
        results = []

        def dot(left, right):
            if len(results) in when:
                if src is not None and len(results) >= back:
                    src[...] = pltpu.bitcast(results[-back][0:8], U32)
                next(job, None)
                left = stack(left[:-8] if len(left) > 8 else None, left[-8:] | dst[...])
            results.append(_dot(pltpu.bitcast(left, BF16), right))
            return results[-1]

        return dot

    spare_qkv, spare_t = stg_qkv.at[3 * GP, 0, 0:8], wo_t.at[GP, 0, 1, 0:8]
    zero_w = wb.bitcast(U32).at[4 * GP, 0, 0:8]

    def a_out(j, dot):
        rhs = _pair_rhs(_tile(oa_s, slice(None)))
        for r0 in range(0, D // 2, RO):
            halves = _pair_matmul(lambda i: lo_a.bitcast(U32)[i, r0 // 2:(r0 + RO) // 2, :], rhs, dot)
            for e in range(2):
                ga_s[j, pl.ds(e * D // 2 + r0, RO), :] = halves[e]

    def a_tile(j, first, dot):
        rhs = _pair_rhs(_tile(xt_v, j))
        logit, prob, outs = {}, {}, {}
        for e0 in range(0, len(entries), RE):
            some = entries[e0:e0 + RE]
            halves = _pair_matmul(
                lambda i: la.bitcast(U32)[i, 4 * e0:4 * (e0 + len(some)), :], rhs, dot)
            for ent, r0 in zip(some, range(0, 8 * RE, 8)):
                pair = [t[r0:r0 + 8] for t in halves]
                if ent is None:
                    gsig = 1.0 / (1.0 + jnp.exp(-halves[0][0:8]))
                    continue
                g, part, n = ent
                if part:
                    prev, cur = exchange((2 * g + part - 1) * (DA // 2) + n, pair, first)
                    back = [cur] + [
                        pltpu.roll(jnp.where(lane >= LANES - DIL * w, prev, cur), DIL * w, 1)
                        for w in range(1, WIN)]
                    back = [pltpu.bitcast(t, BF16).astype(F32) for t in back]
                if part == 2:
                    outs[g, n] = functools.reduce(
                        jnp.add, [stack(p, p) * t for p, t in zip(prob[g], back)]).astype(BF16)
                elif part == 0:
                    terms = [pair[0] * t[0:8] + pair[1] * t[8:16] for t in back]
                    logit[g] = terms if n == 0 else [a + t for a, t in zip(logit[g], terms)]
                if (part, n) == (0, DA // 2 - 1):
                    s = [jnp.where(lane >= DIL * w, t, NEG * DA ** 0.5) if first else t
                         for w, t in enumerate(logit[g])]
                    top = functools.reduce(jnp.maximum, s)
                    ex = [jnp.exp2((t - top) * (DA ** -0.5 * LOG2E)) for t in s]
                    inv = gsig / functools.reduce(jnp.add, ex)
                    prob[g] = [t * inv for t in ex]
        gm_s[j] = 1.0 - gsig
        if not first:
            a_out(j - 1, dot)
        oa_s[...] = stack(*(outs[key] for key in sorted(outs)))

    plain = lambda left, right: _dot(pltpu.bitcast(left, BF16), right)
    wait_all(cp_x[0])
    to_rows(0)
    a_tile(0, True, plain)
    cp_wo.wait()
    wait_all(cp_x[1])
    prep_wo()
    a_tile(1, False, plain)
    to_rows(1)

    def a_loop(first, count, work, spare, loading):
        def body(j, carry):
            if loading:
                for j0 in XCUT[2:]:
                    pl.when(j == j0)(functools.partial(wait_all, cp_x[j0]))
                copy(stg_qkv.at[j - first], stg_qkv.at[j - first], sem_in.at[j - first]).wait()
                to_rows(j)
            job = work(j - first)
            a_tile(j, False, paced(job, spare, zero_w, *(QA if loading else QB)))
            list(job)
            return carry

        lax.fori_loop(first, first + count, body, 0)

    a_loop(2, 3 * GP, prep_qkv, spare_qkv, True)

    qi = lax.broadcasted_iota(jnp.int32, (rows, rows), 0)
    ki = lax.broadcasted_iota(jnp.int32, (rows, rows), 1)
    mask = (qi >= seg) | (ki >= seg) | (qi >= ki)
    part, o_prev, opart, b_rows = (_Carry(r) for r in (part_s, o_s, opart_s, b_s))
    ahead = {}

    def b_step(u, t0, memv, project_only=False, output_only=False):
        odd = u % 2
        keep = lambda slots: [s for s in slots if s["tok"] or memv]
        qs, os_ = keep(_PHASES[odd]), keep(_PHASES[1 - odd])
        lhs, shared, tok, mrow, full, soft, o_mem, o_mix, o_left, o_host, new = ({} for _ in range(11))

        def spread(sums, key, slots, s, tok_rows, mem_rows):
            for nu in range(KB):
                if memv:
                    sums.add(key + (nu, 2), s["c"][nu], mem_rows, sum(abs(o["c"][nu]) for o in slots))
                for mu in range(2 if s["tok"] else 0):
                    sums.add(key + (nu, mu), _C[s["r"]][mu][nu], tok_rows,
                             sum(abs(_C[o["r"]][mu][nu]) for o in slots if o["tok"]))

        x_mix = _Mixer(lambda mu, kk: x32[kk, pl.ds(t0 + mu * seg, seg), :])
        c_mix = _Mixer(lambda mu, _: x32[KB, pl.ds(t0 + mu * seg, seg), :])
        m_mix = _Mixer(lambda _, kk: memv[kk])
        m_tail = memv[KB] + pltpu.roll(memv[KB], 64, 1) if memv else None

        def q_left(e, t):
            s = qs[e]
            if (e, t) not in lhs:
                left = stack(x_mix(_U[s["r"]]) if s["tok"] else None,
                             m_mix([s["a"]]) if memv else None)
                if s["r"] < NH and t < 2:
                    c = stack(c_mix(_TAIL_IN[s["r"]][:, None]),
                              _signed_sum([(sum(s["c"]), m_tail)]) if memv else None)
                    left = jnp.where(_low_half(c.shape[0]), *((c, left), (left, c))[t])
                lhs[e, t] = left
            return lhs[e, t]

        def q_total(key, value):
            i, g, nu, mu = key
            h = g * KB + nu
            if mu == 2:
                mrow[i, h] = value
            elif odd:
                part[i, h, mu] = value
            elif mu == 0:
                tok[i, h] = value + part[i, h, mu]
            else:
                ahead[i, h] = value + part[i, h, mu]
            cur = (ahead if odd else tok).get((i, h))
            if (i, h) in mrow and cur is not None and (i, h) not in full:
                full[i, h] = stack(cur, mrow[i, h]).astype(BF16 if i else F32)

        q_sums = _Sums(q_total)

        def q_pass(e, i, gp, t):
            s = qs[e]
            p = _dot(q_left(e, t), _tile(wb, i * GP + gp, t * NR + s["r"]))
            if t == 2:
                shared[e, i, gp] = p
                return
            if s["r"] < NH:
                p = p + shared[e, i, gp]
            spread(q_sums, (i, 2 * gp + t), qs, s, p[:seg], p[-mem:])

        def scores(h):
            s = jnp.where(mask, _dot_nt(full[0, h], full[1, h]), NEG * DB ** 0.5)
            e = jnp.exp2((s - jnp.max(s, axis=-1, keepdims=True)) * (DB ** -0.5 * LOG2E))
            total = jnp.sum(e, axis=-1, keepdims=True)
            inv = pltpu.reciprocal(total, approx=True)
            soft[h] = e * (inv * (2.0 - total * inv))

        def values(h):
            o = _dot(soft[h], full[2, h])
            o_mem[h] = o[seg:]
            if odd:
                o_prev[0, h], o_prev[1, h] = ahead["o", h], o[:seg]
            else:
                ahead["o", h] = o[:seg]

        def o_rows(e, gp, t):
            s = os_[e]
            if (e, gp, t) not in o_left:
                g = 2 * gp + t
                if t == 2:
                    o_left[e, gp, t] = o_rows(e, gp, 0) + o_rows(e, gp, 1)
                    return o_left[e, gp, t]
                if g not in o_mix:
                    o_mix[g] = (_Mixer(lambda _, kk: o_mem[g * KB + kk]),
                                _Mixer(lambda mu, kk: o_prev[mu, g * KB + kk]))
                o_left[e, gp, t] = stack(o_mix[g][0]([s["a"]]) if memv else None,
                                         o_mix[g][1](_U[s["r"]]) if s["tok"] else None)
            return o_left[e, gp, t]

        def o_total(key, value):
            nu, mu = key
            if mu == 2:
                new[nu] = value
            elif odd:
                opart[nu, mu] = value
            else:
                b_rows[nu, (u - 2) % 4 + mu] = value + opart[nu, mu]

        out_sums = _Sums(o_total)

        def o_product(key, value):
            e, t = key
            s = os_[e]
            if s["r"] < NH:
                o_host[key] = value
                if any((e, t_) not in o_host for t_ in range(3)):
                    return
                lo = _low_half(value.shape[0])
                value = o_host[e, 2] + jnp.where(lo, o_host[e, 1], o_host[e, 0])
                y = jnp.where(lo, o_host[e, 0], o_host[e, 1])
                if memv:
                    out_sums.add((KB, 2), sum(s["a"]), y[:mem], KB)
                for mu in range(2):
                    out_sums.add((KB, mu), _TAIL_OUT[s["r"]][mu], y[-seg:],
                                 sum(abs(_TAIL_OUT[o["r"]][mu]) for o in os_ if o["r"] < NH))
            spread(out_sums, (), os_, s, value[-seg:], value[:mem])

        o_sums = _Sums(o_product)

        def o_pass(e, gp, t):
            host = os_[e]["r"] < NH
            p = _dot(o_rows(e, gp, t), _tile(wb, 3 * GP + gp, t * NR + os_[e]["r"]))
            o_sums.add((e, t if host else 0), 1, p, GP if host else 2 * GP)

        todo = []
        tiles = lambda s: (2, 0, 1) if s["r"] < NH else (0, 1)
        if not output_only:
            todo = [(s["tok"], q_pass, e, i, gp, t) for gp in range(GP) for i in (1, 0, 2)
                    for e, s in enumerate(qs) for t in tiles(s)]
            last = [max(e for e, s in enumerate(_PHASES[odd]) if s["tok"] and s["c"][nu])
                    for nu in range(KB)]
            ready = lambda e, t: 99 if qs[e]["r"] < NH and t < 2 else max(
                last[kk] for kk in range(KB) if qs[e]["a"][kk])
            todo[:HEAD[odd]] = sorted(todo[:HEAD[odd]], key=lambda p: ready(p[2], p[5]))
        if not project_only:
            todo += [(s["tok"], o_pass, e, gp, t) for pairs in ((0, 1), (2, 3)) for e, s in enumerate(os_)
                     for gp in pairs for t in tiles(s)]
        long_, short = ([p[1:] for p in todo if p[0] == tok] for tok in (True, False))
        extra = {}
        for h in range(HB if memv else 0):
            extra.setdefault(SCORE_AT[odd][h // 2], []).append((scores, h))
            extra.setdefault(VALUE_AT[odd][h // 2], []).append((values, h))
        issued = 0
        for n, p in enumerate(long_):
            for fn, *args in extra.get(n, []) + [p]:
                if issued % 4 == 0 and short and n >= SHORT_AT[odd][-len(short) // 4]:
                    for fn_s, *args_s in short[:4]:
                        fn_s(*args_s)
                    del short[:4]
                fn(*args)
                issued += 1
        assert not short
        return new

    def emit_tile(j):
        for nu in range(KB + 1):
            bt = jnp.concatenate([b_s[nu, 0], b_s[nu, 1], b_rows.val.pop((nu, 2)),
                                  b_rows.val.pop((nu, 3))], axis=0).T
            bt = bt if nu < KB else bt[:64] + bt[64:]
            at = pl.ds(nu * LANES, bt.shape[0])
            gm = jnp.concatenate([gm_s[j]] * (bt.shape[0] // 8), axis=0)
            out_v[j, at, :] = (ga_s[j, at, :] + gm * bt).astype(out_v.dtype)

    cp_wot.wait()
    for gp in range(GP):
        turn_out(gp)
    b_step(3, 0, None, project_only=True)
    part.flush()
    for j in range(3 * GP + 2, nt):
        to_rows(j)
    a_loop(3 * GP + 2, GP - 2, prep_out, spare_t, False)
    job = itertools.chain(prep_out(GP - 2), prep_out(GP - 1))
    a_out(nt - 1, paced(job, spare_t, zero_w, *QC))
    list(job)

    def b_body(j, carry):
        memv = {kk: mem_s[kk] for kk in range(KB + 1)}
        for u in range(4):
            t0 = jnp.minimum(j * LANES + (u + 1) // 2 * 2 * seg, seq - 2 * seg)
            memv = b_step(u, pl.multiple_of(t0, seg), memv)
            if u == 0:
                emit_tile(jnp.maximum(j - 1, 0))
        for kk, t in memv.items():
            mem_s[kk] = t
        for c in (part, o_prev, opart, b_rows):
            c.flush()
        pl.when(j > 0)(lambda: cp_out(j - 1).start())
        return carry

    lax.fori_loop(0, nt, b_body, 0)
    b_step(0, None, None, output_only=True)
    emit_tile(nt - 1)
    cp_out(nt - 1).start()
    for j in range(nt):
        cp_out(j).wait()


@functools.partial(jax.jit, static_argnames=("B_seg_len",))
def pallas_gated_mix__sliding_local_dilated__memory_aug_recurrent_mem_tr__prompt_kernel(
    A_x: jax.Array,
    A_wqkv: jax.Array,
    A_wo: jax.Array,
    B_x: jax.Array,
    B_mem0: jax.Array,
    B_Wq: jax.Array,
    B_Wk: jax.Array,
    B_Wv: jax.Array,
    B_Wo: jax.Array,
    B_seg_len: int,
    gate_w: jax.Array,
):
    del B_x
    batch, seq, width = A_x.shape
    mem, seg = B_mem0.shape[1], int(B_seg_len)
    nt = seq // LANES
    assert batch == 1 and width == D and nt == 4 * GP and seq % LANES == 0
    assert B_Wq.shape == (D, HB, DB) and mem == 8 and 4 * seg == LANES

    hbm = pl.BlockSpec(memory_space=pl.ANY)
    out_t = pl.pallas_call(
        functools.partial(_kernel, seq=seq, seg=seg, mem=mem),
        out_shape=jax.ShapeDtypeStruct((D, seq), A_x.dtype),
        in_specs=[hbm] * 9,
        out_specs=hbm,
        scratch_shapes=[
            pltpu.VMEM((nt, D, LANES), BF16),
            pltpu.VMEM((D, 3 * D), BF16),
            pltpu.VMEM((D, D), BF16),
            pltpu.VMEM((3 * GP + 1, KB, D, DB), U32),
            pltpu.VMEM((HB, D, DB), BF16),
            pltpu.VMEM((GP + 1, 2 * KB + 1, KB, 64, LANES), U32),
            pltpu.VMEM((5, 3 * D + 32, LANES), F32),
            pltpu.VMEM((5, D + 32, LANES), F32),
            pltpu.VMEM((12, 3 * D // 2 + 16, LANES), BF16),
            pltpu.VMEM((12, D // 2, LANES), BF16),
            pltpu.VMEM((2 * D, LANES), BF16),
            pltpu.VMEM((D, LANES), BF16),
            pltpu.VMEM((4 * GP + 1, 2 * NR + NH, LANES, LANES), BF16),
            pltpu.VMEM((KB + 1, seq, LANES), F32),
            pltpu.VMEM((nt, D, LANES), F32),
            pltpu.VMEM((nt, 8, LANES), F32),
            pltpu.VMEM((2 * KB, mem, LANES), F32),
            pltpu.VMEM((3, HB, 2, seg, LANES), F32),
            pltpu.VMEM((2, HB, seg, LANES), F32),
            pltpu.VMEM((KB + 1, 2, seg, LANES), F32),
            pltpu.VMEM((KB + 1, 2, seg, LANES), F32),
            pltpu.VMEM((nt, D, LANES), A_x.dtype),
            pltpu.VMEM((mem, D), BF16),
            pltpu.VMEM((D,), BF16),
            pltpu.SemaphoreType.DMA((3 * GP + 9 + len(XCUT),)),
            pltpu.SemaphoreType.DMA(()),
        ],
        compiler_params=pltpu.CompilerParams(vmem_limit_bytes=110 * 1024 * 1024),
        name="gated_mix_kernel",
    )(A_x.reshape(seq, D).T, A_wqkv, A_wo, B_mem0.reshape(mem, D), B_Wq, B_Wk, B_Wv,
      B_Wo.transpose(0, 2, 1), gate_w)
    return out_t.T.reshape(batch, seq, D)
```

```python
import functools
import itertools

import jax
import jax.numpy as jnp
import numpy as np
from jax import lax
import jax.experimental.pallas as pl
import jax.experimental.pallas.tpu as pltpu

F32, BF16, U32 = jnp.float32, jnp.bfloat16, jnp.uint32

D = 576
LANES = 128
HA, DA = 32, 18
WIN, DIL = 8, 2
HB, DB = 32, 128
NEG = -1000000000.0
LOG2E = 1.4426950408889634
NG = HA // 8

KB = 4
GP = HB // (2 * KB)

_HK = (
    (".... +...", "+.-. -... .... -...", "+... +..."),
    ("+... -...", "+-.- .... -... ....", "+... ...."),
    (".+.. .-..", ".... +-.. .+.. ....", ".... .+.."),
    (".+.. ....", ".-.. .+-. .... ....", ".+.. .+.."),
    (".... ..+.", ".... ..-. -.+. .+-.", ".... ..+."),
    ("..+. ....", "..-. ...+ .-+- ....", "..+. ...."),
    ("...+ ...-", ".... ...- ...+ ++.-", ".... ...+"),
    ("...+ ....", "...- ...- .... .+-+", "...+ ...+"),
    (".... ++..", ".... +... .... ....", ".... ++.."),
    ("++.. ....", ".+.. .... .... ....", "++.. ...."),
    (".+.. +...", ".-.. +... .... ....", "+... .-.."),
    ("+.+. -.-.", ".... .... -... ....", ".... +.+."),
    ("+.+. ....", "..+. .... .... ....", "+.+. +.+."),
    ("+.+. -...", "..-. .... +... ....", "+... +.+."),
    (".... +..+", ".... .... .... +...", ".... +..+"),
    ("+..+ ....", "...+ .... .... ....", "+..+ ...."),
    ("...+ +...", "...- .... .... +...", "+... ...-"),
    (".... .++.", ".... ..+. .... .-..", ".++. .++."),
    (".++. .--.", ".... ...- .+.. ....", ".++. ...."),
    (".+.. .--.", ".... ..+. .-.. ....", ".++. .+.."),
    (".... ..++", ".... .... .... .-+.", "..++ ..++"),
    ("..++ ..--", ".... ...- ...+ ....", "..++ ...."),
    ("...+ ..--", ".... ...+ ...- .-+.", "..++ ...+"),
    (".... .+++", ".... .... .... .+..", ".... .+++"),
    (".+++ ....", ".... ...+ .... ....", ".+++ ...."),
    ("...+ .++.", ".... ...- .... .+..", ".++. ...-"),
)
_U, _V, _C = (np.array([[["-.+".index(ch) - 1 for ch in row] for row in prod[i].split()]
                        for prod in _HK]) for i in range(3))
NR = len(_HK)
assert np.array_equal(np.einsum("rak,rln,rbm->akblnm", _U, _V, _C),
                      np.einsum("ab,kl,nm->akblnm", *(np.eye(n, dtype=int) for n in (2, KB, KB))))


def _phase(products):
    tiles = [max(r, ~r) for r in products]
    dual = np.rint(np.linalg.inv(_V[tiles].reshape(len(tiles), -1)).T).astype(int)
    slots = []
    for r, d in zip(products, dual.reshape(-1, KB, KB)):
        i, j = np.argwhere(d)[0]
        a, c = d[:, j] * d[i, j], d[i]
        assert np.array_equal(np.outer(a, c), d)
        slots.append(dict(r=max(r, ~r), tok=r >= 0, a=a.tolist(), c=c.tolist()))
    return slots


_PHASES = (_phase((11, 8, ~9, 4, 2, 23, 17, ~13, 25, 20, 22, 7, ~19, 16, 15, 1)),
           _phase((24, 21, ~16, 18, 19, 3, 10, ~22, 9, 5, 12, 13, ~25, 0, 14, 6)))
assert sorted(s["r"] for ph in _PHASES for s in ph if s["tok"]) == list(range(NR))

NH = 2 * KB
assert all(sorted(s["r"] // 2 for s in ph if s["r"] < NH) == list(range(KB)) for ph in _PHASES)
assert all(np.abs(s[k]).tolist() == np.eye(KB)[s["r"] // 2].tolist()
           for ph in _PHASES for s in ph if s["r"] < NH for k in "ac")
_TAIL_IN, _TAIL_OUT = (
    np.concatenate([np.rint(np.linalg.inv(t[2 * n:2 * n + 2, :, n]).T).astype(int)
                    for n in range(KB)]) for t in (_C, _U))


SCORE_AT = ((76, 94, 116, 138, 162, 184, 206, 228,
             252, 274, 296, 318, 342, 344, 346, 348),
            (72, 94, 116, 138, 162, 184, 206, 228,
             252, 274, 296, 318, 342, 344, 346, 348))
VALUE_AT = ((112, 134, 156, 182, 202, 224, 252, 268,
             294, 314, 336, 358, 382, 384, 386, 388),
            (112, 134, 156, 182, 202, 224, 246, 268,
             292, 310, 336, 356, 382, 384, 386, 388))
SHORT_AT = ((6, 26, 46, 66, 86, 106, 126, 146, 166, 186, 206, 226,
             246, 266, 286, 306, 326, 346, 364, 385, 410, 426, 444, 463),
            (6, 26, 46, 66, 86, 106, 126, 146, 170, 186, 206, 226,
             246, 266, 286, 306, 326, 346, 360, 385, 410, 426, 440, 463))
HEAD = (72, 66)
XCUT = (0, 1, 3, 8)
RE, RO = 8, 48
ORD = (9, 8, 10, 19, 2, 3, 23, 24, 25, 17, 18, 20, 21, 22, 12, 11, 13, 4, 5, 15, 14, 16, 6, 7, 0, 1)
QA = ((4, 10, 22, 26, 39, 42, 63, 80, 94, 149, 158, 162, 165, 169, 172), 24)
QB = ((10, 13, 22, 42, 52, 73, 90, 109, 146, 155, 160, 166, 171, 176, 179), 32)
QC = ((4, 5, 7, 11, 14, 16, 21, 24, 28, 32, 35, 37, 41, 44, 48, 52), 12)


def _signed_sum(terms):
    terms = [(c, t) for c, t in terms if c]
    first = next((i for i, (c, _) in enumerate(terms) if c > 0), 0)
    c, acc = terms.pop(first)
    acc = acc if c > 0 else -acc
    for c, t in terms:
        acc = acc + t if c > 0 else acc - t
    return acc


class _Mixer:
    def __init__(self, block):
        self.block, self.known = block, {}

    def __call__(self, coef):
        want = {(i, k): int(c) for i, row in enumerate(coef) for k, c in enumerate(row) if c}
        key = tuple(sorted(want.items()))
        if key not in self.known:
            terms = []
            for have in sorted(self.known, key=lambda h: -len(h)):
                for sign in (1, -1):
                    if all(want.get(pos) == sign * c for pos, c in have):
                        terms.append((sign, self.known[have]))
                        want = {pos: c for pos, c in want.items() if pos not in dict(have)}
                        break
            for pos, c in sorted(want.items()):
                self.known[((pos, 1),)] = self.block(*pos)
                terms.append((c, self.known[((pos, 1),)]))
            self.known[key] = _signed_sum(terms)
        return self.known[key]


class _Sums:
    def __init__(self, done):
        self.done, self.acc = done, {}

    def add(self, key, sign, value, expected):
        if not sign:
            return
        count, neg, tot = self.acc.pop(key, (0, sign < 0, value))
        if count and neg == (sign < 0):
            tot = tot + value
        elif count:
            tot, neg = (value - tot if neg else tot - value), False
        if count + 1 == expected:
            self.done(key, -tot if neg else tot)
        else:
            self.acc[key] = (count + 1, neg, tot)


class _Carry:
    def __init__(self, ref):
        self.ref, self.val = ref, {}

    def __getitem__(self, key):
        return self.val[key] if key in self.val else self.ref[key]

    def __setitem__(self, key, value):
        self.val[key] = value

    def flush(self):
        for key, value in self.val.items():
            self.ref[key] = value
        self.val = {}


def _dot(a, b):
    return lax.dot_general(a, b, (((1,), (0,)), ((), ())), preferred_element_type=F32)


def _dot_nt(a, b):
    return lax.dot_general(a, b, (((1,), (1,)), ((), ())), preferred_element_type=F32)


def _tile(ref, *idx):
    return pltpu.bitcast(ref.bitcast(U32)[idx], BF16)


def _stack(*parts):
    parts = [t for t in parts if t is not None]
    return parts[0] if len(parts) == 1 else jnp.concatenate(parts, axis=0)


def _low_half(rows):
    return lax.broadcasted_iota(jnp.int32, (rows, LANES), 1) < 64


def _pair_lhs(t1, t2):
    lo = _low_half(t1[3].shape[0])
    diff = t1[3] - t2[3]
    return (t1[:3] + [jnp.where(lo, t1[4], diff)]
            + t2[:3] + [jnp.where(lo, -diff, t2[4])]
            + [jnp.where(lo, t1[3], t2[3])])


def _pair_rhs(x):
    a, b, c = x[384:448], x[448:512], x[512:576]
    cat = lambda u, v: jnp.concatenate([u, v], axis=0)
    return [x[i * 128:(i + 1) * 128] for i in range(3)] + [cat(c, b), cat(a, c), x[384:512]]


def _pair_matmul(lhs, rhs, dot):
    out = [dot(lhs(8), rhs[5])] * 2
    for i in range(8):
        out[i // 4] = out[i // 4] + dot(lhs(i), rhs[i % 4 if i < 7 else 4])
    return out


def _kernel(xt_hbm, wqkv_hbm, wo_hbm, mem0_hbm, wq_hbm, wk_hbm, wv_hbm, wot_hbm, gate_hbm,
            out_hbm,
            xt_v, wqkv_v, wo_v, stg_qkv, stg_o, wo_t, wt32, wo32_s, la, lo_a, kv_prev, oa_s,
            wb, x32, ga_s, gm_s, mem_s, part_s, o_s, opart_s, b_s, out_v, mem0_v, gate_v,
            sem_in, sem_out, *, seq, seg, mem):
    nt = seq // LANES
    rows = mem + seg

    sems = (sem_in.at[n] for n in itertools.count(3 * GP))
    copy = pltpu.make_async_copy
    cp_wqkv = {k: copy(wqkv_hbm.at[k * LANES:min(D, (k + 1) * LANES)],
                       wqkv_v.at[k * LANES:min(D, (k + 1) * LANES)], next(sems))
               for k in (3, 4, 0, 1, 2)}
    cp_wo = copy(wo_hbm, wo_v, next(sems))
    cp_x = {j0: [copy(xt_hbm.at[:, j * LANES:(j + 1) * LANES], xt_v.at[j], sem)
                 for j in range(j0, j1)] for j0, j1, sem in zip(XCUT, XCUT[1:] + (nt,), sems)}
    cp_wot = copy(wot_hbm, stg_o, next(sems))
    cp_small = [copy(mem0_hbm, mem0_v, next(sems)), copy(gate_hbm, gate_v, next(sems))]
    queue = cp_small + list(cp_wqkv.values()) + cp_x[0] + [cp_wo]
    for unit in range(3 * GP):
        src = (wq_hbm, wk_hbm, wv_hbm)[unit // GP].bitcast(U32)
        queue += cp_x.get(unit + 1, []) + [
            copy(src.at[:, KB * (unit % GP) + p, :], stg_qkv.at[unit, p], sem_in.at[unit])
            for p in range(KB)]
    for c in queue + [cp_wot]:
        c.start()

    def wait_all(copies):
        for c in copies:
            c.wait()

    def cp_out(j):
        col = j * LANES if isinstance(j, int) else pl.multiple_of(j * LANES, LANES)
        return copy(out_v.at[j], out_hbm.at[:, pl.ds(col, LANES)], sem_out)

    for ref in (o_s, opart_s, b_s):
        ref[...] = jnp.zeros(ref.shape, ref.dtype)
    wait_all(cp_small)
    m0 = mem0_v[...].astype(F32)
    for kk in range(KB):
        mem_s[kk] = m0[:, kk * LANES:(kk + 1) * LANES]
    mem_s[KB] = jnp.concatenate([m0[:, KB * LANES:], jnp.zeros((mem, 64), F32)], axis=1)
    wb[4 * GP, 0, 0:16, :] = jnp.zeros((16, LANES), BF16)

    gate = jnp.broadcast_to(gate_v[...].astype(F32).reshape(1, D), (8, D))
    gate_t = [gate[:, i * 128:(i + 1) * 128] for i in range(4)]
    gate_t.append(jnp.concatenate([gate[:, 512:], gate[:, 512:]], axis=1))

    entries = [None] * 2 + [(g - part // 2, part, n) for g in range(NG + 1) for n in range(DA // 2)
                            for part in (1, 0, 2) if 0 <= g - part // 2 < NG]

    def feature_rows(k, e):
        return _stack(*(gate_t[k] if ent is None else
                       wt32[k, pl.ds(ent[1] * D + ent[0] * 8 * DA + 2 * ent[2] + e, 8, stride=DA), :]
                       for ent in entries))

    for k in cp_wqkv:
        cp_wqkv[k].wait()
        rows_k = wqkv_v[k * LANES:min(D, (k + 1) * LANES), :]
        wt32[k, 0:3 * D] = (rows_k if k < 4 else _stack(rows_k, rows_k)).T.astype(F32)
        for e in range(2 if k < 3 else 0):
            la[4 * e + k] = feature_rows(k, e).astype(BF16)
        if k == 4:
            mixed = _pair_lhs(*([None] * 3 + [feature_rows(3, e), feature_rows(4, e)]
                                for e in range(2)))
            for i in (3, 7, 8):
                la[i] = mixed[i].astype(BF16)

    def prep_wo():
        wo32 = wo_v[...].astype(F32)
        for n in range(4):
            wo32_s[n, 0:D] = wo32[:, n * LANES:(n + 1) * LANES]
        wo32_s[4, 0:D] = jnp.concatenate([wo32[:, 4 * LANES:]] * 2, axis=1)
        turned = []
        for n in range(5):
            perm = _stack(*(wo32_s[n, pl.ds(g * 8 * DA + d, 8, stride=DA), :]
                           for g in range(NG) for d in range(DA))).astype(BF16)
            turned.append([perm[k * LANES:(k + 1) * LANES].T for k in range(4)]
                          + [_stack(perm[4 * LANES:], perm[4 * LANES:]).T])
        tiles = [_stack(*(t[k] for t in turned))[:D].astype(F32) for k in range(5)]
        for i, t in enumerate(_pair_lhs([t[:D // 2] for t in tiles], [t[D // 2:] for t in tiles])):
            lo_a[i] = t.astype(BF16)

    def prep_qkv(unit):
        src, dst = stg_qkv.at[unit], wb.at[unit]

        def rows(g, r0, nu):
            u = src[2 * g + nu // 2, r0:r0 + 16, :]
            return pltpu.bitcast(u & jnp.uint32(0xFFFF0000) if nu % 2 else u << 16, F32)

        for e in range(8):
            at, own, shared = pl.ds(16 * e, 16), e // 4, {}
            for g in (own, 1 - own):
                mix = _Mixer(lambda kk, nu: rows(g, kk * LANES + 16 * e, nu))
                for r in ORD:
                    w = mix(_V[r])
                    if r < NH and g == own:
                        shared[r] = w.astype(BF16)
                        dst[2 * NR + r, at, :] = shared[r]
                        w = rows(g, KB * LANES + 16 * (e % 4), r // 2)
                    elif r < NH:
                        w = w - shared[r].astype(F32)
                    dst[g * NR + r, at, :] = w.astype(BF16)
                yield

    def turn_out(gp):
        words = lambda head, r0, n: _tile(stg_o, 2 * KB * gp + head, pl.ds(r0 // 2, n // 2))
        for head in range(2 * KB + 1):
            for nu in range(KB):
                if head < 2 * KB:
                    tile = words(head, nu * LANES, LANES)
                else:
                    tile = _stack(*(words(g * KB + nu, KB * LANES, 64) for g in range(2)))
                wo_t[gp, head, nu] = pltpu.bitcast(tile.T, U32)

    def prep_out(gp):
        dst, lo = wb.at[3 * GP + gp], _low_half(16)
        for e in range(8):
            at, first = pl.ds(16 * e, 16), {}
            rows = lambda head, nu: pltpu.bitcast(
                wo_t[gp, head, nu, 8 * e:8 * e + 8, :], BF16).astype(F32)
            for g in range(2):
                mix = _Mixer(lambda kk, nu: rows(g * KB + kk, nu))
                for r in ORD:
                    w = mix(_V[r])
                    if r >= NH:
                        dst[g * NR + r, at, :] = w.astype(BF16)
                    elif g == 0:
                        first[r] = w
                    else:
                        z, t = jnp.where(lo, first[r], w).astype(BF16), rows(2 * KB, r // 2)
                        dst[2 * NR + r, at, :] = z
                        dst[r, at, :] = jnp.where(lo, t, first[r] - z.astype(F32)).astype(BF16)
                        dst[NR + r, at, :] = jnp.where(lo, w - z.astype(F32), t).astype(BF16)
                yield

    lane = lax.broadcasted_iota(jnp.int32, (8, LANES), 1)

    def exchange(idx, pair, first):
        at = pl.ds(8 * idx, 8)
        prev = None if first else kv_prev.bitcast(U32)[at, :]
        kv_prev[16 * idx:16 * idx + 16, :] = jnp.concatenate(pair, axis=0).astype(BF16)
        cur = kv_prev.bitcast(U32)[at, :]
        return (jnp.broadcast_to(cur[:, 0:1], (8, LANES)) if first else prev), cur

    def to_rows(j):
        t0 = j * LANES if isinstance(j, int) else pl.multiple_of(j * LANES, LANES)
        xt = _tile(xt_v, j)
        for kk in range(KB + 1):
            tile = xt[kk * LANES:(kk + 1) * LANES]
            x32[kk, pl.ds(t0, LANES), :] = (tile if kk < KB else _stack(tile, tile)).T.astype(F32)

    def paced(job, src, dst, when, back):
        results = []

        def dot(left, right):
            if len(results) in when:
                if len(results) >= back:
                    src[...] = pltpu.bitcast(results[-back][0:8], U32)
                next(job, None)
                left = _stack(left[:-8] if len(left) > 8 else None, left[-8:] | dst[...])
            results.append(_dot(pltpu.bitcast(left, BF16), right))
            return results[-1]

        return dot

    spare_qkv, spare_t = stg_qkv.at[3 * GP, 0, 0:8], wo_t.at[GP, 0, 1, 0:8]
    zero_w = wb.bitcast(U32).at[4 * GP, 0, 0:8]

    def a_out(j, dot):
        rhs = _pair_rhs(_tile(oa_s, slice(None)))
        for r0 in range(0, D // 2, RO):
            halves = _pair_matmul(lambda i: lo_a.bitcast(U32)[i, r0 // 2:(r0 + RO) // 2, :], rhs, dot)
            for e in range(2):
                ga_s[j, pl.ds(e * D // 2 + r0, RO), :] = halves[e]

    def a_tile(j, first, dot):
        rhs = _pair_rhs(_tile(xt_v, j))
        logit, prob, outs = {}, {}, {}
        for e0 in range(0, len(entries), RE):
            some = entries[e0:e0 + RE]
            halves = _pair_matmul(
                lambda i: la.bitcast(U32)[i, 4 * e0:4 * (e0 + len(some)), :], rhs, dot)
            for ent, r0 in zip(some, range(0, 8 * RE, 8)):
                pair = [t[r0:r0 + 8] for t in halves]
                if ent is None:
                    gsig = 1.0 / (1.0 + jnp.exp(-halves[0][0:8]))
                    continue
                g, part, n = ent
                if part:
                    prev, cur = exchange((2 * g + part - 1) * (DA // 2) + n, pair, first)
                    back = [cur] + [
                        pltpu.roll(jnp.where(lane >= LANES - DIL * w, prev, cur), DIL * w, 1)
                        for w in range(1, WIN)]
                    back = [pltpu.bitcast(t, BF16).astype(F32) for t in back]
                if part == 2:
                    outs[g, n] = functools.reduce(
                        jnp.add, [_stack(p, p) * t for p, t in zip(prob[g], back)]).astype(BF16)
                elif part == 0:
                    terms = [pair[0] * t[0:8] + pair[1] * t[8:16] for t in back]
                    logit[g] = terms if n == 0 else [a + t for a, t in zip(logit[g], terms)]
                if (part, n) == (0, DA // 2 - 1):
                    s = [jnp.where(lane >= DIL * w, t, NEG * DA ** 0.5) if first else t
                         for w, t in enumerate(logit[g])]
                    top = functools.reduce(jnp.maximum, s)
                    ex = [jnp.exp2((t - top) * (DA ** -0.5 * LOG2E)) for t in s]
                    inv = gsig / functools.reduce(jnp.add, ex)
                    prob[g] = [t * inv for t in ex]
        gm_s[j] = 1.0 - gsig
        if not first:
            a_out(j - 1, dot)
        oa_s[...] = _stack(*(outs[key] for key in sorted(outs)))

    plain = lambda left, right: _dot(pltpu.bitcast(left, BF16), right)
    wait_all(cp_x[0])
    to_rows(0)
    a_tile(0, True, plain)
    cp_wo.wait()
    wait_all(cp_x[1])
    prep_wo()
    a_tile(1, False, plain)
    to_rows(1)

    def a_loop(first, count, work, spare, loading):
        def body(j, carry):
            if loading:
                for j0 in XCUT[2:]:
                    pl.when(j == j0)(functools.partial(wait_all, cp_x[j0]))
                copy(stg_qkv.at[j - first], stg_qkv.at[j - first], sem_in.at[j - first]).wait()
                to_rows(j)
            job = work(j - first)
            a_tile(j, False, paced(job, spare, zero_w, *(QA if loading else QB)))
            list(job)
            return carry

        lax.fori_loop(first, first + count, body, 0)

    a_loop(2, 3 * GP, prep_qkv, spare_qkv, True)

    qi = lax.broadcasted_iota(jnp.int32, (rows, rows), 0)
    ki = lax.broadcasted_iota(jnp.int32, (rows, rows), 1)
    mask = (qi >= seg) | (ki >= seg) | (qi >= ki)
    part, o_prev, opart, b_rows = (_Carry(r) for r in (part_s, o_s, opart_s, b_s))
    ahead = {}

    def b_step(u, t0, memv, project_only=False, output_only=False):
        odd = u % 2
        keep = lambda slots: [s for s in slots if s["tok"] or memv]
        qs, os_ = keep(_PHASES[odd]), keep(_PHASES[1 - odd])
        lhs, shared, tok, mrow, full, soft, o_mem, o_mix, o_left, o_host, new = ({} for _ in range(11))

        def spread(sums, key, slots, s, tok_rows, mem_rows):
            for nu in range(KB):
                if memv:
                    sums.add(key + (nu, 2), s["c"][nu], mem_rows, sum(abs(o["c"][nu]) for o in slots))
                for mu in range(2 if s["tok"] else 0):
                    sums.add(key + (nu, mu), _C[s["r"]][mu][nu], tok_rows,
                             sum(abs(_C[o["r"]][mu][nu]) for o in slots if o["tok"]))

        x_mix = _Mixer(lambda mu, kk: x32[kk, pl.ds(t0 + mu * seg, seg), :])
        c_mix = _Mixer(lambda mu, _: x32[KB, pl.ds(t0 + mu * seg, seg), :])
        m_mix = _Mixer(lambda _, kk: memv[kk])
        m_tail = memv[KB] + pltpu.roll(memv[KB], 64, 1) if memv else None

        def q_left(e, t):
            s = qs[e]
            if (e, t) not in lhs:
                left = _stack(x_mix(_U[s["r"]]) if s["tok"] else None,
                             m_mix([s["a"]]) if memv else None)
                if s["r"] < NH and t < 2:
                    c = _stack(c_mix(_TAIL_IN[s["r"]][:, None]),
                              _signed_sum([(sum(s["c"]), m_tail)]) if memv else None)
                    left = jnp.where(_low_half(c.shape[0]), *((c, left), (left, c))[t])
                lhs[e, t] = left
            return lhs[e, t]

        def q_total(key, value):
            i, g, nu, mu = key
            h = g * KB + nu
            if mu == 2:
                mrow[i, h] = value
            elif odd:
                part[i, h, mu] = value
            elif mu == 0:
                tok[i, h] = value + part[i, h, mu]
            else:
                ahead[i, h] = value + part[i, h, mu]
            cur = (ahead if odd else tok).get((i, h))
            if (i, h) in mrow and cur is not None and (i, h) not in full:
                full[i, h] = _stack(cur, mrow[i, h]).astype(BF16 if i else F32)

        q_sums = _Sums(q_total)

        def q_pass(e, i, gp, t):
            s = qs[e]
            p = _dot(q_left(e, t), _tile(wb, i * GP + gp, t * NR + s["r"]))
            if t == 2:
                shared[e, i, gp] = p
                return
            if s["r"] < NH:
                p = p + shared[e, i, gp]
            spread(q_sums, (i, 2 * gp + t), qs, s, p[:seg], p[-mem:])

        def scores(h):
            s = jnp.where(mask, _dot_nt(full[0, h], full[1, h]), NEG * DB ** 0.5)
            e = jnp.exp2((s - jnp.max(s, axis=-1, keepdims=True)) * (DB ** -0.5 * LOG2E))
            total = jnp.sum(e, axis=-1, keepdims=True)
            inv = pltpu.reciprocal(total, approx=True)
            soft[h] = e * (inv * (2.0 - total * inv))

        def values(h):
            o = _dot(soft[h], full[2, h])
            o_mem[h] = o[seg:]
            if odd:
                o_prev[0, h], o_prev[1, h] = ahead["o", h], o[:seg]
            else:
                ahead["o", h] = o[:seg]

        def o_rows(e, gp, t):
            s = os_[e]
            if (e, gp, t) not in o_left:
                g = 2 * gp + t
                if t == 2:
                    o_left[e, gp, t] = o_rows(e, gp, 0) + o_rows(e, gp, 1)
                    return o_left[e, gp, t]
                if g not in o_mix:
                    o_mix[g] = (_Mixer(lambda _, kk: o_mem[g * KB + kk]),
                                _Mixer(lambda mu, kk: o_prev[mu, g * KB + kk]))
                o_left[e, gp, t] = _stack(o_mix[g][0]([s["a"]]) if memv else None,
                                         o_mix[g][1](_U[s["r"]]) if s["tok"] else None)
            return o_left[e, gp, t]

        def o_total(key, value):
            nu, mu = key
            if mu == 2:
                new[nu] = value
            elif odd:
                opart[nu, mu] = value
            else:
                b_rows[nu, (u - 2) % 4 + mu] = value + opart[nu, mu]

        out_sums = _Sums(o_total)

        def o_product(key, value):
            e, t = key
            s = os_[e]
            if s["r"] < NH:
                o_host[key] = value
                if any((e, t_) not in o_host for t_ in range(3)):
                    return
                lo = _low_half(value.shape[0])
                value = o_host[e, 2] + jnp.where(lo, o_host[e, 1], o_host[e, 0])
                y = jnp.where(lo, o_host[e, 0], o_host[e, 1])
                if memv:
                    out_sums.add((KB, 2), sum(s["a"]), y[:mem], KB)
                for mu in range(2):
                    out_sums.add((KB, mu), _TAIL_OUT[s["r"]][mu], y[-seg:],
                                 sum(abs(_TAIL_OUT[o["r"]][mu]) for o in os_ if o["r"] < NH))
            spread(out_sums, (), os_, s, value[-seg:], value[:mem])

        o_sums = _Sums(o_product)

        def o_pass(e, gp, t):
            host = os_[e]["r"] < NH
            p = _dot(o_rows(e, gp, t), _tile(wb, 3 * GP + gp, t * NR + os_[e]["r"]))
            o_sums.add((e, t if host else 0), 1, p, GP if host else 2 * GP)

        todo = []
        tiles = lambda s: (2, 0, 1) if s["r"] < NH else (0, 1)
        if not output_only:
            todo = [(s["tok"], q_pass, e, i, gp, t) for gp in range(GP) for i in (1, 0, 2)
                    for e, s in enumerate(qs) for t in tiles(s)]
            last = [max(e for e, s in enumerate(_PHASES[odd]) if s["tok"] and s["c"][nu])
                    for nu in range(KB)]
            ready = lambda e, t: 99 if qs[e]["r"] < NH and t < 2 else max(
                last[kk] for kk in range(KB) if qs[e]["a"][kk])
            todo[:HEAD[odd]] = sorted(todo[:HEAD[odd]], key=lambda p: ready(p[2], p[5]))
        if not project_only:
            todo += [(s["tok"], o_pass, e, gp, t) for pairs in ((0, 1), (2, 3)) for e, s in enumerate(os_)
                     for gp in pairs for t in tiles(s)]
        long_, short = ([p[1:] for p in todo if p[0] == tok] for tok in (True, False))
        extra = {}
        for h in range(HB if memv else 0):
            extra.setdefault(SCORE_AT[odd][h // 2], []).append((scores, h))
            extra.setdefault(VALUE_AT[odd][h // 2], []).append((values, h))
        issued = 0
        for n, p in enumerate(long_):
            for fn, *args in extra.get(n, []) + [p]:
                if issued % 4 == 0 and short and n >= SHORT_AT[odd][-len(short) // 4]:
                    for fn_s, *args_s in short[:4]:
                        fn_s(*args_s)
                    del short[:4]
                fn(*args)
                issued += 1
        assert not short
        return new

    def emit_tile(j):
        for nu in range(KB + 1):
            bt = jnp.concatenate([b_s[nu, 0], b_s[nu, 1], b_rows.val.pop((nu, 2)),
                                  b_rows.val.pop((nu, 3))], axis=0).T
            bt = bt if nu < KB else bt[:64] + bt[64:]
            at = pl.ds(nu * LANES, bt.shape[0])
            gm = jnp.concatenate([gm_s[j]] * (bt.shape[0] // 8), axis=0)
            out_v[j, at, :] = (ga_s[j, at, :] + gm * bt).astype(out_v.dtype)

    cp_wot.wait()
    for gp in range(GP):
        turn_out(gp)
    b_step(3, 0, None, project_only=True)
    part.flush()
    for j in range(3 * GP + 2, nt):
        to_rows(j)
    a_loop(3 * GP + 2, GP - 2, prep_out, spare_t, False)
    job = itertools.chain(prep_out(GP - 2), prep_out(GP - 1))
    a_out(nt - 1, paced(job, spare_t, zero_w, *QC))
    list(job)

    def b_body(j, carry):
        memv = {kk: mem_s[kk] for kk in range(KB + 1)}
        for u in range(4):
            t0 = jnp.minimum(j * LANES + (u + 1) // 2 * 2 * seg, seq - 2 * seg)
            memv = b_step(u, pl.multiple_of(t0, seg), memv)
            if u == 0:
                emit_tile(jnp.maximum(j - 1, 0))
        for kk, t in memv.items():
            mem_s[kk] = t
        for c in (part, o_prev, opart, b_rows):
            c.flush()
        pl.when(j > 0)(lambda: cp_out(j - 1).start())
        return carry

    lax.fori_loop(0, nt, b_body, 0)
    b_step(0, None, None, output_only=True)
    emit_tile(nt - 1)
    cp_out(nt - 1).start()
    for j in range(nt):
        cp_out(j).wait()


@functools.partial(jax.jit, static_argnames=("B_seg_len",))
def pallas_gated_mix__sliding_local_dilated__memory_aug_recurrent_mem_tr__prompt_kernel(
    A_x: jax.Array,
    A_wqkv: jax.Array,
    A_wo: jax.Array,
    B_x: jax.Array,
    B_mem0: jax.Array,
    B_Wq: jax.Array,
    B_Wk: jax.Array,
    B_Wv: jax.Array,
    B_Wo: jax.Array,
    B_seg_len: int,
    gate_w: jax.Array,
):
    del B_x
    batch, seq, width = A_x.shape
    mem, seg = B_mem0.shape[1], int(B_seg_len)
    nt = seq // LANES
    assert batch == 1 and width == D and nt == 4 * GP and seq % LANES == 0
    assert B_Wq.shape == (D, HB, DB) and mem == 8 and 4 * seg == LANES

    hbm = pl.BlockSpec(memory_space=pl.ANY)
    out_t = pl.pallas_call(
        functools.partial(_kernel, seq=seq, seg=seg, mem=mem),
        out_shape=jax.ShapeDtypeStruct((D, seq), A_x.dtype),
        in_specs=[hbm] * 9,
        out_specs=hbm,
        scratch_shapes=[
            pltpu.VMEM((nt, D, LANES), BF16),
            pltpu.VMEM((D, 3 * D), BF16),
            pltpu.VMEM((D, D), BF16),
            pltpu.VMEM((3 * GP + 1, KB, D, DB), U32),
            pltpu.VMEM((HB, D, DB), BF16),
            pltpu.VMEM((GP + 1, 2 * KB + 1, KB, 64, LANES), U32),
            pltpu.VMEM((5, 3 * D + 32, LANES), F32),
            pltpu.VMEM((5, D + 32, LANES), F32),
            pltpu.VMEM((12, 3 * D // 2 + 16, LANES), BF16),
            pltpu.VMEM((12, D // 2, LANES), BF16),
            pltpu.VMEM((2 * D, LANES), BF16),
            pltpu.VMEM((D, LANES), BF16),
            pltpu.VMEM((4 * GP + 1, 2 * NR + NH, LANES, LANES), BF16),
            pltpu.VMEM((KB + 1, seq, LANES), F32),
            pltpu.VMEM((nt, D, LANES), F32),
            pltpu.VMEM((nt, 8, LANES), F32),
            pltpu.VMEM((2 * KB, mem, LANES), F32),
            pltpu.VMEM((3, HB, 2, seg, LANES), F32),
            pltpu.VMEM((2, HB, seg, LANES), F32),
            pltpu.VMEM((KB + 1, 2, seg, LANES), F32),
            pltpu.VMEM((KB + 1, 2, seg, LANES), F32),
            pltpu.VMEM((nt, D, LANES), A_x.dtype),
            pltpu.VMEM((mem, D), BF16),
            pltpu.VMEM((D,), BF16),
            pltpu.SemaphoreType.DMA((3 * GP + 9 + len(XCUT),)),
            pltpu.SemaphoreType.DMA(()),
        ],
        compiler_params=pltpu.CompilerParams(vmem_limit_bytes=110 * 1024 * 1024),
        name="gated_mix_kernel",
    )(A_x.reshape(seq, D).T, A_wqkv, A_wo, B_mem0.reshape(mem, D), B_Wq, B_Wk, B_Wv,
      B_Wo.transpose(0, 2, 1), gate_w)
    return out_t.T.reshape(batch, seq, D)
```

```python
import functools
import itertools

import jax
import jax.numpy as jnp
import numpy as np
from jax import lax
import jax.experimental.pallas as pl
import jax.experimental.pallas.tpu as pltpu

F32, BF16, U32 = jnp.float32, jnp.bfloat16, jnp.uint32

D = 576
LANES = 128
HA, DA = 32, 18
WIN, DIL = 8, 2
HB, DB = 32, 128
NEG = -1000000000.0
LOG2E = 1.4426950408889634
NG = HA // 8

KB = 4
GP = HB // (2 * KB)

_HK = (
    (".... +...", "+.-. -... .... -...", "+... +..."),
    ("+... -...", "+-.- .... -... ....", "+... ...."),
    (".+.. .-..", ".... +-.. .+.. ....", ".... .+.."),
    (".+.. ....", ".-.. .+-. .... ....", ".+.. .+.."),
    (".... ..+.", ".... ..-. -.+. .+-.", ".... ..+."),
    ("..+. ....", "..-. ...+ .-+- ....", "..+. ...."),
    ("...+ ...-", ".... ...- ...+ ++.-", ".... ...+"),
    ("...+ ....", "...- ...- .... .+-+", "...+ ...+"),
    (".... ++..", ".... +... .... ....", ".... ++.."),
    ("++.. ....", ".+.. .... .... ....", "++.. ...."),
    (".+.. +...", ".-.. +... .... ....", "+... .-.."),
    ("+.+. -.-.", ".... .... -... ....", ".... +.+."),
    ("+.+. ....", "..+. .... .... ....", "+.+. +.+."),
    ("+.+. -...", "..-. .... +... ....", "+... +.+."),
    (".... +..+", ".... .... .... +...", ".... +..+"),
    ("+..+ ....", "...+ .... .... ....", "+..+ ...."),
    ("...+ +...", "...- .... .... +...", "+... ...-"),
    (".... .++.", ".... ..+. .... .-..", ".++. .++."),
    (".++. .--.", ".... ...- .+.. ....", ".++. ...."),
    (".+.. .--.", ".... ..+. .-.. ....", ".++. .+.."),
    (".... ..++", ".... .... .... .-+.", "..++ ..++"),
    ("..++ ..--", ".... ...- ...+ ....", "..++ ...."),
    ("...+ ..--", ".... ...+ ...- .-+.", "..++ ...+"),
    (".... .+++", ".... .... .... .+..", ".... .+++"),
    (".+++ ....", ".... ...+ .... ....", ".+++ ...."),
    ("...+ .++.", ".... ...- .... .+..", ".++. ...-"),
)
_U, _V, _C = (np.array([[["-.+".index(ch) - 1 for ch in row] for row in prod[i].split()]
                        for prod in _HK]) for i in range(3))
NR = len(_HK)
assert np.array_equal(np.einsum("rak,rln,rbm->akblnm", _U, _V, _C),
                      np.einsum("ab,kl,nm->akblnm", *(np.eye(n, dtype=int) for n in (2, KB, KB))))


def _phase(products):
    tiles = [max(r, ~r) for r in products]
    dual = np.rint(np.linalg.inv(_V[tiles].reshape(len(tiles), -1)).T).astype(int)
    slots = []
    for r, d in zip(products, dual.reshape(-1, KB, KB)):
        i, j = np.argwhere(d)[0]
        a, c = d[:, j] * d[i, j], d[i]
        assert np.array_equal(np.outer(a, c), d)
        slots.append(dict(r=max(r, ~r), tok=r >= 0, a=a.tolist(), c=c.tolist()))
    return slots


_PHASES = (_phase((11, 8, ~9, 4, 2, 23, 17, ~13, 25, 20, 22, 7, ~19, 16, 15, 1)),
           _phase((24, 21, ~16, 18, 19, 3, 10, ~22, 9, 5, 12, 13, ~25, 0, 14, 6)))
assert sorted(s["r"] for ph in _PHASES for s in ph if s["tok"]) == list(range(NR))

NH = 2 * KB
assert all(sorted(s["r"] // 2 for s in ph if s["r"] < NH) == list(range(KB)) for ph in _PHASES)
assert all(np.abs(s[k]).tolist() == np.eye(KB)[s["r"] // 2].tolist()
           for ph in _PHASES for s in ph if s["r"] < NH for k in "ac")
_TAIL_IN, _TAIL_OUT = (
    np.concatenate([np.rint(np.linalg.inv(t[2 * n:2 * n + 2, :, n]).T).astype(int)
                    for n in range(KB)]) for t in (_C, _U))


SCORE_AT = ((76, 94, 116, 138, 162, 184, 206, 228,
             252, 274, 296, 318, 342, 344, 346, 348),
            (72, 94, 116, 138, 162, 184, 206, 228,
             252, 274, 296, 318, 342, 344, 346, 348))
VALUE_AT = ((112, 134, 156, 182, 202, 224, 252, 268,
             294, 314, 336, 358, 382, 384, 386, 388),
            (112, 134, 156, 182, 202, 224, 246, 268,
             292, 310, 336, 356, 382, 384, 386, 388))
SHORT_AT = ((6, 26, 46, 66, 86, 106, 126, 146, 166, 186, 206, 226,
             246, 266, 286, 306, 326, 346, 364, 385, 410, 426, 444, 463),
            (6, 26, 46, 66, 86, 106, 126, 146, 170, 186, 206, 226,
             246, 266, 286, 306, 326, 346, 360, 385, 410, 426, 440, 463))
HEAD = (72, 66)
XCUT = (0, 1, 3, 8)
RE, RO = 8, 48
ORD = (9, 8, 10, 19, 2, 3, 23, 24, 25, 17, 18, 20, 21, 22, 12, 11, 13, 4, 5, 15, 14, 16, 6, 7, 0, 1)
QA = ((4, 10, 22, 26, 39, 42, 63, 80, 94, 149, 158, 162, 165, 169, 172), 24)
QB = ((10, 13, 22, 42, 52, 73, 90, 109, 146, 155, 160, 166, 171, 176, 179), 32)
QC = ((4, 5, 7, 11, 14, 16, 21, 24, 28, 32, 35, 37, 41, 44, 48, 52), 12)


def _signed_sum(terms):
    terms = [(c, t) for c, t in terms if c]
    first = next((i for i, (c, _) in enumerate(terms) if c > 0), 0)
    c, acc = terms.pop(first)
    acc = acc if c > 0 else -acc
    for c, t in terms:
        acc = acc + t if c > 0 else acc - t
    return acc


class _Mixer:
    def __init__(self, block):
        self.block, self.known = block, {}

    def __call__(self, coef):
        want = {(i, k): int(c) for i, row in enumerate(coef) for k, c in enumerate(row) if c}
        key = tuple(sorted(want.items()))
        if key not in self.known:
            terms = []
            for have in sorted(self.known, key=lambda h: -len(h)):
                for sign in (1, -1):
                    if all(want.get(pos) == sign * c for pos, c in have):
                        terms.append((sign, self.known[have]))
                        want = {pos: c for pos, c in want.items() if pos not in dict(have)}
                        break
            for pos, c in sorted(want.items()):
                self.known[((pos, 1),)] = self.block(*pos)
                terms.append((c, self.known[((pos, 1),)]))
            self.known[key] = _signed_sum(terms)
        return self.known[key]


class _Sums:
    def __init__(self, done):
        self.done, self.acc = done, {}

    def add(self, key, sign, value, expected):
        if not sign:
            return
        count, neg, tot = self.acc.pop(key, (0, sign < 0, value))
        if count and neg == (sign < 0):
            tot = tot + value
        elif count:
            tot, neg = (value - tot if neg else tot - value), False
        if count + 1 == expected:
            self.done(key, -tot if neg else tot)
        else:
            self.acc[key] = (count + 1, neg, tot)


class _Carry:
    def __init__(self, ref):
        self.ref, self.val = ref, {}

    def __getitem__(self, key):
        return self.val[key] if key in self.val else self.ref[key]

    def put(self, key, value, store):
        self.val[key] = value
        if store:
            self.ref[key] = value


def _dot(a, b):
    return lax.dot_general(a, b, (((1,), (0,)), ((), ())), preferred_element_type=F32)


def _dot_nt(a, b):
    return lax.dot_general(a, b, (((1,), (1,)), ((), ())), preferred_element_type=F32)


def _tile(ref, *idx):
    return pltpu.bitcast(ref.bitcast(U32)[idx], BF16)


def _stack(*parts):
    parts = [t for t in parts if t is not None]
    return parts[0] if len(parts) == 1 else jnp.concatenate(parts, axis=0)


def _low_half(rows):
    return lax.broadcasted_iota(jnp.int32, (rows, LANES), 1) < 64


def _pair_lhs(t1, t2):
    lo = _low_half(t1[3].shape[0])
    diff = t1[3] - t2[3]
    return (t1[:3] + [jnp.where(lo, t1[4], diff)]
            + t2[:3] + [jnp.where(lo, -diff, t2[4])]
            + [jnp.where(lo, t1[3], t2[3])])


def _pair_rhs(x):
    a, b, c = x[384:448], x[448:512], x[512:576]
    cat = lambda u, v: jnp.concatenate([u, v], axis=0)
    return [x[i * 128:(i + 1) * 128] for i in range(3)] + [cat(c, b), cat(a, c), x[384:512]]


def _pair_matmul(lhs, rhs, dot):
    out = [dot(lhs(8), rhs[5])] * 2
    for i in range(8):
        out[i // 4] = out[i // 4] + dot(lhs(i), rhs[i % 4 if i < 7 else 4])
    return out


def _kernel(xt_hbm, wqkv_hbm, wo_hbm, mem0_hbm, wq_hbm, wk_hbm, wv_hbm, wot_hbm, gate_hbm,
            out_hbm,
            xt_v, wqkv_v, wo_v, stg_qkv, stg_o, wo_t, wt32, wo32_s, la, lo_a, kv_prev, oa_s,
            wb, x32, ga_s, gm_s, mem_s, part_s, o_s, opart_s, b_s, out_v, mem0_v, gate_v,
            sem_in, sem_out, *, seq, seg, mem):
    nt = seq // LANES
    rows = mem + seg

    sems = (sem_in.at[n] for n in itertools.count(3 * GP))
    copy = pltpu.make_async_copy
    cp_wqkv = {k: copy(wqkv_hbm.at[k * LANES:min(D, (k + 1) * LANES)],
                       wqkv_v.at[k * LANES:min(D, (k + 1) * LANES)], next(sems))
               for k in (3, 4, 0, 1, 2)}
    cp_wo = copy(wo_hbm, wo_v, next(sems))
    cp_x = {j0: [copy(xt_hbm.at[:, j * LANES:(j + 1) * LANES], xt_v.at[j], sem)
                 for j in range(j0, j1)] for j0, j1, sem in zip(XCUT, XCUT[1:] + (nt,), sems)}
    cp_wot = copy(wot_hbm, stg_o, next(sems))
    cp_small = [copy(mem0_hbm, mem0_v, next(sems)), copy(gate_hbm, gate_v, next(sems))]
    queue = cp_small + list(cp_wqkv.values()) + cp_x[0] + [cp_wo]
    for unit in range(3 * GP):
        src = (wq_hbm, wk_hbm, wv_hbm)[unit // GP].bitcast(U32)
        queue += cp_x.get(unit + 1, []) + [
            copy(src.at[:, KB * (unit % GP) + p, :], stg_qkv.at[unit, p], sem_in.at[unit])
            for p in range(KB)]
    for c in queue + [cp_wot]:
        c.start()

    def wait_all(copies):
        for c in copies:
            c.wait()

    def cp_out(j):
        col = j * LANES if isinstance(j, int) else pl.multiple_of(j * LANES, LANES)
        return copy(out_v.at[j], out_hbm.at[:, pl.ds(col, LANES)], sem_out)

    for ref in (o_s, opart_s, b_s):
        ref[...] = jnp.zeros(ref.shape, ref.dtype)
    wait_all(cp_small)
    m0 = mem0_v[...].astype(F32)
    for kk in range(KB):
        mem_s[kk] = m0[:, kk * LANES:(kk + 1) * LANES]
    mem_s[KB] = jnp.concatenate([m0[:, KB * LANES:], jnp.zeros((mem, 64), F32)], axis=1)
    wb[4 * GP, 0, 0:16, :] = jnp.zeros((16, LANES), BF16)

    gate = jnp.broadcast_to(gate_v[...].astype(F32).reshape(1, D), (8, D))
    gate_t = [gate[:, i * 128:(i + 1) * 128] for i in range(4)]
    gate_t.append(jnp.concatenate([gate[:, 512:], gate[:, 512:]], axis=1))

    entries = [None] * 2 + [(g - part // 2, part, n) for g in range(NG + 1) for n in range(DA // 2)
                            for part in (1, 0, 2) if 0 <= g - part // 2 < NG]

    def feature_rows(k, e):
        return _stack(*(gate_t[k] if ent is None else
                       wt32[k, pl.ds(ent[1] * D + ent[0] * 8 * DA + 2 * ent[2] + e, 8, stride=DA), :]
                       for ent in entries))

    for k in cp_wqkv:
        cp_wqkv[k].wait()
        rows_k = wqkv_v[k * LANES:min(D, (k + 1) * LANES), :]
        wt32[k, 0:3 * D] = (rows_k if k < 4 else _stack(rows_k, rows_k)).T.astype(F32)
        for e in range(2 if k < 3 else 0):
            la[4 * e + k] = feature_rows(k, e).astype(BF16)
        if k == 4:
            mixed = _pair_lhs(*([None] * 3 + [feature_rows(3, e), feature_rows(4, e)]
                                for e in range(2)))
            for i in (3, 7, 8):
                la[i] = mixed[i].astype(BF16)

    def prep_wo():
        wo32 = wo_v[...].astype(F32)
        for n in range(4):
            wo32_s[n, 0:D] = wo32[:, n * LANES:(n + 1) * LANES]
        wo32_s[4, 0:D] = jnp.concatenate([wo32[:, 4 * LANES:]] * 2, axis=1)
        turned = []
        for n in range(5):
            perm = _stack(*(wo32_s[n, pl.ds(g * 8 * DA + d, 8, stride=DA), :]
                           for g in range(NG) for d in range(DA))).astype(BF16)
            turned.append([perm[k * LANES:(k + 1) * LANES].T for k in range(4)]
                          + [_stack(perm[4 * LANES:], perm[4 * LANES:]).T])
        tiles = [_stack(*(t[k] for t in turned))[:D].astype(F32) for k in range(5)]
        for i, t in enumerate(_pair_lhs([t[:D // 2] for t in tiles], [t[D // 2:] for t in tiles])):
            lo_a[i] = t.astype(BF16)

    def prep_qkv(unit):
        src, dst = stg_qkv.at[unit], wb.at[unit]

        def rows(g, r0, nu):
            u = src[2 * g + nu // 2, r0:r0 + 16, :]
            return pltpu.bitcast(u & jnp.uint32(0xFFFF0000) if nu % 2 else u << 16, F32)

        for e in range(8):
            at, own, shared = pl.ds(16 * e, 16), e // 4, {}
            for g in (own, 1 - own):
                mix = _Mixer(lambda kk, nu: rows(g, kk * LANES + 16 * e, nu))
                for r in ORD:
                    w = mix(_V[r])
                    if r < NH and g == own:
                        shared[r] = w.astype(BF16)
                        dst[2 * NR + r, at, :] = shared[r]
                        w = rows(g, KB * LANES + 16 * (e % 4), r // 2)
                    elif r < NH:
                        w = w - shared[r].astype(F32)
                    dst[g * NR + r, at, :] = w.astype(BF16)
                yield

    def turn_out(gp):
        words = lambda head, r0, n: _tile(stg_o, 2 * KB * gp + head, pl.ds(r0 // 2, n // 2))
        for head in range(2 * KB + 1):
            for nu in range(KB):
                if head < 2 * KB:
                    tile = words(head, nu * LANES, LANES)
                else:
                    tile = _stack(*(words(g * KB + nu, KB * LANES, 64) for g in range(2)))
                wo_t[gp, head, nu] = pltpu.bitcast(tile.T, U32)

    def prep_out(gp):
        dst, lo = wb.at[3 * GP + gp], _low_half(16)
        for e in range(8):
            at, first = pl.ds(16 * e, 16), {}
            rows = lambda head, nu: pltpu.bitcast(
                wo_t[gp, head, nu, 8 * e:8 * e + 8, :], BF16).astype(F32)
            for g in range(2):
                mix = _Mixer(lambda kk, nu: rows(g * KB + kk, nu))
                for r in ORD:
                    w = mix(_V[r])
                    if r >= NH:
                        dst[g * NR + r, at, :] = w.astype(BF16)
                    elif g == 0:
                        first[r] = w
                    else:
                        z, t = jnp.where(lo, first[r], w).astype(BF16), rows(2 * KB, r // 2)
                        dst[2 * NR + r, at, :] = z
                        dst[r, at, :] = jnp.where(lo, t, first[r] - z.astype(F32)).astype(BF16)
                        dst[NR + r, at, :] = jnp.where(lo, w - z.astype(F32), t).astype(BF16)
                yield

    lane = lax.broadcasted_iota(jnp.int32, (8, LANES), 1)

    def exchange(idx, pair, first):
        at = pl.ds(8 * idx, 8)
        prev = None if first else kv_prev.bitcast(U32)[at, :]
        kv_prev[16 * idx:16 * idx + 16, :] = jnp.concatenate(pair, axis=0).astype(BF16)
        cur = kv_prev.bitcast(U32)[at, :]
        return (jnp.broadcast_to(cur[:, 0:1], (8, LANES)) if first else prev), cur

    def to_rows(j):
        t0 = j * LANES if isinstance(j, int) else pl.multiple_of(j * LANES, LANES)
        xt = _tile(xt_v, j)
        for kk in range(KB + 1):
            tile = xt[kk * LANES:(kk + 1) * LANES]
            x32[kk, pl.ds(t0, LANES), :] = (tile if kk < KB else _stack(tile, tile)).T.astype(F32)

    def paced(job, src, dst, when, back):
        results = []

        def dot(left, right):
            if len(results) in when:
                if len(results) >= back:
                    src[...] = pltpu.bitcast(results[-back][0:8], U32)
                next(job, None)
                left = _stack(left[:-8] if len(left) > 8 else None, left[-8:] | dst[...])
            results.append(_dot(pltpu.bitcast(left, BF16), right))
            return results[-1]

        return dot

    spare_qkv, spare_t = stg_qkv.at[3 * GP, 0, 0:8], wo_t.at[GP, 0, 1, 0:8]
    zero_w = wb.bitcast(U32).at[4 * GP, 0, 0:8]

    def a_out(j, dot):
        rhs = _pair_rhs(_tile(oa_s, slice(None)))
        for r0 in range(0, D // 2, RO):
            halves = _pair_matmul(lambda i: lo_a.bitcast(U32)[i, r0 // 2:(r0 + RO) // 2, :], rhs, dot)
            for e in range(2):
                ga_s[j, pl.ds(e * D // 2 + r0, RO), :] = halves[e]

    def a_tile(j, first, dot):
        rhs = _pair_rhs(_tile(xt_v, j))
        logit, prob, outs = {}, {}, {}
        for e0 in range(0, len(entries), RE):
            some = entries[e0:e0 + RE]
            halves = _pair_matmul(
                lambda i: la.bitcast(U32)[i, 4 * e0:4 * (e0 + len(some)), :], rhs, dot)
            for ent, r0 in zip(some, range(0, 8 * RE, 8)):
                pair = [t[r0:r0 + 8] for t in halves]
                if ent is None:
                    gsig = 1.0 / (1.0 + jnp.exp(-halves[0][0:8]))
                    continue
                g, part, n = ent
                if part:
                    prev, cur = exchange((2 * g + part - 1) * (DA // 2) + n, pair, first)
                    back = [cur] + [
                        pltpu.roll(jnp.where(lane >= LANES - DIL * w, prev, cur), DIL * w, 1)
                        for w in range(1, WIN)]
                    back = [pltpu.bitcast(t, BF16).astype(F32) for t in back]
                if part == 2:
                    outs[g, n] = functools.reduce(
                        jnp.add, [_stack(p, p) * t for p, t in zip(prob[g], back)]).astype(BF16)
                elif part == 0:
                    terms = [pair[0] * t[0:8] + pair[1] * t[8:16] for t in back]
                    logit[g] = terms if n == 0 else [a + t for a, t in zip(logit[g], terms)]
                if (part, n) == (0, DA // 2 - 1):
                    s = [jnp.where(lane >= DIL * w, t, NEG * DA ** 0.5) if first else t
                         for w, t in enumerate(logit[g])]
                    top = functools.reduce(jnp.maximum, s)
                    ex = [jnp.exp2((t - top) * (DA ** -0.5 * LOG2E)) for t in s]
                    inv = gsig / functools.reduce(jnp.add, ex)
                    prob[g] = [t * inv for t in ex]
        gm_s[j] = 1.0 - gsig
        if not first:
            a_out(j - 1, dot)
        oa_s[...] = _stack(*(outs[key] for key in sorted(outs)))

    plain = lambda left, right: _dot(pltpu.bitcast(left, BF16), right)
    wait_all(cp_x[0])
    to_rows(0)
    a_tile(0, True, plain)
    cp_wo.wait()
    wait_all(cp_x[1])
    prep_wo()
    a_tile(1, False, plain)
    to_rows(1)

    def a_loop(first, count, work, spare, loading):
        def body(j, carry):
            if loading:
                for j0 in XCUT[2:]:
                    pl.when(j == j0)(functools.partial(wait_all, cp_x[j0]))
                copy(stg_qkv.at[j - first], stg_qkv.at[j - first], sem_in.at[j - first]).wait()
                to_rows(j)
            job = work(j - first)
            a_tile(j, False, paced(job, spare, zero_w, *(QA if loading else QB)))
            list(job)
            return carry

        lax.fori_loop(first, first + count, body, 0)

    a_loop(2, 3 * GP, prep_qkv, spare_qkv, True)

    qi = lax.broadcasted_iota(jnp.int32, (rows, rows), 0)
    ki = lax.broadcasted_iota(jnp.int32, (rows, rows), 1)
    mask = (qi >= seg) | (ki >= seg) | (qi >= ki)
    part, o_prev, opart, b_rows = (_Carry(r) for r in (part_s, o_s, opart_s, b_s))
    ahead = {}

    def b_step(u, t0, memv, project_only=False, output_only=False):
        odd = u % 2
        keep = lambda slots: [s for s in slots if s["tok"] or memv]
        qs, os_ = keep(_PHASES[odd]), keep(_PHASES[1 - odd])
        lhs, shared, tok, mrow, full, soft, o_mem, o_mix, o_left, o_host, new = ({} for _ in range(11))

        def spread(sums, key, slots, s, tok_rows, mem_rows):
            for nu in range(KB):
                if memv:
                    sums.add(key + (nu, 2), s["c"][nu], mem_rows, sum(abs(o["c"][nu]) for o in slots))
                for mu in range(2 if s["tok"] else 0):
                    sums.add(key + (nu, mu), _C[s["r"]][mu][nu], tok_rows,
                             sum(abs(_C[o["r"]][mu][nu]) for o in slots if o["tok"]))

        x_mix = _Mixer(lambda mu, kk: x32[kk, pl.ds(t0 + mu * seg, seg), :])
        c_mix = _Mixer(lambda mu, _: x32[KB, pl.ds(t0 + mu * seg, seg), :])
        m_mix = _Mixer(lambda _, kk: memv[kk])
        m_tail = memv[KB] + pltpu.roll(memv[KB], 64, 1) if memv else None

        def q_left(e, t):
            s = qs[e]
            if (e, t) not in lhs:
                left = _stack(x_mix(_U[s["r"]]) if s["tok"] else None,
                             m_mix([s["a"]]) if memv else None)
                if s["r"] < NH and t < 2:
                    c = _stack(c_mix(_TAIL_IN[s["r"]][:, None]),
                              _signed_sum([(sum(s["c"]), m_tail)]) if memv else None)
                    left = jnp.where(_low_half(c.shape[0]), *((c, left), (left, c))[t])
                lhs[e, t] = left
            return lhs[e, t]

        def q_total(key, value):
            i, g, nu, mu = key
            h = g * KB + nu
            if mu == 2:
                mrow[i, h] = value
            elif odd:
                part.put((i, h, mu), value, u == 3)
            elif mu == 0:
                tok[i, h] = value + part[i, h, mu]
            else:
                ahead[i, h] = value + part[i, h, mu]
            cur = (ahead if odd else tok).get((i, h))
            if (i, h) in mrow and cur is not None and (i, h) not in full:
                full[i, h] = _stack(cur, mrow[i, h]).astype(BF16 if i else F32)

        q_sums = _Sums(q_total)

        def q_pass(e, i, gp, t):
            s = qs[e]
            p = _dot(q_left(e, t), _tile(wb, i * GP + gp, t * NR + s["r"]))
            if t == 2:
                shared[e, i, gp] = p
                return
            if s["r"] < NH:
                p = p + shared[e, i, gp]
            spread(q_sums, (i, 2 * gp + t), qs, s, p[:seg], p[-mem:])

        def scores(h):
            s = jnp.where(mask, _dot_nt(full[0, h], full[1, h]), NEG * DB ** 0.5)
            e = jnp.exp2((s - jnp.max(s, axis=-1, keepdims=True)) * (DB ** -0.5 * LOG2E))
            total = jnp.sum(e, axis=-1, keepdims=True)
            inv = pltpu.reciprocal(total, approx=True)
            soft[h] = e * (inv * (2.0 - total * inv))

        def values(h):
            o = _dot(soft[h], full[2, h])
            o_mem[h] = o[seg:]
            if odd:
                o_prev.put((0, h), ahead["o", h], u == 3)
                o_prev.put((1, h), o[:seg], u == 3)
            else:
                ahead["o", h] = o[:seg]

        def o_rows(e, gp, t):
            s = os_[e]
            if (e, gp, t) not in o_left:
                g = 2 * gp + t
                if t == 2:
                    o_left[e, gp, t] = o_rows(e, gp, 0) + o_rows(e, gp, 1)
                    return o_left[e, gp, t]
                if g not in o_mix:
                    o_mix[g] = (_Mixer(lambda _, kk: o_mem[g * KB + kk]),
                                _Mixer(lambda mu, kk: o_prev[mu, g * KB + kk]))
                o_left[e, gp, t] = _stack(o_mix[g][0]([s["a"]]) if memv else None,
                                         o_mix[g][1](_U[s["r"]]) if s["tok"] else None)
            return o_left[e, gp, t]

        def o_total(key, value):
            nu, mu = key
            if mu == 2:
                new[nu] = value
            elif odd:
                opart.put((nu, mu), value, u == 3)
            else:
                b_rows.put((nu, (u - 2) % 4 + mu), value + opart[nu, mu], u == 2)

        out_sums = _Sums(o_total)

        def o_product(key, value):
            e, t = key
            s = os_[e]
            if s["r"] < NH:
                o_host[key] = value
                if any((e, t_) not in o_host for t_ in range(3)):
                    return
                lo = _low_half(value.shape[0])
                value = o_host[e, 2] + jnp.where(lo, o_host[e, 1], o_host[e, 0])
                y = jnp.where(lo, o_host[e, 0], o_host[e, 1])
                if memv:
                    out_sums.add((KB, 2), sum(s["a"]), y[:mem], KB)
                for mu in range(2):
                    out_sums.add((KB, mu), _TAIL_OUT[s["r"]][mu], y[-seg:],
                                 sum(abs(_TAIL_OUT[o["r"]][mu]) for o in os_ if o["r"] < NH))
            spread(out_sums, (), os_, s, value[-seg:], value[:mem])

        o_sums = _Sums(o_product)

        def o_pass(e, gp, t):
            host = os_[e]["r"] < NH
            p = _dot(o_rows(e, gp, t), _tile(wb, 3 * GP + gp, t * NR + os_[e]["r"]))
            o_sums.add((e, t if host else 0), 1, p, GP if host else 2 * GP)

        todo = []
        tiles = lambda s: (2, 0, 1) if s["r"] < NH else (0, 1)
        if not output_only:
            todo = [(s["tok"], q_pass, e, i, gp, t) for gp in range(GP) for i in (1, 0, 2)
                    for e, s in enumerate(qs) for t in tiles(s)]
            last = [max(e for e, s in enumerate(_PHASES[odd]) if s["tok"] and s["c"][nu])
                    for nu in range(KB)]
            ready = lambda e, t: 99 if qs[e]["r"] < NH and t < 2 else max(
                last[kk] for kk in range(KB) if qs[e]["a"][kk])
            todo[:HEAD[odd]] = sorted(todo[:HEAD[odd]], key=lambda p: ready(p[2], p[5]))
        if not project_only:
            todo += [(s["tok"], o_pass, e, gp, t) for pairs in ((0, 1), (2, 3)) for e, s in enumerate(os_)
                     for gp in pairs for t in tiles(s)]
        long_, short = ([p[1:] for p in todo if p[0] == tok] for tok in (True, False))
        extra = {}
        for h in range(HB if memv else 0):
            extra.setdefault(SCORE_AT[odd][h // 2], []).append((scores, h))
            extra.setdefault(VALUE_AT[odd][h // 2], []).append((values, h))
        issued = 0
        for n, p in enumerate(long_):
            for fn, *args in extra.get(n, []) + [p]:
                if issued % 4 == 0 and short and n >= SHORT_AT[odd][-len(short) // 4]:
                    for fn_s, *args_s in short[:4]:
                        fn_s(*args_s)
                    del short[:4]
                fn(*args)
                issued += 1
        assert not short
        return new

    def emit_tile(j):
        for nu in range(KB + 1):
            bt = _stack(*(b_rows[nu, n] for n in range(4))).T
            bt = bt if nu < KB else bt[:64] + bt[64:]
            at = pl.ds(nu * LANES, bt.shape[0])
            gm = jnp.concatenate([gm_s[j]] * (bt.shape[0] // 8), axis=0)
            out_v[j, at, :] = (ga_s[j, at, :] + gm * bt).astype(out_v.dtype)

    cp_wot.wait()
    for gp in range(GP):
        turn_out(gp)
    b_step(3, 0, None, project_only=True)
    part.val.clear()
    for j in range(3 * GP + 2, nt):
        to_rows(j)
    a_loop(3 * GP + 2, GP - 2, prep_out, spare_t, False)
    job = itertools.chain(prep_out(GP - 2), prep_out(GP - 1))
    a_out(nt - 1, paced(job, spare_t, zero_w, *QC))
    list(job)

    def b_body(j, carry):
        memv = {kk: mem_s[kk] for kk in range(KB + 1)}
        for u in range(4):
            t0 = jnp.minimum(j * LANES + (u + 1) // 2 * 2 * seg, seq - 2 * seg)
            memv = b_step(u, pl.multiple_of(t0, seg), memv)
            if u == 0:
                emit_tile(jnp.maximum(j - 1, 0))
        for kk, t in memv.items():
            mem_s[kk] = t
        for c in (part, o_prev, opart, b_rows):
            c.val.clear()
        pl.when(j > 0)(lambda: cp_out(j - 1).start())
        return carry

    lax.fori_loop(0, nt, b_body, 0)
    b_step(0, None, None, output_only=True)
    emit_tile(nt - 1)
    cp_out(nt - 1).start()
    for j in range(nt):
        cp_out(j).wait()


@functools.partial(jax.jit, static_argnames=("B_seg_len",))
def pallas_gated_mix__sliding_local_dilated__memory_aug_recurrent_mem_tr__prompt_kernel(
    A_x: jax.Array,
    A_wqkv: jax.Array,
    A_wo: jax.Array,
    B_x: jax.Array,
    B_mem0: jax.Array,
    B_Wq: jax.Array,
    B_Wk: jax.Array,
    B_Wv: jax.Array,
    B_Wo: jax.Array,
    B_seg_len: int,
    gate_w: jax.Array,
):
    del B_x
    batch, seq, width = A_x.shape
    mem, seg = B_mem0.shape[1], int(B_seg_len)
    nt = seq // LANES
    assert batch == 1 and width == D and nt == 4 * GP and seq % LANES == 0
    assert B_Wq.shape == (D, HB, DB) and mem == 8 and 4 * seg == LANES

    hbm = pl.BlockSpec(memory_space=pl.ANY)
    out_t = pl.pallas_call(
        functools.partial(_kernel, seq=seq, seg=seg, mem=mem),
        out_shape=jax.ShapeDtypeStruct((D, seq), A_x.dtype),
        in_specs=[hbm] * 9,
        out_specs=hbm,
        scratch_shapes=[
            pltpu.VMEM((nt, D, LANES), BF16),
            pltpu.VMEM((D, 3 * D), BF16),
            pltpu.VMEM((D, D), BF16),
            pltpu.VMEM((3 * GP + 1, KB, D, DB), U32),
            pltpu.VMEM((HB, D, DB), BF16),
            pltpu.VMEM((GP + 1, 2 * KB + 1, KB, 64, LANES), U32),
            pltpu.VMEM((5, 3 * D + 32, LANES), F32),
            pltpu.VMEM((5, D + 32, LANES), F32),
            pltpu.VMEM((12, 3 * D // 2 + 16, LANES), BF16),
            pltpu.VMEM((12, D // 2, LANES), BF16),
            pltpu.VMEM((2 * D, LANES), BF16),
            pltpu.VMEM((D, LANES), BF16),
            pltpu.VMEM((4 * GP + 1, 2 * NR + NH, LANES, LANES), BF16),
            pltpu.VMEM((KB + 1, seq, LANES), F32),
            pltpu.VMEM((nt, D, LANES), F32),
            pltpu.VMEM((nt, 8, LANES), F32),
            pltpu.VMEM((2 * KB, mem, LANES), F32),
            pltpu.VMEM((3, HB, 2, seg, LANES), F32),
            pltpu.VMEM((2, HB, seg, LANES), F32),
            pltpu.VMEM((KB + 1, 2, seg, LANES), F32),
            pltpu.VMEM((KB + 1, 2, seg, LANES), F32),
            pltpu.VMEM((nt, D, LANES), A_x.dtype),
            pltpu.VMEM((mem, D), BF16),
            pltpu.VMEM((D,), BF16),
            pltpu.SemaphoreType.DMA((3 * GP + 9 + len(XCUT),)),
            pltpu.SemaphoreType.DMA(()),
        ],
        compiler_params=pltpu.CompilerParams(vmem_limit_bytes=110 * 1024 * 1024),
        name="gated_mix_kernel",
    )(A_x.reshape(seq, D).T, A_wqkv, A_wo, B_mem0.reshape(mem, D), B_Wq, B_Wk, B_Wv,
      B_Wo.transpose(0, 2, 1), gate_w)
    return out_t.T.reshape(batch, seq, D)
```

```python
import functools
import itertools

import jax
import jax.numpy as jnp
import numpy as np
from jax import lax
import jax.experimental.pallas as pl
import jax.experimental.pallas.tpu as pltpu

F32, BF16, U32 = jnp.float32, jnp.bfloat16, jnp.uint32

D = 576
LANES = 128
HA, DA = 32, 18
WIN, DIL = 8, 2
HB, DB = 32, 128
NEG = -1000000000.0
LOG2E = 1.4426950408889634
NG = HA // 8

KB = 4
GP = HB // (2 * KB)

_HK = (
    (".... +...", "+.-. -... .... -...", "+... +..."),
    ("+... -...", "+-.- .... -... ....", "+... ...."),
    (".+.. .-..", ".... +-.. .+.. ....", ".... .+.."),
    (".+.. ....", ".-.. .+-. .... ....", ".+.. .+.."),
    (".... ..+.", ".... ..-. -.+. .+-.", ".... ..+."),
    ("..+. ....", "..-. ...+ .-+- ....", "..+. ...."),
    ("...+ ...-", ".... ...- ...+ ++.-", ".... ...+"),
    ("...+ ....", "...- ...- .... .+-+", "...+ ...+"),
    (".... ++..", ".... +... .... ....", ".... ++.."),
    ("++.. ....", ".+.. .... .... ....", "++.. ...."),
    (".+.. +...", ".-.. +... .... ....", "+... .-.."),
    ("+.+. -.-.", ".... .... -... ....", ".... +.+."),
    ("+.+. ....", "..+. .... .... ....", "+.+. +.+."),
    ("+.+. -...", "..-. .... +... ....", "+... +.+."),
    (".... +..+", ".... .... .... +...", ".... +..+"),
    ("+..+ ....", "...+ .... .... ....", "+..+ ...."),
    ("...+ +...", "...- .... .... +...", "+... ...-"),
    (".... .++.", ".... ..+. .... .-..", ".++. .++."),
    (".++. .--.", ".... ...- .+.. ....", ".++. ...."),
    (".+.. .--.", ".... ..+. .-.. ....", ".++. .+.."),
    (".... ..++", ".... .... .... .-+.", "..++ ..++"),
    ("..++ ..--", ".... ...- ...+ ....", "..++ ...."),
    ("...+ ..--", ".... ...+ ...- .-+.", "..++ ...+"),
    (".... .+++", ".... .... .... .+..", ".... .+++"),
    (".+++ ....", ".... ...+ .... ....", ".+++ ...."),
    ("...+ .++.", ".... ...- .... .+..", ".++. ...-"),
)
_U, _V, _C = (np.array([[["-.+".index(ch) - 1 for ch in row] for row in prod[i].split()]
                        for prod in _HK]) for i in range(3))
NR = len(_HK)
assert np.array_equal(np.einsum("rak,rln,rbm->akblnm", _U, _V, _C),
                      np.einsum("ab,kl,nm->akblnm", *(np.eye(n, dtype=int) for n in (2, KB, KB))))


def _phase(products):
    tiles = [max(r, ~r) for r in products]
    dual = np.rint(np.linalg.inv(_V[tiles].reshape(len(tiles), -1)).T).astype(int)
    slots = []
    for r, d in zip(products, dual.reshape(-1, KB, KB)):
        i, j = np.argwhere(d)[0]
        a, c = d[:, j] * d[i, j], d[i]
        assert np.array_equal(np.outer(a, c), d)
        slots.append(dict(r=max(r, ~r), tok=r >= 0, a=a.tolist(), c=c.tolist()))
    return slots


_PHASES = (_phase((11, 8, ~9, 4, 2, 23, 17, ~13, 25, 20, 22, 7, ~19, 16, 15, 1)),
           _phase((24, 21, ~16, 18, 19, 3, 10, ~22, 9, 5, 12, 13, ~25, 0, 14, 6)))
assert sorted(s["r"] for ph in _PHASES for s in ph if s["tok"]) == list(range(NR))

NH = 2 * KB
assert all(sorted(s["r"] // 2 for s in ph if s["r"] < NH) == list(range(KB)) for ph in _PHASES)
assert all(np.abs(s[k]).tolist() == np.eye(KB)[s["r"] // 2].tolist()
           for ph in _PHASES for s in ph if s["r"] < NH for k in "ac")
_TAIL_IN, _TAIL_OUT = (
    np.concatenate([np.rint(np.linalg.inv(t[2 * n:2 * n + 2, :, n]).T).astype(int)
                    for n in range(KB)]) for t in (_C, _U))


SCORE_AT = ((76, 94, 116, 138, 162, 184, 206, 228,
             252, 274, 296, 318, 342, 344, 346, 348),
            (72, 94, 116, 138, 162, 184, 206, 228,
             252, 274, 296, 318, 342, 344, 346, 348))
VALUE_AT = ((112, 134, 156, 182, 202, 224, 252, 268,
             294, 314, 336, 358, 382, 384, 386, 388),
            (112, 134, 156, 182, 202, 224, 246, 268,
             292, 310, 336, 356, 382, 384, 386, 388))
SHORT_AT = ((6, 26, 46, 66, 86, 106, 126, 146, 166, 186, 206, 226,
             246, 266, 286, 306, 326, 346, 364, 385, 410, 426, 444, 463),
            (6, 26, 46, 66, 86, 106, 126, 146, 170, 186, 206, 226,
             246, 266, 286, 306, 326, 346, 360, 385, 410, 426, 440, 455))
HEAD = (72, 66)
XCUT = (0, 1, 3, 8)
RE, RO = 8, 48
ORD = (9, 8, 10, 19, 2, 3, 23, 24, 25, 17, 18, 20, 21, 22, 12, 11, 13, 4, 5, 15, 14, 16, 6, 7, 0, 1)
QA = ((4, 10, 16, 27, 39, 42, 63, 80, 93, 120, 159, 162, 165, 169, 172), 24)
QB = ((10, 13, 21, 42, 55, 73, 90, 109, 146, 155, 160, 166, 168, 175, 179), 32)
QC = ((4, 5, 7, 11, 14, 16, 21, 24, 28, 29, 32, 37, 41, 44, 48, 52), 8)


def _signed_sum(terms):
    terms = [(c, t) for c, t in terms if c]
    first = next((i for i, (c, _) in enumerate(terms) if c > 0), 0)
    c, acc = terms.pop(first)
    acc = acc if c > 0 else -acc
    for c, t in terms:
        acc = acc + t if c > 0 else acc - t
    return acc


class _Mixer:
    def __init__(self, block):
        self.block, self.known = block, {}

    def __call__(self, coef):
        want = {(i, k): int(c) for i, row in enumerate(coef) for k, c in enumerate(row) if c}
        key = tuple(sorted(want.items()))
        if key not in self.known:
            terms = []
            for have in sorted(self.known, key=lambda h: -len(h)):
                for sign in (1, -1):
                    if all(want.get(pos) == sign * c for pos, c in have):
                        terms.append((sign, self.known[have]))
                        want = {pos: c for pos, c in want.items() if pos not in dict(have)}
                        break
            for pos, c in sorted(want.items()):
                self.known[((pos, 1),)] = self.block(*pos)
                terms.append((c, self.known[((pos, 1),)]))
            self.known[key] = _signed_sum(terms)
        return self.known[key]


class _Sums:
    def __init__(self, done):
        self.done, self.acc = done, {}

    def add(self, key, sign, value, expected):
        if not sign:
            return
        count, neg, tot = self.acc.pop(key, (0, sign < 0, value))
        if count and neg == (sign < 0):
            tot = tot + value
        elif count:
            tot, neg = (value - tot if neg else tot - value), False
        if count + 1 == expected:
            self.done(key, -tot if neg else tot)
        else:
            self.acc[key] = (count + 1, neg, tot)


class _Carry:
    def __init__(self, ref):
        self.ref, self.val = ref, {}

    def __getitem__(self, key):
        return self.val[key] if key in self.val else self.ref[key]

    def put(self, key, value, store):
        self.val[key] = value
        if store:
            self.ref[key] = value


def _dot(a, b):
    return lax.dot_general(a, b, (((1,), (0,)), ((), ())), preferred_element_type=F32)


def _dot_nt(a, b):
    return lax.dot_general(a, b, (((1,), (1,)), ((), ())), preferred_element_type=F32)


def _tile(ref, *idx):
    return pltpu.bitcast(ref.bitcast(U32)[idx], BF16)


def _stack(*parts):
    parts = [t for t in parts if t is not None]
    return parts[0] if len(parts) == 1 else jnp.concatenate(parts, axis=0)


def _low_half(rows):
    return lax.broadcasted_iota(jnp.int32, (rows, LANES), 1) < 64


def _pair_lhs(t1, t2):
    lo = _low_half(t1[3].shape[0])
    diff = t1[3] - t2[3]
    return (t1[:3] + [jnp.where(lo, t1[4], diff)]
            + t2[:3] + [jnp.where(lo, -diff, t2[4])]
            + [jnp.where(lo, t1[3], t2[3])])


def _pair_rhs(x):
    a, b, c = x[384:448], x[448:512], x[512:576]
    cat = lambda u, v: jnp.concatenate([u, v], axis=0)
    return [x[i * 128:(i + 1) * 128] for i in range(3)] + [cat(c, b), cat(a, c), x[384:512]]


def _pair_matmul(lhs, rhs, dot):
    out = [dot(lhs(8), rhs[5])] * 2
    for i in range(8):
        out[i // 4] = out[i // 4] + dot(lhs(i), rhs[i % 4 if i < 7 else 4])
    return out


def _kernel(xt_hbm, wqkv_hbm, wo_hbm, mem0_hbm, wq_hbm, wk_hbm, wv_hbm, wot_hbm, gate_hbm,
            out_hbm,
            xt_v, wqkv_v, wo_v, stg_qkv, stg_o, wo_t, wt32, wo32_s, la, lo_a, kv_prev, oa_s,
            wb, x32, ga_s, gm_s, mem_s, part_s, o_s, opart_s, b_s, out_v, mem0_v, gate_v,
            sem_in, sem_out, *, seq, seg, mem):
    nt = seq // LANES
    rows = mem + seg

    sems = (sem_in.at[n] for n in itertools.count(3 * GP))
    copy = pltpu.make_async_copy
    cp_wqkv = {k: copy(wqkv_hbm.at[k * LANES:min(D, (k + 1) * LANES)],
                       wqkv_v.at[k * LANES:min(D, (k + 1) * LANES)], next(sems))
               for k in (3, 4, 0, 1, 2)}
    cp_wo = copy(wo_hbm, wo_v, next(sems))
    cp_x = {j0: [copy(xt_hbm.at[:, j * LANES:(j + 1) * LANES], xt_v.at[j], sem)
                 for j in range(j0, j1)] for j0, j1, sem in zip(XCUT, XCUT[1:] + (nt,), sems)}
    cp_wot = copy(wot_hbm, stg_o, next(sems))
    cp_small = [copy(mem0_hbm, mem0_v, next(sems)), copy(gate_hbm, gate_v, next(sems))]
    queue = cp_small + list(cp_wqkv.values()) + cp_x[0] + [cp_wo]
    for unit in range(3 * GP):
        src = (wq_hbm, wk_hbm, wv_hbm)[unit // GP].bitcast(U32)
        queue += cp_x.get(unit + 1, []) + [
            copy(src.at[:, KB * (unit % GP) + p, :], stg_qkv.at[unit, p], sem_in.at[unit])
            for p in range(KB)]
    for c in queue + [cp_wot]:
        c.start()

    def wait_all(copies):
        for c in copies:
            c.wait()

    def cp_out(j):
        col = j * LANES if isinstance(j, int) else pl.multiple_of(j * LANES, LANES)
        return copy(out_v.at[j], out_hbm.at[:, pl.ds(col, LANES)], sem_out)

    for ref in (o_s, opart_s, b_s):
        ref[...] = jnp.zeros(ref.shape, ref.dtype)
    wait_all(cp_small)
    m0 = mem0_v[...].astype(F32)
    for kk in range(KB):
        mem_s[kk] = m0[:, kk * LANES:(kk + 1) * LANES]
    mem_s[KB] = jnp.concatenate([m0[:, KB * LANES:], jnp.zeros((mem, 64), F32)], axis=1)
    wb[4 * GP, 0, 0:16, :] = jnp.zeros((16, LANES), BF16)

    gate = jnp.broadcast_to(gate_v[...].astype(F32).reshape(1, D), (8, D))
    gate_t = [gate[:, i * 128:(i + 1) * 128] for i in range(4)]
    gate_t.append(jnp.concatenate([gate[:, 512:], gate[:, 512:]], axis=1))

    entries = [None] * 2 + [(g - part // 2, part, n) for g in range(NG + 1) for n in range(DA // 2)
                            for part in (1, 0, 2) if 0 <= g - part // 2 < NG]

    def feature_rows(k, e):
        return _stack(*(gate_t[k] if ent is None else
                       wt32[k, pl.ds(ent[1] * D + ent[0] * 8 * DA + 2 * ent[2] + e, 8, stride=DA), :]
                       for ent in entries))

    for k in cp_wqkv:
        cp_wqkv[k].wait()
        rows_k = wqkv_v[k * LANES:min(D, (k + 1) * LANES), :]
        wt32[k, 0:3 * D] = (rows_k if k < 4 else _stack(rows_k, rows_k)).T.astype(F32)
        for e in range(2 if k < 3 else 0):
            la[4 * e + k] = feature_rows(k, e).astype(BF16)
        if k == 4:
            mixed = _pair_lhs(*([None] * 3 + [feature_rows(3, e), feature_rows(4, e)]
                                for e in range(2)))
            for i in (3, 7, 8):
                la[i] = mixed[i].astype(BF16)

    def prep_wo():
        wo32 = wo_v[...].astype(F32)
        for n in range(4):
            wo32_s[n, 0:D] = wo32[:, n * LANES:(n + 1) * LANES]
        wo32_s[4, 0:D] = jnp.concatenate([wo32[:, 4 * LANES:]] * 2, axis=1)
        turned = []
        for n in range(5):
            perm = _stack(*(wo32_s[n, pl.ds(g * 8 * DA + d, 8, stride=DA), :]
                           for g in range(NG) for d in range(DA))).astype(BF16)
            turned.append([perm[k * LANES:(k + 1) * LANES].T for k in range(4)]
                          + [_stack(perm[4 * LANES:], perm[4 * LANES:]).T])
        tiles = [_stack(*(t[k] for t in turned))[:D].astype(F32) for k in range(5)]
        for i, t in enumerate(_pair_lhs([t[:D // 2] for t in tiles], [t[D // 2:] for t in tiles])):
            lo_a[i] = t.astype(BF16)

    def prep_qkv(unit):
        src, dst = stg_qkv.at[unit], wb.at[unit]

        def rows(g, r0, nu):
            u = src[2 * g + nu // 2, r0:r0 + 16, :]
            return pltpu.bitcast(u & jnp.uint32(0xFFFF0000) if nu % 2 else u << 16, F32)

        for e in range(8):
            at, own, shared = pl.ds(16 * e, 16), e // 4, {}
            for g in (own, 1 - own):
                mix = _Mixer(lambda kk, nu: rows(g, kk * LANES + 16 * e, nu))
                for r in ORD:
                    w = mix(_V[r])
                    if r < NH and g == own:
                        shared[r] = w.astype(BF16)
                        dst[2 * NR + r, at, :] = shared[r]
                        w = rows(g, KB * LANES + 16 * (e % 4), r // 2)
                    elif r < NH:
                        w = w - shared[r].astype(F32)
                    dst[g * NR + r, at, :] = w.astype(BF16)
                yield

    def turn_out(gp):
        words = lambda head, r0, n: _tile(stg_o, 2 * KB * gp + head, pl.ds(r0 // 2, n // 2))
        for head in range(2 * KB + 1):
            for nu in range(KB):
                if head < 2 * KB:
                    tile = words(head, nu * LANES, LANES)
                else:
                    tile = _stack(*(words(g * KB + nu, KB * LANES, 64) for g in range(2)))
                wo_t[gp, head, nu] = pltpu.bitcast(tile.T, U32)

    def prep_out(gp):
        dst, lo = wb.at[3 * GP + gp], _low_half(16)
        for e in range(8):
            at, first = pl.ds(16 * e, 16), {}
            rows = lambda head, nu: pltpu.bitcast(
                wo_t[gp, head, nu, 8 * e:8 * e + 8, :], BF16).astype(F32)
            for g in range(2):
                mix = _Mixer(lambda kk, nu: rows(g * KB + kk, nu))
                for r in ORD:
                    w = mix(_V[r])
                    if r >= NH:
                        dst[g * NR + r, at, :] = w.astype(BF16)
                    elif g == 0:
                        first[r] = w
                    else:
                        z, t = jnp.where(lo, first[r], w).astype(BF16), rows(2 * KB, r // 2)
                        dst[2 * NR + r, at, :] = z
                        dst[r, at, :] = jnp.where(lo, t, first[r] - z.astype(F32)).astype(BF16)
                        dst[NR + r, at, :] = jnp.where(lo, w - z.astype(F32), t).astype(BF16)
                yield

    lane = lax.broadcasted_iota(jnp.int32, (8, LANES), 1)

    def exchange(idx, pair, first):
        at = pl.ds(8 * idx, 8)
        prev = None if first else kv_prev.bitcast(U32)[at, :]
        kv_prev[16 * idx:16 * idx + 16, :] = jnp.concatenate(pair, axis=0).astype(BF16)
        cur = kv_prev.bitcast(U32)[at, :]
        return (jnp.broadcast_to(cur[:, 0:1], (8, LANES)) if first else prev), cur

    def to_rows(j):
        t0 = j * LANES if isinstance(j, int) else pl.multiple_of(j * LANES, LANES)
        xt = _tile(xt_v, j)
        for kk in range(KB + 1):
            tile = xt[kk * LANES:(kk + 1) * LANES]
            x32[kk, pl.ds(t0, LANES), :] = (tile if kk < KB else _stack(tile, tile)).T.astype(F32)

    def paced(job, src, dst, when, back):
        results = []

        def dot(left, right):
            if len(results) in when:
                if len(results) >= back:
                    src[...] = pltpu.bitcast(results[-back][0:8], U32)
                next(job, None)
                left = _stack(left[:-8] if len(left) > 8 else None, left[-8:] | dst[...])
            results.append(_dot(pltpu.bitcast(left, BF16), right))
            return results[-1]

        return dot

    spare_qkv, spare_t = stg_qkv.at[3 * GP, 0, 0:8], wo_t.at[GP, 0, 1, 0:8]
    zero_w = wb.bitcast(U32).at[4 * GP, 0, 0:8]

    def a_out(j, dot):
        rhs = _pair_rhs(_tile(oa_s, slice(None)))
        for r0 in range(0, D // 2, RO):
            halves = _pair_matmul(lambda i: lo_a.bitcast(U32)[i, r0 // 2:(r0 + RO) // 2, :], rhs, dot)
            for e in range(2):
                ga_s[j, pl.ds(e * D // 2 + r0, RO), :] = halves[e]

    def a_tile(j, first, dot):
        rhs = _pair_rhs(_tile(xt_v, j))
        logit, prob, outs = {}, {}, {}
        for e0 in range(0, len(entries), RE):
            some = entries[e0:e0 + RE]
            halves = _pair_matmul(
                lambda i: la.bitcast(U32)[i, 4 * e0:4 * (e0 + len(some)), :], rhs, dot)
            for ent, r0 in zip(some, range(0, 8 * RE, 8)):
                pair = [t[r0:r0 + 8] for t in halves]
                if ent is None:
                    gsig = 1.0 / (1.0 + jnp.exp(-halves[0][0:8]))
                    continue
                g, part, n = ent
                if part:
                    prev, cur = exchange((2 * g + part - 1) * (DA // 2) + n, pair, first)
                    back = [cur] + [
                        pltpu.roll(jnp.where(lane >= LANES - DIL * w, prev, cur), DIL * w, 1)
                        for w in range(1, WIN)]
                    back = [pltpu.bitcast(t, BF16).astype(F32) for t in back]
                if part == 2:
                    outs[g, n] = functools.reduce(
                        jnp.add, [_stack(p, p) * t for p, t in zip(prob[g], back)]).astype(BF16)
                elif part == 0:
                    terms = [pair[0] * t[0:8] + pair[1] * t[8:16] for t in back]
                    logit[g] = terms if n == 0 else [a + t for a, t in zip(logit[g], terms)]
                if (part, n) == (0, DA // 2 - 1):
                    s = [jnp.where(lane >= DIL * w, t, NEG * DA ** 0.5) if first else t
                         for w, t in enumerate(logit[g])]
                    top = functools.reduce(jnp.maximum, s)
                    ex = [jnp.exp2((t - top) * (DA ** -0.5 * LOG2E)) for t in s]
                    inv = gsig / functools.reduce(jnp.add, ex)
                    prob[g] = [t * inv for t in ex]
        gm_s[j] = 1.0 - gsig
        if not first:
            a_out(j - 1, dot)
        oa_s[...] = _stack(*(outs[key] for key in sorted(outs)))

    plain = lambda left, right: _dot(pltpu.bitcast(left, BF16), right)
    wait_all(cp_x[0])
    to_rows(0)
    a_tile(0, True, plain)
    cp_wo.wait()
    wait_all(cp_x[1])
    prep_wo()
    a_tile(1, False, plain)
    to_rows(1)

    def a_loop(first, count, work, spare, loading):
        def body(j, carry):
            if loading:
                for j0 in XCUT[2:]:
                    pl.when(j == j0)(functools.partial(wait_all, cp_x[j0]))
                copy(stg_qkv.at[j - first], stg_qkv.at[j - first], sem_in.at[j - first]).wait()
                to_rows(j)
            job = work(j - first)
            a_tile(j, False, paced(job, spare, zero_w, *(QA if loading else QB)))
            list(job)
            return carry

        lax.fori_loop(first, first + count, body, 0)

    a_loop(2, 3 * GP, prep_qkv, spare_qkv, True)

    qi = lax.broadcasted_iota(jnp.int32, (rows, rows), 0)
    ki = lax.broadcasted_iota(jnp.int32, (rows, rows), 1)
    mask = (qi >= seg) | (ki >= seg) | (qi >= ki)
    part, o_prev, opart, b_rows = (_Carry(r) for r in (part_s, o_s, opart_s, b_s))
    ahead = {}

    def b_step(u, t0, memv, project_only=False, output_only=False):
        odd = u % 2
        keep = lambda slots: [s for s in slots if s["tok"] or memv]
        qs, os_ = keep(_PHASES[odd]), keep(_PHASES[1 - odd])
        lhs, shared, tok, mrow, full, soft, o_mem, o_mix, o_left, o_host, new = ({} for _ in range(11))

        def spread(sums, key, slots, s, tok_rows, mem_rows):
            for nu in range(KB):
                if memv:
                    sums.add(key + (nu, 2), s["c"][nu], mem_rows, sum(abs(o["c"][nu]) for o in slots))
                for mu in range(2 if s["tok"] else 0):
                    sums.add(key + (nu, mu), _C[s["r"]][mu][nu], tok_rows,
                             sum(abs(_C[o["r"]][mu][nu]) for o in slots if o["tok"]))

        x_mix = _Mixer(lambda mu, kk: x32[kk, pl.ds(t0 + mu * seg, seg), :])
        c_mix = _Mixer(lambda mu, _: x32[KB, pl.ds(t0 + mu * seg, seg), :])
        m_mix = _Mixer(lambda _, kk: memv[kk])
        m_tail = memv[KB] + pltpu.roll(memv[KB], 64, 1) if memv else None

        def q_left(e, t):
            s = qs[e]
            if (e, t) not in lhs:
                left = _stack(x_mix(_U[s["r"]]) if s["tok"] else None,
                             m_mix([s["a"]]) if memv else None)
                if s["r"] < NH and t < 2:
                    c = _stack(c_mix(_TAIL_IN[s["r"]][:, None]),
                              _signed_sum([(sum(s["c"]), m_tail)]) if memv else None)
                    left = jnp.where(_low_half(c.shape[0]), *((c, left), (left, c))[t])
                lhs[e, t] = left
            return lhs[e, t]

        def q_total(key, value):
            i, g, nu, mu = key
            h = g * KB + nu
            if mu == 2:
                mrow[i, h] = value
            elif odd:
                part.put((i, h, mu), value, u == 3)
            elif mu == 0:
                tok[i, h] = value + part[i, h, mu]
            else:
                ahead[i, h] = value + part[i, h, mu]
            cur = (ahead if odd else tok).get((i, h))
            if (i, h) in mrow and cur is not None and (i, h) not in full:
                full[i, h] = _stack(cur, mrow[i, h]).astype(BF16 if i else F32)

        q_sums = _Sums(q_total)

        def q_pass(e, i, gp, t):
            s = qs[e]
            p = _dot(q_left(e, t), _tile(wb, i * GP + gp, t * NR + s["r"]))
            if t == 2:
                shared[e, i, gp] = p
                return
            if s["r"] < NH:
                p = p + shared[e, i, gp]
            spread(q_sums, (i, 2 * gp + t), qs, s, p[:seg], p[-mem:])

        def scores(h):
            s = jnp.where(mask, _dot_nt(full[0, h], full[1, h]), NEG * DB ** 0.5)
            e = jnp.exp2((s - jnp.max(s, axis=-1, keepdims=True)) * (DB ** -0.5 * LOG2E))
            total = jnp.sum(e, axis=-1, keepdims=True)
            inv = pltpu.reciprocal(total, approx=True)
            soft[h] = e * (inv * (2.0 - total * inv))

        def values(h):
            o = _dot(soft[h], full[2, h])
            o_mem[h] = o[seg:]
            if odd:
                o_prev.put((0, h), ahead["o", h], u == 3)
                o_prev.put((1, h), o[:seg], u == 3)
            else:
                ahead["o", h] = o[:seg]

        def o_rows(e, gp, t):
            s = os_[e]
            if (e, gp, t) not in o_left:
                g = 2 * gp + t
                if t == 2:
                    o_left[e, gp, t] = o_rows(e, gp, 0) + o_rows(e, gp, 1)
                    return o_left[e, gp, t]
                if g not in o_mix:
                    o_mix[g] = (_Mixer(lambda _, kk: o_mem[g * KB + kk]),
                                _Mixer(lambda mu, kk: o_prev[mu, g * KB + kk]))
                o_left[e, gp, t] = _stack(o_mix[g][0]([s["a"]]) if memv else None,
                                         o_mix[g][1](_U[s["r"]]) if s["tok"] else None)
            return o_left[e, gp, t]

        def o_total(key, value):
            nu, mu = key
            if mu == 2:
                new[nu] = value
            elif odd:
                opart.put((nu, mu), value, u == 3)
            else:
                b_rows.put((nu, (u - 2) % 4 + mu), value + opart[nu, mu], u == 2)

        out_sums = _Sums(o_total)

        def o_product(key, value):
            e, t = key
            s = os_[e]
            if s["r"] < NH:
                o_host[key] = value
                if any((e, t_) not in o_host for t_ in range(3)):
                    return
                lo = _low_half(value.shape[0])
                value = o_host[e, 2] + jnp.where(lo, o_host[e, 1], o_host[e, 0])
                y = jnp.where(lo, o_host[e, 0], o_host[e, 1])
                if memv:
                    out_sums.add((KB, 2), sum(s["a"]), y[:mem], KB)
                for mu in range(2):
                    out_sums.add((KB, mu), _TAIL_OUT[s["r"]][mu], y[-seg:],
                                 sum(abs(_TAIL_OUT[o["r"]][mu]) for o in os_ if o["r"] < NH))
            spread(out_sums, (), os_, s, value[-seg:], value[:mem])

        o_sums = _Sums(o_product)

        def o_pass(e, gp, t):
            host = os_[e]["r"] < NH
            p = _dot(o_rows(e, gp, t), _tile(wb, 3 * GP + gp, t * NR + os_[e]["r"]))
            o_sums.add((e, t if host else 0), 1, p, GP if host else 2 * GP)

        todo = []
        tiles = lambda s: (2, 0, 1) if s["r"] < NH else (0, 1)
        if not output_only:
            todo = [(s["tok"], q_pass, e, i, gp, t) for gp in range(GP) for i in (1, 0, 2)
                    for e, s in enumerate(qs) for t in tiles(s)]
            last = [max(e for e, s in enumerate(_PHASES[odd]) if s["tok"] and s["c"][nu])
                    for nu in range(KB)]
            ready = lambda e, t: 99 if qs[e]["r"] < NH and t < 2 else max(
                last[kk] for kk in range(KB) if qs[e]["a"][kk])
            todo[:HEAD[odd]] = sorted(todo[:HEAD[odd]], key=lambda p: ready(p[2], p[5]))
        if not project_only:
            todo += [(s["tok"], o_pass, e, gp, t) for pairs in ((0, 1), (2, 3)) for e, s in enumerate(os_)
                     for gp in pairs for t in tiles(s)]
        long_, short = ([p[1:] for p in todo if p[0] == tok] for tok in (True, False))
        extra = {}
        for h in range(HB if memv else 0):
            extra.setdefault(SCORE_AT[odd][h // 2], []).append((scores, h))
            extra.setdefault(VALUE_AT[odd][h // 2], []).append((values, h))
        issued = 0
        for n, p in enumerate(long_):
            for fn, *args in extra.get(n, []) + [p]:
                if issued % 4 == 0 and short and n >= SHORT_AT[odd][-len(short) // 4]:
                    for fn_s, *args_s in short[:4]:
                        fn_s(*args_s)
                    del short[:4]
                fn(*args)
                issued += 1
        assert not short
        return new

    def emit_tile(j):
        for nu in range(KB + 1):
            bt = _stack(*(b_rows[nu, n] for n in range(4))).T
            bt = bt if nu < KB else bt[:64] + bt[64:]
            at = pl.ds(nu * LANES, bt.shape[0])
            gm = jnp.concatenate([gm_s[j]] * (bt.shape[0] // 8), axis=0)
            out_v[j, at, :] = (ga_s[j, at, :] + gm * bt).astype(out_v.dtype)

    cp_wot.wait()
    for gp in range(GP):
        turn_out(gp)
    b_step(3, 0, None, project_only=True)
    part.val.clear()
    for j in range(3 * GP + 2, nt):
        to_rows(j)
    a_loop(3 * GP + 2, GP - 2, prep_out, spare_t, False)
    job = itertools.chain(prep_out(GP - 2), prep_out(GP - 1))
    a_out(nt - 1, paced(job, spare_t, zero_w, *QC))
    list(job)

    def b_body(j, carry):
        memv = {kk: mem_s[kk] for kk in range(KB + 1)}
        for u in range(4):
            t0 = jnp.minimum(j * LANES + (u + 1) // 2 * 2 * seg, seq - 2 * seg)
            memv = b_step(u, pl.multiple_of(t0, seg), memv)
            if u == 0:
                emit_tile(jnp.maximum(j - 1, 0))
        for kk, t in memv.items():
            mem_s[kk] = t
        for c in (part, o_prev, opart, b_rows):
            c.val.clear()
        pl.when(j > 0)(lambda: cp_out(j - 1).start())
        return carry

    lax.fori_loop(0, nt, b_body, 0)
    b_step(0, None, None, output_only=True)
    emit_tile(nt - 1)
    cp_out(nt - 1).start()
    for j in range(nt):
        cp_out(j).wait()


@functools.partial(jax.jit, static_argnames=("B_seg_len",))
def pallas_gated_mix__sliding_local_dilated__memory_aug_recurrent_mem_tr__prompt_kernel(
    A_x: jax.Array,
    A_wqkv: jax.Array,
    A_wo: jax.Array,
    B_x: jax.Array,
    B_mem0: jax.Array,
    B_Wq: jax.Array,
    B_Wk: jax.Array,
    B_Wv: jax.Array,
    B_Wo: jax.Array,
    B_seg_len: int,
    gate_w: jax.Array,
):
    del B_x
    batch, seq, width = A_x.shape
    mem, seg = B_mem0.shape[1], int(B_seg_len)
    nt = seq // LANES
    assert batch == 1 and width == D and nt == 4 * GP and seq % LANES == 0
    assert B_Wq.shape == (D, HB, DB) and mem == 8 and 4 * seg == LANES

    hbm = pl.BlockSpec(memory_space=pl.ANY)
    out_t = pl.pallas_call(
        functools.partial(_kernel, seq=seq, seg=seg, mem=mem),
        out_shape=jax.ShapeDtypeStruct((D, seq), A_x.dtype),
        in_specs=[hbm] * 9,
        out_specs=hbm,
        scratch_shapes=[
            pltpu.VMEM((nt, D, LANES), BF16),
            pltpu.VMEM((D, 3 * D), BF16),
            pltpu.VMEM((D, D), BF16),
            pltpu.VMEM((3 * GP + 1, KB, D, DB), U32),
            pltpu.VMEM((HB, D, DB), BF16),
            pltpu.VMEM((GP + 1, 2 * KB + 1, KB, 64, LANES), U32),
            pltpu.VMEM((5, 3 * D + 32, LANES), F32),
            pltpu.VMEM((5, D + 32, LANES), F32),
            pltpu.VMEM((12, 3 * D // 2 + 16, LANES), BF16),
            pltpu.VMEM((12, D // 2, LANES), BF16),
            pltpu.VMEM((2 * D, LANES), BF16),
            pltpu.VMEM((D, LANES), BF16),
            pltpu.VMEM((4 * GP + 1, 2 * NR + NH, LANES, LANES), BF16),
            pltpu.VMEM((KB + 1, seq, LANES), F32),
            pltpu.VMEM((nt, D, LANES), F32),
            pltpu.VMEM((nt, 8, LANES), F32),
            pltpu.VMEM((2 * KB, mem, LANES), F32),
            pltpu.VMEM((3, HB, 2, seg, LANES), F32),
            pltpu.VMEM((2, HB, seg, LANES), F32),
            pltpu.VMEM((KB + 1, 2, seg, LANES), F32),
            pltpu.VMEM((KB + 1, 2, seg, LANES), F32),
            pltpu.VMEM((nt, D, LANES), A_x.dtype),
            pltpu.VMEM((mem, D), BF16),
            pltpu.VMEM((D,), BF16),
            pltpu.SemaphoreType.DMA((3 * GP + 9 + len(XCUT),)),
            pltpu.SemaphoreType.DMA(()),
        ],
        compiler_params=pltpu.CompilerParams(vmem_limit_bytes=110 * 1024 * 1024),
        name="gated_mix_kernel",
    )(A_x.reshape(seq, D).T, A_wqkv, A_wo, B_mem0.reshape(mem, D), B_Wq, B_Wk, B_Wv,
      B_Wo.transpose(0, 2, 1), gate_w)
    return out_t.T.reshape(batch, seq, D)
```
